```python
import jax
import jax.numpy as jnp

def _softmax(x, axis=-1):
    return jax.nn.softmax(x, axis=axis)

def _gelu(x):
    return jax.nn.gelu(x, approximate=True)

def _silu(x):
    return jax.nn.silu(x)

def _sigmoid(x):
    return jax.nn.sigmoid(x)

def _layernorm(x, axis=-1, eps=1e-05):
    m = jnp.mean(x, axis=axis, keepdims=True)
    v = jnp.var(x, axis=axis, keepdims=True)
    return (x - m) / jnp.sqrt(v + eps)

def _scatter_add(tgt, idx, src, axis=0):
    return tgt.at[idx].add(src)

def _segment_sum(src, seg, n):
    return jax.ops.segment_sum(src, seg, n)

class _Rng:

    def __init__(self, key):
        self._k = key

    def _next(self):
        self._k, sub = jax.random.split(self._k)
        return sub

    def normal(self, shape):
        return jax.random.normal(self._next(), shape, dtype=jnp.bfloat16)

    def randint(self, lo, hi, shape):
        return jax.random.randint(self._next(), shape, lo, hi, dtype=jnp.int32)

    def uniform(self, shape, lo=0.0, hi=1.0):
        return jax.random.uniform(self._next(), shape, jnp.bfloat16, lo, hi)

    def permutation(self, n):
        return jax.random.permutation(self._next(), n)
kernel_name = 'adaLN_cond__gqa_block_cached__moe_arch_mod__prompt'

def setup_inputs():
    _rng = _Rng(jax.random.key(int.from_bytes(__import__("os").urandom(4), "little")))
    _w = lambda a: (lambda t: t.astype(jnp.bfloat16) if jnp.issubdtype(t.dtype, jnp.floating) else t)(jnp.asarray(a))

    def _A_setup():
        B, Sq, D = (1, 2048, 576)
        Hq, Hkv, Sk, Dh = (32, 16, 2048, 128)
        assert Hq % Hkv == 0, (Hq, Hkv)
        return {'x': _w((lambda *s: _rng.normal(s) * 0.05)(B, Sq, D)), 'k_cache': _w((lambda *s: _rng.normal(s) * 0.05)(B, Hkv, Sk, Dh)), 'v_cache': _w((lambda *s: _rng.normal(s) * 0.05)(B, Hkv, Sk, Dh)), 'wq': _w((lambda *s: _rng.normal(s) * 0.05)(D, Hq * Dh) * D ** (-0.5)), 'wo': _w((lambda *s: _rng.normal(s) * 0.05)(Hq * Dh, D) * (Hq * Dh) ** (-0.5))}
    _A_in = _A_setup()

    def _B_setup():
        B, S, D, F, C = (1, 2048, 576, 4608, 8)
        return {'x': _w((lambda *s: _rng.normal(s) * 0.05)(B, S, D)), 'w_r': _w((lambda *s: _rng.normal(s) * 0.05)(D)), 'w_gate': _w((lambda *s: _rng.normal(s) * 0.05)(D, F)), 'w_up': _w((lambda *s: _rng.normal(s) * 0.05)(D, F)), 'w_down': _w((lambda *s: _rng.normal(s) * 0.05)(F, D))}
    _B_in = _B_setup()
    return {'A_x': _A_in['x'], 'A_k_cache': _A_in['k_cache'], 'A_v_cache': _A_in['v_cache'], 'A_wq': _A_in['wq'], 'A_wo': _A_in['wo'], 'B_x': _B_in['x'], 'B_w_r': _B_in['w_r'], 'B_w_gate': _B_in['w_gate'], 'B_w_up': _B_in['w_up'], 'B_w_down': _B_in['w_down'], 'c': _w((lambda *s: _rng.normal(s) * 0.05)(1, 576)), 'w_mod': _w((lambda *s: _rng.normal(s) * 0.05)(576, 6 * 576) * 576 ** (-0.5))}

def reference(A_x, A_k_cache, A_v_cache, A_wq, A_wo, B_x, B_w_r, B_w_gate, B_w_up, B_w_down, c, w_mod):

    def _A_ref(x, k_cache, v_cache, wq, wo):
        B, Sq, D = x.shape
        Hq, Dh = (32, 128)
        Hkv = k_cache.shape[1]
        rep = Hq // Hkv
        q = (lambda x, *d: x.transpose(*d))((x @ wq).reshape(B, Sq, Hq, Dh), 0, 2, 1, 3)
        k = jnp.repeat(k_cache, rep, axis=1)
        v = jnp.repeat(v_cache, rep, axis=1)
        scores = jnp.einsum('bhqd,bhkd->bhqk', q, k) * Dh ** (-0.5)
        p = _softmax(scores, axis=-1)
        o = jnp.einsum('bhqk,bhkd->bhqd', p, v)
        return (lambda x, *d: x.transpose(*d))(o, 0, 2, 1, 3).reshape(B, Sq, Hq * Dh) @ wo

    def _B_ref(x, w_r, w_gate, w_up, w_down):
        B, S, D = x.shape
        C = 8
        r = x @ w_r
        idx = jnp.argsort(-r, axis=-1)[:, :C]
        idx_e = jnp.repeat(idx.reshape(B, C, 1), D, axis=2)
        x_sel = jnp.take_along_axis(x, idx_e, axis=1)
        g = _silu(x_sel @ w_gate)
        u = x_sel @ w_up
        y = g * u @ w_down
        r_sel = _sigmoid(jnp.take_along_axis(r, idx, axis=1))
        y = y * r_sel.reshape(B, C, 1)
        b_off = (jnp.arange(B) * S).reshape(B, 1)
        flat_idx = (idx + b_off).reshape(B * C)
        zero = (x * 0.0).reshape(B * S, D)
        upd = _scatter_add(zero, flat_idx, y.reshape(B * C, D), axis=0)
        return x + upd.reshape(B, S, D)
    x = A_x
    mod = (_silu(c) @ w_mod).reshape(c.shape[0], 6, 1, -1)
    sa, ca, ga, sb, cb, gb = (mod[:, 0].copy(), mod[:, 1].copy(), mod[:, 2].copy(), mod[:, 3].copy(), mod[:, 4].copy(), mod[:, 5].copy())
    h = _layernorm(x, axis=-1) * (1 + ca) + sa
    x = x + ga * _A_ref(h, A_k_cache, A_v_cache, A_wq, A_wo)
    h = _layernorm(x, axis=-1) * (1 + cb) + sb
    x = x + gb * _B_ref(h, B_w_r, B_w_gate, B_w_up, B_w_down)
    return x
```

```python
import functools
import math

import jax
import jax.numpy as jnp
from jax import lax
import jax.experimental.pallas as pl
import jax.experimental.pallas.tpu as pltpu

F32 = jnp.float32
BF16 = jnp.bfloat16

HQ = 32
DH = 128
TOPC = 8
LN_EPS = 1e-5
BQ = 256
LN_ROWS = 256


def _rb(x):
    return x.astype(BF16).astype(F32)


def _sigmoid(x):
    return 1.0 / (1.0 + jnp.exp(-x))


def _kernel(x_ref, k_ref, v_ref, wq_ref, wo_ref, wr_ref, c_ref, wmod_ref,
            wg_hbm, wu_hbm, wd_hbm,
            out_ref,
            mod_ref, h_ref, acc_ref, x2_ref, wg_ref, wu_ref, wd_ref, sems,
            *, S, D, NG, REP):
    g = pl.program_id(0)
    qscale = (DH ** -0.5) * math.log2(math.e)

    def ffn_weight_copies():
        return (pltpu.make_async_copy(wg_hbm, wg_ref, sems.at[0]),
                pltpu.make_async_copy(wu_hbm, wu_ref, sems.at[1]),
                pltpu.make_async_copy(wd_hbm, wd_ref, sems.at[2]))

    @pl.when(g == 0)
    def _prologue():
        for cp in ffn_weight_copies():
            cp.start()
        c = c_ref[...].astype(F32)
        sc = (c * _sigmoid(c)).astype(BF16)
        sc8 = jnp.broadcast_to(sc, (8, D))
        mod = jnp.dot(sc8, wmod_ref[...], preferred_element_type=F32)
        mod = _rb(mod)
        for i in range(6):
            mod_ref[i] = mod[:, i * D:(i + 1) * D]
        sa = mod_ref[0][0:1, :]
        ca1 = _rb(1.0 + mod_ref[1][0:1, :])

        def ln1(i, carry):
            r0 = pl.multiple_of(i * LN_ROWS, LN_ROWS)
            x = x_ref[pl.ds(r0, LN_ROWS), :].astype(F32)
            m = jnp.mean(x, axis=1, keepdims=True)
            d = x - m
            var = jnp.mean(d * d, axis=1, keepdims=True)
            h = d * lax.rsqrt(var + LN_EPS) * ca1 + sa
            h_ref[pl.ds(r0, LN_ROWS), :] = h.astype(BF16)
            acc_ref[pl.ds(r0, LN_ROWS), :] = jnp.zeros((LN_ROWS, D), F32)
            return carry
        lax.fori_loop(0, S // LN_ROWS, ln1, 0)

    k = k_ref[0]
    v = v_ref[0]
    wq = wq_ref[...]
    wo = wo_ref[...]
    for j in range(S // BQ):
        rows = slice(j * BQ, (j + 1) * BQ)
        q2 = jnp.dot(h_ref[rows, :], wq, preferred_element_type=F32)
        q2 = (q2 * qscale).astype(BF16)
        os_ = []
        for r in range(REP):
            q = q2[:, r * DH:(r + 1) * DH]
            s = lax.dot_general(q, k, (((1,), (1,)), ((), ())), preferred_element_type=F32)
            m = jnp.max(s, axis=1, keepdims=True)
            p = jnp.exp2(s - m)
            l = jnp.sum(p, axis=1, keepdims=True)
            o = jnp.dot(p.astype(BF16), v, preferred_element_type=F32)
            os_.append((o * (1.0 / l)).astype(BF16))
        o2 = jnp.concatenate(os_, axis=1)
        acc_ref[rows, :] += jnp.dot(o2, wo, preferred_element_type=F32)

    @pl.when(g == NG - 1)
    def _epilogue():
        ga = mod_ref[2][0:1, :]
        sb = mod_ref[3][0:1, :]
        cb1 = _rb(1.0 + mod_ref[4][0:1, :])
        gb = mod_ref[5][0:1, :]
        eps_b = _rb(jnp.full((1, 1), LN_EPS, F32))

        def ln2(i, carry):
            r0 = pl.multiple_of(i * LN_ROWS, LN_ROWS)
            rows = pl.ds(r0, LN_ROWS)
            x = x_ref[rows, :].astype(F32)
            x2 = _rb(x + _rb(ga * _rb(acc_ref[rows, :])))
            m = jnp.mean(x2, axis=1, keepdims=True)
            dc = x2 - m
            var = jnp.mean(dc * dc, axis=1, keepdims=True)
            sd = _rb(jnp.sqrt(_rb(_rb(var) + eps_b)))
            n = _rb(_rb(x2 - _rb(m)) * (1.0 / sd))
            h2 = _rb(_rb(n * cb1) + sb)
            h_ref[rows, :] = h2.astype(BF16)
            x2_ref[rows, :] = x2.astype(BF16)
            out_ref[rows, :] = (x2 + _rb(gb * h2)).astype(BF16)
            return carry
        lax.fori_loop(0, S // LN_ROWS, ln2, 0)

        wr8 = jnp.broadcast_to(wr_ref[...], (8, D))
        r = lax.dot_general(wr8, h_ref[...], (((1,), (1,)), ((), ())),
                            preferred_element_type=F32)
        r = _rb(r[0:1, :]) + 0.0
        bits = pltpu.bitcast(r, jnp.int32)
        mono = bits ^ ((bits >> 31) & jnp.int32(0x7FFFFFFF))
        col = lax.broadcasted_iota(jnp.int32, (1, S), 1)
        key = (mono & jnp.int32(-65536)) | (jnp.int32(S - 1) - col)
        neg = jnp.int32(-2 ** 31)

        row16 = lax.broadcasted_iota(jnp.int32, (16, D), 0)
        sel_base, sel_off, sel_gate = [], [], []
        xsel = jnp.zeros((16, D), F32)
        for t in range(TOPC):
            kmax = jnp.max(key)
            hit = key == kmax
            rv = jnp.sum(jnp.where(hit, r, 0.0), axis=1, keepdims=True)
            key = jnp.where(hit, neg, key)
            idx = jnp.int32(S - 1) - (kmax & jnp.int32(0xFFFF))
            idx = jnp.clip(idx, 0, S - 1)
            base = pl.multiple_of((idx >> 4) << 4, 16)
            off = idx & 15
            hg = h_ref[pl.ds(base, 16), :].astype(F32)
            row = jnp.sum(jnp.where(row16 == off, hg, 0.0), axis=0, keepdims=True)
            xsel = jnp.where(row16 == t, row, xsel)
            sel_base.append(base)
            sel_off.append(off)
            sel_gate.append(_rb(_sigmoid(rv)))

        for cp in ffn_weight_copies():
            cp.wait()
        xs = xsel.astype(BF16)
        gpre = _rb(jnp.dot(xs, wg_ref[...], preferred_element_type=F32))
        u = _rb(jnp.dot(xs, wu_ref[...], preferred_element_type=F32))
        a = (_rb(gpre * _sigmoid(gpre)) * u).astype(BF16)
        y = _rb(jnp.dot(a, wd_ref[...], preferred_element_type=F32))

        for t in range(TOPC):
            rows = pl.ds(sel_base[t], 16)
            yt = _rb(y[t:t + 1, :] * sel_gate[t])
            hg = h_ref[rows, :].astype(F32)
            xg = x2_ref[rows, :].astype(F32)
            new = xg + _rb(gb * _rb(hg + yt))
            old = out_ref[rows, :].astype(F32)
            out_ref[rows, :] = jnp.where(row16 == sel_off[t], new, old).astype(BF16)


@jax.jit
def pallas_adaLN_cond__gqa_block_cached__moe_arch_mod__prompt_kernel(
    A_x: jax.Array,
    A_k_cache: jax.Array,
    A_v_cache: jax.Array,
    A_wq: jax.Array,
    A_wo: jax.Array,
    B_x: jax.Array,
    B_w_r: jax.Array,
    B_w_gate: jax.Array,
    B_w_up: jax.Array,
    B_w_down: jax.Array,
    c: jax.Array,
    w_mod: jax.Array,
):
    del B_x
    B, S, D = A_x.shape
    assert B == 1
    NG, SK = A_k_cache.shape[1], A_k_cache.shape[2]
    REP = HQ // NG
    FF = B_w_gate.shape[1]
    GW = REP * DH

    x = A_x.reshape(S, D)
    k = A_k_cache.reshape(NG, SK, DH)
    v = A_v_cache.reshape(NG, SK, DH)
    wr = B_w_r.reshape(1, D)

    const2 = lambda g: (0, 0)
    out = pl.pallas_call(
        functools.partial(_kernel, S=S, D=D, NG=NG, REP=REP),
        grid=(NG,),
        in_specs=[
            pl.BlockSpec((S, D), const2),
            pl.BlockSpec((1, SK, DH), lambda g: (g, 0, 0)),
            pl.BlockSpec((1, SK, DH), lambda g: (g, 0, 0)),
            pl.BlockSpec((D, GW), lambda g: (0, g)),
            pl.BlockSpec((GW, D), lambda g: (g, 0)),
            pl.BlockSpec((1, D), const2),
            pl.BlockSpec((1, D), const2),
            pl.BlockSpec((D, 6 * D), const2),
            pl.BlockSpec(memory_space=pl.ANY),
            pl.BlockSpec(memory_space=pl.ANY),
            pl.BlockSpec(memory_space=pl.ANY),
        ],
        out_specs=pl.BlockSpec((S, D), const2),
        out_shape=jax.ShapeDtypeStruct((S, D), BF16),
        scratch_shapes=[
            pltpu.VMEM((6, 8, D), F32),
            pltpu.VMEM((S, D), BF16),
            pltpu.VMEM((S, D), F32),
            pltpu.VMEM((S, D), BF16),
            pltpu.VMEM((D, FF), BF16),
            pltpu.VMEM((D, FF), BF16),
            pltpu.VMEM((FF, D), BF16),
            pltpu.SemaphoreType.DMA((3,)),
        ],
        compiler_params=pltpu.CompilerParams(
            dimension_semantics=("arbitrary",),
            vmem_limit_bytes=110 * 1024 * 1024,
        ),
    )(x, k, v, A_wq, A_wo, wr, c, w_mod, B_w_gate, B_w_up, B_w_down)
    return out.reshape(B, S, D)
```

```python
import functools
import math

import jax
import jax.numpy as jnp
from jax import lax
import jax.experimental.pallas as pl
import jax.experimental.pallas.tpu as pltpu

F32 = jnp.float32
BF16 = jnp.bfloat16

HQ = 32
DH = 128
TOPC = 8
LN_EPS = 1e-5
BQ = 256
LANES = 128

_NT = (((1,), (1,)), ((), ()))


def _rb(x):
    return x.astype(BF16).astype(F32)


def _sigmoid(x):
    return 1.0 / (1.0 + jnp.exp(-x))


def _kernel(xt_ref, k_ref, v_ref, wq_ref, wot_ref, wr_ref, c_ref, wmod_ref,
            wg_hbm, wu_hbm, wdt_hbm,
            out_ref,
            modc_ref, gbrow_ref, h_ref, acc_ref, h2t_ref, x2t_ref, r_ref,
            wg_ref, wu_ref, wdt_ref, sems,
            *, S, D, NG, REP):
    g = pl.program_id(0)
    qscale = (DH ** -0.5) * math.log2(math.e)
    NB = S // BQ

    def ffn_weight_copies():
        return (pltpu.make_async_copy(wg_hbm, wg_ref, sems.at[0]),
                pltpu.make_async_copy(wu_hbm, wu_ref, sems.at[1]),
                pltpu.make_async_copy(wdt_hbm, wdt_ref, sems.at[2]))

    def modcol(i):
        return modc_ref[i * D:(i + 1) * D, :]

    @pl.when(g == 0)
    def _prologue():
        for cp in ffn_weight_copies():
            cp.start()
        c = c_ref[...].astype(F32)
        sc = (c * _sigmoid(c)).astype(BF16)
        sc8 = jnp.broadcast_to(sc, (8, D))
        mod = _rb(jnp.dot(sc8, wmod_ref[...], preferred_element_type=F32))
        gbrow_ref[...] = mod[:, 5 * D:6 * D]
        lane = lax.broadcasted_iota(jnp.int32, mod.shape, 1)
        is_scale = ((lane >= D) & (lane < 2 * D)) | ((lane >= 4 * D) & (lane < 5 * D))
        mod = jnp.where(is_scale, _rb(1.0 + mod), mod)
        modc_ref[...] = jnp.broadcast_to(mod[0:1, :], (LANES, 6 * D)).T

        def ln1(i, carry):
            t0 = pl.multiple_of(i * LANES, LANES)
            x = xt_ref[:, pl.ds(t0, LANES)].astype(F32)
            m = jnp.mean(x, axis=0, keepdims=True)
            d = x - m
            var = jnp.mean(d * d, axis=0, keepdims=True)
            ht = d * lax.rsqrt(var + LN_EPS) * modcol(1) + modcol(0)
            h_ref[pl.ds(t0, LANES), :] = ht.T.astype(BF16)
            acc_ref[:, pl.ds(t0, LANES)] = jnp.zeros((D, LANES), F32)
            return carry
        lax.fori_loop(0, S // LANES, ln1, 0)

    k = k_ref[0]
    v = v_ref[0]
    wq = wq_ref[...]
    wot = wot_ref[...]

    def qproj(j):
        q2 = jnp.dot(h_ref[j * BQ:(j + 1) * BQ, :], wq, preferred_element_type=F32)
        return (q2 * qscale).astype(BF16)

    def qk(q2, r):
        return lax.dot_general(q2[:, r * DH:(r + 1) * DH], k, _NT, preferred_element_type=F32)

    def pv(s):
        m = jnp.max(s, axis=1, keepdims=True)
        p = jnp.exp2(s - m)
        l = jnp.sum(p, axis=1, keepdims=True)
        o = jnp.dot(p.astype(BF16), v, preferred_element_type=F32)
        return (o * (1.0 / l)).astype(BF16)

    def oproj(j, os_):
        o2 = jnp.concatenate(os_, axis=1)
        acc_ref[:, j * BQ:(j + 1) * BQ] += lax.dot_general(
            wot, o2, _NT, preferred_element_type=F32)

    assert REP == 2
    q2 = qproj(0)
    prev = None
    for j in range(NB):
        s0 = qk(q2, 0)
        if prev is not None:
            oproj(j - 1, prev)
        o0 = pv(s0)
        s1 = qk(q2, 1)
        if j + 1 < NB:
            q2 = qproj(j + 1)
        o1 = pv(s1)
        prev = [o0, o1]
    oproj(NB - 1, prev)

    @pl.when(g == NG - 1)
    def _epilogue():
        eps_b = _rb(jnp.full((1, 1), LN_EPS, F32))
        wr8 = jnp.broadcast_to(wr_ref[...], (8, D))

        def ln2(i, carry):
            t0 = pl.multiple_of(i * LANES, LANES)
            cols = pl.ds(t0, LANES)
            x = xt_ref[:, cols].astype(F32)
            x2 = _rb(x + _rb(modcol(2) * _rb(acc_ref[:, cols])))
            m = jnp.mean(x2, axis=0, keepdims=True)
            dc = x2 - m
            var = jnp.mean(dc * dc, axis=0, keepdims=True)
            sd = _rb(jnp.sqrt(_rb(_rb(var) + eps_b)))
            n = _rb(_rb(x2 - _rb(m)) * (1.0 / sd))
            h2 = _rb(_rb(n * modcol(4)) + modcol(3))
            h2b = h2.astype(BF16)
            h2t_ref[:, cols] = h2b
            x2t_ref[:, cols] = x2.astype(BF16)
            out_ref[:, cols] = (x2 + _rb(modcol(5) * h2)).astype(BF16)
            r_ref[:, cols] = jnp.dot(wr8, h2b, preferred_element_type=F32)
            return carry
        lax.fori_loop(0, S // LANES, ln2, 0)

        r = _rb(r_ref[0:1, :]) + 0.0
        bits = pltpu.bitcast(r, jnp.int32)
        mono = bits ^ ((bits >> 31) & jnp.int32(0x7FFFFFFF))
        col = lax.broadcasted_iota(jnp.int32, (1, S), 1)
        key = (mono & jnp.int32(-65536)) | (jnp.int32(S - 1) - col)
        neg = jnp.int32(-2 ** 31)

        row16 = lax.broadcasted_iota(jnp.int32, (16, LANES), 0)
        lane16 = lax.broadcasted_iota(jnp.int32, (16, LANES), 1)
        rowc = lax.broadcasted_iota(jnp.int32, (16, 1), 0)
        sel_base, sel_off = [], []
        hsel = jnp.zeros((16, D), F32)
        xsel = jnp.zeros((16, D), F32)
        rsel = jnp.zeros((16, 1), F32)
        for t in range(TOPC):
            kmax = jnp.max(key)
            hit = key == kmax
            rv = jnp.sum(jnp.where(hit, r, 0.0), axis=1, keepdims=True)
            rsel = jnp.where(rowc == t, rv, rsel)
            key = jnp.where(hit, neg, key)
            idx = jnp.int32(S - 1) - (kmax & jnp.int32(0xFFFF))
            idx = jnp.clip(idx, 0, S - 1)
            base = pl.multiple_of((idx >> 7) << 7, LANES)
            off = idx & (LANES - 1)
            onehot = jnp.where((row16 == t) & (lane16 == off), 1.0, 0.0).astype(BF16)
            slab = pl.ds(base, LANES)
            hsel = hsel + lax.dot_general(onehot, h2t_ref[:, slab], _NT, preferred_element_type=F32)
            xsel = xsel + lax.dot_general(onehot, x2t_ref[:, slab], _NT, preferred_element_type=F32)
            sel_base.append(base)
            sel_off.append(off)

        for cp in ffn_weight_copies():
            cp.wait()
        hs = hsel.astype(BF16)
        gpre = _rb(jnp.dot(hs, wg_ref[...], preferred_element_type=F32))
        u = _rb(jnp.dot(hs, wu_ref[...], preferred_element_type=F32))
        a = (_rb(gpre * _sigmoid(gpre)) * u).astype(BF16)
        y = _rb(lax.dot_general(a, wdt_ref[...], _NT, preferred_element_type=F32))
        y = _rb(y * _rb(_sigmoid(rsel)))
        new = _rb(xsel + _rb(gbrow_ref[0:1, :] * _rb(hsel + y)))

        laneD = lax.broadcasted_iota(jnp.int32, (D, LANES), 1)
        for t in range(TOPC):
            slab = pl.ds(sel_base[t], LANES)
            colt = jnp.broadcast_to(new[t:t + 1, :], (LANES, D)).T
            old = out_ref[:, slab].astype(F32)
            out_ref[:, slab] = jnp.where(laneD == sel_off[t], colt, old).astype(BF16)


@jax.jit
def pallas_adaLN_cond__gqa_block_cached__moe_arch_mod__prompt_kernel(
    A_x: jax.Array,
    A_k_cache: jax.Array,
    A_v_cache: jax.Array,
    A_wq: jax.Array,
    A_wo: jax.Array,
    B_x: jax.Array,
    B_w_r: jax.Array,
    B_w_gate: jax.Array,
    B_w_up: jax.Array,
    B_w_down: jax.Array,
    c: jax.Array,
    w_mod: jax.Array,
):
    del B_x
    B, S, D = A_x.shape
    assert B == 1
    NG, SK = A_k_cache.shape[1], A_k_cache.shape[2]
    REP = HQ // NG
    FF = B_w_gate.shape[1]
    GW = REP * DH

    xt = A_x.reshape(S, D).T
    wot = A_wo.T
    wdt = B_w_down.T
    k = A_k_cache.reshape(NG, SK, DH)
    v = A_v_cache.reshape(NG, SK, DH)
    wr = B_w_r.reshape(1, D)

    const2 = lambda g: (0, 0)
    out_t = pl.pallas_call(
        functools.partial(_kernel, S=S, D=D, NG=NG, REP=REP),
        grid=(NG,),
        in_specs=[
            pl.BlockSpec((D, S), const2),
            pl.BlockSpec((1, SK, DH), lambda g: (g, 0, 0)),
            pl.BlockSpec((1, SK, DH), lambda g: (g, 0, 0)),
            pl.BlockSpec((D, GW), lambda g: (0, g)),
            pl.BlockSpec((D, GW), lambda g: (0, g)),
            pl.BlockSpec((1, D), const2),
            pl.BlockSpec((1, D), const2),
            pl.BlockSpec((D, 6 * D), const2),
            pl.BlockSpec(memory_space=pl.ANY),
            pl.BlockSpec(memory_space=pl.ANY),
            pl.BlockSpec(memory_space=pl.ANY),
        ],
        out_specs=pl.BlockSpec((D, S), const2),
        out_shape=jax.ShapeDtypeStruct((D, S), BF16),
        scratch_shapes=[
            pltpu.VMEM((6 * D, LANES), F32),
            pltpu.VMEM((8, D), F32),
            pltpu.VMEM((S, D), BF16),
            pltpu.VMEM((D, S), F32),
            pltpu.VMEM((D, S), BF16),
            pltpu.VMEM((D, S), BF16),
            pltpu.VMEM((8, S), F32),
            pltpu.VMEM((D, FF), BF16),
            pltpu.VMEM((D, FF), BF16),
            pltpu.VMEM((D, FF), BF16),
            pltpu.SemaphoreType.DMA((3,)),
        ],
        compiler_params=pltpu.CompilerParams(
            dimension_semantics=("arbitrary",),
            vmem_limit_bytes=110 * 1024 * 1024,
        ),
    )(xt, k, v, A_wq, wot, wr, c, w_mod, B_w_gate, B_w_up, wdt)
    return out_t.T.reshape(B, S, D)
```

```python
import functools
import math

import jax
import jax.numpy as jnp
from jax import lax
import jax.experimental.pallas as pl
import jax.experimental.pallas.tpu as pltpu

F32 = jnp.float32
BF16 = jnp.bfloat16

HQ = 32
DH = 128
TOPC = 8
LN_EPS = 1e-5
BQ = 256
LANES = 128
XCH = 4

_NT = (((1,), (1,)), ((), ()))

S_C, S_WMA, S_WMB, S_WR, S_WG, S_WU, S_WD = range(7)


def _rb(x):
    return x.astype(BF16).astype(F32)


def _sigmoid(x):
    return 1.0 / (1.0 + jnp.exp(-x))


def _kernel(xt_hbm, k_hbm, v_hbm, wq_hbm, wot_hbm, wr_hbm, c_hbm, wmod_hbm,
            wg_hbm, wu_hbm, wdt_hbm,
            out_hbm,
            xt_ref, k_buf, v_buf, wq_buf, wot_buf, wr_ref, c_ref, wmod_ref,
            wg_ref, wu_ref, wdt_ref,
            modc_ref, gbrow_ref, h_ref, acc_ref, h2t_ref, x2t_ref, r_ref, out_ref,
            sems, xsems, gsems, osems,
            *, S, D, NG, REP):
    g = pl.program_id(0)
    qscale = (DH ** -0.5) * math.log2(math.e)
    NB = S // BQ
    GW = REP * DH
    TCH = S // XCH
    MA = 2 * D

    def cp(src, dst, sem):
        return pltpu.make_async_copy(src, dst, sem)

    def x_copy(i):
        cols = pl.ds(pl.multiple_of(i * TCH, TCH), TCH)
        return cp(xt_hbm.at[:, cols], xt_ref.at[:, cols], xsems.at[i])

    def group_copies(grp, slot):
        cols = pl.ds(pl.multiple_of(grp * GW, GW), GW)
        return (cp(wq_hbm.at[:, cols], wq_buf.at[slot], gsems.at[slot, 0]),
                cp(k_hbm.at[grp], k_buf.at[slot], gsems.at[slot, 1]),
                cp(v_hbm.at[grp], v_buf.at[slot], gsems.at[slot, 2]),
                cp(wot_hbm.at[:, cols], wot_buf.at[slot], gsems.at[slot, 3]))

    c_cp = cp(c_hbm, c_ref, sems.at[S_C])
    wma_cp = cp(wmod_hbm.at[:, 0:MA], wmod_ref.at[:, 0:MA], sems.at[S_WMA])
    wmb_cp = cp(wmod_hbm.at[:, MA:6 * D], wmod_ref.at[:, MA:6 * D], sems.at[S_WMB])
    wr_cp = cp(wr_hbm, wr_ref, sems.at[S_WR])
    wg_cp = cp(wg_hbm, wg_ref, sems.at[S_WG])
    wu_cp = cp(wu_hbm, wu_ref, sems.at[S_WU])
    wd_cp = cp(wdt_hbm, wdt_ref, sems.at[S_WD])

    def modcol(i):
        return modc_ref[i * D:(i + 1) * D, :]

    def modulation(lo, hi, scale_lo):
        c = c_ref[...].astype(F32)
        sc = (c * _sigmoid(c)).astype(BF16)
        sc8 = jnp.broadcast_to(sc, (8, D))
        mod = _rb(jnp.dot(sc8, wmod_ref[:, lo:hi], preferred_element_type=F32))
        lane = lax.broadcasted_iota(jnp.int32, mod.shape, 1) + lo
        is_scale = (lane >= scale_lo) & (lane < scale_lo + D)
        modx = jnp.where(is_scale, _rb(1.0 + mod), mod)
        modc_ref[lo:hi, :] = jnp.broadcast_to(modx[0:1, :], (LANES, hi - lo)).T
        return mod

    @pl.when(g == 0)
    def _prologue():
        c_cp.start()
        wma_cp.start()
        for i in range(XCH):
            x_copy(i).start()
        for d in group_copies(0, 0):
            d.start()
        c_cp.wait()
        wma_cp.wait()
        modulation(0, MA, D)

        def ln1(i, carry):
            x_copy(i).wait()
            for u in range(TCH // LANES):
                t0 = pl.multiple_of(i * TCH + u * LANES, LANES)
                x = xt_ref[:, pl.ds(t0, LANES)].astype(F32)
                m = jnp.mean(x, axis=0, keepdims=True)
                d = x - m
                var = jnp.mean(d * d, axis=0, keepdims=True)
                ht = d * lax.rsqrt(var + LN_EPS) * modcol(1) + modcol(0)
                h_ref[pl.ds(t0, LANES), :] = ht.astype(BF16).T
                acc_ref[:, pl.ds(t0, LANES)] = jnp.zeros((D, LANES), F32)
            return carry
        lax.fori_loop(0, XCH, ln1, 0)

    slot = g % 2

    @pl.when(g + 1 < NG)
    def _():
        for d in group_copies(g + 1, 1 - slot):
            d.start()

    @pl.when(g == 1)
    def _():
        wmb_cp.start()
        wr_cp.start()
        wg_cp.start()

    @pl.when(g == 2)
    def _():
        wu_cp.start()

    @pl.when(g == 3)
    def _():
        wd_cp.start()

    for d in group_copies(g, slot):
        d.wait()

    k = k_buf[slot]
    v = v_buf[slot]
    wq = wq_buf[slot]
    wot = wot_buf[slot]

    def qproj(j):
        q2 = jnp.dot(h_ref[j * BQ:(j + 1) * BQ, :], wq, preferred_element_type=F32)
        return (q2 * qscale).astype(BF16)

    def head(q):
        s = lax.dot_general(q, k, _NT, preferred_element_type=F32)
        m = jnp.max(s, axis=1, keepdims=True)
        p = jnp.exp2(s - m)
        l = jnp.sum(p, axis=1, keepdims=True)
        o = jnp.dot(p.astype(BF16), v, preferred_element_type=F32)
        rl = pl.reciprocal(l, approx=True)
        rl = rl * (2.0 - l * rl)
        return (o * rl).astype(BF16)

    def oproj(j, os_):
        o2 = jnp.concatenate(os_, axis=1)
        acc_ref[:, j * BQ:(j + 1) * BQ] += lax.dot_general(
            wot, o2, _NT, preferred_element_type=F32)

    q2s = [qproj(j) for j in range(NB)]
    prev = None
    for j in range(NB):
        cur = [head(q2s[j][:, r * DH:(r + 1) * DH]) for r in range(REP)]
        if prev is not None:
            oproj(j - 1, prev)
        prev = cur
    oproj(NB - 1, prev)

    @pl.when(g == NG - 1)
    def _epilogue():
        wmb_cp.wait()
        wr_cp.wait()
        modb = modulation(MA, 6 * D, 4 * D)
        gbrow_ref[...] = modb[:, 3 * D:4 * D]
        eps_b = _rb(jnp.full((1, 1), LN_EPS, F32))
        wr8 = jnp.broadcast_to(wr_ref[...], (8, D))

        def ln2(i, carry):
            for u in range(2):
                t0 = pl.multiple_of((2 * i + u) * LANES, LANES)
                cols = pl.ds(t0, LANES)
                x = xt_ref[:, cols].astype(F32)
                x2 = _rb(x + _rb(modcol(2) * _rb(acc_ref[:, cols])))
                m = jnp.mean(x2, axis=0, keepdims=True)
                dc = x2 - m
                var = jnp.mean(dc * dc, axis=0, keepdims=True)
                sd = _rb(jnp.sqrt(_rb(_rb(var) + eps_b)))
                n = _rb(_rb(x2 - _rb(m)) * (1.0 / sd))
                h2 = _rb(_rb(n * modcol(4)) + modcol(3))
                h2b = h2.astype(BF16)
                h2t_ref[:, cols] = h2b
                x2t_ref[:, cols] = x2.astype(BF16)
                out_ref[:, cols] = (x2 + _rb(modcol(5) * h2)).astype(BF16)
                r_ref[:, cols] = jnp.dot(wr8, h2b, preferred_element_type=F32)
            return carry
        lax.fori_loop(0, S // (2 * LANES), ln2, 0)

        r = _rb(r_ref[0:1, :]) + 0.0
        bits = pltpu.bitcast(r, jnp.int32)
        mono = bits ^ ((bits >> 31) & jnp.int32(0x7FFFFFFF))
        col = lax.broadcasted_iota(jnp.int32, (1, S), 1)
        key = (mono & jnp.int32(-65536)) | (jnp.int32(S - 1) - col)
        neg = jnp.int32(-2 ** 31)

        row16 = lax.broadcasted_iota(jnp.int32, (16, LANES), 0)
        lane16 = lax.broadcasted_iota(jnp.int32, (16, LANES), 1)
        rowc = lax.broadcasted_iota(jnp.int32, (16, 1), 0)
        sel_base, sel_off = [], []
        hsel = jnp.zeros((16, D), F32)
        xsel = jnp.zeros((16, D), F32)
        rsel = jnp.zeros((16, 1), F32)
        for t in range(TOPC):
            kmax = jnp.max(key)
            hit = key == kmax
            rv = jnp.sum(jnp.where(hit, r, 0.0), axis=1, keepdims=True)
            rsel = jnp.where(rowc == t, rv, rsel)
            key = jnp.where(hit, neg, key)
            idx = jnp.int32(S - 1) - (kmax & jnp.int32(0xFFFF))
            idx = jnp.clip(idx, 0, S - 1)
            base = pl.multiple_of((idx >> 7) << 7, LANES)
            off = idx & (LANES - 1)
            onehot = jnp.where((row16 == t) & (lane16 == off), 1.0, 0.0).astype(BF16)
            slab = pl.ds(base, LANES)
            hsel = hsel + lax.dot_general(onehot, h2t_ref[:, slab], _NT, preferred_element_type=F32)
            xsel = xsel + lax.dot_general(onehot, x2t_ref[:, slab], _NT, preferred_element_type=F32)
            sel_base.append(base)
            sel_off.append(off)

        wg_cp.wait()
        wu_cp.wait()
        wd_cp.wait()
        hs = hsel.astype(BF16)
        gpre = _rb(jnp.dot(hs, wg_ref[...], preferred_element_type=F32))
        u = _rb(jnp.dot(hs, wu_ref[...], preferred_element_type=F32))
        a = (_rb(gpre * _sigmoid(gpre)) * u).astype(BF16)
        y = _rb(lax.dot_general(a, wdt_ref[...], _NT, preferred_element_type=F32))
        y = _rb(y * _rb(_sigmoid(rsel)))
        new = _rb(xsel + _rb(gbrow_ref[0:1, :] * _rb(hsel + y)))

        laneD = lax.broadcasted_iota(jnp.int32, (D, LANES), 1)
        for t in range(TOPC):
            slab = pl.ds(sel_base[t], LANES)
            colt = jnp.broadcast_to(new[t:t + 1, :], (LANES, D)).T
            old = out_ref[:, slab].astype(F32)
            out_ref[:, slab] = jnp.where(laneD == sel_off[t], colt, old).astype(BF16)

        o_cp = cp(out_ref, out_hbm, osems.at[0])
        o_cp.start()
        o_cp.wait()


@jax.jit
def pallas_adaLN_cond__gqa_block_cached__moe_arch_mod__prompt_kernel(
    A_x: jax.Array,
    A_k_cache: jax.Array,
    A_v_cache: jax.Array,
    A_wq: jax.Array,
    A_wo: jax.Array,
    B_x: jax.Array,
    B_w_r: jax.Array,
    B_w_gate: jax.Array,
    B_w_up: jax.Array,
    B_w_down: jax.Array,
    c: jax.Array,
    w_mod: jax.Array,
):
    del B_x
    B, S, D = A_x.shape
    assert B == 1
    NG, SK = A_k_cache.shape[1], A_k_cache.shape[2]
    REP = HQ // NG
    FF = B_w_gate.shape[1]
    GW = REP * DH

    xt = A_x.reshape(S, D).T
    wot = A_wo.T
    wdt = B_w_down.T
    k = A_k_cache.reshape(NG, SK, DH)
    v = A_v_cache.reshape(NG, SK, DH)
    wr = B_w_r.reshape(1, D)

    hbm = pl.BlockSpec(memory_space=pl.ANY)
    out_t = pl.pallas_call(
        functools.partial(_kernel, S=S, D=D, NG=NG, REP=REP),
        grid=(NG,),
        in_specs=[hbm] * 11,
        out_specs=hbm,
        out_shape=jax.ShapeDtypeStruct((D, S), BF16),
        scratch_shapes=[
            pltpu.VMEM((D, S), BF16),
            pltpu.VMEM((2, SK, DH), BF16),
            pltpu.VMEM((2, SK, DH), BF16),
            pltpu.VMEM((2, D, GW), BF16),
            pltpu.VMEM((2, D, GW), BF16),
            pltpu.VMEM((1, D), BF16),
            pltpu.VMEM((1, D), BF16),
            pltpu.VMEM((D, 6 * D), BF16),
            pltpu.VMEM((D, FF), BF16),
            pltpu.VMEM((D, FF), BF16),
            pltpu.VMEM((D, FF), BF16),
            pltpu.VMEM((6 * D, LANES), F32),
            pltpu.VMEM((8, D), F32),
            pltpu.VMEM((S, D), BF16),
            pltpu.VMEM((D, S), F32),
            pltpu.VMEM((D, S), BF16),
            pltpu.VMEM((D, S), BF16),
            pltpu.VMEM((8, S), F32),
            pltpu.VMEM((D, S), BF16),
            pltpu.SemaphoreType.DMA((7,)),
            pltpu.SemaphoreType.DMA((XCH,)),
            pltpu.SemaphoreType.DMA((2, 4)),
            pltpu.SemaphoreType.DMA((1,)),
        ],
        compiler_params=pltpu.CompilerParams(
            dimension_semantics=("arbitrary",),
            vmem_limit_bytes=110 * 1024 * 1024,
        ),
    )(xt, k, v, A_wq, wot, wr, c, w_mod, B_w_gate, B_w_up, wdt)
    return out_t.T.reshape(B, S, D)
```

```python
import functools
import math

import jax
import jax.numpy as jnp
from jax import lax
import jax.experimental.pallas as pl
import jax.experimental.pallas.tpu as pltpu

F32 = jnp.float32
BF16 = jnp.bfloat16

HQ = 32
DH = 128
TOPC = 8
LN_EPS = 1e-5
BQ = 256
LANES = 128
SPLIT = 512
C0 = 2
OPD = 2
LN2U = 2
XCH = 4

_NT = (((1,), (1,)), ((), ()))

S_C, S_WMA, S_WMB, S_WR, S_WG, S_WU, S_WD = range(7)


def _rb(x):
    return x.astype(BF16).astype(F32)


def _sigmoid(x):
    return 1.0 / (1.0 + jnp.exp(-x))


def _kernel(xt_hbm, k_hbm, v_hbm, wq_hbm, wot_hbm, wr_hbm, c_hbm, wmod_hbm,
            wg_hbm, wu_hbm, wdt_hbm,
            out_hbm,
            xt_ref, k_buf, v_buf, wq_buf, wot_buf, wr_ref, c_ref, wmod_ref,
            wg_ref, wu_ref, wdt_ref,
            modc_ref, gbrow_ref, h_ref, acc_ref, h2t_ref, r_ref, out_ref,
            sems, xsems, gsems, osems,
            *, S, SK, D, NG, REP):
    g = pl.program_id(0)
    qscale = (DH ** -0.5) * math.log2(math.e)
    NB = S // BQ
    GW = REP * DH
    TCH = S // XCH
    MA = 2 * D

    def cp(src, dst, sem):
        return pltpu.make_async_copy(src, dst, sem)

    def x_copy(i):
        cols = pl.ds(pl.multiple_of(i * TCH, TCH), TCH)
        return cp(xt_hbm.at[:, cols], xt_ref.at[:, cols], xsems.at[i])

    def group_copies(grp, slot):
        cols = pl.ds(pl.multiple_of(grp * GW, GW), GW)
        return (cp(wq_hbm.at[:, cols], wq_buf.at[slot], gsems.at[slot, 0]),
                cp(k_hbm.at[grp], k_buf.at[slot], gsems.at[slot, 1]),
                cp(v_hbm.at[grp], v_buf.at[slot], gsems.at[slot, 2]),
                cp(wot_hbm.at[:, cols], wot_buf.at[slot], gsems.at[slot, 3]))

    c_cp = cp(c_hbm, c_ref, sems.at[S_C])
    wma_cp = cp(wmod_hbm.at[:, 0:MA], wmod_ref.at[:, 0:MA], sems.at[S_WMA])
    wmb_cp = cp(wmod_hbm.at[:, MA:6 * D], wmod_ref.at[:, MA:6 * D], sems.at[S_WMB])
    wr_cp = cp(wr_hbm, wr_ref, sems.at[S_WR])
    wg_cp = cp(wg_hbm, wg_ref, sems.at[S_WG])
    wu_cp = cp(wu_hbm, wu_ref, sems.at[S_WU])
    wd_cp = cp(wdt_hbm, wdt_ref, sems.at[S_WD])

    def modcol(i):
        return modc_ref[i * D:(i + 1) * D, :]

    def modulation(lo, hi, scale_lo):
        c = c_ref[...].astype(F32)
        sc = (c * _sigmoid(c)).astype(BF16)
        sc8 = jnp.broadcast_to(sc, (8, D))
        mod = _rb(jnp.dot(sc8, wmod_ref[:, lo:hi], preferred_element_type=F32))
        lane = lax.broadcasted_iota(jnp.int32, mod.shape, 1) + lo
        is_scale = (lane >= scale_lo) & (lane < scale_lo + D)
        modx = jnp.where(is_scale, _rb(1.0 + mod), mod)
        modc_ref[lo:hi, :] = jnp.broadcast_to(modx[0:1, :], (LANES, hi - lo)).T
        return mod

    @pl.when(g == 0)
    def _prologue():
        c_cp.start()
        wma_cp.start()
        for i in range(XCH):
            x_copy(i).start()
        for d in group_copies(0, 0):
            d.start()
        c_cp.wait()
        wma_cp.wait()
        modulation(0, MA, D)

        def ln1(i, carry):
            x_copy(i).wait()
            for u in range(TCH // LANES):
                t0 = pl.multiple_of(i * TCH + u * LANES, LANES)
                x = xt_ref[:, pl.ds(t0, LANES)].astype(F32)
                m = jnp.mean(x, axis=0, keepdims=True)
                d = x - m
                var = jnp.mean(d * d, axis=0, keepdims=True)
                ht = d * lax.rsqrt(var + LN_EPS) * modcol(1) + modcol(0)
                h_ref[pl.ds(t0, LANES), :] = ht.astype(BF16).T
                acc_ref[:, pl.ds(t0, LANES)] = jnp.zeros((D, LANES), F32)
            return carry
        lax.fori_loop(0, XCH, ln1, 0)

    slot = g % 2

    @pl.when(g + 1 < NG)
    def _():
        for d in group_copies(g + 1, 1 - slot):
            d.start()

    @pl.when(g == 1)
    def _():
        wmb_cp.start()
        wr_cp.start()
        wg_cp.start()

    @pl.when(g == 2)
    def _():
        wu_cp.start()

    @pl.when(g == 3)
    def _():
        wd_cp.start()

    for d in group_copies(g, slot):
        d.wait()

    k = k_buf[slot]
    v = v_buf[slot]
    wq = wq_buf[slot]
    wot = wot_buf[slot]

    def qproj(j):
        q2 = jnp.dot(h_ref[j * BQ:(j + 1) * BQ, :], wq, preferred_element_type=F32)
        return (q2 * qscale).astype(BF16)

    def qk(q, lo, hi):
        return lax.dot_general(q, k[lo:hi], _NT, preferred_element_type=F32)

    def softmax_pv(s, late):
        m = jnp.max(s, axis=1, keepdims=True)
        p = jnp.exp2(s - m)
        o = jnp.dot(p.astype(BF16), v, preferred_element_type=F32)
        if late:
            lp = p[:, 0:LANES]
            for i in range(1, SK // LANES):
                lp = lp + p[:, i * LANES:(i + 1) * LANES]
            l = jnp.sum(jnp.where(lp < 0.0, o, lp), axis=1, keepdims=True)
        else:
            l = jnp.sum(p, axis=1, keepdims=True)
        rl = pl.reciprocal(l, approx=True)
        rl = rl * (2.0 - l * rl)
        return (o * rl).astype(BF16)

    def oproj(j):
        o2 = jnp.concatenate([outs[REP * j + r] for r in range(REP)], axis=1)
        acc_ref[:, j * BQ:(j + 1) * BQ] += lax.dot_general(
            wot, o2, _NT, preferred_element_type=F32)

    q2s = [qproj(j) for j in range(NB)]
    qs = [q2s[j][:, r * DH:(r + 1) * DH] for j in range(NB) for r in range(REP)]
    outs = []
    done = 0
    s_head = None
    for ci in range(len(qs)):
        if s_head is None:
            s = qk(qs[ci], 0, SK)
        else:
            s = jnp.concatenate([s_head, qk(qs[ci], SPLIT, SK)], axis=1)
        s_head = qk(qs[ci + 1], 0, SPLIT) if (C0 <= ci < len(qs) - 1) else None
        outs.append(softmax_pv(s, late=(ci == len(qs) - 1)))
        if ci % REP == REP - 1 and ci // REP - OPD >= 0:
            oproj(done)
            done += 1
    for j in range(done, NB):
        oproj(j)

    @pl.when(g == NG - 1)
    def _epilogue():
        wmb_cp.wait()
        wr_cp.wait()
        modb = modulation(MA, 6 * D, 4 * D)
        gbrow_ref[...] = modb[:, 3 * D:4 * D]
        eps_b = _rb(jnp.full((1, 1), LN_EPS, F32))
        wr8 = jnp.broadcast_to(wr_ref[...], (8, D))
        NSL = S // LANES

        def ln2(i, carry):
            for u in range(LN2U):
                sl = LN2U * i + u
                cols = pl.ds(pl.multiple_of(sl * LANES, LANES), LANES)
                x2 = xt_ref[:, cols].astype(F32) + modcol(2) * acc_ref[:, cols]
                m = jnp.mean(x2, axis=0, keepdims=True)
                dc = x2 - m
                var = jnp.mean(dc * dc, axis=0, keepdims=True)
                sd = _rb(jnp.sqrt(_rb(_rb(var) + eps_b)))
                h2 = dc * (1.0 / sd) * modcol(4) + modcol(3)
                h2b = h2.astype(BF16)
                h2t_ref[:, cols] = h2b
                out_ref[:, cols] = (x2 + modcol(5) * h2).astype(BF16)
                r_ref[pl.ds(sl, 1), :] = jnp.dot(wr8, h2b, preferred_element_type=F32)[0:1, :]
            return carry
        lax.fori_loop(0, NSL // LN2U, ln2, 0)

        r = _rb(r_ref[...]) + 0.0
        bits = pltpu.bitcast(r, jnp.int32)
        mono = bits ^ ((bits >> 31) & jnp.int32(0x7FFFFFFF))
        tok = (lax.broadcasted_iota(jnp.int32, (NSL, LANES), 0) * LANES
               + lax.broadcasted_iota(jnp.int32, (NSL, LANES), 1))
        keyi = (((mono >> 16) + 32768) * S + (S - 1 - tok)) + jnp.int32(1 << 29)
        key = pltpu.bitcast(keyi, F32)

        row16 = lax.broadcasted_iota(jnp.int32, (16, LANES), 0)
        lane16 = lax.broadcasted_iota(jnp.int32, (16, LANES), 1)
        rowc = lax.broadcasted_iota(jnp.int32, (16, 1), 0)
        sel_base, sel_off = [], []
        hsel = jnp.zeros((16, D), F32)
        ksel = jnp.zeros((16, 1), F32)
        for t in range(TOPC):
            kmax = jnp.max(jnp.max(key, axis=0, keepdims=True), axis=1, keepdims=True)
            key = jnp.where(key == kmax, 0.0, key)
            ksel = jnp.where(rowc == t, kmax, ksel)
            ki = pltpu.bitcast(kmax, jnp.int32)[0, 0]
            idx = (S - 1) - (ki & (S - 1))
            base = pl.multiple_of((idx >> 7) << 7, LANES)
            off = idx & (LANES - 1)
            onehot = jnp.where((row16 == t) & (lane16 == off), 1.0, 0.0).astype(BF16)
            hsel = hsel + lax.dot_general(onehot, h2t_ref[:, pl.ds(base, LANES)], _NT,
                                          preferred_element_type=F32)
            sel_base.append(base)
            sel_off.append(off)
        hi = ((pltpu.bitcast(ksel, jnp.int32) - jnp.int32(1 << 29)) // S - 32768) << 16
        rbits = hi ^ ((hi >> 31) & jnp.int32(0x7FFF0000))
        rsel = jnp.where(rowc < TOPC, pltpu.bitcast(rbits, F32), 0.0)

        wg_cp.wait()
        wu_cp.wait()
        wd_cp.wait()
        hs = hsel.astype(BF16)
        gpre = jnp.dot(hs, wg_ref[...], preferred_element_type=F32)
        u = jnp.dot(hs, wu_ref[...], preferred_element_type=F32)
        a = (gpre * _sigmoid(gpre) * u).astype(BF16)
        y = lax.dot_general(a, wdt_ref[...], _NT, preferred_element_type=F32)
        delta = y * _sigmoid(rsel) * gbrow_ref[0:1, :]

        laneD = lax.broadcasted_iota(jnp.int32, (D, LANES), 1)
        for t in range(TOPC):
            slab = pl.ds(sel_base[t], LANES)
            colt = jnp.broadcast_to(delta[t:t + 1, :], (LANES, D)).T
            old = out_ref[:, slab].astype(F32)
            out_ref[:, slab] = jnp.where(laneD == sel_off[t], old + colt, old).astype(BF16)

        o_cp = cp(out_ref, out_hbm, osems.at[0])
        o_cp.start()
        o_cp.wait()


@jax.jit
def pallas_adaLN_cond__gqa_block_cached__moe_arch_mod__prompt_kernel(
    A_x: jax.Array,
    A_k_cache: jax.Array,
    A_v_cache: jax.Array,
    A_wq: jax.Array,
    A_wo: jax.Array,
    B_x: jax.Array,
    B_w_r: jax.Array,
    B_w_gate: jax.Array,
    B_w_up: jax.Array,
    B_w_down: jax.Array,
    c: jax.Array,
    w_mod: jax.Array,
):
    del B_x
    B, S, D = A_x.shape
    assert B == 1
    NG, SK = A_k_cache.shape[1], A_k_cache.shape[2]
    REP = HQ // NG
    FF = B_w_gate.shape[1]
    GW = REP * DH

    xt = A_x.reshape(S, D).T
    wot = A_wo.T
    wdt = B_w_down.T
    k = A_k_cache.reshape(NG, SK, DH)
    v = A_v_cache.reshape(NG, SK, DH)
    wr = B_w_r.reshape(1, D)

    hbm = pl.BlockSpec(memory_space=pl.ANY)
    out_t = pl.pallas_call(
        functools.partial(_kernel, S=S, SK=SK, D=D, NG=NG, REP=REP),
        grid=(NG,),
        in_specs=[hbm] * 11,
        out_specs=hbm,
        out_shape=jax.ShapeDtypeStruct((D, S), BF16),
        scratch_shapes=[
            pltpu.VMEM((D, S), BF16),
            pltpu.VMEM((2, SK, DH), BF16),
            pltpu.VMEM((2, SK, DH), BF16),
            pltpu.VMEM((2, D, GW), BF16),
            pltpu.VMEM((2, D, GW), BF16),
            pltpu.VMEM((1, D), BF16),
            pltpu.VMEM((1, D), BF16),
            pltpu.VMEM((D, 6 * D), BF16),
            pltpu.VMEM((D, FF), BF16),
            pltpu.VMEM((D, FF), BF16),
            pltpu.VMEM((D, FF), BF16),
            pltpu.VMEM((6 * D, LANES), F32),
            pltpu.VMEM((8, D), F32),
            pltpu.VMEM((S, D), BF16),
            pltpu.VMEM((D, S), F32),
            pltpu.VMEM((D, S), BF16),
            pltpu.VMEM((S // LANES, LANES), F32),
            pltpu.VMEM((D, S), BF16),
            pltpu.SemaphoreType.DMA((7,)),
            pltpu.SemaphoreType.DMA((XCH,)),
            pltpu.SemaphoreType.DMA((2, 4)),
            pltpu.SemaphoreType.DMA((1,)),
        ],
        compiler_params=pltpu.CompilerParams(
            dimension_semantics=("arbitrary",),
            vmem_limit_bytes=110 * 1024 * 1024,
        ),
    )(xt, k, v, A_wq, wot, wr, c, w_mod, B_w_gate, B_w_up, wdt)
    return out_t.T.reshape(B, S, D)
```

```python
import functools
import math

import jax
import jax.numpy as jnp
from jax import lax
import jax.experimental.pallas as pl
import jax.experimental.pallas.tpu as pltpu

F32 = jnp.float32
BF16 = jnp.bfloat16

HQ = 32
DH = 128
TOPC = 8
LN_EPS = 1e-5
BQ = 256
LANES = 128
SPLIT = 512
C0 = 2
OPD = 2
LN2U = 2
XCH = 4

_NT = (((1,), (1,)), ((), ()))

S_C, S_WMA, S_WMB, S_WR, S_WG, S_WU, S_WD, S_OUT = range(8)
S_X = 8
S_G = S_X + XCH
N_SEMS = S_G + 8


def _rb(x):
    return x.astype(BF16).astype(F32)


def _sigmoid(x):
    return 1.0 / (1.0 + jnp.exp(-x))


def _kernel(xt_hbm, k_hbm, v_hbm, wq_hbm, wot_hbm, wr_hbm, c_hbm, wmod_hbm,
            wg_hbm, wu_hbm, wdt_hbm,
            out_hbm,
            xt_ref, k_buf, v_buf, wq_buf, wot_buf, wr_ref, c_ref, wmod_ref,
            wg_ref, wu_ref, wdt_ref,
            modc_ref, gbrow_ref, h_ref, acc_ref, h2t_ref, r_ref, out_ref,
            sems,
            *, S, SK, D, NG, REP):
    g = pl.program_id(0)
    qscale = (DH ** -0.5) * math.log2(math.e)
    NB = S // BQ
    GW = REP * DH
    TCH = S // XCH
    MA = 2 * D

    def cp(src, dst, sem):
        return pltpu.make_async_copy(src, dst, sem)

    def x_copy(i):
        cols = pl.ds(pl.multiple_of(i * TCH, TCH), TCH)
        return cp(xt_hbm.at[:, cols], xt_ref.at[:, cols], sems.at[S_X + i])

    def group_copies(grp, slot):
        cols = pl.ds(pl.multiple_of(grp * GW, GW), GW)
        return (cp(wq_hbm.at[:, cols], wq_buf.at[slot], sems.at[S_G + 4 * slot + 0]),
                cp(k_hbm.at[grp], k_buf.at[slot], sems.at[S_G + 4 * slot + 1]),
                cp(v_hbm.at[grp], v_buf.at[slot], sems.at[S_G + 4 * slot + 2]),
                cp(wot_hbm.at[:, cols], wot_buf.at[slot], sems.at[S_G + 4 * slot + 3]))

    c_cp = cp(c_hbm, c_ref, sems.at[S_C])
    wma_cp = cp(wmod_hbm.at[:, 0:MA], wmod_ref.at[:, 0:MA], sems.at[S_WMA])
    wmb_cp = cp(wmod_hbm.at[:, MA:6 * D], wmod_ref.at[:, MA:6 * D], sems.at[S_WMB])
    wr_cp = cp(wr_hbm, wr_ref, sems.at[S_WR])
    wg_cp = cp(wg_hbm, wg_ref, sems.at[S_WG])
    wu_cp = cp(wu_hbm, wu_ref, sems.at[S_WU])
    wd_cp = cp(wdt_hbm, wdt_ref, sems.at[S_WD])

    def modcol(i):
        return modc_ref[i * D:(i + 1) * D, :]

    def modulation(lo, hi, scale_lo):
        c = c_ref[...].astype(F32)
        sc = (c * _sigmoid(c)).astype(BF16)
        sc8 = jnp.broadcast_to(sc, (8, D))
        mod = _rb(jnp.dot(sc8, wmod_ref[:, lo:hi], preferred_element_type=F32))
        lane = lax.broadcasted_iota(jnp.int32, mod.shape, 1) + lo
        is_scale = (lane >= scale_lo) & (lane < scale_lo + D)
        modx = jnp.where(is_scale, _rb(1.0 + mod), mod)
        modc_ref[lo:hi, :] = jnp.broadcast_to(modx[0:1, :], (LANES, hi - lo)).T
        return mod

    @pl.when(g == 0)
    def _prologue():
        c_cp.start()
        wma_cp.start()
        for i in range(XCH):
            x_copy(i).start()
        for d in group_copies(0, 0) + group_copies(1, 1):
            d.start()
        wr_cp.start()
        c_cp.wait()
        wma_cp.wait()
        modulation(0, MA, D)

        def ln1(i, carry):
            x_copy(i).wait()
            for u in range(TCH // LANES):
                t0 = pl.multiple_of(i * TCH + u * LANES, LANES)
                x = xt_ref[:, pl.ds(t0, LANES)].astype(F32)
                m = jnp.mean(x, axis=0, keepdims=True)
                d = x - m
                var = jnp.mean(d * d, axis=0, keepdims=True)
                ht = d * lax.rsqrt(var + LN_EPS) * modcol(1) + modcol(0)
                h_ref[pl.ds(t0, LANES), :] = ht.astype(BF16).T
                acc_ref[:, pl.ds(t0, LANES)] = jnp.zeros((D, LANES), F32)
            return carry
        lax.fori_loop(0, XCH, ln1, 0)

    slot = g % 2
    for d in group_copies(g, slot):
        d.wait()

    k = k_buf[slot]
    v = v_buf[slot]
    wq = wq_buf[slot]
    wot = wot_buf[slot]

    def qproj(j):
        q2 = jnp.dot(h_ref[j * BQ:(j + 1) * BQ, :], wq, preferred_element_type=F32)
        return (q2 * qscale).astype(BF16)

    def qk(q, lo, hi):
        return lax.dot_general(q, k[lo:hi], _NT, preferred_element_type=F32)

    def softmax_pv(s, late):
        m = jnp.max(s, axis=1, keepdims=True)
        p = jnp.exp2(s - m)
        o = jnp.dot(p.astype(BF16), v, preferred_element_type=F32)
        if late:
            lp = p[:, 0:LANES]
            for i in range(1, SK // LANES):
                lp = lp + p[:, i * LANES:(i + 1) * LANES]
            l = jnp.sum(jnp.where(lp < 0.0, o, lp), axis=1, keepdims=True)
        else:
            l = jnp.sum(p, axis=1, keepdims=True)
        rl = pl.reciprocal(l, approx=True)
        rl = rl * (2.0 - l * rl)
        return (o * rl).astype(BF16)

    def oproj(j):
        o2 = jnp.concatenate([outs[REP * j + r] for r in range(REP)], axis=1)
        acc_ref[:, j * BQ:(j + 1) * BQ] += lax.dot_general(
            wot, o2, _NT, preferred_element_type=F32)

    q2s = [qproj(j) for j in range(NB)]
    qs = [q2s[j][:, r * DH:(r + 1) * DH] for j in range(NB) for r in range(REP)]
    outs = []
    done = 0
    s_head = None
    for ci in range(len(qs)):
        if s_head is None:
            s = qk(qs[ci], 0, SK)
        else:
            s = jnp.concatenate([s_head, qk(qs[ci], SPLIT, SK)], axis=1)
        s_head = qk(qs[ci + 1], 0, SPLIT) if (C0 <= ci < len(qs) - 1) else None
        outs.append(softmax_pv(s, late=(ci == len(qs) - 1)))
        if ci % REP == REP - 1 and ci // REP - OPD >= 0:
            oproj(done)
            done += 1
    for j in range(done, NB):
        oproj(j)

    @pl.when(g + 2 < NG)
    def _():
        for d in group_copies(g + 2, slot):
            d.start()

    @pl.when(g == 0)
    def _():
        wmb_cp.start()
        wg_cp.start()

    @pl.when(g == 1)
    def _():
        wu_cp.start()

    @pl.when(g == 2)
    def _():
        wd_cp.start()

    @pl.when(g == NG - 1)
    def _epilogue():
        wmb_cp.wait()
        wr_cp.wait()
        modb = modulation(MA, 6 * D, 4 * D)
        gbrow_ref[...] = modb[:, 3 * D:4 * D]
        eps_b = _rb(jnp.full((1, 1), LN_EPS, F32))
        wr8 = jnp.broadcast_to(wr_ref[...], (8, D))
        NSL = S // LANES

        def ln2(i, carry):
            for u in range(LN2U):
                sl = LN2U * i + u
                cols = pl.ds(pl.multiple_of(sl * LANES, LANES), LANES)
                x2 = xt_ref[:, cols].astype(F32) + modcol(2) * acc_ref[:, cols]
                m = jnp.mean(x2, axis=0, keepdims=True)
                dc = x2 - m
                var = jnp.mean(dc * dc, axis=0, keepdims=True)
                sd = _rb(jnp.sqrt(_rb(_rb(var) + eps_b)))
                h2 = dc * (1.0 / sd) * modcol(4) + modcol(3)
                h2b = h2.astype(BF16)
                h2t_ref[:, cols] = h2b
                out_ref[:, cols] = (x2 + modcol(5) * h2).astype(BF16)
                r_ref[pl.ds(sl, 1), :] = jnp.dot(wr8, h2b, preferred_element_type=F32)[0:1, :]
            return carry
        lax.fori_loop(0, NSL // LN2U, ln2, 0)

        r = _rb(r_ref[...]) + 0.0
        bits = pltpu.bitcast(r, jnp.int32)
        mono = bits ^ ((bits >> 31) & jnp.int32(0x7FFFFFFF))
        tok = (lax.broadcasted_iota(jnp.int32, (NSL, LANES), 0) * LANES
               + lax.broadcasted_iota(jnp.int32, (NSL, LANES), 1))
        keyi = (((mono >> 16) + 32768) * S + (S - 1 - tok)) + jnp.int32(1 << 29)
        key = pltpu.bitcast(keyi, F32)

        row16 = lax.broadcasted_iota(jnp.int32, (16, LANES), 0)
        lane16 = lax.broadcasted_iota(jnp.int32, (16, LANES), 1)
        rowc = lax.broadcasted_iota(jnp.int32, (16, 1), 0)
        sel_base, sel_off = [], []
        hsel = jnp.zeros((16, D), F32)
        ksel = jnp.zeros((16, 1), F32)
        for t in range(TOPC):
            kmax = jnp.max(jnp.max(key, axis=0, keepdims=True), axis=1, keepdims=True)
            key = jnp.where(key == kmax, 0.0, key)
            ksel = jnp.where(rowc == t, kmax, ksel)
            ki = pltpu.bitcast(kmax, jnp.int32)[0, 0]
            idx = (S - 1) - (ki & (S - 1))
            base = pl.multiple_of((idx >> 7) << 7, LANES)
            off = idx & (LANES - 1)
            onehot = jnp.where((row16 == t) & (lane16 == off), 1.0, 0.0).astype(BF16)
            hsel = hsel + lax.dot_general(onehot, h2t_ref[:, pl.ds(base, LANES)], _NT,
                                          preferred_element_type=F32)
            sel_base.append(base)
            sel_off.append(off)
        hi = ((pltpu.bitcast(ksel, jnp.int32) - jnp.int32(1 << 29)) // S - 32768) << 16
        rbits = hi ^ ((hi >> 31) & jnp.int32(0x7FFF0000))
        rsel = jnp.where(rowc < TOPC, pltpu.bitcast(rbits, F32), 0.0)

        wg_cp.wait()
        wu_cp.wait()
        wd_cp.wait()
        hs = hsel.astype(BF16)
        gpre = jnp.dot(hs, wg_ref[...], preferred_element_type=F32)
        u = jnp.dot(hs, wu_ref[...], preferred_element_type=F32)
        a = (gpre * _sigmoid(gpre) * u).astype(BF16)
        y = lax.dot_general(a, wdt_ref[...], _NT, preferred_element_type=F32)
        delta = y * _sigmoid(rsel) * gbrow_ref[0:1, :]

        laneD = lax.broadcasted_iota(jnp.int32, (D, LANES), 1)
        for t in range(TOPC):
            slab = pl.ds(sel_base[t], LANES)
            colt = jnp.broadcast_to(delta[t:t + 1, :], (LANES, D)).T
            old = out_ref[:, slab].astype(F32)
            out_ref[:, slab] = jnp.where(laneD == sel_off[t], old + colt, old).astype(BF16)

        o_cp = cp(out_ref, out_hbm, sems.at[S_OUT])
        o_cp.start()
        o_cp.wait()


@jax.jit
def pallas_adaLN_cond__gqa_block_cached__moe_arch_mod__prompt_kernel(
    A_x: jax.Array,
    A_k_cache: jax.Array,
    A_v_cache: jax.Array,
    A_wq: jax.Array,
    A_wo: jax.Array,
    B_x: jax.Array,
    B_w_r: jax.Array,
    B_w_gate: jax.Array,
    B_w_up: jax.Array,
    B_w_down: jax.Array,
    c: jax.Array,
    w_mod: jax.Array,
):
    del B_x
    B, S, D = A_x.shape
    assert B == 1
    NG, SK = A_k_cache.shape[1], A_k_cache.shape[2]
    REP = HQ // NG
    FF = B_w_gate.shape[1]
    GW = REP * DH

    xt = A_x.reshape(S, D).T
    wot = A_wo.T
    wdt = B_w_down.T
    k = A_k_cache.reshape(NG, SK, DH)
    v = A_v_cache.reshape(NG, SK, DH)
    wr = B_w_r.reshape(1, D)

    hbm = pl.BlockSpec(memory_space=pl.ANY)
    out_t = pl.pallas_call(
        functools.partial(_kernel, S=S, SK=SK, D=D, NG=NG, REP=REP),
        grid=(NG,),
        in_specs=[hbm] * 11,
        out_specs=hbm,
        out_shape=jax.ShapeDtypeStruct((D, S), BF16),
        scratch_shapes=[
            pltpu.VMEM((D, S), BF16),
            pltpu.VMEM((2, SK, DH), BF16),
            pltpu.VMEM((2, SK, DH), BF16),
            pltpu.VMEM((2, D, GW), BF16),
            pltpu.VMEM((2, D, GW), BF16),
            pltpu.VMEM((1, D), BF16),
            pltpu.VMEM((1, D), BF16),
            pltpu.VMEM((D, 6 * D), BF16),
            pltpu.VMEM((D, FF), BF16),
            pltpu.VMEM((D, FF), BF16),
            pltpu.VMEM((D, FF), BF16),
            pltpu.VMEM((6 * D, LANES), F32),
            pltpu.VMEM((8, D), F32),
            pltpu.VMEM((S, D), BF16),
            pltpu.VMEM((D, S), F32),
            pltpu.VMEM((D, S), BF16),
            pltpu.VMEM((S // LANES, LANES), F32),
            pltpu.VMEM((D, S), BF16),
            pltpu.SemaphoreType.DMA((N_SEMS,)),
        ],
        compiler_params=pltpu.CompilerParams(
            dimension_semantics=("arbitrary",),
            vmem_limit_bytes=110 * 1024 * 1024,
            disable_bounds_checks=True,
        ),
    )(xt, k, v, A_wq, wot, wr, c, w_mod, B_w_gate, B_w_up, wdt)
    return out_t.T.reshape(B, S, D)
```

```python
import functools
import math

import jax
import jax.numpy as jnp
from jax import lax
import jax.experimental.pallas as pl
import jax.experimental.pallas.tpu as pltpu

F32 = jnp.float32
BF16 = jnp.bfloat16

HQ = 32
DH = 128
TOPC = 8
LN_EPS = 1e-5
BQ = 256
LANES = 128
SPLIT = 512
C0 = 2
OPD = 2
LN2U = 4
XCH = 4

_NT = (((1,), (1,)), ((), ()))

S_C, S_WMA, S_WMB, S_WR, S_WG, S_WU, S_WD, S_OUT = range(8)
S_X = 8
S_G = S_X + XCH
N_SEMS = S_G + 8


def _rb(x):
    return x.astype(BF16).astype(F32)


def _sigmoid(x):
    return 1.0 / (1.0 + jnp.exp(-x))


def _kernel(xt_hbm, k_hbm, v_hbm, wq_hbm, wot_hbm, wr_hbm, c_hbm, wmod_hbm,
            wg_hbm, wu_hbm, wdt_hbm,
            out_hbm,
            xt_ref, k_buf, v_buf, wq_buf, wot_buf, wr_ref, c_ref, wmod_ref,
            wg_ref, wu_ref, wdt_ref,
            modc_ref, gbrow_ref, h_ref, acc_ref, h2t_ref, st_ref, r_ref, out_ref,
            sems,
            *, S, SK, D, NG, REP):
    g = pl.program_id(0)
    qscale = (DH ** -0.5) * math.log2(math.e)
    NB = S // BQ
    GW = REP * DH
    TCH = S // XCH
    MA = 2 * D

    def cp(src, dst, sem):
        return pltpu.make_async_copy(src, dst, sem)

    def x_copy(i):
        cols = pl.ds(pl.multiple_of(i * TCH, TCH), TCH)
        return cp(xt_hbm.at[:, cols], xt_ref.at[:, cols], sems.at[S_X + i])

    def group_copies(grp, slot):
        cols = pl.ds(pl.multiple_of(grp * GW, GW), GW)
        return (cp(wq_hbm.at[:, cols], wq_buf.at[slot], sems.at[S_G + 4 * slot + 0]),
                cp(k_hbm.at[grp], k_buf.at[slot], sems.at[S_G + 4 * slot + 1]),
                cp(v_hbm.at[grp], v_buf.at[slot], sems.at[S_G + 4 * slot + 2]),
                cp(wot_hbm.at[:, cols], wot_buf.at[slot], sems.at[S_G + 4 * slot + 3]))

    c_cp = cp(c_hbm, c_ref, sems.at[S_C])
    wma_cp = cp(wmod_hbm.at[:, 0:MA], wmod_ref.at[:, 0:MA], sems.at[S_WMA])
    wmb_cp = cp(wmod_hbm.at[:, MA:6 * D], wmod_ref.at[:, MA:6 * D], sems.at[S_WMB])
    wr_cp = cp(wr_hbm, wr_ref, sems.at[S_WR])
    wg_cp = cp(wg_hbm, wg_ref, sems.at[S_WG])
    wu_cp = cp(wu_hbm, wu_ref, sems.at[S_WU])
    wd_cp = cp(wdt_hbm, wdt_ref, sems.at[S_WD])

    def modcol(i):
        return modc_ref[i * D:(i + 1) * D, :]

    def modulation(lo, hi, scale_lo):
        c = c_ref[...].astype(F32)
        sc = (c * _sigmoid(c)).astype(BF16)
        sc8 = jnp.broadcast_to(sc, (8, D))
        mod = _rb(jnp.dot(sc8, wmod_ref[:, lo:hi], preferred_element_type=F32))
        lane = lax.broadcasted_iota(jnp.int32, mod.shape, 1) + lo
        is_scale = (lane >= scale_lo) & (lane < scale_lo + D)
        modx = jnp.where(is_scale, _rb(1.0 + mod), mod)
        modc_ref[lo:hi, :] = jnp.broadcast_to(modx[0:1, :], (LANES, hi - lo)).T
        return mod

    @pl.when(g == 0)
    def _prologue():
        c_cp.start()
        wma_cp.start()
        for i in range(XCH):
            x_copy(i).start()
        for d in group_copies(0, 0) + group_copies(1, 1):
            d.start()
        wr_cp.start()
        c_cp.wait()
        wma_cp.wait()
        modulation(0, MA, D)

        def ln1(i, carry):
            x_copy(i).wait()
            for u in range(TCH // LANES):
                t0 = pl.multiple_of(i * TCH + u * LANES, LANES)
                x = xt_ref[:, pl.ds(t0, LANES)].astype(F32)
                m = jnp.mean(x, axis=0, keepdims=True)
                d = x - m
                var = jnp.mean(d * d, axis=0, keepdims=True)
                ht = d * lax.rsqrt(var + LN_EPS) * modcol(1) + modcol(0)
                h_ref[pl.ds(t0, LANES), :] = ht.astype(BF16).T
                acc_ref[:, pl.ds(t0, LANES)] = jnp.zeros((D, LANES), F32)
            return carry
        lax.fori_loop(0, XCH, ln1, 0)

    slot = g % 2
    for d in group_copies(g, slot):
        d.wait()

    k = k_buf[slot]
    v = v_buf[slot]
    wq = wq_buf[slot]
    wot = wot_buf[slot]

    def qproj(j):
        q2 = jnp.dot(h_ref[j * BQ:(j + 1) * BQ, :], wq, preferred_element_type=F32)
        return (q2 * qscale).astype(BF16)

    def qk(q, lo, hi):
        return lax.dot_general(q, k[lo:hi], _NT, preferred_element_type=F32)

    def softmax_pv(s, late):
        m = jnp.max(s, axis=1, keepdims=True)
        p = jnp.exp2(s - m)
        o = jnp.dot(p.astype(BF16), v, preferred_element_type=F32)
        if late:
            lp = p[:, 0:LANES]
            for i in range(1, SK // LANES):
                lp = lp + p[:, i * LANES:(i + 1) * LANES]
            l = jnp.sum(jnp.where(lp < 0.0, o, lp), axis=1, keepdims=True)
        else:
            l = jnp.sum(p, axis=1, keepdims=True)
        rl = pl.reciprocal(l, approx=True)
        rl = rl * (2.0 - l * rl)
        return (o * rl).astype(BF16)

    def oproj(j):
        o2 = jnp.concatenate([outs[REP * j + r] for r in range(REP)], axis=1)
        acc_ref[:, j * BQ:(j + 1) * BQ] += lax.dot_general(
            wot, o2, _NT, preferred_element_type=F32)

    q2s = [qproj(j) for j in range(NB)]
    qs = [q2s[j][:, r * DH:(r + 1) * DH] for j in range(NB) for r in range(REP)]
    outs = []
    done = 0
    s_head = None
    for ci in range(len(qs)):
        if s_head is None:
            s = qk(qs[ci], 0, SK)
        else:
            s = jnp.concatenate([s_head, qk(qs[ci], SPLIT, SK)], axis=1)
        s_head = qk(qs[ci + 1], 0, SPLIT) if (C0 <= ci < len(qs) - 1) else None
        outs.append(softmax_pv(s, late=(ci == len(qs) - 1)))
        if ci % REP == REP - 1 and ci // REP - OPD >= 0:
            oproj(done)
            done += 1
    for j in range(done, NB):
        oproj(j)

    @pl.when(g + 2 < NG)
    def _():
        for d in group_copies(g + 2, slot):
            d.start()

    @pl.when(g == 0)
    def _():
        wmb_cp.start()
        wg_cp.start()

    @pl.when(g == 1)
    def _():
        wu_cp.start()

    @pl.when(g == 2)
    def _():
        wd_cp.start()

    @pl.when(g == NG - 1)
    def _epilogue():
        wmb_cp.wait()
        wr_cp.wait()
        modb = modulation(MA, 6 * D, 4 * D)
        gbrow_ref[...] = modb[:, 3 * D:4 * D]
        eps_b = _rb(jnp.full((1, 1), LN_EPS, F32))
        wr8 = jnp.broadcast_to(wr_ref[...], (8, D))
        NSL = S // LANES

        W2 = LN2U * LANES

        def tile_cols(col):
            return jnp.concatenate([col] * LN2U, axis=1)

        def ln2_stats(i, carry):
            cols = pl.ds(pl.multiple_of(i * W2, W2), W2)
            x2 = xt_ref[:, cols].astype(F32) + tile_cols(modcol(2)) * acc_ref[:, cols]
            acc_ref[:, cols] = x2
            piv = x2[0:1, :]
            d = x2 - piv
            md = jnp.mean(d, axis=0, keepdims=True)
            var = jnp.maximum(jnp.mean(d * d, axis=0, keepdims=True) - md * md, 0.0)
            sd = _rb(jnp.sqrt(_rb(_rb(var) + eps_b)))
            rs = 1.0 / sd
            st_ref[0:1, cols] = rs
            st_ref[1:2, cols] = (piv + md) * rs
            return carry
        lax.fori_loop(0, S // W2, ln2_stats, 0)

        def ln2_apply(i, carry):
            cols = pl.ds(pl.multiple_of(i * W2, W2), W2)
            x2 = acc_ref[:, cols]
            n = x2 * st_ref[0:1, cols] - st_ref[1:2, cols]
            h2 = n * tile_cols(modcol(4)) + tile_cols(modcol(3))
            h2b = h2.astype(BF16)
            h2t_ref[:, cols] = pltpu.bitcast(h2b, jnp.uint32)
            out_ref[:, cols] = (x2 + tile_cols(modcol(5)) * h2).astype(BF16)
            rr = jnp.dot(wr8, h2b, preferred_element_type=F32)
            for u in range(LN2U):
                r_ref[pl.ds(LN2U * i + u, 1), :] = rr[0:1, u * LANES:(u + 1) * LANES]
            return carry
        lax.fori_loop(0, S // W2, ln2_apply, 0)

        r = _rb(r_ref[...]) + 0.0
        bits = pltpu.bitcast(r, jnp.int32)
        mono = bits ^ ((bits >> 31) & jnp.int32(0x7FFFFFFF))
        tok = (lax.broadcasted_iota(jnp.int32, (NSL, LANES), 0) * LANES
               + lax.broadcasted_iota(jnp.int32, (NSL, LANES), 1))
        keyi = (((mono >> 16) + 32768) * S + (S - 1 - tok)) + jnp.int32(1 << 29)
        key = pltpu.bitcast(keyi, F32)

        row16 = lax.broadcasted_iota(jnp.int32, (16, LANES), 0)
        lane16 = lax.broadcasted_iota(jnp.int32, (16, LANES), 1)
        rowc = lax.broadcasted_iota(jnp.int32, (16, 1), 0)
        sel_base, sel_off = [], []
        hsel = jnp.zeros((16, D), F32)
        ksel = jnp.zeros((16, 1), F32)
        for t in range(TOPC):
            kmax = jnp.max(jnp.max(key, axis=0, keepdims=True), axis=1, keepdims=True)
            key = jnp.where(key == kmax, 0.0, key)
            ksel = jnp.where(rowc == t, kmax, ksel)
            ki = pltpu.bitcast(kmax, jnp.int32)[0, 0]
            idx = (S - 1) - (ki & (S - 1))
            base = pl.multiple_of((idx >> 7) << 7, LANES)
            off = idx & (LANES - 1)
            onehot = jnp.where((row16 == t) & (lane16 == off), 1.0, 0.0).astype(BF16)
            hsel = hsel + lax.dot_general(onehot, pltpu.bitcast(h2t_ref[:, pl.ds(base, LANES)], BF16), _NT,
                                          preferred_element_type=F32)
            sel_base.append(base)
            sel_off.append(off)
        hi = ((pltpu.bitcast(ksel, jnp.int32) - jnp.int32(1 << 29)) // S - 32768) << 16
        rbits = hi ^ ((hi >> 31) & jnp.int32(0x7FFF0000))
        rsel = jnp.where(rowc < TOPC, pltpu.bitcast(rbits, F32), 0.0)

        wg_cp.wait()
        wu_cp.wait()
        wd_cp.wait()
        hs = hsel.astype(BF16)
        gpre = jnp.dot(hs, wg_ref[...], preferred_element_type=F32)
        u = jnp.dot(hs, wu_ref[...], preferred_element_type=F32)
        a = (gpre * _sigmoid(gpre) * u).astype(BF16)
        y = lax.dot_general(a, wdt_ref[...], _NT, preferred_element_type=F32)
        delta = y * _sigmoid(rsel) * gbrow_ref[0:1, :]

        laneD = lax.broadcasted_iota(jnp.int32, (D, LANES), 1)
        for t in range(TOPC):
            slab = pl.ds(sel_base[t], LANES)
            colt = jnp.broadcast_to(delta[t:t + 1, :], (LANES, D)).T
            old = out_ref[:, slab].astype(F32)
            out_ref[:, slab] = jnp.where(laneD == sel_off[t], old + colt, old).astype(BF16)

        o_cp = cp(out_ref, out_hbm, sems.at[S_OUT])
        o_cp.start()
        o_cp.wait()


@jax.jit
def pallas_adaLN_cond__gqa_block_cached__moe_arch_mod__prompt_kernel(
    A_x: jax.Array,
    A_k_cache: jax.Array,
    A_v_cache: jax.Array,
    A_wq: jax.Array,
    A_wo: jax.Array,
    B_x: jax.Array,
    B_w_r: jax.Array,
    B_w_gate: jax.Array,
    B_w_up: jax.Array,
    B_w_down: jax.Array,
    c: jax.Array,
    w_mod: jax.Array,
):
    del B_x
    B, S, D = A_x.shape
    assert B == 1
    NG, SK = A_k_cache.shape[1], A_k_cache.shape[2]
    REP = HQ // NG
    FF = B_w_gate.shape[1]
    GW = REP * DH

    xt = A_x.reshape(S, D).T
    wot = A_wo.T
    wdt = B_w_down.T
    k = A_k_cache.reshape(NG, SK, DH)
    v = A_v_cache.reshape(NG, SK, DH)
    wr = B_w_r.reshape(1, D)

    hbm = pl.BlockSpec(memory_space=pl.ANY)
    out_t = pl.pallas_call(
        functools.partial(_kernel, S=S, SK=SK, D=D, NG=NG, REP=REP),
        grid=(NG,),
        in_specs=[hbm] * 11,
        out_specs=hbm,
        out_shape=jax.ShapeDtypeStruct((D, S), BF16),
        scratch_shapes=[
            pltpu.VMEM((D, S), BF16),
            pltpu.VMEM((2, SK, DH), BF16),
            pltpu.VMEM((2, SK, DH), BF16),
            pltpu.VMEM((2, D, GW), BF16),
            pltpu.VMEM((2, D, GW), BF16),
            pltpu.VMEM((1, D), BF16),
            pltpu.VMEM((1, D), BF16),
            pltpu.VMEM((D, 6 * D), BF16),
            pltpu.VMEM((D, FF), BF16),
            pltpu.VMEM((D, FF), BF16),
            pltpu.VMEM((D, FF), BF16),
            pltpu.VMEM((6 * D, LANES), F32),
            pltpu.VMEM((8, D), F32),
            pltpu.VMEM((S, D), BF16),
            pltpu.VMEM((D, S), F32),
            pltpu.VMEM((D // 2, S), jnp.uint32),
            pltpu.VMEM((8, S), F32),
            pltpu.VMEM((S // LANES, LANES), F32),
            pltpu.VMEM((D, S), BF16),
            pltpu.SemaphoreType.DMA((N_SEMS,)),
        ],
        compiler_params=pltpu.CompilerParams(
            dimension_semantics=("arbitrary",),
            vmem_limit_bytes=110 * 1024 * 1024,
            disable_bounds_checks=True,
        ),
    )(xt, k, v, A_wq, wot, wr, c, w_mod, B_w_gate, B_w_up, wdt)
    return out_t.T.reshape(B, S, D)
```

```python
import functools
import math

import jax
import jax.numpy as jnp
from jax import lax
import jax.experimental.pallas as pl
import jax.experimental.pallas.tpu as pltpu

F32 = jnp.float32
BF16 = jnp.bfloat16

HQ = 32
DH = 128
TOPC = 8
LN_EPS = 1e-5
BQ = 256
LANES = 128
SPLIT = 512
C0 = 2
OPD = 2
XCH = 4
MT = 3
PR = 8
EPR = 64
MOD_S0 = 2

_NT = (((1,), (1,)), ((), ()))

S_C, S_WMA, S_WMB, S_WR, S_WG, S_WU, S_WD = range(7)
S_X = 7
S_G = S_X + XCH
S_O = S_G + 16
S_P = S_O + 8
N_SEMS = S_P + TOPC


def _rb(x):
    return x.astype(BF16).astype(F32)


def _sigmoid(x):
    return 1.0 / (1.0 + jnp.exp(-x))


def _tile(col, n):
    return jnp.concatenate([col] * n, axis=1)


def _as_cols(row):
    return jnp.broadcast_to(row, (LANES, row.shape[1])).T


def _moments(x):
    piv = x[0:1, :]
    d = x - piv
    md = jnp.mean(d, axis=0, keepdims=True)
    var = jnp.maximum(jnp.mean(d * d, axis=0, keepdims=True) - md * md, 0.0)
    return piv + md, var


def _kernel(xt_hbm, k_hbm, v_hbm, wq_hbm, wot_hbm, wr_hbm, c_hbm, wmod_hbm,
            wg_hbm, wu_hbm, wdt_hbm,
            out_hbm,
            xt_ref, kx_ref, v_all, wq_all, wot_all, wr_ref, c_ref, wmod_ref,
            wg_ref, wu_ref, wdt_ref,
            scc_ref, wrc_ref, rc_ref, h_ref, acc_ref,
            sems,
            *, S, SK, D, NG, REP):
    step = pl.program_id(0)
    qscale = (DH ** -0.5) * math.log2(math.e)
    NB = S // BQ
    GW = REP * DH
    TCH = S // XCH
    MA = 2 * D
    NSL = S // LANES
    SPB = BQ // LANES
    assert NG == 2 * NB and (4 * D) % (MT * LANES) == 0 and MA % LANES == 0
    MOD_STEPS = 4 * D // (MT * LANES)
    assert MOD_S0 + MOD_STEPS <= NB
    OUT0 = NG * SK
    H20 = OUT0 + NSL * D
    R0 = H20 + NSL * D
    MOD0 = R0 + NSL * 16

    def rows(start, n):
        return pl.ds(pl.multiple_of(start, 16), n)

    def cp(src, dst, sem):
        return pltpu.make_async_copy(src, dst, sems.at[sem])

    def x_copy(i):
        cols = pl.ds(pl.multiple_of(i * TCH, TCH), TCH)
        return cp(xt_hbm.at[:, cols], xt_ref.at[:, cols], S_X + i)

    def group_copies(grp):
        cols = pl.ds(pl.multiple_of(grp * GW, GW), GW)
        return (cp(wq_hbm.at[:, cols], wq_all.at[grp], S_G + grp),
                cp(k_hbm.at[grp], kx_ref.at[rows(grp * SK, SK), :], S_G + grp),
                cp(v_hbm.at[grp], v_all.at[grp], S_G + grp),
                cp(wot_hbm.at[:, cols], wot_all.at[grp], S_G + grp))

    def slab_copy(sl, sem):
        cols = pl.ds(pl.multiple_of(sl * LANES, LANES), LANES)
        return cp(kx_ref.at[rows(OUT0 + sl * D, D), :], out_hbm.at[:, cols], sem)

    def out_copies(jb):
        return [slab_copy(SPB * jb + u, S_O + jb) for u in range(SPB)]

    c_cp = lambda: cp(c_hbm, c_ref, S_C)
    wma_cp = lambda: cp(wmod_hbm.at[:, 0:MA], wmod_ref.at[:, 0:MA], S_WMA)
    wmb_cp = lambda: cp(wmod_hbm.at[:, MA:6 * D], wmod_ref.at[:, MA:6 * D], S_WMB)
    wr_cp = lambda: cp(wr_hbm, wr_ref, S_WR)
    wg_cp = lambda: cp(wg_hbm, wg_ref, S_WG)
    wu_cp = lambda: cp(wu_hbm, wu_ref, S_WU)
    wd_cp = lambda: cp(wdt_hbm, wdt_ref, S_WD)

    def modcol(i):
        return kx_ref[MOD0 + i * D:MOD0 + (i + 1) * D, :].astype(F32)

    def finish_mod(mod, col0):
        mod = _rb(mod)
        lane = lax.broadcasted_iota(jnp.int32, mod.shape, 1) + col0
        is_scale = ((lane >= D) & (lane < 2 * D)) | ((lane >= 4 * D) & (lane < 5 * D))
        return jnp.where(is_scale, _rb(1.0 + mod), mod)

    def ln2(jb, pr, paced):
        cols = pl.ds(pl.multiple_of(jb * BQ, BQ), BQ)

        def mc(i, r0):
            return kx_ref[MOD0 + i * D + r0:MOD0 + i * D + r0 + pr, :].astype(F32)

        x2s = []
        for r0 in range(0, D, pr):
            a = acc_ref[r0:r0 + pr, cols]
            if paced and r0 > 0:
                a = jnp.where(s2 < 0.0, s2, a)
            x2 = xt_ref[r0:r0 + pr, cols].astype(F32) + _tile(mc(2, r0), SPB) * a
            if r0 == 0:
                piv = x2[0:1, :]
            d = x2 - piv
            t = d * _tile(wrc_ref[r0:r0 + pr, :], SPB)
            s1, s2, s3 = (d, d * d, t) if r0 == 0 else (s1 + d, s2 + d * d, s3 + t)
            x2s.append(x2)
        md = jnp.sum(s1, axis=0, keepdims=True) * (1.0 / D)
        var = jnp.maximum(jnp.sum(s2, axis=0, keepdims=True) * (1.0 / D) - md * md, 0.0)
        eps_b = _rb(jnp.full((1, 1), LN_EPS, F32))
        rs = 1.0 / _rb(jnp.sqrt(_rb(_rb(var) + eps_b)))
        mrs = (piv + md) * rs
        rr = ((jnp.sum(s3, axis=0, keepdims=True) - md * _tile(rc_ref[0:1, :], SPB)) * rs
              + _tile(rc_ref[1:2, :], SPB))
        h2v, ov = [], []
        for u in range(SPB):
            sl = SPB * jb + u
            kx_ref[rows(R0 + sl * 16, 16), :] = jnp.broadcast_to(
                rr[:, u * LANES:(u + 1) * LANES], (16, LANES)).astype(BF16)
            h2v.append(kx_ref.at[rows(H20 + sl * D, D), :])
            ov.append(kx_ref.at[rows(OUT0 + sl * D, D), :])
        for n, r0 in enumerate(range(0, D, pr)):
            cb, sb, gb = mc(4, r0), mc(3, r0), mc(5, r0)
            for u in range(SPB):
                lanes = slice(u * LANES, (u + 1) * LANES)
                x2 = x2s[n][:, lanes]
                h2 = (x2 * rs[:, lanes] - mrs[:, lanes]) * cb + sb
                h2v[u][r0:r0 + pr, :] = h2.astype(BF16)
                ov[u][r0:r0 + pr, :] = (x2 + gb * h2).astype(BF16)

    @pl.when(step == 0)
    def _prologue():
        c_cp().start()
        wr_cp().start()
        wma_cp().start()
        for i in range(XCH):
            x_copy(i).start()
        for d in group_copies(0) + group_copies(1):
            d.start()
        wmb_cp().start()
        c_cp().wait()
        wr_cp().wait()
        c = c_ref[...].astype(F32)
        sc = (c * _sigmoid(c)).astype(BF16)
        scc_ref[...] = _as_cols(sc.astype(F32))
        wrc_ref[...] = _as_cols(wr_ref[...].astype(F32))
        acc_ref[...] = jnp.zeros((D, S), F32)
        wma_cp().wait()
        mod = jnp.dot(jnp.broadcast_to(sc, (8, D)), wmod_ref[:, 0:MA], preferred_element_type=F32)
        kx_ref[MOD0:MOD0 + MA, :] = _as_cols(finish_mod(mod, 0)[0:1, :]).astype(BF16)

        def ln1(i, carry):
            x_copy(i).wait()
            t0 = pl.multiple_of(i * TCH, TCH)
            x = xt_ref[:, pl.ds(t0, TCH)].astype(F32)
            m, var = _moments(x)
            rs = lax.rsqrt(var + LN_EPS)
            n = TCH // LANES
            ht = (x * rs - m * rs) * _tile(modcol(1), n) + _tile(modcol(0), n)
            h_ref[pl.ds(t0, TCH), :] = ht.astype(BF16).T
            return carry
        lax.fori_loop(0, XCH, ln1, 0)

    phase1 = step < NB

    @pl.when(phase1)
    def _():
        for d in group_copies(step):
            d.wait()

    @pl.when(step == MOD_S0)
    def _():
        wmb_cp().wait()

    @pl.when(step == NB)
    def _():
        for grp in range(NB, NG):
            for d in group_copies(grp):
                d.wait()
        wg_cp().wait()
        wu_cp().wait()
        wd_cp().wait()
        wr = wrc_ref[...]
        a = wr * modcol(4)
        wrc_ref[...] = a
        rc_ref[0:1, :] = jnp.sum(a, axis=0, keepdims=True)
        rc_ref[1:2, :] = jnp.sum(wr * modcol(3), axis=0, keepdims=True)

    in_win = (step >= MOD_S0) & (step < MOD_S0 + MOD_STEPS)
    mc0 = pl.multiple_of(jnp.where(in_win, MA + (step - MOD_S0) * (MT * LANES), 0), LANES)
    for r0 in range(0, D, PR):
        sc8 = scc_ref[r0:r0 + PR, :]
        if r0 > 0:
            g8 = macc[:, 0:LANES]
            sc8 = jnp.where(g8 * g8 < 0.0, g8, sc8)
        t = wmod_ref[r0:r0 + PR, pl.ds(mc0, MT * LANES)].astype(F32) * _tile(sc8, MT)
        macc = t if r0 == 0 else macc + t
    mrow = jnp.sum(macc, axis=0, keepdims=True)
    kx_ref[rows(MOD0 + mc0, MT * LANES), :] = _as_cols(finish_mod(mrow, mc0)).astype(BF16)
    ln2(jnp.maximum(step - (NB + 1), 0), PR, True)

    ujs = [jnp.where(phase1, u, step - NB) for u in range(NB)]
    ugs = [jnp.where(phase1, step, NB + u) for u in range(NB)]

    def qproj(u):
        q2 = jnp.dot(h_ref[rows(ujs[u] * BQ, BQ), :], wq_all[ugs[u]], preferred_element_type=F32)
        return (q2 * qscale).astype(BF16)

    def qk(ci, lo, hi):
        return lax.dot_general(qs[ci], kx_ref[rows(ugs[ci // REP] * SK + lo, hi - lo), :], _NT,
                               preferred_element_type=F32)

    def softmax_pv(ci, s, late):
        m = jnp.max(s, axis=1, keepdims=True)
        p = jnp.exp2(s - m)
        o = jnp.dot(p.astype(BF16), v_all[ugs[ci // REP]], preferred_element_type=F32)
        if late:
            lp = p[:, 0:LANES]
            for i in range(1, SK // LANES):
                lp = lp + p[:, i * LANES:(i + 1) * LANES]
            l = jnp.sum(jnp.where(lp < 0.0, o, lp), axis=1, keepdims=True)
        else:
            l = jnp.sum(p, axis=1, keepdims=True)
        rl = pl.reciprocal(l, approx=True)
        rl = rl * (2.0 - l * rl)
        return (o * rl).astype(BF16)

    def oproj(u):
        cols = pl.ds(pl.multiple_of(ujs[u] * BQ, BQ), BQ)
        o2 = jnp.concatenate([outs[REP * u + r] for r in range(REP)], axis=1)
        acc_ref[:, cols] += lax.dot_general(wot_all[ugs[u]], o2, _NT, preferred_element_type=F32)

    q2s = [qproj(u) for u in range(NB)]
    qs = [q2s[u][:, r * DH:(r + 1) * DH] for u in range(NB) for r in range(REP)]
    outs = []
    done = 0
    s_head = None
    for ci in range(len(qs)):
        if s_head is None:
            s = qk(ci, 0, SK)
        else:
            s = jnp.concatenate([s_head, qk(ci, SPLIT, SK)], axis=1)
        s_head = qk(ci + 1, 0, SPLIT) if (C0 <= ci < len(qs) - 1) else None
        outs.append(softmax_pv(ci, s, late=(ci == len(qs) - 1)))
        if ci % REP == REP - 1 and ci // REP - OPD >= 0:
            oproj(done)
            done += 1
    for u in range(done, NB):
        oproj(u)

    @pl.when(step < NB - 1)
    def _():
        for d in group_copies(jnp.where(step + 2 < NB, step + 2, NG - 1)) + group_copies(NB + step):
            d.start()

    @pl.when(step == 0)
    def _():
        wg_cp().start()

    @pl.when(step == 1)
    def _():
        wu_cp().start()

    @pl.when(step == 2)
    def _():
        wd_cp().start()

    @pl.when(step > NB)
    def _():
        for d in out_copies(step - (NB + 1)):
            d.start()

    @pl.when(step == NG - 1)
    def _epilogue():
        ln2(NB - 1, EPR, False)
        for d in out_copies(NB - 1):
            d.start()

        row16 = lax.broadcasted_iota(jnp.int32, (16, LANES), 0)
        assert NSL == 16
        r = kx_ref[R0:R0 + 16, :].astype(F32)
        for sl in range(1, NSL):
            r = jnp.where(row16 == sl, kx_ref[R0 + 16 * sl:R0 + 16 * (sl + 1), :].astype(F32), r)
        r = r + 0.0
        bits = pltpu.bitcast(r, jnp.int32)
        mono = bits ^ ((bits >> 31) & jnp.int32(0x7FFFFFFF))
        tok = (lax.broadcasted_iota(jnp.int32, (NSL, LANES), 0) * LANES
               + lax.broadcasted_iota(jnp.int32, (NSL, LANES), 1))
        keyi = (((mono >> 16) + 32768) * S + (S - 1 - tok)) + jnp.int32(1 << 29)
        key = pltpu.bitcast(keyi, F32)

        lane16 = lax.broadcasted_iota(jnp.int32, (16, LANES), 1)
        rowc = lax.broadcasted_iota(jnp.int32, (16, 1), 0)
        sel_base, sel_off = [], []
        hsel = jnp.zeros((16, D), F32)
        ksel = jnp.zeros((16, 1), F32)
        for t in range(TOPC):
            kmax = jnp.max(jnp.max(key, axis=0, keepdims=True), axis=1, keepdims=True)
            key = jnp.where(key == kmax, 0.0, key)
            ksel = jnp.where(rowc == t, kmax, ksel)
            ki = pltpu.bitcast(kmax, jnp.int32)[0, 0]
            idx = (S - 1) - (ki & (S - 1))
            base = idx >> 7
            off = idx & (LANES - 1)
            onehot = jnp.where((row16 == t) & (lane16 == off), 1.0, 0.0).astype(BF16)
            hsel = hsel + lax.dot_general(
                onehot, kx_ref[rows(H20 + base * D, D), :], _NT,
                preferred_element_type=F32)
            sel_base.append(base)
            sel_off.append(off)
        hi = ((pltpu.bitcast(ksel, jnp.int32) - jnp.int32(1 << 29)) // S - 32768) << 16
        rbits = hi ^ ((hi >> 31) & jnp.int32(0x7FFF0000))
        rsel = jnp.where(rowc < TOPC, pltpu.bitcast(rbits, F32), 0.0)

        hs = hsel.astype(BF16)
        gpre = jnp.dot(hs, wg_ref[...], preferred_element_type=F32)
        u = jnp.dot(hs, wu_ref[...], preferred_element_type=F32)
        a = (gpre * _sigmoid(gpre) * u).astype(BF16)
        y = lax.dot_general(a, wdt_ref[...], _NT, preferred_element_type=F32)
        y = y * _sigmoid(rsel)

        for jb in range(NB):
            for d in out_copies(jb):
                d.wait()
        laneD = lax.broadcasted_iota(jnp.int32, (D, LANES), 1)
        for t in range(TOPC):
            slab = rows(OUT0 + sel_base[t] * D, D)
            colt = _as_cols(y[t:t + 1, :]) * modcol(5)
            old = kx_ref[slab, :].astype(F32)
            kx_ref[slab, :] = jnp.where(laneD == sel_off[t], old + colt, old).astype(BF16)

        def patch_copy(t):
            return slab_copy(sel_base[t], S_P + t)

        fresh = []
        for t in range(TOPC):
            f = jnp.bool_(True)
            for t2 in range(t):
                f = f & (sel_base[t] != sel_base[t2])
            fresh.append(f)
            pl.when(f)(lambda t=t: patch_copy(t).start())
        for t in range(TOPC):
            pl.when(fresh[t])(lambda t=t: patch_copy(t).wait())


@jax.jit
def pallas_adaLN_cond__gqa_block_cached__moe_arch_mod__prompt_kernel(
    A_x: jax.Array,
    A_k_cache: jax.Array,
    A_v_cache: jax.Array,
    A_wq: jax.Array,
    A_wo: jax.Array,
    B_x: jax.Array,
    B_w_r: jax.Array,
    B_w_gate: jax.Array,
    B_w_up: jax.Array,
    B_w_down: jax.Array,
    c: jax.Array,
    w_mod: jax.Array,
):
    del B_x
    B, S, D = A_x.shape
    assert B == 1
    NG, SK = A_k_cache.shape[1], A_k_cache.shape[2]
    REP = HQ // NG
    FF = B_w_gate.shape[1]
    GW = REP * DH

    xt = A_x.reshape(S, D).T
    wot = A_wo.T
    wdt = B_w_down.T
    k = A_k_cache.reshape(NG, SK, DH)
    v = A_v_cache.reshape(NG, SK, DH)
    wr = B_w_r.reshape(1, D)

    hbm = pl.BlockSpec(memory_space=pl.ANY)
    out_t = pl.pallas_call(
        functools.partial(_kernel, S=S, SK=SK, D=D, NG=NG, REP=REP),
        grid=(NG,),
        in_specs=[hbm] * 11,
        out_specs=hbm,
        out_shape=jax.ShapeDtypeStruct((D, S), BF16),
        scratch_shapes=[
            pltpu.VMEM((D, S), BF16),
            pltpu.VMEM((NG * SK + (S // LANES) * (2 * D + 16) + 6 * D, DH), BF16),
            pltpu.VMEM((NG, SK, DH), BF16),
            pltpu.VMEM((NG, D, GW), BF16),
            pltpu.VMEM((NG, D, GW), BF16),
            pltpu.VMEM((1, D), BF16),
            pltpu.VMEM((1, D), BF16),
            pltpu.VMEM((D, 6 * D), BF16),
            pltpu.VMEM((D, FF), BF16),
            pltpu.VMEM((D, FF), BF16),
            pltpu.VMEM((D, FF), BF16),
            pltpu.VMEM((D, LANES), F32),
            pltpu.VMEM((D, LANES), F32),
            pltpu.VMEM((8, LANES), F32),
            pltpu.VMEM((S, D), BF16),
            pltpu.VMEM((D, S), F32),
            pltpu.SemaphoreType.DMA((N_SEMS,)),
        ],
        compiler_params=pltpu.CompilerParams(
            dimension_semantics=("arbitrary",),
            vmem_limit_bytes=110 * 1024 * 1024,
            disable_bounds_checks=True,
        ),
    )(xt, k, v, A_wq, wot, wr, c, w_mod, B_w_gate, B_w_up, wdt)
    return out_t.T.reshape(B, S, D)
```

```python
import functools
import math

import jax
import jax.numpy as jnp
from jax import lax
import jax.experimental.pallas as pl
import jax.experimental.pallas.tpu as pltpu

F32 = jnp.float32
BF16 = jnp.bfloat16
U32 = jnp.uint32

HQ = 32
DH = 128
TOPC = 8
LN_EPS = 1e-5
BQ = 256
LANES = 128
SPLIT = 512
C0 = 2
OPD = 2
XCH = 4
LN2U = 4
MOD_STEP = 4

_NT = (((1,), (1,)), ((), ()))

S_C, S_WMA, S_WMB, S_WR, S_WG, S_WU, S_WD = range(7)
S_X = 7
S_G = S_X + XCH
S_O = S_G + 2
S_P = S_O + 16
N_SEMS = S_P + TOPC


def _rb(x):
    return x.astype(BF16).astype(F32)


def _sigmoid(x):
    return 1.0 / (1.0 + jnp.exp(-x))


def _tile(col, n):
    return jnp.concatenate([col] * n, axis=1)


def _as_cols(row):
    return jnp.broadcast_to(row, (LANES, row.shape[1])).T


def _kernel(xt_hbm, k_hbm, v_hbm, wq_hbm, wot_hbm, wr_hbm, c_hbm, wmod_hbm,
            wg_hbm, wu_hbm, wdt_hbm,
            out_hbm,
            xt_ref, k_buf, v_buf, wq_buf, wot_buf, wr_ref, c_ref, wmod_ref,
            wg_ref, wu_ref, wx_ref,
            modc_ref, wrc_ref, rc_ref, h_ref, acc_ref, h2t_ref, st_ref, r_ref,
            sems,
            *, S, SK, D, FF, NG, REP):
    step = pl.program_id(0)
    qscale = (DH ** -0.5) * math.log2(math.e)
    NB = S // BQ
    GW = REP * DH
    TCH = S // XCH
    MA = 2 * D
    NSL = S // LANES

    def cp(src, dst, sem):
        return pltpu.make_async_copy(src, dst, sems.at[sem])

    def x_copy(i):
        cols = pl.ds(pl.multiple_of(i * TCH, TCH), TCH)
        return cp(xt_hbm.at[:, cols], xt_ref.at[:, cols], S_X + i)

    def group_copies(grp):
        slot = grp % 2
        cols = pl.ds(pl.multiple_of(grp * GW, GW), GW)
        return (cp(wq_hbm.at[:, cols], wq_buf.at[slot], S_G + slot),
                cp(k_hbm.at[grp], k_buf.at[slot], S_G + slot),
                cp(v_hbm.at[grp], v_buf.at[slot], S_G + slot),
                cp(wot_hbm.at[:, cols], wot_buf.at[slot], S_G + slot))

    c_cp = lambda: cp(c_hbm, c_ref, S_C)
    wma_cp = lambda: cp(wmod_hbm.at[:, 0:MA], wmod_ref.at[:, 0:MA], S_WMA)
    wmb_cp = lambda: cp(wmod_hbm.at[:, MA:6 * D], wmod_ref.at[:, MA:6 * D], S_WMB)
    wr_cp = lambda: cp(wr_hbm, wr_ref, S_WR)
    wg_cp = lambda: cp(wg_hbm, wg_ref, S_WG)
    wu_cp = lambda: cp(wu_hbm, wu_ref, S_WU)
    wd_cp = lambda: cp(wdt_hbm, wx_ref.at[:, 0:FF], S_WD)

    def modcol(i):
        return modc_ref[i * D:(i + 1) * D, :]

    def modulation(lo, hi):
        c = c_ref[...].astype(F32)
        sc8 = jnp.broadcast_to((c * _sigmoid(c)).astype(BF16), (8, D))
        for a in range(lo, hi, MA):
            mod = _rb(jnp.dot(sc8, wmod_ref[:, a:a + MA], preferred_element_type=F32))
            lane = lax.broadcasted_iota(jnp.int32, mod.shape, 1) + a
            is_scale = ((lane >= D) & (lane < 2 * D)) | ((lane >= 4 * D) & (lane < 5 * D))
            mod = jnp.where(is_scale, _rb(1.0 + mod), mod)
            modc_ref[a:a + MA, :] = _as_cols(mod[0:1, :])

    @pl.when(step == 0)
    def _prologue():
        c_cp().start()
        wr_cp().start()
        wma_cp().start()
        for i in range(XCH):
            x_copy(i).start()
        for d in group_copies(0) + group_copies(1):
            d.start()
        c_cp().wait()
        wr_cp().wait()
        wrc_ref[...] = _as_cols(wr_ref[...].astype(F32))
        acc_ref[...] = jnp.zeros((D, S), F32)
        wma_cp().wait()
        modulation(0, MA)

        def ln1(i, carry):
            x_copy(i).wait()
            x = xt_ref[:, pl.ds(pl.multiple_of(i * TCH, TCH), TCH)].astype(F32)
            piv = x[0:1, :]
            d = x - piv
            md = jnp.mean(d, axis=0, keepdims=True)
            var = jnp.maximum(jnp.mean(d * d, axis=0, keepdims=True) - md * md, 0.0)
            rs = lax.rsqrt(var + LN_EPS)
            n = TCH // LANES
            ht = (x * rs - (piv + md) * rs) * _tile(modcol(1), n) + _tile(modcol(0), n)
            h_ref[pl.ds(pl.multiple_of(i * (TCH // 2), TCH // 2), TCH // 2), :] = pltpu.bitcast(
                ht.astype(BF16).T, U32)
            return carry
        lax.fori_loop(0, XCH, ln1, 0)

    @pl.when(step == MOD_STEP)
    def _late_modulation():
        wmb_cp().wait()
        wg_cp().wait()
        wu_cp().wait()
        wd_cp().wait()
        modulation(MA, 6 * D)
        wr = wrc_ref[...]
        a = wr * modcol(4)
        wrc_ref[...] = a
        rc_ref[0:1, :] = jnp.sum(a, axis=0, keepdims=True)
        rc_ref[1:2, :] = jnp.sum(wr * modcol(3), axis=0, keepdims=True)

    for d in group_copies(step):
        d.wait()

    slot = step % 2
    k = k_buf[slot]
    v = v_buf[slot]
    wq = wq_buf[slot]
    wot = wot_buf[slot]

    def qproj(j):
        hb = pltpu.bitcast(h_ref[j * (BQ // 2):(j + 1) * (BQ // 2), :], BF16)
        q2 = jnp.dot(hb, wq, preferred_element_type=F32)
        return (q2 * qscale).astype(BF16)

    def qk(ci, lo, hi):
        return lax.dot_general(qs[ci], k[lo:hi], _NT, preferred_element_type=F32)

    def softmax_pv(s, late):
        m = jnp.max(s, axis=1, keepdims=True)
        p = jnp.exp2(s - m)
        o = jnp.dot(p.astype(BF16), v, preferred_element_type=F32)
        if late:
            lp = p[:, 0:LANES]
            for i in range(1, SK // LANES):
                lp = lp + p[:, i * LANES:(i + 1) * LANES]
            l = jnp.sum(jnp.where(lp < 0.0, o, lp), axis=1, keepdims=True)
        else:
            l = jnp.sum(p, axis=1, keepdims=True)
        rl = pl.reciprocal(l, approx=True)
        rl = rl * (2.0 - l * rl)
        return (o * rl).astype(BF16)

    def oproj(j):
        o2 = jnp.concatenate([outs[REP * j + r] for r in range(REP)], axis=1)
        acc_ref[:, j * BQ:(j + 1) * BQ] += lax.dot_general(wot, o2, _NT, preferred_element_type=F32)

    q2s = [qproj(j) for j in range(NB)]
    qs = [q2s[j][:, r * DH:(r + 1) * DH] for j in range(NB) for r in range(REP)]
    outs = []
    done = 0
    s_head = None
    for ci in range(len(qs)):
        if s_head is None:
            s = qk(ci, 0, SK)
        else:
            s = jnp.concatenate([s_head, qk(ci, SPLIT, SK)], axis=1)
        s_head = qk(ci + 1, 0, SPLIT) if (C0 <= ci < len(qs) - 1) else None
        outs.append(softmax_pv(s, late=(ci == len(qs) - 1)))
        if ci % REP == REP - 1 and ci // REP - OPD >= 0:
            oproj(done)
            done += 1
    for j in range(done, NB):
        oproj(j)

    @pl.when(step + 2 < NG)
    def _():
        for d in group_copies(step + 2):
            d.start()

    @pl.when(step == 0)
    def _():
        wmb_cp().start()
        wg_cp().start()

    @pl.when(step == 1)
    def _():
        wu_cp().start()

    @pl.when(step == 2)
    def _():
        wd_cp().start()

    @pl.when(step == NG - 1)
    def _epilogue():
        W2 = LN2U * LANES
        eps_b = _rb(jnp.full((1, 1), LN_EPS, F32))

        def ln2_stats(i, carry):
            cols = pl.ds(pl.multiple_of(i * W2, W2), W2)
            x2 = xt_ref[:, cols].astype(F32) + _tile(modcol(2), LN2U) * acc_ref[:, cols]
            acc_ref[:, cols] = x2
            piv = x2[0:1, :]
            d = x2 - piv
            md = jnp.mean(d, axis=0, keepdims=True)
            var = jnp.maximum(jnp.mean(d * d, axis=0, keepdims=True) - md * md, 0.0)
            rs = 1.0 / _rb(jnp.sqrt(_rb(_rb(var) + eps_b)))
            st_ref[0:1, cols] = rs
            st_ref[1:2, cols] = (piv + md) * rs
            s3 = jnp.sum(d * _tile(wrc_ref[...], LN2U), axis=0, keepdims=True)
            rr = (s3 - md * _tile(rc_ref[0:1, :], LN2U)) * rs + _tile(rc_ref[1:2, :], LN2U)
            for u in range(LN2U):
                r_ref[pl.ds(LN2U * i + u, 1), :] = rr[:, u * LANES:(u + 1) * LANES]
            return carry
        lax.fori_loop(0, S // W2, ln2_stats, 0)

        def ln2_apply(i, carry):
            c0 = pl.multiple_of(i * W2, W2)
            cols = pl.ds(c0, W2)
            x2 = acc_ref[:, cols]
            n = x2 * st_ref[0:1, cols] - st_ref[1:2, cols]
            h2 = n * _tile(modcol(4), LN2U) + _tile(modcol(3), LN2U)
            h2t_ref[:, cols] = pltpu.bitcast(h2.astype(BF16), U32)
            wx_ref[:, pl.ds(pl.multiple_of(FF + c0, LANES), W2)] = (
                x2 + _tile(modcol(5), LN2U) * h2).astype(BF16)
            return carry
        lax.fori_loop(0, S // W2, ln2_apply, 0)

        r = _rb(r_ref[...]) + 0.0
        bits = pltpu.bitcast(r, jnp.int32)
        mono = bits ^ ((bits >> 31) & jnp.int32(0x7FFFFFFF))
        tok = (lax.broadcasted_iota(jnp.int32, (NSL, LANES), 0) * LANES
               + lax.broadcasted_iota(jnp.int32, (NSL, LANES), 1))
        keyi = (((mono >> 16) + 32768) * S + (S - 1 - tok)) + jnp.int32(1 << 29)
        key = pltpu.bitcast(keyi, F32)

        row16 = lax.broadcasted_iota(jnp.int32, (16, LANES), 0)
        lane16 = lax.broadcasted_iota(jnp.int32, (16, LANES), 1)
        rowc = lax.broadcasted_iota(jnp.int32, (16, 1), 0)
        sel_slab, sel_off = [], []
        hsel = jnp.zeros((16, D), F32)
        ksel = jnp.zeros((16, 1), F32)
        for t in range(TOPC):
            kmax = jnp.max(jnp.max(key, axis=0, keepdims=True), axis=1, keepdims=True)
            key = jnp.where(key == kmax, 0.0, key)
            ksel = jnp.where(rowc == t, kmax, ksel)
            ki = pltpu.bitcast(kmax, jnp.int32)[0, 0]
            idx = (S - 1) - (ki & (S - 1))
            slab = idx >> 7
            off = idx & (LANES - 1)
            onehot = jnp.where((row16 == t) & (lane16 == off), 1.0, 0.0).astype(BF16)
            hslab = h2t_ref[:, pl.ds(pl.multiple_of(slab * LANES, LANES), LANES)]
            hsel = hsel + lax.dot_general(onehot, pltpu.bitcast(hslab, BF16), _NT,
                                          preferred_element_type=F32)
            sel_slab.append(slab)
            sel_off.append(off)
        hi = ((pltpu.bitcast(ksel, jnp.int32) - jnp.int32(1 << 29)) // S - 32768) << 16
        rbits = hi ^ ((hi >> 31) & jnp.int32(0x7FFF0000))
        gate = _sigmoid(jnp.where(rowc < TOPC, pltpu.bitcast(rbits, F32), 0.0))

        def out_copy(sl, r0, nr, sem):
            c0 = pl.multiple_of(sl * LANES, LANES)
            return cp(wx_ref.at[r0:r0 + nr, pl.ds(pl.multiple_of(FF + c0, LANES), LANES)],
                      out_hbm.at[r0:r0 + nr, pl.ds(c0, LANES)], sem)

        plain = []
        for sl in range(NSL):
            f = sel_slab[0] != sl
            for t in range(1, TOPC):
                f = f & (sel_slab[t] != sl)
            plain.append(f)
            pl.when(f)(lambda sl=sl: out_copy(sl, 0, D, S_O + sl).start())
        fresh = []
        for t in range(TOPC):
            f = jnp.bool_(True)
            for t2 in range(t):
                f = f & (sel_slab[t] != sel_slab[t2])
            fresh.append(f)

        hs = hsel.astype(BF16)
        gpre = jnp.dot(hs, wg_ref[...], preferred_element_type=F32)
        u = jnp.dot(hs, wu_ref[...], preferred_element_type=F32)
        a = (gpre * _sigmoid(gpre) * u).astype(BF16)

        pieces = [(r0, min(LANES, D - r0)) for r0 in range(0, D, LANES)]

        def down(r0, nr):
            y = lax.dot_general(a, wx_ref[r0:r0 + nr, 0:FF], _NT, preferred_element_type=F32)
            y = jnp.concatenate([y * gate, jnp.zeros((LANES - 16, nr), F32)], axis=0)
            return y.T * modc_ref[5 * D + r0:5 * D + r0 + nr, :]

        def patch(r0, nr, yt):
            lane = lax.broadcasted_iota(jnp.int32, (nr, LANES), 1)
            for t in range(TOPC):
                cols = pl.ds(pl.multiple_of(FF + sel_slab[t] * LANES, LANES), LANES)
                old = wx_ref[r0:r0 + nr, cols].astype(F32)
                upd = pltpu.roll(yt, (sel_off[t] + (LANES - t)) & (LANES - 1), 1)
                wx_ref[r0:r0 + nr, cols] = jnp.where(lane == sel_off[t], old + upd, old).astype(BF16)
            for t in range(TOPC):
                pl.when(fresh[t])(lambda t=t: out_copy(sel_slab[t], r0, nr, S_P + t).start())

        yts = [down(*pieces[0])]
        for n in range(len(pieces)):
            if n + 1 < len(pieces):
                yts.append(down(*pieces[n + 1]))
            patch(*pieces[n], yts[n])

        for sl in range(NSL):
            pl.when(plain[sl])(lambda sl=sl: out_copy(sl, 0, D, S_O + sl).wait())
        for t in range(TOPC):
            @pl.when(fresh[t])
            def _(t=t):
                for r0, nr in pieces:
                    out_copy(sel_slab[t], r0, nr, S_P + t).wait()


@jax.jit
def pallas_adaLN_cond__gqa_block_cached__moe_arch_mod__prompt_kernel(
    A_x: jax.Array,
    A_k_cache: jax.Array,
    A_v_cache: jax.Array,
    A_wq: jax.Array,
    A_wo: jax.Array,
    B_x: jax.Array,
    B_w_r: jax.Array,
    B_w_gate: jax.Array,
    B_w_up: jax.Array,
    B_w_down: jax.Array,
    c: jax.Array,
    w_mod: jax.Array,
):
    del B_x
    B, S, D = A_x.shape
    assert B == 1
    NG, SK = A_k_cache.shape[1], A_k_cache.shape[2]
    REP = HQ // NG
    FF = B_w_gate.shape[1]
    GW = REP * DH

    xt = A_x.reshape(S, D).T
    wot = A_wo.T
    wdt = B_w_down.T
    k = A_k_cache.reshape(NG, SK, DH)
    v = A_v_cache.reshape(NG, SK, DH)
    wr = B_w_r.reshape(1, D)

    hbm = pl.BlockSpec(memory_space=pl.ANY)
    out_t = pl.pallas_call(
        functools.partial(_kernel, S=S, SK=SK, D=D, FF=FF, NG=NG, REP=REP),
        grid=(NG,),
        in_specs=[hbm] * 11,
        out_specs=hbm,
        out_shape=jax.ShapeDtypeStruct((D, S), BF16),
        scratch_shapes=[
            pltpu.VMEM((D, S), BF16),
            pltpu.VMEM((2, SK, DH), BF16),
            pltpu.VMEM((2, SK, DH), BF16),
            pltpu.VMEM((2, D, GW), BF16),
            pltpu.VMEM((2, D, GW), BF16),
            pltpu.VMEM((1, D), BF16),
            pltpu.VMEM((1, D), BF16),
            pltpu.VMEM((D, 6 * D), BF16),
            pltpu.VMEM((D, FF), BF16),
            pltpu.VMEM((D, FF), BF16),
            pltpu.VMEM((D, FF + S), BF16),
            pltpu.VMEM((6 * D, LANES), F32),
            pltpu.VMEM((D, LANES), F32),
            pltpu.VMEM((8, LANES), F32),
            pltpu.VMEM((S // 2, D), U32),
            pltpu.VMEM((D, S), F32),
            pltpu.VMEM((D // 2, S), U32),
            pltpu.VMEM((8, S), F32),
            pltpu.VMEM((S // LANES, LANES), F32),
            pltpu.SemaphoreType.DMA((N_SEMS,)),
        ],
        compiler_params=pltpu.CompilerParams(
            dimension_semantics=("arbitrary",),
            vmem_limit_bytes=100 * 1024 * 1024,
            disable_bounds_checks=True,
        ),
    )(xt, k, v, A_wq, wot, wr, c, w_mod, B_w_gate, B_w_up, wdt)
    return out_t.T.reshape(B, S, D)
```

```python
import functools
import math

import jax
import jax.numpy as jnp
from jax import lax
import jax.experimental.pallas as pl
import jax.experimental.pallas.tpu as pltpu

F32 = jnp.float32
BF16 = jnp.bfloat16
U32 = jnp.uint32

HQ = 32
DH = 128
TOPC = 8
LN_EPS = 1e-5
BQ = 256
LANES = 128
SPLIT = 512
C0 = 2
OPD = 2
XCH = 4
LN2U = 4
MOD_STEP = 4

_NT = (((1,), (1,)), ((), ()))

S_C, S_WMA, S_WMB, S_WR, S_WG, S_WU, S_WD = range(7)
S_X = 7
S_G = S_X + XCH
S_O = S_G + 2
S_P = S_O + 16
N_SEMS = S_P + TOPC


def _rb(x):
    return x.astype(BF16).astype(F32)


def _sigmoid(x):
    return 1.0 / (1.0 + jnp.exp(-x))


def _tile(col, n):
    return jnp.concatenate([col] * n, axis=1)


def _as_cols(row):
    return jnp.broadcast_to(row, (LANES, row.shape[1])).astype(BF16).T


def _kernel(xt_hbm, k_hbm, v_hbm, wq_hbm, wot_hbm, wr_hbm, c_hbm, wmod_hbm,
            wg_hbm, wu_hbm, wdt_hbm,
            out_hbm,
            xt_ref, k_buf, v_buf, wq_buf, wot_buf, wr_ref, c_ref, wmod_ref,
            wg_ref, wu_ref, wx_ref,
            modc_ref, gb_ref, wrc_ref, rc_ref, h_ref, acc_ref, h2t_ref, st_ref, r_ref,
            sems,
            *, S, SK, D, FF, NG, REP):
    step = pl.program_id(0)
    qscale = (DH ** -0.5) * math.log2(math.e)
    NB = S // BQ
    GW = REP * DH
    TCH = S // XCH
    MA = 2 * D
    NSL = S // LANES

    def cp(src, dst, sem):
        return pltpu.make_async_copy(src, dst, sems.at[sem])

    def x_copy(i):
        cols = pl.ds(pl.multiple_of(i * TCH, TCH), TCH)
        return cp(xt_hbm.at[:, cols], xt_ref.at[:, cols], S_X + i)

    def group_copies(grp):
        slot = grp % 2
        cols = pl.ds(pl.multiple_of(grp * GW, GW), GW)
        return (cp(wq_hbm.at[:, cols], wq_buf.at[slot], S_G + slot),
                cp(k_hbm.at[grp], k_buf.at[slot], S_G + slot),
                cp(v_hbm.at[grp], v_buf.at[slot], S_G + slot),
                cp(wot_hbm.at[:, cols], wot_buf.at[slot], S_G + slot))

    c_cp = lambda: cp(c_hbm, c_ref, S_C)
    wma_cp = lambda: cp(wmod_hbm.at[:, 0:MA], wmod_ref.at[:, 0:MA], S_WMA)
    wmb_cp = lambda: cp(wmod_hbm.at[:, MA:6 * D], wmod_ref.at[:, MA:6 * D], S_WMB)
    wr_cp = lambda: cp(wr_hbm, wr_ref, S_WR)
    wg_cp = lambda: cp(wg_hbm, wg_ref, S_WG)
    wu_cp = lambda: cp(wu_hbm, wu_ref, S_WU)
    wd_cp = lambda: cp(wdt_hbm, wx_ref.at[:, 0:FF], S_WD)

    def modcol(i):
        return modc_ref[i * D:(i + 1) * D, :]

    def modulation(lo, hi):
        c = c_ref[...].astype(F32)
        sc8 = jnp.broadcast_to((c * _sigmoid(c)).astype(BF16), (8, D))
        for a in range(lo, hi, MA):
            mod = _rb(jnp.dot(sc8, wmod_ref[:, a:a + MA], preferred_element_type=F32))
            lane = lax.broadcasted_iota(jnp.int32, mod.shape, 1) + a
            is_scale = ((lane >= D) & (lane < 2 * D)) | ((lane >= 4 * D) & (lane < 5 * D))
            mod = jnp.where(is_scale, _rb(1.0 + mod), mod)
            modc_ref[a:a + MA, :] = _as_cols(mod[0:1, :]).astype(F32)
        return mod

    @pl.when(step == 0)
    def _prologue():
        c_cp().start()
        wr_cp().start()
        wma_cp().start()
        for i in range(XCH):
            x_copy(i).start()
        for d in group_copies(0) + group_copies(1):
            d.start()
        c_cp().wait()
        wr_cp().wait()
        wrc_ref[...] = _as_cols(wr_ref[...].astype(F32)).astype(F32)
        acc_ref[...] = jnp.zeros((D, S), F32)
        wma_cp().wait()
        modulation(0, MA)

        def ln1(i, carry):
            x_copy(i).wait()
            x = xt_ref[:, pl.ds(pl.multiple_of(i * TCH, TCH), TCH)].astype(F32)
            piv = x[0:1, :]
            d = x - piv
            md = jnp.mean(d, axis=0, keepdims=True)
            var = jnp.maximum(jnp.mean(d * d, axis=0, keepdims=True) - md * md, 0.0)
            rs = lax.rsqrt(var + LN_EPS)
            n = TCH // LANES
            ht = (x * rs - (piv + md) * rs) * _tile(modcol(1), n) + _tile(modcol(0), n)
            h_ref[pl.ds(pl.multiple_of(i * (TCH // 2), TCH // 2), TCH // 2), :] = pltpu.bitcast(
                ht.astype(BF16).T, U32)
            return carry
        lax.fori_loop(0, XCH, ln1, 0)

    @pl.when(step == MOD_STEP)
    def _late_modulation():
        wmb_cp().wait()
        wg_cp().wait()
        wu_cp().wait()
        wd_cp().wait()
        gb_ref[...] = modulation(MA, 6 * D)[:, D:2 * D]
        wr = wrc_ref[...]
        a = wr * modcol(4)
        wrc_ref[...] = a
        rc_ref[0:1, :] = jnp.sum(a, axis=0, keepdims=True)
        rc_ref[1:2, :] = jnp.sum(wr * modcol(3), axis=0, keepdims=True)

    for d in group_copies(step):
        d.wait()

    slot = step % 2
    k = k_buf[slot]
    v = v_buf[slot]
    wq = wq_buf[slot]
    wot = wot_buf[slot]

    def qproj(j):
        hb = pltpu.bitcast(h_ref[j * (BQ // 2):(j + 1) * (BQ // 2), :], BF16)
        q2 = jnp.dot(hb, wq, preferred_element_type=F32)
        return (q2 * qscale).astype(BF16)

    def qk(ci, lo, hi):
        return lax.dot_general(qs[ci], k[lo:hi], _NT, preferred_element_type=F32)

    def softmax_pv(s, late):
        m = jnp.max(s, axis=1, keepdims=True)
        p = jnp.exp2(s - m)
        o = jnp.dot(p.astype(BF16), v, preferred_element_type=F32)
        if late:
            lp = p[:, 0:LANES]
            for i in range(1, SK // LANES):
                lp = lp + p[:, i * LANES:(i + 1) * LANES]
            l = jnp.sum(jnp.where(lp < 0.0, o, lp), axis=1, keepdims=True)
        else:
            l = jnp.sum(p, axis=1, keepdims=True)
        rl = pl.reciprocal(l, approx=True)
        rl = rl * (2.0 - l * rl)
        return (o * rl).astype(BF16)

    def oproj(j):
        o2 = jnp.concatenate([outs[REP * j + r] for r in range(REP)], axis=1)
        acc_ref[:, j * BQ:(j + 1) * BQ] += lax.dot_general(wot, o2, _NT, preferred_element_type=F32)

    q2s = [qproj(j) for j in range(NB)]
    qs = [q2s[j][:, r * DH:(r + 1) * DH] for j in range(NB) for r in range(REP)]
    outs = []
    done = 0
    s_head = None
    for ci in range(len(qs)):
        if s_head is None:
            s = qk(ci, 0, SK)
        else:
            s = jnp.concatenate([s_head, qk(ci, SPLIT, SK)], axis=1)
        s_head = qk(ci + 1, 0, SPLIT) if (C0 <= ci < len(qs) - 1) else None
        outs.append(softmax_pv(s, late=(ci == len(qs) - 1)))
        if ci % REP == REP - 1 and ci // REP - OPD >= 0:
            oproj(done)
            done += 1
    for j in range(done, NB):
        oproj(j)

    @pl.when(step + 2 < NG)
    def _():
        for d in group_copies(step + 2):
            d.start()

    @pl.when(step == 0)
    def _():
        wmb_cp().start()
        wg_cp().start()

    @pl.when(step == 1)
    def _():
        wu_cp().start()

    @pl.when(step == 2)
    def _():
        wd_cp().start()

    @pl.when(step == NG - 1)
    def _epilogue():
        W2 = LN2U * LANES
        eps_b = _rb(jnp.full((1, 1), LN_EPS, F32))

        def ln2_stats(i, carry):
            cols = pl.ds(pl.multiple_of(i * W2, W2), W2)
            x2 = xt_ref[:, cols].astype(F32) + _tile(modcol(2), LN2U) * acc_ref[:, cols]
            acc_ref[:, cols] = x2
            piv = x2[0:1, :]
            d = x2 - piv
            md = jnp.mean(d, axis=0, keepdims=True)
            var = jnp.maximum(jnp.mean(d * d, axis=0, keepdims=True) - md * md, 0.0)
            rs = 1.0 / _rb(jnp.sqrt(_rb(_rb(var) + eps_b)))
            st_ref[0:1, cols] = rs
            st_ref[1:2, cols] = (piv + md) * rs
            s3 = jnp.sum(d * _tile(wrc_ref[...], LN2U), axis=0, keepdims=True)
            rr = (s3 - md * _tile(rc_ref[0:1, :], LN2U)) * rs + _tile(rc_ref[1:2, :], LN2U)
            for u in range(LN2U):
                r_ref[pl.ds(LN2U * i + u, 1), :] = rr[:, u * LANES:(u + 1) * LANES]
            return carry
        lax.fori_loop(0, S // W2, ln2_stats, 0)

        def ln2_apply(i, carry):
            c0 = pl.multiple_of(i * W2, W2)
            cols = pl.ds(c0, W2)
            x2 = acc_ref[:, cols]
            n = x2 * st_ref[0:1, cols] - st_ref[1:2, cols]
            h2 = n * _tile(modcol(4), LN2U) + _tile(modcol(3), LN2U)
            h2t_ref[:, cols] = pltpu.bitcast(h2.astype(BF16), U32)
            wx_ref[:, pl.ds(pl.multiple_of(FF + c0, LANES), W2)] = (
                x2 + _tile(modcol(5), LN2U) * h2).astype(BF16)
            return carry
        lax.fori_loop(0, S // W2, ln2_apply, 0)

        r = _rb(r_ref[...]) + 0.0
        bits = pltpu.bitcast(r, jnp.int32)
        mono = bits ^ ((bits >> 31) & jnp.int32(0x7FFFFFFF))
        tok = (lax.broadcasted_iota(jnp.int32, (NSL, LANES), 0) * LANES
               + lax.broadcasted_iota(jnp.int32, (NSL, LANES), 1))
        keyi = (((mono >> 16) + 32768) * S + (S - 1 - tok)) + jnp.int32(1 << 29)
        key = pltpu.bitcast(keyi, F32)

        row16 = lax.broadcasted_iota(jnp.int32, (16, LANES), 0)
        lane16 = lax.broadcasted_iota(jnp.int32, (16, LANES), 1)
        rowc = lax.broadcasted_iota(jnp.int32, (16, 1), 0)
        sel_slab, sel_off = [], []
        hsel = jnp.zeros((16, D), F32)
        osel = jnp.zeros((16, D), F32)
        ksel = jnp.zeros((16, 1), F32)
        for t in range(TOPC):
            kmax = jnp.max(jnp.max(key, axis=0, keepdims=True), axis=1, keepdims=True)
            key = jnp.where(key == kmax, 0.0, key)
            ksel = jnp.where(rowc == t, kmax, ksel)
            ki = pltpu.bitcast(kmax, jnp.int32)[0, 0]
            idx = (S - 1) - (ki & (S - 1))
            slab = idx >> 7
            off = idx & (LANES - 1)
            onehot = jnp.where((row16 == t) & (lane16 == off), 1.0, 0.0).astype(BF16)
            hslab = h2t_ref[:, pl.ds(pl.multiple_of(slab * LANES, LANES), LANES)]
            hsel = hsel + lax.dot_general(onehot, pltpu.bitcast(hslab, BF16), _NT,
                                          preferred_element_type=F32)
            oslab = wx_ref[:, pl.ds(pl.multiple_of(FF + slab * LANES, LANES), LANES)]
            osel = osel + lax.dot_general(onehot, oslab, _NT, preferred_element_type=F32)
            sel_slab.append(slab)
            sel_off.append(off)
        hi = ((pltpu.bitcast(ksel, jnp.int32) - jnp.int32(1 << 29)) // S - 32768) << 16
        rbits = hi ^ ((hi >> 31) & jnp.int32(0x7FFF0000))
        gate = _sigmoid(jnp.where(rowc < TOPC, pltpu.bitcast(rbits, F32), 0.0))

        def out_copy(sl, r0, nr, sem):
            c0 = pl.multiple_of(sl * LANES, LANES)
            return cp(wx_ref.at[r0:r0 + nr, pl.ds(pl.multiple_of(FF + c0, LANES), LANES)],
                      out_hbm.at[r0:r0 + nr, pl.ds(c0, LANES)], sem)

        fresh = []
        seen = jnp.int32(0)
        for t in range(TOPC):
            fresh.append(((seen >> sel_slab[t]) & 1) == 0)
            seen = seen | (1 << sel_slab[t])
        plain = [((seen >> sl) & 1) == 0 for sl in range(NSL)]
        for sl in range(NSL):
            pl.when(plain[sl])(lambda sl=sl: out_copy(sl, 0, D, S_O + sl).start())

        hs = hsel.astype(BF16)
        gpre = jnp.dot(hs, wg_ref[...], preferred_element_type=F32)
        u = jnp.dot(hs, wu_ref[...], preferred_element_type=F32)
        a = (gpre * _sigmoid(gpre) * u).astype(BF16)

        pieces = [(r0, min(LANES, D - r0)) for r0 in range(0, D, LANES)]

        coef = gate * gb_ref[0:1, :]

        def down(r0, nr):
            y = lax.dot_general(a, wx_ref[r0:r0 + nr, 0:FF], _NT, preferred_element_type=F32)
            return osel[:, r0:r0 + nr] + y * coef[:, r0:r0 + nr]

        def patch(r0, nr, new):
            lane = lax.broadcasted_iota(jnp.int32, (nr // 2, LANES), 1)
            for t in range(TOPC):
                cols = pl.ds(pl.multiple_of(FF + sel_slab[t] * LANES, LANES), LANES)
                old = pltpu.bitcast(wx_ref[r0:r0 + nr, cols], U32)
                upd = pltpu.bitcast(_as_cols(new[t:t + 1, :]), U32)
                wx_ref[r0:r0 + nr, cols] = pltpu.bitcast(jnp.where(lane == sel_off[t], upd, old), BF16)
            for t in range(TOPC):
                pl.when(fresh[t])(lambda t=t: out_copy(sel_slab[t], r0, nr, S_P + t).start())

        yts = [down(*pieces[0])]
        for n in range(len(pieces)):
            if n + 1 < len(pieces):
                yts.append(down(*pieces[n + 1]))
            patch(*pieces[n], yts[n])

        for sl in range(NSL):
            pl.when(plain[sl])(lambda sl=sl: out_copy(sl, 0, D, S_O + sl).wait())
        for t in range(TOPC):
            @pl.when(fresh[t])
            def _(t=t):
                for r0, nr in pieces:
                    out_copy(sel_slab[t], r0, nr, S_P + t).wait()


@jax.jit
def pallas_adaLN_cond__gqa_block_cached__moe_arch_mod__prompt_kernel(
    A_x: jax.Array,
    A_k_cache: jax.Array,
    A_v_cache: jax.Array,
    A_wq: jax.Array,
    A_wo: jax.Array,
    B_x: jax.Array,
    B_w_r: jax.Array,
    B_w_gate: jax.Array,
    B_w_up: jax.Array,
    B_w_down: jax.Array,
    c: jax.Array,
    w_mod: jax.Array,
):
    del B_x
    B, S, D = A_x.shape
    assert B == 1
    NG, SK = A_k_cache.shape[1], A_k_cache.shape[2]
    REP = HQ // NG
    FF = B_w_gate.shape[1]
    GW = REP * DH

    xt = A_x.reshape(S, D).T
    wot = A_wo.T
    wdt = B_w_down.T
    k = A_k_cache.reshape(NG, SK, DH)
    v = A_v_cache.reshape(NG, SK, DH)
    wr = B_w_r.reshape(1, D)

    hbm = pl.BlockSpec(memory_space=pl.ANY)
    out_t = pl.pallas_call(
        functools.partial(_kernel, S=S, SK=SK, D=D, FF=FF, NG=NG, REP=REP),
        grid=(NG,),
        in_specs=[hbm] * 11,
        out_specs=hbm,
        out_shape=jax.ShapeDtypeStruct((D, S), BF16),
        scratch_shapes=[
            pltpu.VMEM((D, S), BF16),
            pltpu.VMEM((2, SK, DH), BF16),
            pltpu.VMEM((2, SK, DH), BF16),
            pltpu.VMEM((2, D, GW), BF16),
            pltpu.VMEM((2, D, GW), BF16),
            pltpu.VMEM((1, D), BF16),
            pltpu.VMEM((1, D), BF16),
            pltpu.VMEM((D, 6 * D), BF16),
            pltpu.VMEM((D, FF), BF16),
            pltpu.VMEM((D, FF), BF16),
            pltpu.VMEM((D, FF + S), BF16),
            pltpu.VMEM((6 * D, LANES), F32),
            pltpu.VMEM((8, D), F32),
            pltpu.VMEM((D, LANES), F32),
            pltpu.VMEM((8, LANES), F32),
            pltpu.VMEM((S // 2, D), U32),
            pltpu.VMEM((D, S), F32),
            pltpu.VMEM((D // 2, S), U32),
            pltpu.VMEM((8, S), F32),
            pltpu.VMEM((S // LANES, LANES), F32),
            pltpu.SemaphoreType.DMA((N_SEMS,)),
        ],
        compiler_params=pltpu.CompilerParams(
            dimension_semantics=("arbitrary",),
            vmem_limit_bytes=100 * 1024 * 1024,
            disable_bounds_checks=True,
        ),
    )(xt, k, v, A_wq, wot, wr, c, w_mod, B_w_gate, B_w_up, wdt)
    return out_t.T.reshape(B, S, D)
```

```python
import functools
import math

import jax
import jax.numpy as jnp
from jax import lax
import jax.experimental.pallas as pl
import jax.experimental.pallas.tpu as pltpu

F32 = jnp.float32
BF16 = jnp.bfloat16
U32 = jnp.uint32

HQ = 32
DH = 128
TOPC = 8
LN_EPS = 1e-5
BQ = 256
LANES = 128
SPLIT = 512
C0 = 2
OPD = 2
XCH = 4
LN2U = 4
UNROLL_STATS = 0
UNROLL_APPLY = 0
MOD_STEP = 4

_NT = (((1,), (1,)), ((), ()))

S_C, S_WMA, S_WMB, S_WR, S_WG, S_WU, S_WD = range(7)
S_X = 7
S_G = S_X + XCH
S_O = S_G + 2
N_SEMS = S_O + 1


def _rb(x):
    return x.astype(BF16).astype(F32)


def _sigmoid(x):
    return 1.0 / (1.0 + jnp.exp(-x))


def _mo(x, n):
    return x if isinstance(x, int) else pl.multiple_of(x, n)


def _tile(col, n):
    return jnp.concatenate([col] * n, axis=1)


def _as_cols(row):
    return jnp.broadcast_to(row, (LANES, row.shape[1])).astype(BF16).T


def _kernel(xt_hbm, k_hbm, v_hbm, wq_hbm, wot_hbm, wr_hbm, c_hbm, wmod_hbm,
            wg_hbm, wu_hbm, wdt_hbm,
            out_hbm,
            xt_ref, k_buf, v_buf, wq_buf, wot_buf, wr_ref, c_ref, wmod_ref,
            wg_ref, wu_ref, wx_ref,
            modc_ref, gb_ref, wrc_ref, rc_ref, h_ref, acc_ref, h2t_ref, st_ref, r_ref,
            sems,
            *, S, SK, D, FF, NG, REP):
    step = pl.program_id(0)
    qscale = (DH ** -0.5) * math.log2(math.e)
    NB = S // BQ
    GW = REP * DH
    TCH = S // XCH
    MA = 2 * D
    NSL = S // LANES

    def cp(src, dst, sem):
        return pltpu.make_async_copy(src, dst, sems.at[sem])

    def x_copy(i):
        cols = pl.ds(pl.multiple_of(i * TCH, TCH), TCH)
        return cp(xt_hbm.at[:, cols], xt_ref.at[:, cols], S_X + i)

    def group_copies(grp):
        slot = grp % 2
        cols = pl.ds(pl.multiple_of(grp * GW, GW), GW)
        return (cp(wq_hbm.at[:, cols], wq_buf.at[slot], S_G + slot),
                cp(k_hbm.at[grp], k_buf.at[slot], S_G + slot),
                cp(v_hbm.at[grp], v_buf.at[slot], S_G + slot),
                cp(wot_hbm.at[:, cols], wot_buf.at[slot], S_G + slot))

    c_cp = lambda: cp(c_hbm, c_ref, S_C)
    wma_cp = lambda: cp(wmod_hbm.at[:, 0:MA], wmod_ref.at[:, 0:MA], S_WMA)
    wmb_cp = lambda: cp(wmod_hbm.at[:, MA:6 * D], wmod_ref.at[:, MA:6 * D], S_WMB)
    wr_cp = lambda: cp(wr_hbm, wr_ref, S_WR)
    wg_cp = lambda: cp(wg_hbm, wg_ref, S_WG)
    wu_cp = lambda: cp(wu_hbm, wu_ref, S_WU)
    wd_cp = lambda: cp(wdt_hbm, wx_ref.at[:, 0:FF], S_WD)

    def modcol(i):
        return modc_ref[i * D:(i + 1) * D, :]

    def modulation(lo, hi):
        c = c_ref[...].astype(F32)
        sc8 = jnp.broadcast_to((c * _sigmoid(c)).astype(BF16), (8, D))
        for a in range(lo, hi, MA):
            mod = _rb(jnp.dot(sc8, wmod_ref[:, a:a + MA], preferred_element_type=F32))
            lane = lax.broadcasted_iota(jnp.int32, mod.shape, 1) + a
            is_scale = ((lane >= D) & (lane < 2 * D)) | ((lane >= 4 * D) & (lane < 5 * D))
            mod = jnp.where(is_scale, _rb(1.0 + mod), mod)
            modc_ref[a:a + MA, :] = _as_cols(mod[0:1, :]).astype(F32)
        return mod

    @pl.when(step == 0)
    def _prologue():
        wma_cp().start()
        c_cp().start()
        for i in range(XCH):
            x_copy(i).start()
        for d in group_copies(0) + group_copies(1):
            d.start()
        wr_cp().start()
        acc_ref[...] = jnp.zeros((D, S), F32)
        wma_cp().wait()
        c_cp().wait()
        modulation(0, MA)

        def ln1(i, carry):
            x_copy(i).wait()
            x = xt_ref[:, pl.ds(pl.multiple_of(i * TCH, TCH), TCH)].astype(F32)
            piv = x[0:1, :]
            d = x - piv
            md = jnp.mean(d, axis=0, keepdims=True)
            var = jnp.maximum(jnp.mean(d * d, axis=0, keepdims=True) - md * md, 0.0)
            rs = lax.rsqrt(var + LN_EPS)
            n = TCH // LANES
            ht = (x * rs - (piv + md) * rs) * _tile(modcol(1), n) + _tile(modcol(0), n)
            h_ref[pl.ds(pl.multiple_of(i * (TCH // 2), TCH // 2), TCH // 2), :] = pltpu.bitcast(
                ht.astype(BF16).T, U32)
            return carry
        lax.fori_loop(0, XCH, ln1, 0)

    @pl.when(step == MOD_STEP)
    def _late_modulation():
        wr_cp().wait()
        wmb_cp().wait()
        wg_cp().wait()
        wu_cp().wait()
        wd_cp().wait()
        gb_ref[...] = modulation(MA, 6 * D)[:, D:2 * D]
        wr = _as_cols(wr_ref[...].astype(F32).reshape(1, D)).astype(F32)
        a = wr * modcol(4)
        wrc_ref[...] = a
        rc_ref[0:1, :] = jnp.sum(a, axis=0, keepdims=True)
        rc_ref[1:2, :] = jnp.sum(wr * modcol(3), axis=0, keepdims=True)

    for d in group_copies(step):
        d.wait()

    slot = step % 2
    k = k_buf[slot]
    v = v_buf[slot]
    wq = wq_buf[slot]
    wot = wot_buf[slot]

    def qproj(j):
        hb = pltpu.bitcast(h_ref[j * (BQ // 2):(j + 1) * (BQ // 2), :], BF16)
        q2 = jnp.dot(hb, wq, preferred_element_type=F32)
        return (q2 * qscale).astype(BF16)

    def qk(ci, lo, hi):
        return lax.dot_general(qs[ci], k[lo:hi], _NT, preferred_element_type=F32)

    def softmax_pv(s, late):
        m = jnp.max(s, axis=1, keepdims=True)
        p = jnp.exp2(s - m)
        o = jnp.dot(p.astype(BF16), v, preferred_element_type=F32)
        if late:
            lp = p[:, 0:LANES]
            for i in range(1, SK // LANES):
                lp = lp + p[:, i * LANES:(i + 1) * LANES]
            l = jnp.sum(jnp.where(lp < 0.0, o, lp), axis=1, keepdims=True)
        else:
            l = jnp.sum(p, axis=1, keepdims=True)
        rl = pl.reciprocal(l, approx=True)
        rl = rl * (2.0 - l * rl)
        return (o * rl).astype(BF16)

    def oproj(j):
        o2 = jnp.concatenate([outs[REP * j + r] for r in range(REP)], axis=1)
        acc_ref[:, j * BQ:(j + 1) * BQ] += lax.dot_general(wot, o2, _NT, preferred_element_type=F32)

    q2s = [qproj(j) for j in range(NB)]
    qs = [q2s[j][:, r * DH:(r + 1) * DH] for j in range(NB) for r in range(REP)]
    outs = []
    done = 0
    s_head = None
    for ci in range(len(qs)):
        if s_head is None:
            s = qk(ci, 0, SK)
        else:
            s = jnp.concatenate([s_head, qk(ci, SPLIT, SK)], axis=1)
        s_head = qk(ci + 1, 0, SPLIT) if (C0 <= ci < len(qs) - 1) else None
        outs.append(softmax_pv(s, late=(ci == len(qs) - 1)))
        if ci % REP == REP - 1 and ci // REP - OPD >= 0:
            oproj(done)
            done += 1
    for j in range(done, NB):
        oproj(j)

    @pl.when(step + 2 < NG)
    def _():
        for d in group_copies(step + 2):
            d.start()

    @pl.when(step == 0)
    def _():
        wmb_cp().start()
        wg_cp().start()

    @pl.when(step == 1)
    def _():
        wu_cp().start()

    @pl.when(step == 2)
    def _():
        wd_cp().start()

    @pl.when(step == NG - 1)
    def _epilogue():
        W2 = LN2U * LANES
        eps_b = _rb(jnp.full((1, 1), LN_EPS, F32))

        def ln2_stats(i, carry):
            cols = pl.ds(_mo(i * W2, W2), W2)
            x2 = xt_ref[:, cols].astype(F32) + _tile(modcol(2), LN2U) * acc_ref[:, cols]
            acc_ref[:, cols] = x2
            piv = x2[0:1, :]
            d = x2 - piv
            md = jnp.mean(d, axis=0, keepdims=True)
            var = jnp.maximum(jnp.mean(d * d, axis=0, keepdims=True) - md * md, 0.0)
            rs = 1.0 / _rb(jnp.sqrt(_rb(_rb(var) + eps_b)))
            st_ref[0:1, cols] = rs
            st_ref[1:2, cols] = (piv + md) * rs
            s3 = jnp.sum(d * _tile(wrc_ref[...], LN2U), axis=0, keepdims=True)
            rr = (s3 - md * _tile(rc_ref[0:1, :], LN2U)) * rs + _tile(rc_ref[1:2, :], LN2U)
            for u in range(LN2U):
                r_ref[pl.ds(LN2U * i + u, 1), :] = rr[:, u * LANES:(u + 1) * LANES]
            return carry
        if UNROLL_STATS:
            @pl.when(step > 0)
            def _():
                for i in range(S // W2):
                    ln2_stats(i, 0)
        else:
            lax.fori_loop(0, S // W2, ln2_stats, 0)

        def ln2_apply(i, carry):
            c0 = _mo(i * W2, W2)
            cols = pl.ds(c0, W2)
            x2 = acc_ref[:, cols]
            n = x2 * st_ref[0:1, cols] - st_ref[1:2, cols]
            h2 = n * _tile(modcol(4), LN2U) + _tile(modcol(3), LN2U)
            h2t_ref[:, cols] = pltpu.bitcast(h2.astype(BF16), U32)
            wx_ref[:, pl.ds(_mo(FF + c0, LANES), W2)] = (
                x2 + _tile(modcol(5), LN2U) * h2).astype(BF16)
            return carry
        if UNROLL_APPLY:
            for i in range(S // W2):
                ln2_apply(i, 0)
        else:
            lax.fori_loop(0, S // W2, ln2_apply, 0)

        r = _rb(r_ref[...]) + 0.0
        bits = pltpu.bitcast(r, jnp.int32)
        mono = bits ^ ((bits >> 31) & jnp.int32(0x7FFFFFFF))
        tok = (lax.broadcasted_iota(jnp.int32, (NSL, LANES), 0) * LANES
               + lax.broadcasted_iota(jnp.int32, (NSL, LANES), 1))
        keyi = (((mono >> 16) + 32768) * S + (S - 1 - tok)) + jnp.int32(1 << 29)
        key = pltpu.bitcast(keyi, F32)

        row16 = lax.broadcasted_iota(jnp.int32, (16, LANES), 0)
        lane16 = lax.broadcasted_iota(jnp.int32, (16, LANES), 1)
        rowc = lax.broadcasted_iota(jnp.int32, (16, 1), 0)
        sel_slab, sel_off = [], []
        hsel = jnp.zeros((16, D), F32)
        osel = jnp.zeros((16, D), F32)
        ksel = jnp.zeros((16, 1), F32)
        for t in range(TOPC):
            kmax = jnp.max(jnp.max(key, axis=0, keepdims=True), axis=1, keepdims=True)
            key = jnp.where(key == kmax, 0.0, key)
            ksel = jnp.where(rowc == t, kmax, ksel)
            ki = pltpu.bitcast(kmax, jnp.int32)[0, 0]
            idx = (S - 1) - (ki & (S - 1))
            slab = idx >> 7
            off = idx & (LANES - 1)
            onehot = jnp.where((row16 == t) & (lane16 == off), 1.0, 0.0).astype(BF16)
            hslab = h2t_ref[:, pl.ds(pl.multiple_of(slab * LANES, LANES), LANES)]
            hsel = hsel + lax.dot_general(onehot, pltpu.bitcast(hslab, BF16), _NT,
                                          preferred_element_type=F32)
            oslab = wx_ref[:, pl.ds(pl.multiple_of(FF + slab * LANES, LANES), LANES)]
            osel = osel + lax.dot_general(onehot, oslab, _NT, preferred_element_type=F32)
            sel_slab.append(slab)
            sel_off.append(off)
        hi = ((pltpu.bitcast(ksel, jnp.int32) - jnp.int32(1 << 29)) // S - 32768) << 16
        rbits = hi ^ ((hi >> 31) & jnp.int32(0x7FFF0000))
        gate = _sigmoid(jnp.where(rowc < TOPC, pltpu.bitcast(rbits, F32), 0.0))

        def out_copy(sl, r0, nr):
            c0 = pl.multiple_of(sl * LANES, LANES)
            return cp(wx_ref.at[r0:r0 + nr, pl.ds(pl.multiple_of(FF + c0, LANES), LANES)],
                      out_hbm.at[r0:r0 + nr, pl.ds(c0, LANES)], S_O)

        fresh = []
        seen = jnp.int32(0)
        for t in range(TOPC):
            fresh.append(((seen >> sel_slab[t]) & 1) == 0)
            seen = seen | (1 << sel_slab[t])
        plain = [((seen >> sl) & 1) == 0 for sl in range(NSL)]
        for sl in range(NSL):
            pl.when(plain[sl])(lambda sl=sl: out_copy(sl, 0, D).start())

        hs = hsel.astype(BF16)
        gpre = jnp.dot(hs, wg_ref[...], preferred_element_type=F32)
        u = jnp.dot(hs, wu_ref[...], preferred_element_type=F32)
        a = (gpre * _sigmoid(gpre) * u).astype(BF16)

        pieces = [(r0, min(LANES, D - r0)) for r0 in range(0, D, LANES)]

        coef = gate * gb_ref[0:1, :]

        def down(r0, nr):
            y = lax.dot_general(a, wx_ref[r0:r0 + nr, 0:FF], _NT, preferred_element_type=F32)
            return osel[:, r0:r0 + nr] + y * coef[:, r0:r0 + nr]

        def patch(r0, nr, new):
            lane = lax.broadcasted_iota(jnp.int32, (nr // 2, LANES), 1)
            for t in range(TOPC):
                cols = pl.ds(pl.multiple_of(FF + sel_slab[t] * LANES, LANES), LANES)
                old = pltpu.bitcast(wx_ref[r0:r0 + nr, cols], U32)
                upd = pltpu.bitcast(_as_cols(new[t:t + 1, :]), U32)
                wx_ref[r0:r0 + nr, cols] = pltpu.bitcast(jnp.where(lane == sel_off[t], upd, old), BF16)
            for t in range(TOPC):
                pl.when(fresh[t])(lambda t=t: out_copy(sel_slab[t], r0, nr).start())

        yts = [down(*pieces[0])]
        for n in range(len(pieces)):
            if n + 1 < len(pieces):
                yts.append(down(*pieces[n + 1]))
            patch(*pieces[n], yts[n])

        cp(wx_ref.at[:, FF:FF + S], out_hbm, S_O).wait()


@jax.jit
def pallas_adaLN_cond__gqa_block_cached__moe_arch_mod__prompt_kernel(
    A_x: jax.Array,
    A_k_cache: jax.Array,
    A_v_cache: jax.Array,
    A_wq: jax.Array,
    A_wo: jax.Array,
    B_x: jax.Array,
    B_w_r: jax.Array,
    B_w_gate: jax.Array,
    B_w_up: jax.Array,
    B_w_down: jax.Array,
    c: jax.Array,
    w_mod: jax.Array,
):
    del B_x
    B, S, D = A_x.shape
    assert B == 1
    NG, SK = A_k_cache.shape[1], A_k_cache.shape[2]
    REP = HQ // NG
    FF = B_w_gate.shape[1]
    GW = REP * DH

    xt = A_x.reshape(S, D).T
    wot = A_wo.T
    wdt = B_w_down.T
    k = A_k_cache.reshape(NG, SK, DH)
    v = A_v_cache.reshape(NG, SK, DH)

    hbm = pl.BlockSpec(memory_space=pl.ANY)
    out_t = pl.pallas_call(
        functools.partial(_kernel, S=S, SK=SK, D=D, FF=FF, NG=NG, REP=REP),
        grid=(NG,),
        in_specs=[hbm] * 11,
        out_specs=hbm,
        out_shape=jax.ShapeDtypeStruct((D, S), BF16),
        scratch_shapes=[
            pltpu.VMEM((D, S), BF16),
            pltpu.VMEM((2, SK, DH), BF16),
            pltpu.VMEM((2, SK, DH), BF16),
            pltpu.VMEM((2, D, GW), BF16),
            pltpu.VMEM((2, D, GW), BF16),
            pltpu.VMEM((D,), BF16),
            pltpu.VMEM((1, D), BF16),
            pltpu.VMEM((D, 6 * D), BF16),
            pltpu.VMEM((D, FF), BF16),
            pltpu.VMEM((D, FF), BF16),
            pltpu.VMEM((D, FF + S), BF16),
            pltpu.VMEM((6 * D, LANES), F32),
            pltpu.VMEM((8, D), F32),
            pltpu.VMEM((D, LANES), F32),
            pltpu.VMEM((8, LANES), F32),
            pltpu.VMEM((S // 2, D), U32),
            pltpu.VMEM((D, S), F32),
            pltpu.VMEM((D // 2, S), U32),
            pltpu.VMEM((8, S), F32),
            pltpu.VMEM((S // LANES, LANES), F32),
            pltpu.SemaphoreType.DMA((N_SEMS,)),
        ],
        compiler_params=pltpu.CompilerParams(
            dimension_semantics=("arbitrary",),
            vmem_limit_bytes=100 * 1024 * 1024,
            disable_bounds_checks=True,
        ),
    )(xt, k, v, A_wq, wot, B_w_r, c, w_mod, B_w_gate, B_w_up, wdt)
    return out_t.T.reshape(B, S, D)
```

```python
import functools
import math

import jax
import jax.numpy as jnp
from jax import lax
import jax.experimental.pallas as pl
import jax.experimental.pallas.tpu as pltpu

F32 = jnp.float32
BF16 = jnp.bfloat16
U32 = jnp.uint32

HQ = 32
DH = 128
TOPC = 8
LN_EPS = 1e-5
BQ = 256
LANES = 128
SPLIT = 512
C0 = 2
OPD = 2
XCH = 4
LN2U = 1
OUW = 2
GATED = 0
TK_TIES = [0, 2, 3, 5, 6]
OPR = 16
SPR = 128
UNROLL_STATS = 1
MOD_STEP = 4

_NT = (((1,), (1,)), ((), ()))

S_C, S_WMA, S_WMB, S_WR, S_WG, S_WU, S_WD = range(7)
S_X = 7
S_G = S_X + XCH
S_O = S_G + 2
N_SEMS = S_O + 1


def _rb(x):
    return x.astype(BF16).astype(F32)


def _sigmoid(x):
    return 1.0 / (1.0 + jnp.exp(-x))


def _mo(x, n):
    return x if isinstance(x, int) else pl.multiple_of(x, n)


def _tile(col, n):
    return jnp.concatenate([col] * n, axis=1)


def _as_cols(row):
    return jnp.broadcast_to(row, (LANES, row.shape[1])).astype(BF16).T


def _kernel(xt_hbm, k_hbm, v_hbm, wq_hbm, wot_hbm, wr_hbm, c_hbm, wmod_hbm,
            wg_hbm, wu_hbm, wdt_hbm,
            out_hbm,
            xt_ref, k_buf, v_buf, wq_buf, wot_buf, wr_ref, c_ref, wmod_ref,
            wg_ref, wu_ref, wx_ref,
            modc_ref, mrow_ref, lhs_ref, rc_ref, h_ref, acc_ref, db_ref, st_ref, r_ref,
            sems,
            *, S, SK, D, FF, NG, REP):
    step = pl.program_id(0)
    qscale = (DH ** -0.5) * math.log2(math.e)
    NB = S // BQ
    GW = REP * DH
    TCH = S // XCH
    MA = 2 * D
    NSL = S // LANES

    def cp(src, dst, sem):
        return pltpu.make_async_copy(src, dst, sems.at[sem])

    def x_copy(i):
        cols = pl.ds(pl.multiple_of(i * TCH, TCH), TCH)
        return cp(xt_hbm.at[:, cols], xt_ref.at[:, cols], S_X + i)

    def group_copies(grp):
        slot = grp % 2
        cols = pl.ds(pl.multiple_of(grp * GW, GW), GW)
        return (cp(wq_hbm.at[:, cols], wq_buf.at[slot], S_G + slot),
                cp(k_hbm.at[grp], k_buf.at[slot], S_G + slot),
                cp(v_hbm.at[grp], v_buf.at[slot], S_G + slot),
                cp(wot_hbm.at[:, cols], wot_buf.at[slot], S_G + slot))

    c_cp = lambda: cp(c_hbm, c_ref, S_C)
    wma_cp = lambda: cp(wmod_hbm.at[:, 0:MA], wmod_ref.at[:, 0:MA], S_WMA)
    wmb_cp = lambda: cp(wmod_hbm.at[:, MA:6 * D], wmod_ref.at[:, MA:6 * D], S_WMB)
    wr_cp = lambda: cp(wr_hbm, wr_ref, S_WR)
    wg_cp = lambda: cp(wg_hbm, wg_ref, S_WG)
    wu_cp = lambda: cp(wu_hbm, wu_ref, S_WU)
    wd_cp = lambda: cp(wdt_hbm, wx_ref.at[:, 0:FF], S_WD)

    def modcol(i):
        return modc_ref[i * D:(i + 1) * D, :]

    def modulation(lo, hi):
        c = c_ref[...].astype(F32)
        sc8 = jnp.broadcast_to((c * _sigmoid(c)).astype(BF16), (8, D))
        mods = []
        for a in range(lo, hi, MA):
            mod = _rb(jnp.dot(sc8, wmod_ref[:, a:a + MA], preferred_element_type=F32))
            lane = lax.broadcasted_iota(jnp.int32, mod.shape, 1) + a
            is_scale = ((lane >= D) & (lane < 2 * D)) | ((lane >= 4 * D) & (lane < 5 * D))
            mods.append(jnp.where(is_scale, _rb(1.0 + mod), mod))
        return mods

    @pl.when(step == 0)
    def _prologue():
        wma_cp().start()
        c_cp().start()
        for i in range(XCH):
            x_copy(i).start()
        for d in group_copies(0) + group_copies(1):
            d.start()
        wr_cp().start()
        acc_ref[...] = jnp.zeros((D, S), F32)
        wma_cp().wait()
        c_cp().wait()
        modc_ref[0:MA, :] = _as_cols(modulation(0, MA)[0][0:1, :]).astype(F32)

        def ln1(i, carry):
            x_copy(i).wait()
            x = xt_ref[:, pl.ds(pl.multiple_of(i * TCH, TCH), TCH)].astype(F32)
            piv = x[0:1, :]
            d = x - piv
            md = jnp.mean(d, axis=0, keepdims=True)
            var = jnp.maximum(jnp.mean(d * d, axis=0, keepdims=True) - md * md, 0.0)
            rs = lax.rsqrt(var + LN_EPS)
            st_ref[2:3, pl.ds(pl.multiple_of(i * TCH, TCH), TCH)] = piv + md
            n = TCH // LANES
            ht = (x * rs - (piv + md) * rs) * _tile(modcol(1), n) + _tile(modcol(0), n)
            h_ref[pl.ds(pl.multiple_of(i * (TCH // 2), TCH // 2), TCH // 2), :] = pltpu.bitcast(
                ht.astype(BF16).T, U32)
            return carry
        lax.fori_loop(0, XCH, ln1, 0)

    @pl.when(step == MOD_STEP)
    def _late_modulation():
        wr_cp().wait()
        wmb_cp().wait()
        wg_cp().wait()
        wu_cp().wait()
        wd_cp().wait()
        m23, m45 = modulation(MA, 6 * D)
        sb, cb, gb = m23[:, D:MA], m45[:, 0:D], m45[:, D:MA]
        mrow_ref[0] = sb
        mrow_ref[1] = cb
        mrow_ref[2] = gb
        c23 = _as_cols(m23[0:1, :]).astype(F32)
        c45 = _as_cols(m45[0:1, :]).astype(F32)
        modc_ref[0:D, :] = c23[0:D]
        modc_ref[D:MA, :] = c45[D:MA] * c45[0:D]
        modc_ref[MA:3 * D, :] = c45[D:MA] * c23[D:MA]
        wr = wr_ref[...].astype(F32).reshape(1, D)
        wc = wr * cb[0:1, :]
        whi = _rb(wc)
        row = lax.broadcasted_iota(jnp.int32, (16, D), 0)
        lhs_ref[...] = jnp.where(row == 0, 1.0, jnp.where(row == 1, whi, jnp.where(
            row == 2, wc - whi, 0.0))).astype(BF16)
        rc_ref[0:1, :] = jnp.broadcast_to(jnp.sum(wc, axis=1, keepdims=True), (1, LANES))
        rc_ref[1:2, :] = jnp.broadcast_to(jnp.sum(wr * sb[0:1, :], axis=1, keepdims=True), (1, LANES))

    for d in group_copies(step):
        d.wait()

    slot = step % 2
    k = k_buf[slot]
    v = v_buf[slot]
    wq = wq_buf[slot]
    wot = wot_buf[slot]

    def qproj(j):
        hb = pltpu.bitcast(h_ref[j * (BQ // 2):(j + 1) * (BQ // 2), :], BF16)
        q2 = jnp.dot(hb, wq, preferred_element_type=F32)
        return (q2 * qscale).astype(BF16)

    def qk(ci, lo, hi):
        return lax.dot_general(qs[ci], k[lo:hi], _NT, preferred_element_type=F32)

    def softmax_pv(s, late):
        m = jnp.max(s, axis=1, keepdims=True)
        p = jnp.exp2(s - m)
        o = jnp.dot(p.astype(BF16), v, preferred_element_type=F32)
        if late:
            lp = p[:, 0:LANES]
            for i in range(1, SK // LANES):
                lp = lp + p[:, i * LANES:(i + 1) * LANES]
            l = jnp.sum(jnp.where(lp < 0.0, o, lp), axis=1, keepdims=True)
        else:
            l = jnp.sum(p, axis=1, keepdims=True)
        rl = pl.reciprocal(l, approx=True)
        rl = rl * (2.0 - l * rl)
        return (o * rl).astype(BF16)

    def oproj(j):
        o2 = jnp.concatenate([outs[REP * j + r] for r in range(REP)], axis=1)
        acc_ref[:, j * BQ:(j + 1) * BQ] += lax.dot_general(wot, o2, _NT, preferred_element_type=F32)

    q2s = [qproj(j) for j in range(NB)]
    qs = [q2s[j][:, r * DH:(r + 1) * DH] for j in range(NB) for r in range(REP)]
    outs = []
    done = 0
    s_head = None
    for ci in range(len(qs)):
        if s_head is None:
            s = qk(ci, 0, SK)
        else:
            s = jnp.concatenate([s_head, qk(ci, SPLIT, SK)], axis=1)
        s_head = qk(ci + 1, 0, SPLIT) if (C0 <= ci < len(qs) - 1) else None
        outs.append(softmax_pv(s, late=(ci == len(qs) - 1)))
        if ci % REP == REP - 1 and ci // REP - OPD >= 0:
            oproj(done)
            done += 1
    for j in range(done, NB):
        oproj(j)

    @pl.when(step + 2 < NG)
    def _():
        for d in group_copies(step + 2):
            d.start()

    @pl.when(step == 0)
    def _():
        wmb_cp().start()
        wg_cp().start()

    @pl.when(step == 1)
    def _():
        wu_cp().start()

    @pl.when(step == 2)
    def _():
        wd_cp().start()

    @pl.when(step == NG - 1)
    def _epilogue():
        W2 = LN2U * LANES
        eps_b = _rb(jnp.full((1, 1), LN_EPS, F32))

        def ln2_stats(i, carry):
            cols = pl.ds(_mo(i * W2, W2), W2)
            piv = st_ref[2:3, cols]
            s2 = sums = None
            for r0 in range(0, D, SPR):
                r1 = min(r0 + SPR, D)
                x2 = (xt_ref[r0:r1, cols].astype(F32)
                      + _tile(modc_ref[r0:r1, :], LN2U) * acc_ref[r0:r1, cols])
                acc_ref[r0:r1, cols] = x2
                d = x2 - piv
                db = d.astype(BF16)
                db_ref[r0 // 2:r1 // 2, cols] = pltpu.bitcast(db, U32)
                t = jnp.dot(lhs_ref[:, r0:r1], db, preferred_element_type=F32)
                dd = jnp.sum((d * d).reshape((r1 - r0) // 8, 8, W2), axis=0)
                s2, sums = (dd, t) if r0 == 0 else (s2 + dd, sums + t)
            md = sums[0:1, :] * (1.0 / D)
            var = jnp.maximum(jnp.sum(s2, axis=0, keepdims=True) * (1.0 / D) - md * md, 0.0)
            sd = _rb(jnp.sqrt(_rb(_rb(var) + eps_b)))
            rs = 1.0 / sd
            st_ref[0:1, cols] = rs
            st_ref[1:2, cols] = (piv + md) * rs
            rr = ((sums[1:2, :] + sums[2:3, :] - md * _tile(rc_ref[0:1, :], LN2U)) * rs
                  + _tile(rc_ref[1:2, :], LN2U))
            for u in range(LN2U):
                r_ref[pl.ds(LN2U * i + u, 1), :] = rr[:, u * LANES:(u + 1) * LANES]
            row = lax.broadcasted_iota(jnp.int32, (16, W2), 0)
            ext = jnp.where(row == 0, sd, 0.0)
            for n, val in enumerate((md, piv)):
                hi = _rb(val)
                ext = jnp.where(row == 1 + 2 * n, hi, jnp.where(row == 2 + 2 * n, val - hi, ext))
            db_ref[D // 2:D // 2 + 8, cols] = pltpu.bitcast(ext.astype(BF16), U32)
            return carry
        if UNROLL_STATS:
            @pl.when(step > 0)
            def _():
                for i in range(S // W2):
                    ln2_stats(i, 0)
        else:
            lax.fori_loop(0, S // W2, ln2_stats, 0)

        lane16 = lax.broadcasted_iota(jnp.int32, (16, LANES), 1)

        never = lane16 > step + LANES

        def out_unit(n, gate):
            w = OUW * LANES
            cols = slice(n * w, (n + 1) * w)
            rs = st_ref[0:1, cols]
            if gate is not None:
                rs = jnp.where(_tile(never[0:1, :], OUW), _tile(gate[0:1, :], OUW), rs)
            mrs = st_ref[1:2, cols]
            for r0 in range(0, D, OPR):
                x2 = acc_ref[r0:r0 + OPR, cols]
                o = x2 + ((x2 * rs - mrs) * _tile(modc_ref[D + r0:D + r0 + OPR, :], OUW)
                          + _tile(modc_ref[MA + r0:MA + r0 + OPR, :], OUW))
                wx_ref[r0:r0 + OPR, FF + n * w:FF + (n + 1) * w] = o.astype(BF16)
            dyn0 = pl.multiple_of(FF + (step - (NG - 1)) * LANES, LANES)
            return wx_ref[0:16, pl.ds(dyn0, LANES)].astype(F32)

        r = _rb(r_ref[...]) + 0.0
        bits = pltpu.bitcast(r, jnp.int32)
        mono = bits ^ ((bits >> 31) & jnp.int32(0x7FFFFFFF))
        tok = (lax.broadcasted_iota(jnp.int32, (NSL, LANES), 0) * LANES
               + lax.broadcasted_iota(jnp.int32, (NSL, LANES), 1))
        keyi = (((mono >> 16) + 32768) * S + (S - 1 - tok)) + jnp.int32(1 << 29)
        key = pltpu.bitcast(keyi, F32)

        row16 = lax.broadcasted_iota(jnp.int32, (16, LANES), 0)
        rowc = lax.broadcasted_iota(jnp.int32, (16, 1), 0)
        sel_slab, sel_off = [], []
        tie, nunit = None, 0
        gsel = jnp.zeros((16, D + 16), F32)
        ksel = jnp.zeros((16, 1), F32)
        for t in range(TOPC):
            kmax = jnp.max(jnp.max(key, axis=0, keepdims=True), axis=1, keepdims=True)
            key = jnp.where(key == kmax, 0.0, key)
            for _ in range(TK_TIES.count(t)):
                tie = out_unit(nunit, tie if GATED else None)
                nunit += 1
                key = jnp.where(never, tie, key)
            ksel = jnp.where(rowc == t, kmax, ksel)
            ki = pltpu.bitcast(kmax, jnp.int32)[0, 0]
            idx = (S - 1) - (ki & (S - 1))
            slab = idx >> 7
            off = idx & (LANES - 1)
            onehot = jnp.where((row16 == t) & (lane16 == off), 1.0, 0.0).astype(BF16)
            dslab = db_ref[:, pl.ds(pl.multiple_of(slab * LANES, LANES), LANES)]
            gsel = gsel + lax.dot_general(onehot, pltpu.bitcast(dslab, BF16), _NT,
                                          preferred_element_type=F32)
            sel_slab.append(slab)
            sel_off.append(off)
        dsel = gsel[:, 0:D]
        sd = jnp.where(rowc < TOPC, gsel[:, D:D + 1], 1.0)
        md = gsel[:, D + 1:D + 2] + gsel[:, D + 2:D + 3]
        piv = gsel[:, D + 3:D + 4] + gsel[:, D + 4:D + 5]
        hsel = (dsel - md) * (1.0 / sd) * mrow_ref[1, 0:1, :] + mrow_ref[0, 0:1, :]
        osel = dsel + piv + mrow_ref[2, 0:1, :] * hsel
        hi = ((pltpu.bitcast(ksel, jnp.int32) - jnp.int32(1 << 29)) // S - 32768) << 16
        rbits = hi ^ ((hi >> 31) & jnp.int32(0x7FFF0000))
        gate = _sigmoid(jnp.where(rowc < TOPC, pltpu.bitcast(rbits, F32), 0.0))

        def out_copy(sl, r0, nr):
            c0 = pl.multiple_of(sl * LANES, LANES)
            return cp(wx_ref.at[r0:r0 + nr, pl.ds(pl.multiple_of(FF + c0, LANES), LANES)],
                      out_hbm.at[r0:r0 + nr, pl.ds(c0, LANES)], S_O)

        fresh = []
        seen = jnp.int32(0)
        for t in range(TOPC):
            fresh.append(((seen >> sel_slab[t]) & 1) == 0)
            seen = seen | (1 << sel_slab[t])
        plain = [((seen >> sl) & 1) == 0 for sl in range(NSL)]

        for n in range(nunit, NSL // OUW):
            tie = out_unit(n, tie if GATED else None)
        for sl in range(NSL):
            pl.when(plain[sl])(lambda sl=sl: out_copy(sl, 0, D).start())

        h0 = jnp.where(never, tie, hsel[:, 0:LANES])
        hs = jnp.concatenate([h0, hsel[:, LANES:]], axis=1).astype(BF16)
        gpre = jnp.dot(hs, wg_ref[...], preferred_element_type=F32)
        u = jnp.dot(hs, wu_ref[...], preferred_element_type=F32)
        a = (gpre * _sigmoid(gpre) * u).astype(BF16)

        pieces = [(r0, min(LANES, D - r0)) for r0 in range(0, D, LANES)]

        coef = gate * mrow_ref[2, 0:1, :]

        def down(r0, nr):
            y = lax.dot_general(a, wx_ref[r0:r0 + nr, 0:FF], _NT, preferred_element_type=F32)
            return osel[:, r0:r0 + nr] + y * coef[:, r0:r0 + nr]

        def patch(r0, nr, new):
            lane = lax.broadcasted_iota(jnp.int32, (nr // 2, LANES), 1)
            for t in range(TOPC):
                cols = pl.ds(pl.multiple_of(FF + sel_slab[t] * LANES, LANES), LANES)
                old = pltpu.bitcast(wx_ref[r0:r0 + nr, cols], U32)
                upd = pltpu.bitcast(_as_cols(new[t:t + 1, :]), U32)
                wx_ref[r0:r0 + nr, cols] = pltpu.bitcast(jnp.where(lane == sel_off[t], upd, old), BF16)
            for t in range(TOPC):
                pl.when(fresh[t])(lambda t=t: out_copy(sel_slab[t], r0, nr).start())

        yts = [down(*pieces[0])]
        for n in range(len(pieces)):
            if n + 1 < len(pieces):
                yts.append(down(*pieces[n + 1]))
            patch(*pieces[n], yts[n])

        cp(wx_ref.at[:, FF:FF + S], out_hbm, S_O).wait()


@jax.jit
def pallas_adaLN_cond__gqa_block_cached__moe_arch_mod__prompt_kernel(
    A_x: jax.Array,
    A_k_cache: jax.Array,
    A_v_cache: jax.Array,
    A_wq: jax.Array,
    A_wo: jax.Array,
    B_x: jax.Array,
    B_w_r: jax.Array,
    B_w_gate: jax.Array,
    B_w_up: jax.Array,
    B_w_down: jax.Array,
    c: jax.Array,
    w_mod: jax.Array,
):
    del B_x
    B, S, D = A_x.shape
    assert B == 1
    NG, SK = A_k_cache.shape[1], A_k_cache.shape[2]
    REP = HQ // NG
    FF = B_w_gate.shape[1]
    GW = REP * DH

    xt = A_x.reshape(S, D).T
    wot = A_wo.T
    wdt = B_w_down.T
    k = A_k_cache.reshape(NG, SK, DH)
    v = A_v_cache.reshape(NG, SK, DH)

    hbm = pl.BlockSpec(memory_space=pl.ANY)
    out_t = pl.pallas_call(
        functools.partial(_kernel, S=S, SK=SK, D=D, FF=FF, NG=NG, REP=REP),
        grid=(NG,),
        in_specs=[hbm] * 11,
        out_specs=hbm,
        out_shape=jax.ShapeDtypeStruct((D, S), BF16),
        scratch_shapes=[
            pltpu.VMEM((D, S), BF16),
            pltpu.VMEM((2, SK, DH), BF16),
            pltpu.VMEM((2, SK, DH), BF16),
            pltpu.VMEM((2, D, GW), BF16),
            pltpu.VMEM((2, D, GW), BF16),
            pltpu.VMEM((D,), BF16),
            pltpu.VMEM((1, D), BF16),
            pltpu.VMEM((D, 6 * D), BF16),
            pltpu.VMEM((D, FF), BF16),
            pltpu.VMEM((D, FF), BF16),
            pltpu.VMEM((D, FF + S), BF16),
            pltpu.VMEM((3 * D, LANES), F32),
            pltpu.VMEM((3, 8, D), F32),
            pltpu.VMEM((16, D), BF16),
            pltpu.VMEM((8, LANES), F32),
            pltpu.VMEM((S // 2, D), U32),
            pltpu.VMEM((D, S), F32),
            pltpu.VMEM((D // 2 + 8, S), U32),
            pltpu.VMEM((8, S), F32),
            pltpu.VMEM((S // LANES, LANES), F32),
            pltpu.SemaphoreType.DMA((N_SEMS,)),
        ],
        compiler_params=pltpu.CompilerParams(
            dimension_semantics=("arbitrary",),
            vmem_limit_bytes=100 * 1024 * 1024,
            disable_bounds_checks=True,
        ),
    )(xt, k, v, A_wq, wot, B_w_r, c, w_mod, B_w_gate, B_w_up, wdt)
    return out_t.T.reshape(B, S, D)
```

```python
import functools
import math

import jax
import jax.numpy as jnp
from jax import lax
import jax.experimental.pallas as pl
import jax.experimental.pallas.tpu as pltpu

F32 = jnp.float32
BF16 = jnp.bfloat16
U32 = jnp.uint32

HQ = 32
DH = 128
TOPC = 8
LN_EPS = 1e-5
BQ = 256
LANES = 128
SPLIT = 512
C0 = 2
OPD = 2
XCH = 4
LN2U = 1
OUW = 2
GATED = 0
TK_TIES = [0, 2, 3, 5, 6]
OPR = 16
SPR = 128
UNROLL_STATS = 1
MOD_STEP = 4

_NT = (((1,), (1,)), ((), ()))

S_C, S_WMA, S_WMB, S_WR, S_WG, S_WU, S_WD = range(7)
S_X = 7
S_G = S_X + XCH
S_O = S_G + 2
N_SEMS = S_O + 1


def _rb(x):
    return x.astype(BF16).astype(F32)


def _sigmoid(x):
    return 1.0 / (1.0 + jnp.exp(-x))


def _ln_rows(mean, var):
    eps = _rb(jnp.full((1, 1), LN_EPS, F32))
    return _rb(mean), _rb(jnp.sqrt(_rb(_rb(var) + eps)))


def _mo(x, n):
    return x if isinstance(x, int) else pl.multiple_of(x, n)


def _tile(col, n):
    return jnp.concatenate([col] * n, axis=1)


def _as_cols(row):
    return jnp.broadcast_to(row, (LANES, row.shape[1])).astype(BF16).T


def _kernel(xt_hbm, k_hbm, v_hbm, wq_hbm, wot_hbm, wr_hbm, c_hbm, wmod_hbm,
            wg_hbm, wu_hbm, wdt_hbm,
            out_hbm,
            xt_ref, k_buf, v_buf, wq_buf, wot_buf, wr_ref, c_ref, wmod_ref,
            wg_ref, wu_ref, wx_ref,
            modc_ref, mrow_ref, lhs_ref, rc_ref, h_ref, acc_ref, db_ref, st_ref, r_ref,
            sems,
            *, S, SK, D, FF, NG, REP):
    step = pl.program_id(0)
    qscale = (DH ** -0.5) * math.log2(math.e)
    NB = S // BQ
    GW = REP * DH
    TCH = S // XCH
    MA = 2 * D
    NSL = S // LANES

    def cp(src, dst, sem):
        return pltpu.make_async_copy(src, dst, sems.at[sem])

    def x_copy(i):
        cols = pl.ds(pl.multiple_of(i * TCH, TCH), TCH)
        return cp(xt_hbm.at[:, cols], xt_ref.at[:, cols], S_X + i)

    def group_copies(grp):
        slot = grp % 2
        cols = pl.ds(pl.multiple_of(grp * GW, GW), GW)
        return (cp(wq_hbm.at[:, cols], wq_buf.at[slot], S_G + slot),
                cp(k_hbm.at[grp], k_buf.at[slot], S_G + slot),
                cp(v_hbm.at[grp], v_buf.at[slot], S_G + slot),
                cp(wot_hbm.at[:, cols], wot_buf.at[slot], S_G + slot))

    c_cp = lambda: cp(c_hbm, c_ref, S_C)
    wma_cp = lambda: cp(wmod_hbm.at[:, 0:MA], wmod_ref.at[:, 0:MA], S_WMA)
    wmb_cp = lambda: cp(wmod_hbm.at[:, MA:6 * D], wmod_ref.at[:, MA:6 * D], S_WMB)
    wr_cp = lambda: cp(wr_hbm, wr_ref, S_WR)
    wg_cp = lambda: cp(wg_hbm, wg_ref, S_WG)
    wu_cp = lambda: cp(wu_hbm, wu_ref, S_WU)
    wd_cp = lambda: cp(wdt_hbm, wx_ref.at[:, 0:FF], S_WD)

    def modcol(i):
        return modc_ref[i * D:(i + 1) * D, :]

    def modulation(lo, hi):
        c = c_ref[...].astype(F32)
        sc8 = jnp.broadcast_to((c * _sigmoid(c)).astype(BF16), (8, D))
        mods = []
        for a in range(lo, hi, MA):
            mod = _rb(jnp.dot(sc8, wmod_ref[:, a:a + MA], preferred_element_type=F32))
            lane = lax.broadcasted_iota(jnp.int32, mod.shape, 1) + a
            is_scale = ((lane >= D) & (lane < 2 * D)) | ((lane >= 4 * D) & (lane < 5 * D))
            mods.append(jnp.where(is_scale, _rb(1.0 + mod), mod))
        return mods

    @pl.when(step == 0)
    def _prologue():
        wma_cp().start()
        c_cp().start()
        for i in range(XCH):
            x_copy(i).start()
        for d in group_copies(0) + group_copies(1):
            d.start()
        wr_cp().start()
        acc_ref[...] = jnp.zeros((D, S), F32)
        wma_cp().wait()
        c_cp().wait()
        modc_ref[0:MA, :] = _as_cols(modulation(0, MA)[0][0:1, :]).astype(F32)

        def ln1(i, carry):
            x_copy(i).wait()
            x = xt_ref[:, pl.ds(pl.multiple_of(i * TCH, TCH), TCH)].astype(F32)
            piv = x[0:1, :]
            d = x - piv
            md = jnp.mean(d, axis=0, keepdims=True)
            var = jnp.maximum(jnp.mean(d * d, axis=0, keepdims=True) - md * md, 0.0)
            mb, sd = _ln_rows(piv + md, var)
            rs = 1.0 / sd
            st_ref[2:3, pl.ds(pl.multiple_of(i * TCH, TCH), TCH)] = mb
            n = TCH // LANES
            ht = (x * rs - mb * rs) * _tile(modcol(1), n) + _tile(modcol(0), n)
            h_ref[pl.ds(pl.multiple_of(i * (TCH // 2), TCH // 2), TCH // 2), :] = pltpu.bitcast(
                ht.astype(BF16).T, U32)
            return carry
        lax.fori_loop(0, XCH, ln1, 0)

    @pl.when(step == MOD_STEP)
    def _late_modulation():
        wr_cp().wait()
        wmb_cp().wait()
        wg_cp().wait()
        wu_cp().wait()
        wd_cp().wait()
        m23, m45 = modulation(MA, 6 * D)
        sb, cb, gb = m23[:, D:MA], m45[:, 0:D], m45[:, D:MA]
        mrow_ref[0] = sb
        mrow_ref[1] = cb
        mrow_ref[2] = gb
        c23 = _as_cols(m23[0:1, :]).astype(F32)
        c45 = _as_cols(m45[0:1, :]).astype(F32)
        modc_ref[0:D, :] = c23[0:D]
        modc_ref[D:MA, :] = c45[D:MA] * c45[0:D]
        modc_ref[MA:3 * D, :] = c45[D:MA] * c23[D:MA]
        wr = wr_ref[...].astype(F32).reshape(1, D)
        wc = wr * cb[0:1, :]
        whi = _rb(wc)
        wlo = _rb(wc - whi)
        row = lax.broadcasted_iota(jnp.int32, (16, D), 0)
        lhs_ref[...] = jnp.where(row == 0, 1.0, jnp.where(row == 1, whi, jnp.where(
            row == 2, wlo, 0.0))).astype(BF16)
        rc_ref[0:1, :] = jnp.broadcast_to(jnp.sum(whi + wlo, axis=1, keepdims=True), (1, LANES))
        rc_ref[1:2, :] = jnp.broadcast_to(jnp.sum(wr * sb[0:1, :], axis=1, keepdims=True), (1, LANES))

    for d in group_copies(step):
        d.wait()

    slot = step % 2
    k = k_buf[slot]
    v = v_buf[slot]
    wq = wq_buf[slot]
    wot = wot_buf[slot]

    def qproj(j):
        hb = pltpu.bitcast(h_ref[j * (BQ // 2):(j + 1) * (BQ // 2), :], BF16)
        q2 = jnp.dot(hb, wq, preferred_element_type=F32)
        return (q2 * qscale).astype(BF16)

    def qk(ci, lo, hi):
        return lax.dot_general(qs[ci], k[lo:hi], _NT, preferred_element_type=F32)

    def softmax_pv(s, late):
        m = jnp.max(s, axis=1, keepdims=True)
        p = jnp.exp2(s - m)
        o = jnp.dot(p.astype(BF16), v, preferred_element_type=F32)
        if late:
            lp = p[:, 0:LANES]
            for i in range(1, SK // LANES):
                lp = lp + p[:, i * LANES:(i + 1) * LANES]
            l = jnp.sum(jnp.where(lp < 0.0, o, lp), axis=1, keepdims=True)
        else:
            l = jnp.sum(p, axis=1, keepdims=True)
        rl = pl.reciprocal(l, approx=True)
        rl = rl * (2.0 - l * rl)
        return (o * rl).astype(BF16)

    def oproj(j):
        o2 = jnp.concatenate([outs[REP * j + r] for r in range(REP)], axis=1)
        acc_ref[:, j * BQ:(j + 1) * BQ] += lax.dot_general(wot, o2, _NT, preferred_element_type=F32)

    q2s = [qproj(j) for j in range(NB)]
    qs = [q2s[j][:, r * DH:(r + 1) * DH] for j in range(NB) for r in range(REP)]
    outs = []
    done = 0
    s_head = None
    for ci in range(len(qs)):
        if s_head is None:
            s = qk(ci, 0, SK)
        else:
            s = jnp.concatenate([s_head, qk(ci, SPLIT, SK)], axis=1)
        s_head = qk(ci + 1, 0, SPLIT) if (C0 <= ci < len(qs) - 1) else None
        outs.append(softmax_pv(s, late=(ci == len(qs) - 1)))
        if ci % REP == REP - 1 and ci // REP - OPD >= 0:
            oproj(done)
            done += 1
    for j in range(done, NB):
        oproj(j)

    @pl.when(step + 2 < NG)
    def _():
        for d in group_copies(step + 2):
            d.start()

    @pl.when(step == 0)
    def _():
        wmb_cp().start()
        wg_cp().start()

    @pl.when(step == 1)
    def _():
        wu_cp().start()

    @pl.when(step == 2)
    def _():
        wd_cp().start()

    @pl.when(step == NG - 1)
    def _epilogue():
        W2 = LN2U * LANES

        def ln2_stats(i, carry):
            cols = pl.ds(_mo(i * W2, W2), W2)
            piv = st_ref[2:3, cols]
            s2 = sums = None
            for r0 in range(0, D, SPR):
                r1 = min(r0 + SPR, D)
                x2 = (xt_ref[r0:r1, cols].astype(F32)
                      + _tile(modc_ref[r0:r1, :], LN2U) * acc_ref[r0:r1, cols])
                acc_ref[r0:r1, cols] = x2
                d = x2 - piv
                db = x2.astype(BF16)
                db_ref[r0 // 2:r1 // 2, cols] = pltpu.bitcast(db, U32)
                t = jnp.dot(lhs_ref[:, r0:r1], db, preferred_element_type=F32)
                dd = jnp.sum((d * d).reshape((r1 - r0) // 8, 8, W2), axis=0)
                s2, sums = (dd, t) if r0 == 0 else (s2 + dd, sums + t)
            mean = sums[0:1, :] * (1.0 / D)
            md = mean - piv
            var = jnp.maximum(jnp.sum(s2, axis=0, keepdims=True) * (1.0 / D) - md * md, 0.0)
            mb, sd = _ln_rows(mean, var)
            rs = 1.0 / sd
            st_ref[0:1, cols] = rs
            st_ref[1:2, cols] = mb * rs
            rr = ((sums[1:2, :] + sums[2:3, :] - mb * _tile(rc_ref[0:1, :], LN2U)) * rs
                  + _tile(rc_ref[1:2, :], LN2U))
            for u in range(LN2U):
                r_ref[pl.ds(LN2U * i + u, 1), :] = rr[:, u * LANES:(u + 1) * LANES]
            row = lax.broadcasted_iota(jnp.int32, (16, W2), 0)
            ext = jnp.where(row == 0, sd, jnp.where(row == 1, mb, 0.0))
            db_ref[D // 2:D // 2 + 8, cols] = pltpu.bitcast(ext.astype(BF16), U32)
            return carry
        if UNROLL_STATS:
            @pl.when(step > 0)
            def _():
                for i in range(S // W2):
                    ln2_stats(i, 0)
        else:
            lax.fori_loop(0, S // W2, ln2_stats, 0)

        lane16 = lax.broadcasted_iota(jnp.int32, (16, LANES), 1)

        never = lane16 > step + LANES

        def out_unit(n, gate):
            w = OUW * LANES
            cols = slice(n * w, (n + 1) * w)
            rs = st_ref[0:1, cols]
            if gate is not None:
                rs = jnp.where(_tile(never[0:1, :], OUW), _tile(gate[0:1, :], OUW), rs)
            mrs = st_ref[1:2, cols]
            for r0 in range(0, D, OPR):
                x2 = acc_ref[r0:r0 + OPR, cols]
                o = x2 + ((x2 * rs - mrs) * _tile(modc_ref[D + r0:D + r0 + OPR, :], OUW)
                          + _tile(modc_ref[MA + r0:MA + r0 + OPR, :], OUW))
                wx_ref[r0:r0 + OPR, FF + n * w:FF + (n + 1) * w] = o.astype(BF16)
            dyn0 = pl.multiple_of(FF + (step - (NG - 1)) * LANES, LANES)
            return wx_ref[0:16, pl.ds(dyn0, LANES)].astype(F32)

        r = _rb(r_ref[...]) + 0.0
        bits = pltpu.bitcast(r, jnp.int32)
        mono = bits ^ ((bits >> 31) & jnp.int32(0x7FFFFFFF))
        tok = (lax.broadcasted_iota(jnp.int32, (NSL, LANES), 0) * LANES
               + lax.broadcasted_iota(jnp.int32, (NSL, LANES), 1))
        keyi = (((mono >> 16) + 32768) * S + (S - 1 - tok)) + jnp.int32(1 << 29)
        key = pltpu.bitcast(keyi, F32)

        row16 = lax.broadcasted_iota(jnp.int32, (16, LANES), 0)
        rowc = lax.broadcasted_iota(jnp.int32, (16, 1), 0)
        sel_slab, sel_off = [], []
        tie, nunit = None, 0
        gsel = jnp.zeros((16, D + 16), F32)
        ksel = jnp.zeros((16, 1), F32)
        for t in range(TOPC):
            kmax = jnp.max(jnp.max(key, axis=0, keepdims=True), axis=1, keepdims=True)
            key = jnp.where(key == kmax, 0.0, key)
            for _ in range(TK_TIES.count(t)):
                tie = out_unit(nunit, tie if GATED else None)
                nunit += 1
                key = jnp.where(never, tie, key)
            ksel = jnp.where(rowc == t, kmax, ksel)
            ki = pltpu.bitcast(kmax, jnp.int32)[0, 0]
            idx = (S - 1) - (ki & (S - 1))
            slab = idx >> 7
            off = idx & (LANES - 1)
            onehot = jnp.where((row16 == t) & (lane16 == off), 1.0, 0.0).astype(BF16)
            dslab = db_ref[:, pl.ds(pl.multiple_of(slab * LANES, LANES), LANES)]
            gsel = gsel + lax.dot_general(onehot, pltpu.bitcast(dslab, BF16), _NT,
                                          preferred_element_type=F32)
            sel_slab.append(slab)
            sel_off.append(off)
        xsel = gsel[:, 0:D]
        sd = jnp.where(rowc < TOPC, gsel[:, D:D + 1], 1.0)
        nsel = _rb(_rb(xsel - gsel[:, D + 1:D + 2]) * (1.0 / sd))
        hsel = _rb(_rb(nsel * mrow_ref[1, 0:1, :]) + mrow_ref[0, 0:1, :])
        hi = ((pltpu.bitcast(ksel, jnp.int32) - jnp.int32(1 << 29)) // S - 32768) << 16
        rbits = hi ^ ((hi >> 31) & jnp.int32(0x7FFF0000))
        gate = _rb(_sigmoid(jnp.where(rowc < TOPC, pltpu.bitcast(rbits, F32), 0.0)))

        def out_copy(sl, r0, nr):
            c0 = pl.multiple_of(sl * LANES, LANES)
            return cp(wx_ref.at[r0:r0 + nr, pl.ds(pl.multiple_of(FF + c0, LANES), LANES)],
                      out_hbm.at[r0:r0 + nr, pl.ds(c0, LANES)], S_O)

        fresh = []
        seen = jnp.int32(0)
        for t in range(TOPC):
            fresh.append(((seen >> sel_slab[t]) & 1) == 0)
            seen = seen | (1 << sel_slab[t])
        plain = [((seen >> sl) & 1) == 0 for sl in range(NSL)]

        for n in range(nunit, NSL // OUW):
            tie = out_unit(n, tie if GATED else None)
        for sl in range(NSL):
            pl.when(plain[sl])(lambda sl=sl: out_copy(sl, 0, D).start())

        h0 = jnp.where(never, tie, hsel[:, 0:LANES])
        hs = jnp.concatenate([h0, hsel[:, LANES:]], axis=1).astype(BF16)
        gpre = _rb(jnp.dot(hs, wg_ref[...], preferred_element_type=F32))
        u = _rb(jnp.dot(hs, wu_ref[...], preferred_element_type=F32))
        a = (_rb(gpre * _sigmoid(gpre)) * u).astype(BF16)

        pieces = [(r0, min(LANES, D - r0)) for r0 in range(0, D, LANES)]

        gb = mrow_ref[2, 0:1, :]

        def down(r0, nr):
            y = lax.dot_general(a, wx_ref[r0:r0 + nr, 0:FF], _NT, preferred_element_type=F32)
            c = slice(r0, r0 + nr)
            return xsel[:, c] + gb[:, c] * (hsel[:, c] + y * gate)

        def patch(r0, nr, new):
            lane = lax.broadcasted_iota(jnp.int32, (nr // 2, LANES), 1)
            for t in range(TOPC):
                cols = pl.ds(pl.multiple_of(FF + sel_slab[t] * LANES, LANES), LANES)
                old = pltpu.bitcast(wx_ref[r0:r0 + nr, cols], U32)
                upd = pltpu.bitcast(_as_cols(new[t:t + 1, :]), U32)
                wx_ref[r0:r0 + nr, cols] = pltpu.bitcast(jnp.where(lane == sel_off[t], upd, old), BF16)
            for t in range(TOPC):
                pl.when(fresh[t])(lambda t=t: out_copy(sel_slab[t], r0, nr).start())

        yts = [down(*pieces[0])]
        for n in range(len(pieces)):
            if n + 1 < len(pieces):
                yts.append(down(*pieces[n + 1]))
            patch(*pieces[n], yts[n])

        cp(wx_ref.at[:, FF:FF + S], out_hbm, S_O).wait()


@jax.jit
def pallas_adaLN_cond__gqa_block_cached__moe_arch_mod__prompt_kernel(
    A_x: jax.Array,
    A_k_cache: jax.Array,
    A_v_cache: jax.Array,
    A_wq: jax.Array,
    A_wo: jax.Array,
    B_x: jax.Array,
    B_w_r: jax.Array,
    B_w_gate: jax.Array,
    B_w_up: jax.Array,
    B_w_down: jax.Array,
    c: jax.Array,
    w_mod: jax.Array,
):
    del B_x
    B, S, D = A_x.shape
    assert B == 1
    NG, SK = A_k_cache.shape[1], A_k_cache.shape[2]
    REP = HQ // NG
    FF = B_w_gate.shape[1]
    GW = REP * DH

    xt = A_x.reshape(S, D).T
    wot = A_wo.T
    wdt = B_w_down.T
    k = A_k_cache.reshape(NG, SK, DH)
    v = A_v_cache.reshape(NG, SK, DH)

    hbm = pl.BlockSpec(memory_space=pl.ANY)
    out_t = pl.pallas_call(
        functools.partial(_kernel, S=S, SK=SK, D=D, FF=FF, NG=NG, REP=REP),
        grid=(NG,),
        in_specs=[hbm] * 11,
        out_specs=hbm,
        out_shape=jax.ShapeDtypeStruct((D, S), BF16),
        scratch_shapes=[
            pltpu.VMEM((D, S), BF16),
            pltpu.VMEM((2, SK, DH), BF16),
            pltpu.VMEM((2, SK, DH), BF16),
            pltpu.VMEM((2, D, GW), BF16),
            pltpu.VMEM((2, D, GW), BF16),
            pltpu.VMEM((D,), BF16),
            pltpu.VMEM((1, D), BF16),
            pltpu.VMEM((D, 6 * D), BF16),
            pltpu.VMEM((D, FF), BF16),
            pltpu.VMEM((D, FF), BF16),
            pltpu.VMEM((D, FF + S), BF16),
            pltpu.VMEM((3 * D, LANES), F32),
            pltpu.VMEM((3, 8, D), F32),
            pltpu.VMEM((16, D), BF16),
            pltpu.VMEM((8, LANES), F32),
            pltpu.VMEM((S // 2, D), U32),
            pltpu.VMEM((D, S), F32),
            pltpu.VMEM((D // 2 + 8, S), U32),
            pltpu.VMEM((8, S), F32),
            pltpu.VMEM((S // LANES, LANES), F32),
            pltpu.SemaphoreType.DMA((N_SEMS,)),
        ],
        compiler_params=pltpu.CompilerParams(
            dimension_semantics=("arbitrary",),
            vmem_limit_bytes=100 * 1024 * 1024,
            disable_bounds_checks=True,
        ),
    )(xt, k, v, A_wq, wot, B_w_r, c, w_mod, B_w_gate, B_w_up, wdt)
    return out_t.T.reshape(B, S, D)
```

```python
import functools
import math

import jax
import jax.numpy as jnp
from jax import lax
import jax.experimental.pallas as pl
import jax.experimental.pallas.tpu as pltpu

F32 = jnp.float32
BF16 = jnp.bfloat16
U32 = jnp.uint32

HQ = 32
DH = 128
TOPC = 8
LN_EPS = 1e-5
BQ = 256
LANES = 128
SPLIT = 512
C0 = 2
OPD = 2
XCH = 4
LN2U = 1
SQ_MXU = 1
OUW = 2
GATED = 0
TK_TIES = [0, 2, 3, 5, 6]
OPR = 16
SPR = 128
UNROLL_STATS = 1
MOD_STEP = 4

_NT = (((1,), (1,)), ((), ()))

S_C, S_WMA, S_WMB, S_WR, S_WG, S_WU, S_WD = range(7)
S_X = 7
S_G = S_X + XCH
S_O = S_G + 2
N_SEMS = S_O + 1


def _rb(x):
    return x.astype(BF16).astype(F32)


def _sigmoid(x):
    return 1.0 / (1.0 + jnp.exp(-x))


def _ln_rows(mean, var):
    eps = _rb(jnp.full((1, 1), LN_EPS, F32))
    return _rb(mean), _rb(jnp.sqrt(_rb(_rb(var) + eps)))


def _mo(x, n):
    return x if isinstance(x, int) else pl.multiple_of(x, n)


def _tile(col, n):
    return jnp.concatenate([col] * n, axis=1)


def _as_cols(row):
    return jnp.broadcast_to(row, (LANES, row.shape[1])).astype(BF16).T


def _kernel(xt_hbm, k_hbm, v_hbm, wq_hbm, wot_hbm, wr_hbm, c_hbm, wmod_hbm,
            wg_hbm, wu_hbm, wdt_hbm,
            out_hbm,
            xt_ref, k_buf, v_buf, wq_buf, wot_buf, wr_ref, c_ref, wmod_ref,
            wg_ref, wu_ref, wx_ref,
            modc_ref, mrow_ref, lhs_ref, rc_ref, h_ref, acc_ref, db_ref, st_ref, r_ref,
            sems,
            *, S, SK, D, FF, NG, REP):
    step = pl.program_id(0)
    qscale = (DH ** -0.5) * math.log2(math.e)
    NB = S // BQ
    GW = REP * DH
    TCH = S // XCH
    MA = 2 * D
    NSL = S // LANES

    def cp(src, dst, sem):
        return pltpu.make_async_copy(src, dst, sems.at[sem])

    def x_copy(i):
        cols = pl.ds(pl.multiple_of(i * TCH, TCH), TCH)
        return cp(xt_hbm.at[:, cols], xt_ref.at[:, cols], S_X + i)

    def group_copies(grp):
        slot = grp % 2
        cols = pl.ds(pl.multiple_of(grp * GW, GW), GW)
        return (cp(wq_hbm.at[:, cols], wq_buf.at[slot], S_G + slot),
                cp(k_hbm.at[grp], k_buf.at[slot], S_G + slot),
                cp(v_hbm.at[grp], v_buf.at[slot], S_G + slot),
                cp(wot_hbm.at[:, cols], wot_buf.at[slot], S_G + slot))

    c_cp = lambda: cp(c_hbm, c_ref, S_C)
    wma_cp = lambda: cp(wmod_hbm.at[:, 0:MA], wmod_ref.at[:, 0:MA], S_WMA)
    wmb_cp = lambda: cp(wmod_hbm.at[:, MA:6 * D], wmod_ref.at[:, MA:6 * D], S_WMB)
    wr_cp = lambda: cp(wr_hbm, wr_ref, S_WR)
    wg_cp = lambda: cp(wg_hbm, wg_ref, S_WG)
    wu_cp = lambda: cp(wu_hbm, wu_ref, S_WU)
    wd_cp = lambda: cp(wdt_hbm, wx_ref.at[:, 0:FF], S_WD)

    def modcol(i):
        return modc_ref[i * D:(i + 1) * D, :]

    def modulation(lo, hi):
        c = c_ref[...].astype(F32)
        sc8 = jnp.broadcast_to((c * _sigmoid(c)).astype(BF16), (8, D))
        mods = []
        for a in range(lo, hi, MA):
            mod = _rb(jnp.dot(sc8, wmod_ref[:, a:a + MA], preferred_element_type=F32))
            lane = lax.broadcasted_iota(jnp.int32, mod.shape, 1) + a
            is_scale = ((lane >= D) & (lane < 2 * D)) | ((lane >= 4 * D) & (lane < 5 * D))
            mods.append(jnp.where(is_scale, _rb(1.0 + mod), mod))
        return mods

    @pl.when(step == 0)
    def _prologue():
        wma_cp().start()
        c_cp().start()
        for i in range(XCH):
            x_copy(i).start()
        for d in group_copies(0) + group_copies(1):
            d.start()
        wr_cp().start()
        acc_ref[...] = jnp.zeros((D, S), F32)
        wma_cp().wait()
        c_cp().wait()
        modc_ref[0:MA, :] = _as_cols(modulation(0, MA)[0][0:1, :]).astype(F32)

        def ln1(i, carry):
            x_copy(i).wait()
            x = xt_ref[:, pl.ds(pl.multiple_of(i * TCH, TCH), TCH)].astype(F32)
            piv = x[0:1, :]
            d = x - piv
            md = jnp.mean(d, axis=0, keepdims=True)
            var = jnp.maximum(jnp.mean(d * d, axis=0, keepdims=True) - md * md, 0.0)
            mb, sd = _ln_rows(piv + md, var)
            rs = 1.0 / sd
            st_ref[2:3, pl.ds(pl.multiple_of(i * TCH, TCH), TCH)] = mb
            n = TCH // LANES
            ht = (x * rs - mb * rs) * _tile(modcol(1), n) + _tile(modcol(0), n)
            h_ref[pl.ds(pl.multiple_of(i * (TCH // 2), TCH // 2), TCH // 2), :] = pltpu.bitcast(
                ht.astype(BF16).T, U32)
            return carry
        lax.fori_loop(0, XCH, ln1, 0)

    @pl.when(step == MOD_STEP)
    def _late_modulation():
        wr_cp().wait()
        wmb_cp().wait()
        wg_cp().wait()
        wu_cp().wait()
        wd_cp().wait()
        m23, m45 = modulation(MA, 6 * D)
        sb, cb, gb = m23[:, D:MA], m45[:, 0:D], m45[:, D:MA]
        mrow_ref[0] = sb
        mrow_ref[1] = cb
        mrow_ref[2] = gb
        c23 = _as_cols(m23[0:1, :]).astype(F32)
        c45 = _as_cols(m45[0:1, :]).astype(F32)
        modc_ref[0:D, :] = c23[0:D]
        modc_ref[D:MA, :] = c45[D:MA] * c45[0:D]
        modc_ref[MA:3 * D, :] = c45[D:MA] * c23[D:MA]
        wr = wr_ref[...].astype(F32).reshape(1, D)
        wc = wr * cb[0:1, :]
        whi = _rb(wc)
        wlo = _rb(wc - whi)
        row = lax.broadcasted_iota(jnp.int32, (16, D), 0)
        lhs_ref[...] = jnp.where(row == 0, 1.0, jnp.where(row == 1, whi, jnp.where(
            row == 2, wlo, 0.0))).astype(BF16)
        rc_ref[0:1, :] = jnp.broadcast_to(jnp.sum(whi + wlo, axis=1, keepdims=True), (1, LANES))
        rc_ref[1:2, :] = jnp.broadcast_to(jnp.sum(wr * sb[0:1, :], axis=1, keepdims=True), (1, LANES))

    for d in group_copies(step):
        d.wait()

    slot = step % 2
    k = k_buf[slot]
    v = v_buf[slot]
    wq = wq_buf[slot]
    wot = wot_buf[slot]

    def qproj(j):
        hb = pltpu.bitcast(h_ref[j * (BQ // 2):(j + 1) * (BQ // 2), :], BF16)
        q2 = jnp.dot(hb, wq, preferred_element_type=F32)
        return (q2 * qscale).astype(BF16)

    def qk(ci, lo, hi):
        return lax.dot_general(qs[ci], k[lo:hi], _NT, preferred_element_type=F32)

    def softmax_pv(s, late):
        m = jnp.max(s, axis=1, keepdims=True)
        p = jnp.exp2(s - m)
        o = jnp.dot(p.astype(BF16), v, preferred_element_type=F32)
        if late:
            lp = p[:, 0:LANES]
            for i in range(1, SK // LANES):
                lp = lp + p[:, i * LANES:(i + 1) * LANES]
            l = jnp.sum(jnp.where(lp < 0.0, o, lp), axis=1, keepdims=True)
        else:
            l = jnp.sum(p, axis=1, keepdims=True)
        rl = pl.reciprocal(l, approx=True)
        rl = rl * (2.0 - l * rl)
        return (o * rl).astype(BF16)

    def oproj(j):
        o2 = jnp.concatenate([outs[REP * j + r] for r in range(REP)], axis=1)
        acc_ref[:, j * BQ:(j + 1) * BQ] += lax.dot_general(wot, o2, _NT, preferred_element_type=F32)

    q2s = [qproj(j) for j in range(NB)]
    qs = [q2s[j][:, r * DH:(r + 1) * DH] for j in range(NB) for r in range(REP)]
    outs = []
    done = 0
    s_head = None
    for ci in range(len(qs)):
        if s_head is None:
            s = qk(ci, 0, SK)
        else:
            s = jnp.concatenate([s_head, qk(ci, SPLIT, SK)], axis=1)
        s_head = qk(ci + 1, 0, SPLIT) if (C0 <= ci < len(qs) - 1) else None
        outs.append(softmax_pv(s, late=(ci == len(qs) - 1)))
        if ci % REP == REP - 1 and ci // REP - OPD >= 0:
            oproj(done)
            done += 1
    for j in range(done, NB):
        oproj(j)

    @pl.when(step + 2 < NG)
    def _():
        for d in group_copies(step + 2):
            d.start()

    @pl.when(step == 0)
    def _():
        wmb_cp().start()
        wg_cp().start()

    @pl.when(step == 1)
    def _():
        wu_cp().start()

    @pl.when(step == 2)
    def _():
        wd_cp().start()

    @pl.when(step == NG - 1)
    def _epilogue():
        W2 = LN2U * LANES

        def ln2_stats(i, carry):
            cols = pl.ds(_mo(i * W2, W2), W2)
            piv = st_ref[2:3, cols]
            s2 = sums = None
            for r0 in range(0, D, SPR):
                r1 = min(r0 + SPR, D)
                x2 = (xt_ref[r0:r1, cols].astype(F32)
                      + _tile(modc_ref[r0:r1, :], LN2U) * acc_ref[r0:r1, cols])
                acc_ref[r0:r1, cols] = x2
                d = x2 - piv
                db = x2.astype(BF16)
                db_ref[r0 // 2:r1 // 2, cols] = pltpu.bitcast(db, U32)
                t = jnp.dot(lhs_ref[:, r0:r1], db, preferred_element_type=F32)
                if SQ_MXU:
                    dd = jnp.dot(lhs_ref[:, r0:r1], (d * d).astype(BF16),
                                 preferred_element_type=F32)[0:1, :]
                else:
                    dd = jnp.sum((d * d).reshape((r1 - r0) // 8, 8, W2), axis=0)
                s2, sums = (dd, t) if r0 == 0 else (s2 + dd, sums + t)
            mean = sums[0:1, :] * (1.0 / D)
            md = mean - piv
            var = jnp.maximum(jnp.sum(s2, axis=0, keepdims=True) * (1.0 / D) - md * md, 0.0)
            mb, sd = _ln_rows(mean, var)
            rs = 1.0 / sd
            st_ref[0:1, cols] = rs
            st_ref[1:2, cols] = mb * rs
            rr = ((sums[1:2, :] + sums[2:3, :] - mb * _tile(rc_ref[0:1, :], LN2U)) * rs
                  + _tile(rc_ref[1:2, :], LN2U))
            for u in range(LN2U):
                r_ref[pl.ds(LN2U * i + u, 1), :] = rr[:, u * LANES:(u + 1) * LANES]
            row = lax.broadcasted_iota(jnp.int32, (16, W2), 0)
            ext = jnp.where(row == 0, sd, jnp.where(row == 1, mb, 0.0))
            db_ref[D // 2:D // 2 + 8, cols] = pltpu.bitcast(ext.astype(BF16), U32)
            return carry
        if UNROLL_STATS:
            @pl.when(step > 0)
            def _():
                for i in range(S // W2):
                    ln2_stats(i, 0)
        else:
            lax.fori_loop(0, S // W2, ln2_stats, 0)

        lane16 = lax.broadcasted_iota(jnp.int32, (16, LANES), 1)

        never = lane16 > step + LANES

        def out_unit(n, gate):
            w = OUW * LANES
            cols = slice(n * w, (n + 1) * w)
            rs = st_ref[0:1, cols]
            if gate is not None:
                rs = jnp.where(_tile(never[0:1, :], OUW), _tile(gate[0:1, :], OUW), rs)
            mrs = st_ref[1:2, cols]
            for r0 in range(0, D, OPR):
                x2 = acc_ref[r0:r0 + OPR, cols]
                o = x2 + ((x2 * rs - mrs) * _tile(modc_ref[D + r0:D + r0 + OPR, :], OUW)
                          + _tile(modc_ref[MA + r0:MA + r0 + OPR, :], OUW))
                wx_ref[r0:r0 + OPR, FF + n * w:FF + (n + 1) * w] = o.astype(BF16)
            dyn0 = pl.multiple_of(FF + (step - (NG - 1)) * LANES, LANES)
            return wx_ref[0:16, pl.ds(dyn0, LANES)].astype(F32)

        r = _rb(r_ref[...]) + 0.0
        bits = pltpu.bitcast(r, jnp.int32)
        mono = bits ^ ((bits >> 31) & jnp.int32(0x7FFFFFFF))
        tok = (lax.broadcasted_iota(jnp.int32, (NSL, LANES), 0) * LANES
               + lax.broadcasted_iota(jnp.int32, (NSL, LANES), 1))
        keyi = (((mono >> 16) + 32768) * S + (S - 1 - tok)) + jnp.int32(1 << 29)
        key = pltpu.bitcast(keyi, F32)

        row16 = lax.broadcasted_iota(jnp.int32, (16, LANES), 0)
        rowc = lax.broadcasted_iota(jnp.int32, (16, 1), 0)
        sel_slab, sel_off = [], []
        tie, nunit = None, 0
        gsel = jnp.zeros((16, D + 16), F32)
        ksel = jnp.zeros((16, 1), F32)
        for t in range(TOPC):
            kmax = jnp.max(jnp.max(key, axis=0, keepdims=True), axis=1, keepdims=True)
            key = jnp.where(key == kmax, 0.0, key)
            for _ in range(TK_TIES.count(t)):
                tie = out_unit(nunit, tie if GATED else None)
                nunit += 1
                key = jnp.where(never, tie, key)
            ksel = jnp.where(rowc == t, kmax, ksel)
            ki = pltpu.bitcast(kmax, jnp.int32)[0, 0]
            idx = (S - 1) - (ki & (S - 1))
            slab = idx >> 7
            off = idx & (LANES - 1)
            onehot = jnp.where((row16 == t) & (lane16 == off), 1.0, 0.0).astype(BF16)
            dslab = db_ref[:, pl.ds(pl.multiple_of(slab * LANES, LANES), LANES)]
            gsel = gsel + lax.dot_general(onehot, pltpu.bitcast(dslab, BF16), _NT,
                                          preferred_element_type=F32)
            sel_slab.append(slab)
            sel_off.append(off)
        xsel = gsel[:, 0:D]
        sd = jnp.where(rowc < TOPC, gsel[:, D:D + 1], 1.0)
        nsel = _rb(_rb(xsel - gsel[:, D + 1:D + 2]) * (1.0 / sd))
        hsel = _rb(_rb(nsel * mrow_ref[1, 0:1, :]) + mrow_ref[0, 0:1, :])
        hi = ((pltpu.bitcast(ksel, jnp.int32) - jnp.int32(1 << 29)) // S - 32768) << 16
        rbits = hi ^ ((hi >> 31) & jnp.int32(0x7FFF0000))
        gate = _rb(_sigmoid(jnp.where(rowc < TOPC, pltpu.bitcast(rbits, F32), 0.0)))

        def out_copy(sl, r0, nr):
            c0 = pl.multiple_of(sl * LANES, LANES)
            return cp(wx_ref.at[r0:r0 + nr, pl.ds(pl.multiple_of(FF + c0, LANES), LANES)],
                      out_hbm.at[r0:r0 + nr, pl.ds(c0, LANES)], S_O)

        fresh = []
        seen = jnp.int32(0)
        for t in range(TOPC):
            fresh.append(((seen >> sel_slab[t]) & 1) == 0)
            seen = seen | (1 << sel_slab[t])
        plain = [((seen >> sl) & 1) == 0 for sl in range(NSL)]

        for n in range(nunit, NSL // OUW):
            tie = out_unit(n, tie if GATED else None)
        for sl in range(NSL):
            pl.when(plain[sl])(lambda sl=sl: out_copy(sl, 0, D).start())

        h0 = jnp.where(never, tie, hsel[:, 0:LANES])
        hs = jnp.concatenate([h0, hsel[:, LANES:]], axis=1).astype(BF16)
        gpre = _rb(jnp.dot(hs, wg_ref[...], preferred_element_type=F32))
        u = _rb(jnp.dot(hs, wu_ref[...], preferred_element_type=F32))
        a = (_rb(gpre * _sigmoid(gpre)) * u).astype(BF16)

        pieces = [(r0, min(LANES, D - r0)) for r0 in range(0, D, LANES)]

        gb = mrow_ref[2, 0:1, :]

        def down(r0, nr):
            y = lax.dot_general(a, wx_ref[r0:r0 + nr, 0:FF], _NT, preferred_element_type=F32)
            c = slice(r0, r0 + nr)
            return xsel[:, c] + gb[:, c] * (hsel[:, c] + y * gate)

        def patch(r0, nr, new):
            lane = lax.broadcasted_iota(jnp.int32, (nr // 2, LANES), 1)
            for t in range(TOPC):
                cols = pl.ds(pl.multiple_of(FF + sel_slab[t] * LANES, LANES), LANES)
                old = pltpu.bitcast(wx_ref[r0:r0 + nr, cols], U32)
                upd = pltpu.bitcast(_as_cols(new[t:t + 1, :]), U32)
                wx_ref[r0:r0 + nr, cols] = pltpu.bitcast(jnp.where(lane == sel_off[t], upd, old), BF16)
            for t in range(TOPC):
                pl.when(fresh[t])(lambda t=t: out_copy(sel_slab[t], r0, nr).start())

        yts = [down(*pieces[0])]
        for n in range(len(pieces)):
            if n + 1 < len(pieces):
                yts.append(down(*pieces[n + 1]))
            patch(*pieces[n], yts[n])

        cp(wx_ref.at[:, FF:FF + S], out_hbm, S_O).wait()


@jax.jit
def pallas_adaLN_cond__gqa_block_cached__moe_arch_mod__prompt_kernel(
    A_x: jax.Array,
    A_k_cache: jax.Array,
    A_v_cache: jax.Array,
    A_wq: jax.Array,
    A_wo: jax.Array,
    B_x: jax.Array,
    B_w_r: jax.Array,
    B_w_gate: jax.Array,
    B_w_up: jax.Array,
    B_w_down: jax.Array,
    c: jax.Array,
    w_mod: jax.Array,
):
    del B_x
    B, S, D = A_x.shape
    assert B == 1
    NG, SK = A_k_cache.shape[1], A_k_cache.shape[2]
    REP = HQ // NG
    FF = B_w_gate.shape[1]
    GW = REP * DH

    xt = A_x.reshape(S, D).T
    wot = A_wo.T
    wdt = B_w_down.T
    k = A_k_cache.reshape(NG, SK, DH)
    v = A_v_cache.reshape(NG, SK, DH)

    hbm = pl.BlockSpec(memory_space=pl.ANY)
    out_t = pl.pallas_call(
        functools.partial(_kernel, S=S, SK=SK, D=D, FF=FF, NG=NG, REP=REP),
        grid=(NG,),
        in_specs=[hbm] * 11,
        out_specs=hbm,
        out_shape=jax.ShapeDtypeStruct((D, S), BF16),
        scratch_shapes=[
            pltpu.VMEM((D, S), BF16),
            pltpu.VMEM((2, SK, DH), BF16),
            pltpu.VMEM((2, SK, DH), BF16),
            pltpu.VMEM((2, D, GW), BF16),
            pltpu.VMEM((2, D, GW), BF16),
            pltpu.VMEM((D,), BF16),
            pltpu.VMEM((1, D), BF16),
            pltpu.VMEM((D, 6 * D), BF16),
            pltpu.VMEM((D, FF), BF16),
            pltpu.VMEM((D, FF), BF16),
            pltpu.VMEM((D, FF + S), BF16),
            pltpu.VMEM((3 * D, LANES), F32),
            pltpu.VMEM((3, 8, D), F32),
            pltpu.VMEM((16, D), BF16),
            pltpu.VMEM((8, LANES), F32),
            pltpu.VMEM((S // 2, D), U32),
            pltpu.VMEM((D, S), F32),
            pltpu.VMEM((D // 2 + 8, S), U32),
            pltpu.VMEM((8, S), F32),
            pltpu.VMEM((S // LANES, LANES), F32),
            pltpu.SemaphoreType.DMA((N_SEMS,)),
        ],
        compiler_params=pltpu.CompilerParams(
            dimension_semantics=("arbitrary",),
            vmem_limit_bytes=100 * 1024 * 1024,
            disable_bounds_checks=True,
        ),
    )(xt, k, v, A_wq, wot, B_w_r, c, w_mod, B_w_gate, B_w_up, wdt)
    return out_t.T.reshape(B, S, D)
```

```python
import functools
import math

import jax
import jax.numpy as jnp
from jax import lax
import jax.experimental.pallas as pl
import jax.experimental.pallas.tpu as pltpu

F32 = jnp.float32
BF16 = jnp.bfloat16
U32 = jnp.uint32

HQ = 32
DH = 128
TOPC = 8
LN_EPS = 1e-5
BQ = 256
LANES = 128
SPLIT = 512
C0 = 2
OPD = 2
XCH = 4
OUW = 2
TK_TIES = [0, 2, 3, 5, 6]
OPR = 16
MOD_STEP = 4

_NT = (((1,), (1,)), ((), ()))

S_C, S_WMA, S_WMB, S_WR, S_WG, S_WU, S_WD = range(7)
S_X = 7
S_G = S_X + XCH
S_O = S_G + 2
N_SEMS = S_O + 1


def _rb(x):
    return x.astype(BF16).astype(F32)


def _sigmoid(x):
    return 1.0 / (1.0 + jnp.exp(-x))


def _ln_rows(mean, var):
    eps = _rb(jnp.full((1, 1), LN_EPS, F32))
    return _rb(mean), _rb(jnp.sqrt(_rb(_rb(var) + eps)))


def _tile(col, n):
    return jnp.concatenate([col] * n, axis=1)


def _as_cols(row):
    return jnp.broadcast_to(row, (LANES, row.shape[1])).astype(BF16).T


def _kernel(xt_hbm, k_hbm, v_hbm, wq_hbm, wot_hbm, wr_hbm, c_hbm, wmod_hbm,
            wg_hbm, wu_hbm, wdt_hbm,
            out_hbm,
            xt_ref, k_buf, v_buf, wq_buf, wot_buf, wr_ref, c_ref, wmod_ref,
            wg_ref, wu_ref, wx_ref,
            modc_ref, mrow_ref, lhs_ref, rc_ref, h_ref, acc_ref, xb_ref, st_ref,
            sems,
            *, S, SK, D, FF, NG, REP):
    step = pl.program_id(0)
    qscale = (DH ** -0.5) * math.log2(math.e)
    NB = S // BQ
    GW = REP * DH
    TCH = S // XCH
    MA = 2 * D
    NSL = S // LANES

    def cp(src, dst, sem):
        return pltpu.make_async_copy(src, dst, sems.at[sem])

    def x_copy(i):
        cols = pl.ds(pl.multiple_of(i * TCH, TCH), TCH)
        return cp(xt_hbm.at[:, cols], xt_ref.at[:, cols], S_X + i)

    def group_copies(grp):
        slot = grp % 2
        cols = pl.ds(pl.multiple_of(grp * GW, GW), GW)
        return (cp(wq_hbm.at[:, cols], wq_buf.at[slot], S_G + slot),
                cp(k_hbm.at[grp], k_buf.at[slot], S_G + slot),
                cp(v_hbm.at[grp], v_buf.at[slot], S_G + slot),
                cp(wot_hbm.at[:, cols], wot_buf.at[slot], S_G + slot))

    c_cp = lambda: cp(c_hbm, c_ref, S_C)
    wma_cp = lambda: cp(wmod_hbm.at[:, 0:MA], wmod_ref.at[:, 0:MA], S_WMA)
    wmb_cp = lambda: cp(wmod_hbm.at[:, MA:6 * D], wmod_ref.at[:, MA:6 * D], S_WMB)
    wr_cp = lambda: cp(wr_hbm, wr_ref, S_WR)
    wg_cp = lambda: cp(wg_hbm, wg_ref, S_WG)
    wu_cp = lambda: cp(wu_hbm, wu_ref, S_WU)
    wd_cp = lambda: cp(wdt_hbm, wx_ref.at[:, 0:FF], S_WD)

    def modcol(i):
        return modc_ref[i * D:(i + 1) * D, :]

    def modulation(lo, hi):
        c = c_ref[...].astype(F32)
        sc8 = jnp.broadcast_to((c * _sigmoid(c)).astype(BF16), (8, D))
        mods = []
        for a in range(lo, hi, MA):
            mod = _rb(jnp.dot(sc8, wmod_ref[:, a:a + MA], preferred_element_type=F32))
            lane = lax.broadcasted_iota(jnp.int32, mod.shape, 1) + a
            is_scale = ((lane >= D) & (lane < 2 * D)) | ((lane >= 4 * D) & (lane < 5 * D))
            mods.append(jnp.where(is_scale, _rb(1.0 + mod), mod))
        return mods

    @pl.when(step == 0)
    def _prologue():
        wma_cp().start()
        c_cp().start()
        for i in range(XCH):
            x_copy(i).start()
        for d in group_copies(0) + group_copies(1):
            d.start()
        wr_cp().start()
        acc_ref[...] = jnp.zeros((D, S), F32)
        wma_cp().wait()
        c_cp().wait()
        modc_ref[0:MA, :] = _as_cols(modulation(0, MA)[0][0:1, :]).astype(F32)

        def ln1(i, carry):
            x_copy(i).wait()
            x = xt_ref[:, pl.ds(pl.multiple_of(i * TCH, TCH), TCH)].astype(F32)
            piv = x[0:1, :]
            d = x - piv
            md = jnp.mean(d, axis=0, keepdims=True)
            var = jnp.maximum(jnp.mean(d * d, axis=0, keepdims=True) - md * md, 0.0)
            mb, sd = _ln_rows(piv + md, var)
            rs = 1.0 / sd
            n = TCH // LANES
            for u in range(n):
                st_ref[0, pl.ds(n * i + u, 1), :] = mb[:, u * LANES:(u + 1) * LANES]
            ht = (x * rs - mb * rs) * _tile(modcol(1), n) + _tile(modcol(0), n)
            h_ref[pl.ds(pl.multiple_of(i * (TCH // 2), TCH // 2), TCH // 2), :] = pltpu.bitcast(
                ht.astype(BF16).T, U32)
            return carry
        lax.fori_loop(0, XCH, ln1, 0)

    @pl.when(step == MOD_STEP)
    def _late_modulation():
        wr_cp().wait()
        wmb_cp().wait()
        wg_cp().wait()
        wu_cp().wait()
        wd_cp().wait()
        m23, m45 = modulation(MA, 6 * D)
        sb, cb, gb = m23[:, D:MA], m45[:, 0:D], m45[:, D:MA]
        mrow_ref[0] = sb
        mrow_ref[1] = cb
        mrow_ref[2] = gb
        c23 = _as_cols(m23[0:1, :]).astype(F32)
        c45 = _as_cols(m45[0:1, :]).astype(F32)
        modc_ref[0:D, :] = c23[0:D]
        modc_ref[D:MA, :] = c45[D:MA] * c45[0:D]
        modc_ref[MA:3 * D, :] = c45[D:MA] * c23[D:MA]
        wr = wr_ref[...].astype(F32).reshape(1, D)
        wc = wr * cb[0:1, :]
        whi = _rb(wc)
        wlo = _rb(wc - whi)
        row = lax.broadcasted_iota(jnp.int32, (16, D), 0)
        lhs_ref[...] = jnp.where(row == 0, 1.0, jnp.where(row == 1, whi, jnp.where(
            row == 2, wlo, 0.0))).astype(BF16)
        rc_ref[0:1, :] = jnp.broadcast_to(jnp.sum(whi + wlo, axis=1, keepdims=True), (1, LANES))
        rc_ref[1:2, :] = jnp.broadcast_to(jnp.sum(wr * sb[0:1, :], axis=1, keepdims=True), (1, LANES))

    for d in group_copies(step):
        d.wait()

    slot = step % 2
    k = k_buf[slot]
    v = v_buf[slot]
    wq = wq_buf[slot]
    wot = wot_buf[slot]

    def qproj(j):
        hb = pltpu.bitcast(h_ref[j * (BQ // 2):(j + 1) * (BQ // 2), :], BF16)
        q2 = jnp.dot(hb, wq, preferred_element_type=F32)
        return (q2 * qscale).astype(BF16)

    def qk(ci, lo, hi):
        return lax.dot_general(qs[ci], k[lo:hi], _NT, preferred_element_type=F32)

    def softmax_pv(s, late):
        m = jnp.max(s, axis=1, keepdims=True)
        p = jnp.exp2(s - m)
        o = jnp.dot(p.astype(BF16), v, preferred_element_type=F32)
        if late:
            lp = p[:, 0:LANES]
            for i in range(1, SK // LANES):
                lp = lp + p[:, i * LANES:(i + 1) * LANES]
            l = jnp.sum(jnp.where(lp < 0.0, o, lp), axis=1, keepdims=True)
        else:
            l = jnp.sum(p, axis=1, keepdims=True)
        rl = pl.reciprocal(l, approx=True)
        rl = rl * (2.0 - l * rl)
        return (o * rl).astype(BF16)

    def oproj(j):
        o2 = jnp.concatenate([outs[REP * j + r] for r in range(REP)], axis=1)
        acc_ref[:, j * BQ:(j + 1) * BQ] += lax.dot_general(wot, o2, _NT, preferred_element_type=F32)

    q2s = [qproj(j) for j in range(NB)]
    qs = [q2s[j][:, r * DH:(r + 1) * DH] for j in range(NB) for r in range(REP)]
    outs = []
    done = 0
    s_head = None
    for ci in range(len(qs)):
        if s_head is None:
            s = qk(ci, 0, SK)
        else:
            s = jnp.concatenate([s_head, qk(ci, SPLIT, SK)], axis=1)
        s_head = qk(ci + 1, 0, SPLIT) if (C0 <= ci < len(qs) - 1) else None
        outs.append(softmax_pv(s, late=(ci == len(qs) - 1)))
        if ci % REP == REP - 1 and ci // REP - OPD >= 0:
            oproj(done)
            done += 1
    for j in range(done, NB):
        oproj(j)

    @pl.when(step + 2 < NG)
    def _():
        for d in group_copies(step + 2):
            d.start()

    @pl.when(step == 0)
    def _():
        wmb_cp().start()
        wg_cp().start()

    @pl.when(step == 1)
    def _():
        wu_cp().start()

    @pl.when(step == 2)
    def _():
        wd_cp().start()

    @pl.when(step == NG - 1)
    def _epilogue():
        @pl.when(step > 0)
        def _ln2_sums():
            for sl in range(NSL):
                cols = slice(sl * LANES, (sl + 1) * LANES)
                piv = st_ref[0, sl:sl + 1, :]
                for r0 in range(0, D, LANES):
                    r1 = min(r0 + LANES, D)
                    x2 = xt_ref[r0:r1, cols].astype(F32) + modc_ref[r0:r1, :] * acc_ref[r0:r1, cols]
                    acc_ref[r0:r1, cols] = x2
                    xb = x2.astype(BF16)
                    xb_ref[r0 // 2:r1 // 2, cols] = pltpu.bitcast(xb, U32)
                    d = x2 - piv
                    lhs = lhs_ref[:, r0:r1]
                    t1 = jnp.dot(lhs, xb, preferred_element_type=F32)[0:8, :]
                    t2 = jnp.dot(lhs, (d * d).astype(BF16), preferred_element_type=F32)[0:8, :]
                    s1, s2 = (t1, t2) if r0 == 0 else (s1 + t1, s2 + t2)
                for n in range(3):
                    st_ref[1 + n, sl:sl + 1, :] = s1[n:n + 1, :]
                st_ref[4, sl:sl + 1, :] = s2[0:1, :]

        mean = st_ref[1] * (1.0 / D)
        md = mean - st_ref[0]
        mb, sd = _ln_rows(mean, jnp.maximum(st_ref[4] * (1.0 / D) - md * md, 0.0))
        rs = 1.0 / sd
        st_ref[5] = rs
        st_ref[6] = mb * rs
        r = (st_ref[2] + st_ref[3] - mb * rc_ref[0:1, :]) * rs + rc_ref[1:2, :]

        lane16 = lax.broadcasted_iota(jnp.int32, (16, LANES), 1)
        never = lane16 > step + LANES

        def out_unit(n):
            w = OUW * LANES
            cols = slice(n * w, (n + 1) * w)
            rs, mrs = (jnp.concatenate([st_ref[k, n * OUW + u:n * OUW + u + 1, :]
                                        for u in range(OUW)], axis=1) for k in (5, 6))
            for r0 in range(0, D, OPR):
                x2 = acc_ref[r0:r0 + OPR, cols]
                o = x2 + ((x2 * rs - mrs) * _tile(modc_ref[D + r0:D + r0 + OPR, :], OUW)
                          + _tile(modc_ref[MA + r0:MA + r0 + OPR, :], OUW))
                wx_ref[r0:r0 + OPR, FF + n * w:FF + (n + 1) * w] = o.astype(BF16)
            dyn0 = pl.multiple_of(FF + (step - (NG - 1)) * LANES, LANES)
            return wx_ref[0:16, pl.ds(dyn0, LANES)].astype(F32)

        r = _rb(r) + 0.0
        bits = pltpu.bitcast(r, jnp.int32)
        mono = bits ^ ((bits >> 31) & jnp.int32(0x7FFFFFFF))
        tok = (lax.broadcasted_iota(jnp.int32, (NSL, LANES), 0) * LANES
               + lax.broadcasted_iota(jnp.int32, (NSL, LANES), 1))
        keyi = (((mono >> 16) + 32768) * S + (S - 1 - tok)) + jnp.int32(1 << 29)
        key = pltpu.bitcast(keyi, F32)

        row16 = lax.broadcasted_iota(jnp.int32, (16, LANES), 0)
        rowc = lax.broadcasted_iota(jnp.int32, (16, 1), 0)
        sel_slab, sel_off = [], []
        tie, nunit = None, 0
        xsel = jnp.zeros((16, D), F32)
        mbsel = jnp.zeros((16, 1), F32)
        rssel = jnp.zeros((16, 1), F32)
        ksel = jnp.zeros((16, 1), F32)
        for t in range(TOPC):
            kmax = jnp.max(jnp.max(key, axis=0, keepdims=True), axis=1, keepdims=True)
            hit = key == kmax
            key = jnp.where(hit, 0.0, key)
            pick = lambda z: jnp.sum(jnp.sum(jnp.where(hit, z, 0.0), axis=0, keepdims=True),
                                     axis=1, keepdims=True)
            mbsel = jnp.where(rowc == t, pick(mb), mbsel)
            rssel = jnp.where(rowc == t, pick(rs), rssel)
            for _ in range(TK_TIES.count(t)):
                tie = out_unit(nunit)
                nunit += 1
                key = jnp.where(never, tie, key)
            ksel = jnp.where(rowc == t, kmax, ksel)
            ki = pltpu.bitcast(kmax, jnp.int32)[0, 0]
            idx = (S - 1) - (ki & (S - 1))
            slab = idx >> 7
            off = idx & (LANES - 1)
            onehot = jnp.where((row16 == t) & (lane16 == off), 1.0, 0.0).astype(BF16)
            dslab = xb_ref[:, pl.ds(pl.multiple_of(slab * LANES, LANES), LANES)]
            xsel = xsel + lax.dot_general(onehot, pltpu.bitcast(dslab, BF16), _NT,
                                          preferred_element_type=F32)
            sel_slab.append(slab)
            sel_off.append(off)
        nsel = _rb(_rb(xsel - mbsel) * rssel)
        hsel = _rb(_rb(nsel * mrow_ref[1, 0:1, :]) + mrow_ref[0, 0:1, :])
        hi = ((pltpu.bitcast(ksel, jnp.int32) - jnp.int32(1 << 29)) // S - 32768) << 16
        rbits = hi ^ ((hi >> 31) & jnp.int32(0x7FFF0000))
        gate = _rb(_sigmoid(jnp.where(rowc < TOPC, pltpu.bitcast(rbits, F32), 0.0)))

        def out_copy(sl, r0, nr):
            c0 = pl.multiple_of(sl * LANES, LANES)
            return cp(wx_ref.at[r0:r0 + nr, pl.ds(pl.multiple_of(FF + c0, LANES), LANES)],
                      out_hbm.at[r0:r0 + nr, pl.ds(c0, LANES)], S_O)

        fresh = []
        seen = jnp.int32(0)
        for t in range(TOPC):
            fresh.append(((seen >> sel_slab[t]) & 1) == 0)
            seen = seen | (1 << sel_slab[t])
        plain = [((seen >> sl) & 1) == 0 for sl in range(NSL)]

        for n in range(nunit, NSL // OUW):
            tie = out_unit(n)
        for sl in range(NSL):
            pl.when(plain[sl])(lambda sl=sl: out_copy(sl, 0, D).start())

        h0 = jnp.where(never, tie, hsel[:, 0:LANES])
        hs = jnp.concatenate([h0, hsel[:, LANES:]], axis=1).astype(BF16)
        gpre = _rb(jnp.dot(hs, wg_ref[...], preferred_element_type=F32))
        u = _rb(jnp.dot(hs, wu_ref[...], preferred_element_type=F32))
        a = (_rb(gpre * _sigmoid(gpre)) * u).astype(BF16)

        pieces = [(r0, min(LANES, D - r0)) for r0 in range(0, D, LANES)]

        gb = mrow_ref[2, 0:1, :]

        def down(r0, nr):
            y = lax.dot_general(a, wx_ref[r0:r0 + nr, 0:FF], _NT, preferred_element_type=F32)
            c = slice(r0, r0 + nr)
            return xsel[:, c] + gb[:, c] * (hsel[:, c] + y * gate)

        def patch(r0, nr, new):
            lane = lax.broadcasted_iota(jnp.int32, (nr // 2, LANES), 1)
            for t in range(TOPC):
                cols = pl.ds(pl.multiple_of(FF + sel_slab[t] * LANES, LANES), LANES)
                old = pltpu.bitcast(wx_ref[r0:r0 + nr, cols], U32)
                upd = pltpu.bitcast(_as_cols(new[t:t + 1, :]), U32)
                wx_ref[r0:r0 + nr, cols] = pltpu.bitcast(jnp.where(lane == sel_off[t], upd, old), BF16)
            for t in range(TOPC):
                pl.when(fresh[t])(lambda t=t: out_copy(sel_slab[t], r0, nr).start())

        yts = [down(*pieces[0])]
        for n in range(len(pieces)):
            if n + 1 < len(pieces):
                yts.append(down(*pieces[n + 1]))
            patch(*pieces[n], yts[n])

        cp(wx_ref.at[:, FF:FF + S], out_hbm, S_O).wait()


@jax.jit
def pallas_adaLN_cond__gqa_block_cached__moe_arch_mod__prompt_kernel(
    A_x: jax.Array,
    A_k_cache: jax.Array,
    A_v_cache: jax.Array,
    A_wq: jax.Array,
    A_wo: jax.Array,
    B_x: jax.Array,
    B_w_r: jax.Array,
    B_w_gate: jax.Array,
    B_w_up: jax.Array,
    B_w_down: jax.Array,
    c: jax.Array,
    w_mod: jax.Array,
):
    del B_x
    B, S, D = A_x.shape
    assert B == 1
    NG, SK = A_k_cache.shape[1], A_k_cache.shape[2]
    REP = HQ // NG
    FF = B_w_gate.shape[1]
    GW = REP * DH

    xt = A_x.reshape(S, D).T
    wot = A_wo.T
    wdt = B_w_down.T
    k = A_k_cache.reshape(NG, SK, DH)
    v = A_v_cache.reshape(NG, SK, DH)

    hbm = pl.BlockSpec(memory_space=pl.ANY)
    out_t = pl.pallas_call(
        functools.partial(_kernel, S=S, SK=SK, D=D, FF=FF, NG=NG, REP=REP),
        grid=(NG,),
        in_specs=[hbm] * 11,
        out_specs=hbm,
        out_shape=jax.ShapeDtypeStruct((D, S), BF16),
        scratch_shapes=[
            pltpu.VMEM((D, S), BF16),
            pltpu.VMEM((2, SK, DH), BF16),
            pltpu.VMEM((2, SK, DH), BF16),
            pltpu.VMEM((2, D, GW), BF16),
            pltpu.VMEM((2, D, GW), BF16),
            pltpu.VMEM((D,), BF16),
            pltpu.VMEM((1, D), BF16),
            pltpu.VMEM((D, 6 * D), BF16),
            pltpu.VMEM((D, FF), BF16),
            pltpu.VMEM((D, FF), BF16),
            pltpu.VMEM((D, FF + S), BF16),
            pltpu.VMEM((3 * D, LANES), F32),
            pltpu.VMEM((3, 8, D), F32),
            pltpu.VMEM((16, D), BF16),
            pltpu.VMEM((8, LANES), F32),
            pltpu.VMEM((S // 2, D), U32),
            pltpu.VMEM((D, S), F32),
            pltpu.VMEM((D // 2, S), U32),
            pltpu.VMEM((7, S // LANES, LANES), F32),
            pltpu.SemaphoreType.DMA((N_SEMS,)),
        ],
        compiler_params=pltpu.CompilerParams(
            dimension_semantics=("arbitrary",),
            vmem_limit_bytes=100 * 1024 * 1024,
            disable_bounds_checks=True,
        ),
    )(xt, k, v, A_wq, wot, B_w_r, c, w_mod, B_w_gate, B_w_up, wdt)
    return out_t.T.reshape(B, S, D)
```

```python
import functools
import math

import jax
import jax.numpy as jnp
from jax import lax
import jax.experimental.pallas as pl
import jax.experimental.pallas.tpu as pltpu

F32 = jnp.float32
BF16 = jnp.bfloat16
U32 = jnp.uint32

HQ = 32
DH = 128
TOPC = 8
LN_EPS = 1e-5
BQ = 256
LANES = 128
SPLIT = 512
C0 = 2
OPD = 2
XCH = 4
DIST = 2
TIEC = 2048
PIECES = [(0, 128), (128, 128), (256, 128), (384, 128), (512, 64)]
OUW = 2
TK_TIES = [0, 2, 3, 5, 6]
OPR = 16
MOD_STEP = 4

_NT = (((1,), (1,)), ((), ()))

S_C, S_WMA, S_WMB, S_WR, S_WG, S_WU, S_WD = range(7)
S_X = 7
S_G = S_X + XCH
S_O = S_G + 2
N_SEMS = S_O + 1


def _rb(x):
    return x.astype(BF16).astype(F32)


def _sigmoid(x):
    return 1.0 / (1.0 + jnp.exp(-x))


def _ln_rows(mean, var):
    eps = _rb(jnp.full((1, 1), LN_EPS, F32))
    return _rb(mean), _rb(jnp.sqrt(_rb(_rb(var) + eps)))


def _tile(col, n):
    return jnp.concatenate([col] * n, axis=1)


def _as_cols(row):
    return jnp.broadcast_to(row, (LANES, row.shape[1])).astype(BF16).T


def _kernel(xt_hbm, k_hbm, v_hbm, wq_hbm, wot_hbm, wr_hbm, c_hbm, wmod_hbm,
            wg_hbm, wu_hbm, wdt_hbm,
            out_hbm,
            xt_ref, k_buf, v_buf, wq_buf, wot_buf, wr_ref, c_ref, wmod_ref,
            wg_ref, wu_ref, wdt_ref, out_ref,
            modc_ref, mrow_ref, lhs_ref, rc_ref, h_ref, acc_ref, xb_ref, st_ref,
            sems,
            *, S, SK, D, FF, NG, REP):
    step = pl.program_id(0)
    qscale = (DH ** -0.5) * math.log2(math.e)
    NB = S // BQ
    GW = REP * DH
    TCH = S // XCH
    MA = 2 * D
    NSL = S // LANES

    def cp(src, dst, sem):
        return pltpu.make_async_copy(src, dst, sems.at[sem])

    def x_copy(i):
        cols = pl.ds(pl.multiple_of(i * TCH, TCH), TCH)
        return cp(xt_hbm.at[:, cols], xt_ref.at[:, cols], S_X + i)

    def group_copies(grp):
        slot = grp % 2
        cols = pl.ds(pl.multiple_of(grp * GW, GW), GW)
        return (cp(wq_hbm.at[:, cols], wq_buf.at[slot], S_G + slot),
                cp(k_hbm.at[grp], k_buf.at[slot], S_G + slot),
                cp(v_hbm.at[grp], v_buf.at[slot], S_G + slot),
                cp(wot_hbm.at[:, cols], wot_buf.at[slot], S_G + slot))

    c_cp = lambda: cp(c_hbm, c_ref, S_C)
    wma_cp = lambda: cp(wmod_hbm.at[:, 0:MA], wmod_ref.at[:, 0:MA], S_WMA)
    wmb_cp = lambda: cp(wmod_hbm.at[:, MA:6 * D], wmod_ref.at[:, MA:6 * D], S_WMB)
    wr_cp = lambda: cp(wr_hbm, wr_ref, S_WR)
    wg_cp = lambda: cp(wg_hbm, wg_ref, S_WG)
    wu_cp = lambda: cp(wu_hbm, wu_ref, S_WU)
    wd_cp = lambda: cp(wdt_hbm, wdt_ref, S_WD)

    def modcol(i):
        return modc_ref[i * D:(i + 1) * D, :]

    def modulation(lo, hi):
        c = c_ref[...].astype(F32)
        sc8 = jnp.broadcast_to((c * _sigmoid(c)).astype(BF16), (8, D))
        mods = []
        for a in range(lo, hi, MA):
            mod = _rb(jnp.dot(sc8, wmod_ref[:, a:a + MA], preferred_element_type=F32))
            lane = lax.broadcasted_iota(jnp.int32, mod.shape, 1) + a
            is_scale = ((lane >= D) & (lane < 2 * D)) | ((lane >= 4 * D) & (lane < 5 * D))
            mods.append(jnp.where(is_scale, _rb(1.0 + mod), mod))
        return mods

    @pl.when(step == 0)
    def _prologue():
        wma_cp().start()
        c_cp().start()
        for i in range(XCH):
            x_copy(i).start()
        for d in group_copies(0) + group_copies(1):
            d.start()
        wr_cp().start()
        acc_ref[...] = jnp.zeros((D, S), F32)
        wma_cp().wait()
        c_cp().wait()
        modc_ref[0:MA, :] = _as_cols(modulation(0, MA)[0][0:1, :]).astype(F32)

        def ln1(i, carry):
            x_copy(i).wait()
            x = xt_ref[:, pl.ds(pl.multiple_of(i * TCH, TCH), TCH)].astype(F32)
            piv = x[0:1, :]
            d = x - piv
            md = jnp.mean(d, axis=0, keepdims=True)
            var = jnp.maximum(jnp.mean(d * d, axis=0, keepdims=True) - md * md, 0.0)
            mb, sd = _ln_rows(piv + md, var)
            rs = 1.0 / sd
            n = TCH // LANES
            for u in range(n):
                st_ref[0, pl.ds(n * i + u, 1), :] = mb[:, u * LANES:(u + 1) * LANES]
            ht = (x * rs - mb * rs) * _tile(modcol(1), n) + _tile(modcol(0), n)
            h_ref[pl.ds(pl.multiple_of(i * (TCH // 2), TCH // 2), TCH // 2), :] = pltpu.bitcast(
                ht.astype(BF16).T, U32)
            return carry
        lax.fori_loop(0, XCH, ln1, 0)

    @pl.when(step == MOD_STEP)
    def _late_modulation():
        wr_cp().wait()
        wmb_cp().wait()
        wg_cp().wait()
        wu_cp().wait()
        wd_cp().wait()
        m23, m45 = modulation(MA, 6 * D)
        sb, cb, gb = m23[:, D:MA], m45[:, 0:D], m45[:, D:MA]
        mrow_ref[0] = sb
        mrow_ref[1] = cb
        mrow_ref[2] = gb
        c23 = _as_cols(m23[0:1, :]).astype(F32)
        c45 = _as_cols(m45[0:1, :]).astype(F32)
        modc_ref[0:D, :] = c23[0:D]
        modc_ref[D:MA, :] = c45[D:MA] * c45[0:D]
        modc_ref[MA:3 * D, :] = c45[D:MA] * c23[D:MA]
        wr = wr_ref[...].astype(F32).reshape(1, D)
        wc = wr * cb[0:1, :]
        whi = _rb(wc)
        wlo = _rb(wc - whi)
        row = lax.broadcasted_iota(jnp.int32, (16, D), 0)
        lhs_ref[...] = jnp.where(row == 0, 1.0, jnp.where(row == 1, whi, jnp.where(
            row == 2, wlo, 0.0))).astype(BF16)
        rc_ref[0:1, :] = jnp.broadcast_to(jnp.sum(whi + wlo, axis=1, keepdims=True), (1, LANES))
        rc_ref[1:2, :] = jnp.broadcast_to(jnp.sum(wr * sb[0:1, :], axis=1, keepdims=True), (1, LANES))

    for d in group_copies(step):
        d.wait()

    slot = step % 2
    k = k_buf[slot]
    v = v_buf[slot]
    wq = wq_buf[slot]
    wot = wot_buf[slot]

    def qproj(j):
        hb = pltpu.bitcast(h_ref[j * (BQ // 2):(j + 1) * (BQ // 2), :], BF16)
        q2 = jnp.dot(hb, wq, preferred_element_type=F32)
        return (q2 * qscale).astype(BF16)

    def qk(ci, lo, hi):
        return lax.dot_general(qs[ci], k[lo:hi], _NT, preferred_element_type=F32)

    def softmax_pv(s, late):
        m = jnp.max(s, axis=1, keepdims=True)
        p = jnp.exp2(s - m)
        o = jnp.dot(p.astype(BF16), v, preferred_element_type=F32)
        if late:
            lp = p[:, 0:LANES]
            for i in range(1, SK // LANES):
                lp = lp + p[:, i * LANES:(i + 1) * LANES]
            l = jnp.sum(jnp.where(lp < 0.0, o, lp), axis=1, keepdims=True)
        else:
            l = jnp.sum(p, axis=1, keepdims=True)
        rl = pl.reciprocal(l, approx=True)
        rl = rl * (2.0 - l * rl)
        return (o * rl).astype(BF16)

    def oproj(j):
        o2 = jnp.concatenate([outs[REP * j + r] for r in range(REP)], axis=1)
        acc_ref[:, j * BQ:(j + 1) * BQ] += lax.dot_general(wot, o2, _NT, preferred_element_type=F32)

    q2s = [qproj(j) for j in range(NB)]
    qs = [q2s[j][:, r * DH:(r + 1) * DH] for j in range(NB) for r in range(REP)]
    outs = []
    done = 0
    s_head = None
    for ci in range(len(qs)):
        if s_head is None:
            s = qk(ci, 0, SK)
        else:
            s = jnp.concatenate([s_head, qk(ci, SPLIT, SK)], axis=1)
        s_head = qk(ci + 1, 0, SPLIT) if (C0 <= ci < len(qs) - 1) else None
        outs.append(softmax_pv(s, late=(ci == len(qs) - 1)))
        if ci % REP == REP - 1 and ci // REP - OPD >= 0:
            oproj(done)
            done += 1
    for j in range(done, NB):
        oproj(j)

    @pl.when(step + 2 < NG)
    def _():
        for d in group_copies(step + 2):
            d.start()

    @pl.when(step == 0)
    def _():
        wmb_cp().start()
        wg_cp().start()

    @pl.when(step == 1)
    def _():
        wu_cp().start()

    @pl.when(step == 2)
    def _():
        wd_cp().start()

    @pl.when(step == NG - 1)
    def _epilogue():
        @pl.when(step > 0)
        def _ln2_sums():
            for sl in range(NSL):
                cols = slice(sl * LANES, (sl + 1) * LANES)
                piv = st_ref[0, sl:sl + 1, :]
                for r0 in range(0, D, LANES):
                    r1 = min(r0 + LANES, D)
                    x2 = xt_ref[r0:r1, cols].astype(F32) + modc_ref[r0:r1, :] * acc_ref[r0:r1, cols]
                    acc_ref[r0:r1, cols] = x2
                    xb = x2.astype(BF16)
                    xb_ref[r0 // 2:r1 // 2, cols] = pltpu.bitcast(xb, U32)
                    d = x2 - piv
                    lhs = lhs_ref[:, r0:r1]
                    t1 = jnp.dot(lhs, xb, preferred_element_type=F32)[0:8, :]
                    t2 = jnp.dot(lhs, (d * d).astype(BF16), preferred_element_type=F32)[0:8, :]
                    s1, s2 = (t1, t2) if r0 == 0 else (s1 + t1, s2 + t2)
                for n in range(3):
                    st_ref[1 + n, sl:sl + 1, :] = s1[n:n + 1, :]
                st_ref[4, sl:sl + 1, :] = s2[0:1, :]

        mean = st_ref[1] * (1.0 / D)
        md = mean - st_ref[0]
        mb, sd = _ln_rows(mean, jnp.maximum(st_ref[4] * (1.0 / D) - md * md, 0.0))
        rs = 1.0 / sd
        st_ref[5] = rs
        st_ref[6] = mb * rs
        r = (st_ref[2] + st_ref[3] - mb * rc_ref[0:1, :]) * rs + rc_ref[1:2, :]

        lane16 = lax.broadcasted_iota(jnp.int32, (16, LANES), 1)
        never = lane16 > step + LANES

        def after_out_stores():
            dyn0 = pl.multiple_of((step - (NG - 1)) * LANES, LANES)
            return out_ref[0:16, pl.ds(dyn0, LANES)]

        def out_unit(n):
            w = OUW * LANES
            cols = slice(n * w, (n + 1) * w)
            rs, mrs = (jnp.concatenate([st_ref[k, n * OUW + u:n * OUW + u + 1, :]
                                        for u in range(OUW)], axis=1) for k in (5, 6))
            for r0 in range(0, D, OPR):
                x2 = acc_ref[r0:r0 + OPR, cols]
                o = x2 + ((x2 * rs - mrs) * _tile(modc_ref[D + r0:D + r0 + OPR, :], OUW)
                          + _tile(modc_ref[MA + r0:MA + r0 + OPR, :], OUW))
                out_ref[r0:r0 + OPR, cols] = o.astype(BF16)
            return after_out_stores().astype(F32)

        r = _rb(r) + 0.0
        bits = pltpu.bitcast(r, jnp.int32)
        mono = bits ^ ((bits >> 31) & jnp.int32(0x7FFFFFFF))
        tok = (lax.broadcasted_iota(jnp.int32, (NSL, LANES), 0) * LANES
               + lax.broadcasted_iota(jnp.int32, (NSL, LANES), 1))
        keyi = (((mono >> 16) + 32768) * S + (S - 1 - tok)) + jnp.int32(1 << 29)
        key = pltpu.bitcast(keyi, F32)

        row16 = lax.broadcasted_iota(jnp.int32, (16, LANES), 0)
        rowc = lax.broadcasted_iota(jnp.int32, (16, 1), 0)
        sel_slab, sel_off = [], []
        tie, nunit = None, 0
        xsel = jnp.zeros((16, D), F32)
        mbsel = jnp.zeros((16, 1), F32)
        rssel = jnp.zeros((16, 1), F32)
        ksel = jnp.zeros((16, 1), F32)
        for t in range(TOPC):
            kmax = jnp.max(jnp.max(key, axis=0, keepdims=True), axis=1, keepdims=True)
            hit = key == kmax
            key = jnp.where(hit, 0.0, key)
            pick = lambda z: jnp.sum(jnp.sum(jnp.where(hit, z, 0.0), axis=0, keepdims=True),
                                     axis=1, keepdims=True)
            mbsel = jnp.where(rowc == t, pick(mb), mbsel)
            rssel = jnp.where(rowc == t, pick(rs), rssel)
            for _ in range(TK_TIES.count(t)):
                tie = out_unit(nunit)
                nunit += 1
                key = jnp.where(never, tie, key)
            ksel = jnp.where(rowc == t, kmax, ksel)
            ki = pltpu.bitcast(kmax, jnp.int32)[0, 0]
            idx = (S - 1) - (ki & (S - 1))
            slab = idx >> 7
            off = idx & (LANES - 1)
            onehot = jnp.where((row16 == t) & (lane16 == off), 1.0, 0.0).astype(BF16)
            dslab = xb_ref[:, pl.ds(pl.multiple_of(slab * LANES, LANES), LANES)]
            xsel = xsel + lax.dot_general(onehot, pltpu.bitcast(dslab, BF16), _NT,
                                          preferred_element_type=F32)
            sel_slab.append(slab)
            sel_off.append(off)
        nsel = _rb(_rb(xsel - mbsel) * rssel)
        hsel = _rb(_rb(nsel * mrow_ref[1, 0:1, :]) + mrow_ref[0, 0:1, :])
        hi = ((pltpu.bitcast(ksel, jnp.int32) - jnp.int32(1 << 29)) // S - 32768) << 16
        rbits = hi ^ ((hi >> 31) & jnp.int32(0x7FFF0000))
        gate = _rb(_sigmoid(jnp.where(rowc < TOPC, pltpu.bitcast(rbits, F32), 0.0)))

        def out_copy(sl, r0, nr):
            c0 = pl.multiple_of(sl * LANES, LANES)
            return cp(out_ref.at[r0:r0 + nr, pl.ds(c0, LANES)],
                      out_hbm.at[r0:r0 + nr, pl.ds(c0, LANES)], S_O)

        fresh = []
        seen = jnp.int32(0)
        for t in range(TOPC):
            fresh.append(((seen >> sel_slab[t]) & 1) == 0)
            seen = seen | (1 << sel_slab[t])
        plain = [((seen >> sl) & 1) == 0 for sl in range(NSL)]

        for n in range(nunit, NSL // OUW):
            tie = out_unit(n)
        for sl in range(NSL):
            pl.when(plain[sl])(lambda sl=sl: out_copy(sl, 0, D).start())

        h0 = jnp.where(never, tie, hsel[:, 0:LANES])
        hs = jnp.concatenate([h0, hsel[:, LANES:]], axis=1).astype(BF16)
        gpre = _rb(jnp.dot(hs, wg_ref[...], preferred_element_type=F32))
        u = _rb(jnp.dot(hs, wu_ref[...], preferred_element_type=F32))
        a = (_rb(gpre * _sigmoid(gpre)) * u).astype(BF16)

        pieces = PIECES

        gb = mrow_ref[2, 0:1, :]

        def down(r0, nr, tied):
            lhs = a
            if tied:
                a0 = jnp.where(never[0:8, :], pltpu.bitcast(after_out_stores(), U32),
                               pltpu.bitcast(a[:, TIEC:TIEC + LANES], U32))
                lhs = jnp.concatenate(([a[:, 0:TIEC]] if TIEC else []) + [pltpu.bitcast(a0, BF16)] + ([a[:, TIEC + LANES:]] if TIEC + LANES < FF else []), axis=1)
            y = lax.dot_general(lhs, wdt_ref[r0:r0 + nr, :], _NT, preferred_element_type=F32)
            c = slice(r0, r0 + nr)
            return xsel[:, c] + gb[:, c] * (hsel[:, c] + y * gate)

        def patch(r0, nr, new):
            lane = lax.broadcasted_iota(jnp.int32, (nr // 2, LANES), 1)
            for t in range(TOPC):
                cols = pl.ds(pl.multiple_of(sel_slab[t] * LANES, LANES), LANES)
                old = pltpu.bitcast(out_ref[r0:r0 + nr, cols], U32)
                upd = pltpu.bitcast(_as_cols(new[t:t + 1, :]), U32)
                out_ref[r0:r0 + nr, cols] = pltpu.bitcast(jnp.where(lane == sel_off[t], upd, old), BF16)
            for t in range(TOPC):
                pl.when(fresh[t])(lambda t=t: out_copy(sel_slab[t], r0, nr).start())

        if DIST == 1:
            for n in range(len(pieces)):
                patch(*pieces[n], down(*pieces[n], n > 0))
        else:
            yts = [down(*pieces[0], False)]
            for n in range(len(pieces)):
                if n + 1 < len(pieces):
                    yts.append(down(*pieces[n + 1], n > 0))
                patch(*pieces[n], yts[n])

        cp(out_ref, out_hbm, S_O).wait()


@jax.jit
def pallas_adaLN_cond__gqa_block_cached__moe_arch_mod__prompt_kernel(
    A_x: jax.Array,
    A_k_cache: jax.Array,
    A_v_cache: jax.Array,
    A_wq: jax.Array,
    A_wo: jax.Array,
    B_x: jax.Array,
    B_w_r: jax.Array,
    B_w_gate: jax.Array,
    B_w_up: jax.Array,
    B_w_down: jax.Array,
    c: jax.Array,
    w_mod: jax.Array,
):
    del B_x
    B, S, D = A_x.shape
    assert B == 1
    NG, SK = A_k_cache.shape[1], A_k_cache.shape[2]
    REP = HQ // NG
    FF = B_w_gate.shape[1]
    GW = REP * DH

    xt = A_x.reshape(S, D).T
    wot = A_wo.T
    wdt = B_w_down.T
    k = A_k_cache.reshape(NG, SK, DH)
    v = A_v_cache.reshape(NG, SK, DH)

    hbm = pl.BlockSpec(memory_space=pl.ANY)
    out_t = pl.pallas_call(
        functools.partial(_kernel, S=S, SK=SK, D=D, FF=FF, NG=NG, REP=REP),
        grid=(NG,),
        in_specs=[hbm] * 11,
        out_specs=hbm,
        out_shape=jax.ShapeDtypeStruct((D, S), BF16),
        scratch_shapes=[
            pltpu.VMEM((D, S), BF16),
            pltpu.VMEM((2, SK, DH), BF16),
            pltpu.VMEM((2, SK, DH), BF16),
            pltpu.VMEM((2, D, GW), BF16),
            pltpu.VMEM((2, D, GW), BF16),
            pltpu.VMEM((D,), BF16),
            pltpu.VMEM((1, D), BF16),
            pltpu.VMEM((D, 6 * D), BF16),
            pltpu.VMEM((D, FF), BF16),
            pltpu.VMEM((D, FF), BF16),
            pltpu.VMEM((D, FF), BF16),
            pltpu.VMEM((D, S), BF16),
            pltpu.VMEM((3 * D, LANES), F32),
            pltpu.VMEM((3, 8, D), F32),
            pltpu.VMEM((16, D), BF16),
            pltpu.VMEM((8, LANES), F32),
            pltpu.VMEM((S // 2, D), U32),
            pltpu.VMEM((D, S), F32),
            pltpu.VMEM((D // 2, S), U32),
            pltpu.VMEM((7, S // LANES, LANES), F32),
            pltpu.SemaphoreType.DMA((N_SEMS,)),
        ],
        compiler_params=pltpu.CompilerParams(
            dimension_semantics=("arbitrary",),
            vmem_limit_bytes=100 * 1024 * 1024,
            disable_bounds_checks=True,
        ),
    )(xt, k, v, A_wq, wot, B_w_r, c, w_mod, B_w_gate, B_w_up, wdt)
    return out_t.T.reshape(B, S, D)
```

```python
import functools
import math

import jax
import jax.numpy as jnp
from jax import lax
import jax.experimental.pallas as pl
import jax.experimental.pallas.tpu as pltpu

F32 = jnp.float32
BF16 = jnp.bfloat16
U32 = jnp.uint32

HQ = 32
DH = 128
TOPC = 8
LN_EPS = 1e-5
BQ = 256
LANES = 128
HEAD = [768, 512, 512, 1024, 768, 512, 512, 512, 768, 768, 512, 512, 512, 512, 512, 0]
MODE = [2, 1, 2, 2, 0, 0, 0, 0, 0, 1, 0, 0, 0, 2, 0, 1]
QP_POS = [-1, -1, -1, -1, -1, 3, -1, -1]
OP_POS = [11, 15, 21, 23, 30, 31, 31, 31]
XCH = 4
DIST = 2
TIEC = 2048
PIECES = [(0, 128), (128, 128), (256, 128), (384, 128), (512, 64)]
OUW = 2
TK_TIES = [0, 2, 3, 5, 6]
OPR = 16
MOD_STEP = 4

_NT = (((1,), (1,)), ((), ()))

S_C, S_WMA, S_WMB, S_WR, S_WG, S_WU, S_WD = range(7)
S_X = 7
S_G = S_X + XCH
S_O = S_G + 2
N_SEMS = S_O + 1


def _rb(x):
    return x.astype(BF16).astype(F32)


def _sigmoid(x):
    return 1.0 / (1.0 + jnp.exp(-x))


def _ln_rows(mean, var):
    eps = _rb(jnp.full((1, 1), LN_EPS, F32))
    return _rb(mean), _rb(jnp.sqrt(_rb(_rb(var) + eps)))


def _tile(col, n):
    return jnp.concatenate([col] * n, axis=1)


def _as_cols(row):
    return jnp.broadcast_to(row, (LANES, row.shape[1])).astype(BF16).T


def _kernel(xt_hbm, k_hbm, v_hbm, wq_hbm, wot_hbm, wr_hbm, c_hbm, wmod_hbm,
            wg_hbm, wu_hbm, wdt_hbm,
            out_hbm,
            xt_ref, k_buf, v_buf, wq_buf, wot_buf, wr_ref, c_ref, wmod_ref,
            wg_ref, wu_ref, wdt_ref, out_ref,
            modc_ref, mrow_ref, lhs_ref, rc_ref, h_ref, acc_ref, xb_ref, st_ref,
            sems,
            *, S, SK, D, FF, NG, REP):
    step = pl.program_id(0)
    qscale = (DH ** -0.5) * math.log2(math.e)
    NB = S // BQ
    GW = REP * DH
    TCH = S // XCH
    MA = 2 * D
    NSL = S // LANES

    def cp(src, dst, sem):
        return pltpu.make_async_copy(src, dst, sems.at[sem])

    def x_copy(i):
        cols = pl.ds(pl.multiple_of(i * TCH, TCH), TCH)
        return cp(xt_hbm.at[:, cols], xt_ref.at[:, cols], S_X + i)

    def group_copies(grp):
        slot = grp % 2
        cols = pl.ds(pl.multiple_of(grp * GW, GW), GW)
        return (cp(wq_hbm.at[:, cols], wq_buf.at[slot], S_G + slot),
                cp(k_hbm.at[grp], k_buf.at[slot], S_G + slot),
                cp(v_hbm.at[grp], v_buf.at[slot], S_G + slot),
                cp(wot_hbm.at[:, cols], wot_buf.at[slot], S_G + slot))

    c_cp = lambda: cp(c_hbm, c_ref, S_C)
    wma_cp = lambda: cp(wmod_hbm.at[:, 0:MA], wmod_ref.at[:, 0:MA], S_WMA)
    wmb_cp = lambda: cp(wmod_hbm.at[:, MA:6 * D], wmod_ref.at[:, MA:6 * D], S_WMB)
    wr_cp = lambda: cp(wr_hbm, wr_ref, S_WR)
    wg_cp = lambda: cp(wg_hbm, wg_ref, S_WG)
    wu_cp = lambda: cp(wu_hbm, wu_ref, S_WU)
    wd_cp = lambda: cp(wdt_hbm, wdt_ref, S_WD)

    def modcol(i):
        return modc_ref[i * D:(i + 1) * D, :]

    def modulation(lo, hi):
        c = c_ref[...].astype(F32)
        sc8 = jnp.broadcast_to((c * _sigmoid(c)).astype(BF16), (8, D))
        mods = []
        for a in range(lo, hi, MA):
            mod = _rb(jnp.dot(sc8, wmod_ref[:, a:a + MA], preferred_element_type=F32))
            lane = lax.broadcasted_iota(jnp.int32, mod.shape, 1) + a
            is_scale = ((lane >= D) & (lane < 2 * D)) | ((lane >= 4 * D) & (lane < 5 * D))
            mods.append(jnp.where(is_scale, _rb(1.0 + mod), mod))
        return mods

    @pl.when(step == 0)
    def _prologue():
        wma_cp().start()
        c_cp().start()
        for i in range(XCH):
            x_copy(i).start()
        for d in group_copies(0) + group_copies(1):
            d.start()
        wr_cp().start()
        acc_ref[...] = jnp.zeros((D, S), F32)
        wma_cp().wait()
        c_cp().wait()
        modc_ref[0:MA, :] = _as_cols(modulation(0, MA)[0][0:1, :]).astype(F32)

        def ln1(i, carry):
            x_copy(i).wait()
            x = xt_ref[:, pl.ds(pl.multiple_of(i * TCH, TCH), TCH)].astype(F32)
            piv = x[0:1, :]
            d = x - piv
            md = jnp.mean(d, axis=0, keepdims=True)
            var = jnp.maximum(jnp.mean(d * d, axis=0, keepdims=True) - md * md, 0.0)
            mb, sd = _ln_rows(piv + md, var)
            rs = 1.0 / sd
            n = TCH // LANES
            for u in range(n):
                st_ref[0, pl.ds(n * i + u, 1), :] = mb[:, u * LANES:(u + 1) * LANES]
            ht = (x * rs - mb * rs) * _tile(modcol(1), n) + _tile(modcol(0), n)
            h_ref[pl.ds(pl.multiple_of(i * (TCH // 2), TCH // 2), TCH // 2), :] = pltpu.bitcast(
                ht.astype(BF16).T, U32)
            return carry
        lax.fori_loop(0, XCH, ln1, 0)

    @pl.when(step == MOD_STEP)
    def _late_modulation():
        wr_cp().wait()
        wmb_cp().wait()
        wg_cp().wait()
        wu_cp().wait()
        wd_cp().wait()
        m23, m45 = modulation(MA, 6 * D)
        sb, cb, gb = m23[:, D:MA], m45[:, 0:D], m45[:, D:MA]
        mrow_ref[0] = sb
        mrow_ref[1] = cb
        mrow_ref[2] = gb
        c23 = _as_cols(m23[0:1, :]).astype(F32)
        c45 = _as_cols(m45[0:1, :]).astype(F32)
        modc_ref[0:D, :] = c23[0:D]
        modc_ref[D:MA, :] = c45[D:MA] * c45[0:D]
        modc_ref[MA:3 * D, :] = c45[D:MA] * c23[D:MA]
        wr = wr_ref[...].astype(F32).reshape(1, D)
        wc = wr * cb[0:1, :]
        whi = _rb(wc)
        wlo = _rb(wc - whi)
        row = lax.broadcasted_iota(jnp.int32, (16, D), 0)
        lhs_ref[...] = jnp.where(row == 0, 1.0, jnp.where(row == 1, whi, jnp.where(
            row == 2, wlo, 0.0))).astype(BF16)
        rc_ref[0:1, :] = jnp.broadcast_to(jnp.sum(whi + wlo, axis=1, keepdims=True), (1, LANES))
        rc_ref[1:2, :] = jnp.broadcast_to(jnp.sum(wr * sb[0:1, :], axis=1, keepdims=True), (1, LANES))

    for d in group_copies(step):
        d.wait()

    slot = step % 2
    k = k_buf[slot]
    v = v_buf[slot]
    wq = wq_buf[slot]
    wot = wot_buf[slot]

    def qproj(j):
        hb = pltpu.bitcast(h_ref[j * (BQ // 2):(j + 1) * (BQ // 2), :], BF16)
        q2 = jnp.dot(hb, wq, preferred_element_type=F32)
        return (q2 * qscale).astype(BF16)

    def qk(ci, lo, hi):
        return lax.dot_general(qs[ci], k[lo:hi], _NT, preferred_element_type=F32)

    def softmax_pv(s, mode):
        m = jnp.max(s, axis=1, keepdims=True)
        p = jnp.exp2(s - m)
        parts = [p[:, i * LANES:(i + 1) * LANES] for i in range(SK // LANES)]
        if mode == 2:
            lp = None
            for c in range(0, len(parts), 4):
                t = (parts[c] + parts[c + 1]) + (parts[c + 2] + parts[c + 3])
                lp = t if lp is None else lp + t
                parts[c + 3] = jnp.where(lp < 0.0, lp, parts[c + 3])
            p = jnp.concatenate(parts, axis=1)
        o = jnp.dot(p.astype(BF16), v, preferred_element_type=F32)
        if mode == 0:
            l = jnp.sum(p, axis=1, keepdims=True)
        elif mode == 1:
            lp = functools.reduce(lambda x, y: x + y, parts)
            l = jnp.sum(jnp.where(lp < 0.0, o, lp), axis=1, keepdims=True)
        else:
            l = jnp.sum(lp, axis=1, keepdims=True)
        rl = pl.reciprocal(l, approx=True)
        rl = rl * (2.0 - l * rl)
        return (o * rl).astype(BF16)

    def oproj(j):
        o2 = jnp.concatenate([outs[REP * j + r] for r in range(REP)], axis=1)
        acc_ref[:, j * BQ:(j + 1) * BQ] += lax.dot_general(wot, o2, _NT, preferred_element_type=F32)

    qs, outs = {}, []

    def fill(pos):
        for j in range(NB):
            if QP_POS[j] == pos:
                q2 = qproj(j)
                for r in range(REP):
                    qs[REP * j + r] = q2[:, r * DH:(r + 1) * DH]
        for j in range(NB):
            if OP_POS[j] == pos:
                oproj(j)

    NC = NB * REP
    fill(-1)
    s_head = None
    for ci in range(NC):
        lo = HEAD[ci - 1] if ci else 0
        s = qk(ci, lo, SK)
        if lo:
            s = jnp.concatenate([s_head, s], axis=1)
        fill(2 * ci)
        if HEAD[ci]:
            s_head = qk(ci + 1, 0, HEAD[ci])
        outs.append(softmax_pv(s, MODE[ci]))
        fill(2 * ci + 1)

    @pl.when(step + 2 < NG)
    def _():
        for d in group_copies(step + 2):
            d.start()

    @pl.when(step == 0)
    def _():
        wmb_cp().start()
        wg_cp().start()

    @pl.when(step == 1)
    def _():
        wu_cp().start()

    @pl.when(step == 2)
    def _():
        wd_cp().start()

    @pl.when(step == NG - 1)
    def _epilogue():
        @pl.when(step > 0)
        def _ln2_sums():
            for sl in range(NSL):
                cols = slice(sl * LANES, (sl + 1) * LANES)
                piv = st_ref[0, sl:sl + 1, :]
                for r0 in range(0, D, LANES):
                    r1 = min(r0 + LANES, D)
                    x2 = xt_ref[r0:r1, cols].astype(F32) + modc_ref[r0:r1, :] * acc_ref[r0:r1, cols]
                    acc_ref[r0:r1, cols] = x2
                    xb = x2.astype(BF16)
                    xb_ref[r0 // 2:r1 // 2, cols] = pltpu.bitcast(xb, U32)
                    d = x2 - piv
                    lhs = lhs_ref[:, r0:r1]
                    t1 = jnp.dot(lhs, xb, preferred_element_type=F32)[0:8, :]
                    t2 = jnp.dot(lhs, (d * d).astype(BF16), preferred_element_type=F32)[0:8, :]
                    s1, s2 = (t1, t2) if r0 == 0 else (s1 + t1, s2 + t2)
                for n in range(3):
                    st_ref[1 + n, sl:sl + 1, :] = s1[n:n + 1, :]
                st_ref[4, sl:sl + 1, :] = s2[0:1, :]

        mean = st_ref[1] * (1.0 / D)
        md = mean - st_ref[0]
        mb, sd = _ln_rows(mean, jnp.maximum(st_ref[4] * (1.0 / D) - md * md, 0.0))
        rs = 1.0 / sd
        st_ref[5] = rs
        st_ref[6] = mb * rs
        r = (st_ref[2] + st_ref[3] - mb * rc_ref[0:1, :]) * rs + rc_ref[1:2, :]

        lane16 = lax.broadcasted_iota(jnp.int32, (16, LANES), 1)
        never = lane16 > step + LANES

        def after_out_stores():
            dyn0 = pl.multiple_of((step - (NG - 1)) * LANES, LANES)
            return out_ref[0:16, pl.ds(dyn0, LANES)]

        def out_unit(n):
            w = OUW * LANES
            cols = slice(n * w, (n + 1) * w)
            rs, mrs = (jnp.concatenate([st_ref[k, n * OUW + u:n * OUW + u + 1, :]
                                        for u in range(OUW)], axis=1) for k in (5, 6))
            for r0 in range(0, D, OPR):
                x2 = acc_ref[r0:r0 + OPR, cols]
                o = x2 + ((x2 * rs - mrs) * _tile(modc_ref[D + r0:D + r0 + OPR, :], OUW)
                          + _tile(modc_ref[MA + r0:MA + r0 + OPR, :], OUW))
                out_ref[r0:r0 + OPR, cols] = o.astype(BF16)
            return after_out_stores().astype(F32)

        r = _rb(r) + 0.0
        bits = pltpu.bitcast(r, jnp.int32)
        mono = bits ^ ((bits >> 31) & jnp.int32(0x7FFFFFFF))
        tok = (lax.broadcasted_iota(jnp.int32, (NSL, LANES), 0) * LANES
               + lax.broadcasted_iota(jnp.int32, (NSL, LANES), 1))
        keyi = (((mono >> 16) + 32768) * S + (S - 1 - tok)) + jnp.int32(1 << 29)
        key = pltpu.bitcast(keyi, F32)

        row16 = lax.broadcasted_iota(jnp.int32, (16, LANES), 0)
        rowc = lax.broadcasted_iota(jnp.int32, (16, 1), 0)
        sel_slab, sel_off = [], []
        tie, nunit = None, 0
        xsel = jnp.zeros((16, D), F32)
        mbsel = jnp.zeros((16, 1), F32)
        rssel = jnp.zeros((16, 1), F32)
        ksel = jnp.zeros((16, 1), F32)
        for t in range(TOPC):
            kmax = jnp.max(jnp.max(key, axis=0, keepdims=True), axis=1, keepdims=True)
            hit = key == kmax
            key = jnp.where(hit, 0.0, key)
            pick = lambda z: jnp.sum(jnp.sum(jnp.where(hit, z, 0.0), axis=0, keepdims=True),
                                     axis=1, keepdims=True)
            mbsel = jnp.where(rowc == t, pick(mb), mbsel)
            rssel = jnp.where(rowc == t, pick(rs), rssel)
            for _ in range(TK_TIES.count(t)):
                tie = out_unit(nunit)
                nunit += 1
                key = jnp.where(never, tie, key)
            ksel = jnp.where(rowc == t, kmax, ksel)
            ki = pltpu.bitcast(kmax, jnp.int32)[0, 0]
            idx = (S - 1) - (ki & (S - 1))
            slab = idx >> 7
            off = idx & (LANES - 1)
            onehot = jnp.where((row16 == t) & (lane16 == off), 1.0, 0.0).astype(BF16)
            dslab = xb_ref[:, pl.ds(pl.multiple_of(slab * LANES, LANES), LANES)]
            xsel = xsel + lax.dot_general(onehot, pltpu.bitcast(dslab, BF16), _NT,
                                          preferred_element_type=F32)
            sel_slab.append(slab)
            sel_off.append(off)
        nsel = _rb(_rb(xsel - mbsel) * rssel)
        hsel = _rb(_rb(nsel * mrow_ref[1, 0:1, :]) + mrow_ref[0, 0:1, :])
        hi = ((pltpu.bitcast(ksel, jnp.int32) - jnp.int32(1 << 29)) // S - 32768) << 16
        rbits = hi ^ ((hi >> 31) & jnp.int32(0x7FFF0000))
        gate = _rb(_sigmoid(jnp.where(rowc < TOPC, pltpu.bitcast(rbits, F32), 0.0)))

        def out_copy(sl, r0, nr):
            c0 = pl.multiple_of(sl * LANES, LANES)
            return cp(out_ref.at[r0:r0 + nr, pl.ds(c0, LANES)],
                      out_hbm.at[r0:r0 + nr, pl.ds(c0, LANES)], S_O)

        fresh = []
        seen = jnp.int32(0)
        for t in range(TOPC):
            fresh.append(((seen >> sel_slab[t]) & 1) == 0)
            seen = seen | (1 << sel_slab[t])
        plain = [((seen >> sl) & 1) == 0 for sl in range(NSL)]

        for n in range(nunit, NSL // OUW):
            tie = out_unit(n)
        for sl in range(NSL):
            pl.when(plain[sl])(lambda sl=sl: out_copy(sl, 0, D).start())

        h0 = jnp.where(never, tie, hsel[:, 0:LANES])
        hs = jnp.concatenate([h0, hsel[:, LANES:]], axis=1).astype(BF16)
        gpre = _rb(jnp.dot(hs, wg_ref[...], preferred_element_type=F32))
        u = _rb(jnp.dot(hs, wu_ref[...], preferred_element_type=F32))
        a = (_rb(gpre * _sigmoid(gpre)) * u).astype(BF16)

        pieces = PIECES

        gb = mrow_ref[2, 0:1, :]

        def down(r0, nr, tied):
            lhs = a
            if tied:
                a0 = jnp.where(never[0:8, :], pltpu.bitcast(after_out_stores(), U32),
                               pltpu.bitcast(a[:, TIEC:TIEC + LANES], U32))
                lhs = jnp.concatenate(([a[:, 0:TIEC]] if TIEC else []) + [pltpu.bitcast(a0, BF16)] + ([a[:, TIEC + LANES:]] if TIEC + LANES < FF else []), axis=1)
            y = lax.dot_general(lhs, wdt_ref[r0:r0 + nr, :], _NT, preferred_element_type=F32)
            c = slice(r0, r0 + nr)
            return xsel[:, c] + gb[:, c] * (hsel[:, c] + y * gate)

        def patch(r0, nr, new):
            lane = lax.broadcasted_iota(jnp.int32, (nr // 2, LANES), 1)
            for t in range(TOPC):
                cols = pl.ds(pl.multiple_of(sel_slab[t] * LANES, LANES), LANES)
                old = pltpu.bitcast(out_ref[r0:r0 + nr, cols], U32)
                upd = pltpu.bitcast(_as_cols(new[t:t + 1, :]), U32)
                out_ref[r0:r0 + nr, cols] = pltpu.bitcast(jnp.where(lane == sel_off[t], upd, old), BF16)
            for t in range(TOPC):
                pl.when(fresh[t])(lambda t=t: out_copy(sel_slab[t], r0, nr).start())

        if DIST == 1:
            for n in range(len(pieces)):
                patch(*pieces[n], down(*pieces[n], n > 0))
        else:
            yts = [down(*pieces[0], False)]
            for n in range(len(pieces)):
                if n + 1 < len(pieces):
                    yts.append(down(*pieces[n + 1], n > 0))
                patch(*pieces[n], yts[n])

        cp(out_ref, out_hbm, S_O).wait()


@jax.jit
def pallas_adaLN_cond__gqa_block_cached__moe_arch_mod__prompt_kernel(
    A_x: jax.Array,
    A_k_cache: jax.Array,
    A_v_cache: jax.Array,
    A_wq: jax.Array,
    A_wo: jax.Array,
    B_x: jax.Array,
    B_w_r: jax.Array,
    B_w_gate: jax.Array,
    B_w_up: jax.Array,
    B_w_down: jax.Array,
    c: jax.Array,
    w_mod: jax.Array,
):
    del B_x
    B, S, D = A_x.shape
    assert B == 1
    NG, SK = A_k_cache.shape[1], A_k_cache.shape[2]
    REP = HQ // NG
    FF = B_w_gate.shape[1]
    GW = REP * DH

    xt = A_x.reshape(S, D).T
    wot = A_wo.T
    wdt = B_w_down.T
    k = A_k_cache.reshape(NG, SK, DH)
    v = A_v_cache.reshape(NG, SK, DH)

    hbm = pl.BlockSpec(memory_space=pl.ANY)
    out_t = pl.pallas_call(
        functools.partial(_kernel, S=S, SK=SK, D=D, FF=FF, NG=NG, REP=REP),
        grid=(NG,),
        in_specs=[hbm] * 11,
        out_specs=hbm,
        out_shape=jax.ShapeDtypeStruct((D, S), BF16),
        scratch_shapes=[
            pltpu.VMEM((D, S), BF16),
            pltpu.VMEM((2, SK, DH), BF16),
            pltpu.VMEM((2, SK, DH), BF16),
            pltpu.VMEM((2, D, GW), BF16),
            pltpu.VMEM((2, D, GW), BF16),
            pltpu.VMEM((D,), BF16),
            pltpu.VMEM((1, D), BF16),
            pltpu.VMEM((D, 6 * D), BF16),
            pltpu.VMEM((D, FF), BF16),
            pltpu.VMEM((D, FF), BF16),
            pltpu.VMEM((D, FF), BF16),
            pltpu.VMEM((D, S), BF16),
            pltpu.VMEM((3 * D, LANES), F32),
            pltpu.VMEM((3, 8, D), F32),
            pltpu.VMEM((16, D), BF16),
            pltpu.VMEM((8, LANES), F32),
            pltpu.VMEM((S // 2, D), U32),
            pltpu.VMEM((D, S), F32),
            pltpu.VMEM((D // 2, S), U32),
            pltpu.VMEM((7, S // LANES, LANES), F32),
            pltpu.SemaphoreType.DMA((N_SEMS,)),
        ],
        compiler_params=pltpu.CompilerParams(
            dimension_semantics=("arbitrary",),
            vmem_limit_bytes=100 * 1024 * 1024,
            disable_bounds_checks=True,
        ),
    )(xt, k, v, A_wq, wot, B_w_r, c, w_mod, B_w_gate, B_w_up, wdt)
    return out_t.T.reshape(B, S, D)
```

```python
import functools
import math

import jax
import jax.numpy as jnp
from jax import lax
import jax.experimental.pallas as pl
import jax.experimental.pallas.tpu as pltpu

F32 = jnp.float32
BF16 = jnp.bfloat16
U32 = jnp.uint32

HQ = 32
DH = 128
TOPC = 8
LN_EPS = 1e-5
BQ = 256
LANES = 128
HEAD = [768, 512, 512, 1024, 768, 512, 512, 512, 768, 768, 512, 512, 512, 512, 512, 0]
MODE = [2, 1, 2, 2, 0, 0, 0, 0, 0, 1, 0, 0, 0, 2, 0, 1]
QP_POS = [-1, -1, -1, -1, -1, 3, -1, -1]
OP_POS = [11, 15, 21, 23, 30, 31, 31, 31]
XCH = 4
DIST = 2
TIEC = 2048
PIECES = [(0, 128), (128, 128), (256, 128), (384, 128), (512, 64)]
OUW = 2
TK_TIES = [0, 2, 3, 5, 6]
OPR = 16
WT_W = 384
WT_R = 256
WT_TIE = 0
MOD_STEP = 4

_NT = (((1,), (1,)), ((), ()))

S_C, S_WMA, S_WMB, S_WR, S_WG, S_WU, S_WD = range(7)
S_X = 7
S_G = S_X + XCH
S_O = S_G + 2
N_SEMS = S_O + 1


def _rb(x):
    return x.astype(BF16).astype(F32)


def _sigmoid(x):
    return 1.0 / (1.0 + jnp.exp(-x))


def _ln_rows(mean, var):
    eps = _rb(jnp.full((1, 1), LN_EPS, F32))
    return _rb(mean), _rb(jnp.sqrt(_rb(_rb(var) + eps)))


def _tile(col, n):
    return jnp.concatenate([col] * n, axis=1)


def _as_cols(row):
    return jnp.broadcast_to(row, (LANES, row.shape[1])).astype(BF16).T


def _kernel(xt_hbm, k_hbm, v_hbm, wq_hbm, wot_hbm, wr_hbm, c_hbm, wmod_hbm,
            wg_hbm, wu_hbm, wdt_hbm,
            out_hbm,
            xt_ref, k_buf, v_buf, wq_buf, wot_buf, wr_ref, c_ref, wmod_ref,
            wg_ref, wu_ref, wdt_ref, wd_ref, out_ref,
            modc_ref, mrow_ref, lhs_ref, rc_ref, h_ref, acc_ref, xb_ref, st_ref,
            sems,
            *, S, SK, D, FF, NG, REP):
    step = pl.program_id(0)
    qscale = (DH ** -0.5) * math.log2(math.e)
    NB = S // BQ
    GW = REP * DH
    TCH = S // XCH
    MA = 2 * D
    NSL = S // LANES

    def cp(src, dst, sem):
        return pltpu.make_async_copy(src, dst, sems.at[sem])

    def x_copy(i):
        cols = pl.ds(pl.multiple_of(i * TCH, TCH), TCH)
        return cp(xt_hbm.at[:, cols], xt_ref.at[:, cols], S_X + i)

    def group_copies(grp):
        slot = grp % 2
        cols = pl.ds(pl.multiple_of(grp * GW, GW), GW)
        return (cp(wq_hbm.at[:, cols], wq_buf.at[slot], S_G + slot),
                cp(k_hbm.at[grp], k_buf.at[slot], S_G + slot),
                cp(v_hbm.at[grp], v_buf.at[slot], S_G + slot),
                cp(wot_hbm.at[:, cols], wot_buf.at[slot], S_G + slot))

    c_cp = lambda: cp(c_hbm, c_ref, S_C)
    wma_cp = lambda: cp(wmod_hbm.at[:, 0:MA], wmod_ref.at[:, 0:MA], S_WMA)
    wmb_cp = lambda: cp(wmod_hbm.at[:, MA:6 * D], wmod_ref.at[:, MA:6 * D], S_WMB)
    wr_cp = lambda: cp(wr_hbm, wr_ref, S_WR)
    wg_cp = lambda: cp(wg_hbm, wg_ref, S_WG)
    wu_cp = lambda: cp(wu_hbm, wu_ref, S_WU)
    wd_cp = lambda: cp(wdt_hbm, wdt_ref.at[:, 0:FF], S_WD)

    def modcol(i):
        return modc_ref[i * D:(i + 1) * D, :]

    def modulation(lo, hi):
        c = c_ref[...].astype(F32)
        sc8 = jnp.broadcast_to((c * _sigmoid(c)).astype(BF16), (8, D))
        mods = []
        for a in range(lo, hi, MA):
            mod = _rb(jnp.dot(sc8, wmod_ref[:, a:a + MA], preferred_element_type=F32))
            lane = lax.broadcasted_iota(jnp.int32, mod.shape, 1) + a
            is_scale = ((lane >= D) & (lane < 2 * D)) | ((lane >= 4 * D) & (lane < 5 * D))
            mods.append(jnp.where(is_scale, _rb(1.0 + mod), mod))
        return mods

    @pl.when(step == 0)
    def _prologue():
        wma_cp().start()
        c_cp().start()
        for i in range(XCH):
            x_copy(i).start()
        for d in group_copies(0) + group_copies(1):
            d.start()
        wr_cp().start()
        acc_ref[...] = jnp.zeros((D, S), F32)
        wma_cp().wait()
        c_cp().wait()
        modc_ref[0:MA, :] = _as_cols(modulation(0, MA)[0][0:1, :]).astype(F32)

        def ln1(i, carry):
            x_copy(i).wait()
            x = xt_ref[:, pl.ds(pl.multiple_of(i * TCH, TCH), TCH)].astype(F32)
            piv = x[0:1, :]
            d = x - piv
            md = jnp.mean(d, axis=0, keepdims=True)
            var = jnp.maximum(jnp.mean(d * d, axis=0, keepdims=True) - md * md, 0.0)
            mb, sd = _ln_rows(piv + md, var)
            rs = 1.0 / sd
            n = TCH // LANES
            for u in range(n):
                st_ref[0, pl.ds(n * i + u, 1), :] = mb[:, u * LANES:(u + 1) * LANES]
            ht = (x * rs - mb * rs) * _tile(modcol(1), n) + _tile(modcol(0), n)
            h_ref[pl.ds(pl.multiple_of(i * (TCH // 2), TCH // 2), TCH // 2), :] = pltpu.bitcast(
                ht.astype(BF16).T, U32)
            return carry
        lax.fori_loop(0, XCH, ln1, 0)

    @pl.when(step == MOD_STEP)
    def _late_modulation():
        wr_cp().wait()
        wmb_cp().wait()
        wg_cp().wait()
        wu_cp().wait()
        wd_cp().wait()
        m23, m45 = modulation(MA, 6 * D)
        sb, cb, gb = m23[:, D:MA], m45[:, 0:D], m45[:, D:MA]
        mrow_ref[0] = sb
        mrow_ref[1] = cb
        mrow_ref[2] = gb
        c23 = _as_cols(m23[0:1, :]).astype(F32)
        c45 = _as_cols(m45[0:1, :]).astype(F32)
        modc_ref[0:D, :] = c23[0:D]
        modc_ref[D:MA, :] = c45[D:MA] * c45[0:D]
        modc_ref[MA:3 * D, :] = c45[D:MA] * c23[D:MA]
        wr = wr_ref[...].astype(F32).reshape(1, D)
        wc = wr * cb[0:1, :]
        whi = _rb(wc)
        wlo = _rb(wc - whi)
        row = lax.broadcasted_iota(jnp.int32, (16, D), 0)
        lhs_ref[...] = jnp.where(row == 0, 1.0, jnp.where(row == 1, whi, jnp.where(
            row == 2, wlo, 0.0))).astype(BF16)
        rc_ref[0:1, :] = jnp.broadcast_to(jnp.sum(whi + wlo, axis=1, keepdims=True), (1, LANES))
        rc_ref[1:2, :] = jnp.broadcast_to(jnp.sum(wr * sb[0:1, :], axis=1, keepdims=True), (1, LANES))

    for d in group_copies(step):
        d.wait()

    slot = step % 2
    k = k_buf[slot]
    v = v_buf[slot]
    wq = wq_buf[slot]
    wot = wot_buf[slot]

    def qproj(j):
        hb = pltpu.bitcast(h_ref[j * (BQ // 2):(j + 1) * (BQ // 2), :], BF16)
        q2 = jnp.dot(hb, wq, preferred_element_type=F32)
        return (q2 * qscale).astype(BF16)

    def qk(ci, lo, hi):
        return lax.dot_general(qs[ci], k[lo:hi], _NT, preferred_element_type=F32)

    def softmax_pv(s, mode):
        m = jnp.max(s, axis=1, keepdims=True)
        p = jnp.exp2(s - m)
        parts = [p[:, i * LANES:(i + 1) * LANES] for i in range(SK // LANES)]
        if mode == 2:
            lp = None
            for c in range(0, len(parts), 4):
                t = (parts[c] + parts[c + 1]) + (parts[c + 2] + parts[c + 3])
                lp = t if lp is None else lp + t
                parts[c + 3] = jnp.where(lp < 0.0, lp, parts[c + 3])
            p = jnp.concatenate(parts, axis=1)
        o = jnp.dot(p.astype(BF16), v, preferred_element_type=F32)
        if mode == 0:
            l = jnp.sum(p, axis=1, keepdims=True)
        elif mode == 1:
            lp = functools.reduce(lambda x, y: x + y, parts)
            l = jnp.sum(jnp.where(lp < 0.0, o, lp), axis=1, keepdims=True)
        else:
            l = jnp.sum(lp, axis=1, keepdims=True)
        rl = pl.reciprocal(l, approx=True)
        rl = rl * (2.0 - l * rl)
        return (o * rl).astype(BF16)

    def oproj(j):
        o2 = jnp.concatenate([outs[REP * j + r] for r in range(REP)], axis=1)
        acc_ref[:, j * BQ:(j + 1) * BQ] += lax.dot_general(wot, o2, _NT, preferred_element_type=F32)

    qs, outs = {}, []

    def fill(pos):
        for j in range(NB):
            if QP_POS[j] == pos:
                q2 = qproj(j)
                for r in range(REP):
                    qs[REP * j + r] = q2[:, r * DH:(r + 1) * DH]
        for j in range(NB):
            if OP_POS[j] == pos:
                oproj(j)

    NC = NB * REP
    assert (NG - MOD_STEP) * WT_W == FF
    wc0 = jnp.where(step >= MOD_STEP, (step - MOD_STEP) * WT_W, FF)
    never8 = lax.broadcasted_iota(jnp.int32, (8, LANES), 1) > step + LANES
    wtie = None
    for t0 in range(0, WT_W, LANES):
        for r0 in range(0, D, WT_R):
            r1 = min(r0 + WT_R, D)
            blk = pltpu.bitcast(wdt_ref[r0:r1, pl.ds(pl.multiple_of(wc0 + t0, LANES), LANES)], U32)
            if wtie is not None:
                blk = jnp.concatenate([jnp.where(never8, wtie, blk[0:8]), blk[8:]], axis=0)
            tb = pltpu.bitcast(pltpu.bitcast(blk, BF16).T, U32)
            wd_ref[pl.ds(pl.multiple_of((wc0 + t0) // 2, LANES // 2), LANES // 2), r0:r1] = tb
            wtie = wd_ref[pl.ds(pl.multiple_of(wc0 // 2, LANES // 2), 8), 0:LANES]
    fill(-1)
    qt = pltpu.bitcast(qs[WT_TIE], U32)
    qs[WT_TIE] = pltpu.bitcast(
        jnp.concatenate([jnp.where(never8, wtie, qt[0:8]), qt[8:]], axis=0), BF16)
    s_head = None
    for ci in range(NC):
        lo = HEAD[ci - 1] if ci else 0
        s = qk(ci, lo, SK)
        if lo:
            s = jnp.concatenate([s_head, s], axis=1)
        fill(2 * ci)
        if HEAD[ci]:
            s_head = qk(ci + 1, 0, HEAD[ci])
        outs.append(softmax_pv(s, MODE[ci]))
        fill(2 * ci + 1)

    @pl.when(step + 2 < NG)
    def _():
        for d in group_copies(step + 2):
            d.start()

    @pl.when(step == 0)
    def _():
        wmb_cp().start()
        wg_cp().start()

    @pl.when(step == 1)
    def _():
        wu_cp().start()

    @pl.when(step == 2)
    def _():
        wd_cp().start()

    @pl.when(step == NG - 1)
    def _epilogue():
        @pl.when(step > 0)
        def _ln2_sums():
            for sl in range(NSL):
                cols = slice(sl * LANES, (sl + 1) * LANES)
                piv = st_ref[0, sl:sl + 1, :]
                for r0 in range(0, D, LANES):
                    r1 = min(r0 + LANES, D)
                    x2 = xt_ref[r0:r1, cols].astype(F32) + modc_ref[r0:r1, :] * acc_ref[r0:r1, cols]
                    acc_ref[r0:r1, cols] = x2
                    xb = x2.astype(BF16)
                    xb_ref[r0 // 2:r1 // 2, cols] = pltpu.bitcast(xb, U32)
                    d = x2 - piv
                    lhs = lhs_ref[:, r0:r1]
                    t1 = jnp.dot(lhs, xb, preferred_element_type=F32)[0:8, :]
                    t2 = jnp.dot(lhs, (d * d).astype(BF16), preferred_element_type=F32)[0:8, :]
                    s1, s2 = (t1, t2) if r0 == 0 else (s1 + t1, s2 + t2)
                for n in range(3):
                    st_ref[1 + n, sl:sl + 1, :] = s1[n:n + 1, :]
                st_ref[4, sl:sl + 1, :] = s2[0:1, :]

        mean = st_ref[1] * (1.0 / D)
        md = mean - st_ref[0]
        mb, sd = _ln_rows(mean, jnp.maximum(st_ref[4] * (1.0 / D) - md * md, 0.0))
        rs = 1.0 / sd
        st_ref[5] = rs
        st_ref[6] = mb * rs
        r = (st_ref[2] + st_ref[3] - mb * rc_ref[0:1, :]) * rs + rc_ref[1:2, :]

        lane16 = lax.broadcasted_iota(jnp.int32, (16, LANES), 1)
        never = lane16 > step + LANES

        def after_out_stores():
            dyn0 = pl.multiple_of((step - (NG - 1)) * LANES, LANES)
            return out_ref[0:16, pl.ds(dyn0, LANES)]

        def out_unit(n):
            w = OUW * LANES
            cols = slice(n * w, (n + 1) * w)
            rs, mrs = (jnp.concatenate([st_ref[k, n * OUW + u:n * OUW + u + 1, :]
                                        for u in range(OUW)], axis=1) for k in (5, 6))
            for r0 in range(0, D, OPR):
                x2 = acc_ref[r0:r0 + OPR, cols]
                o = x2 + ((x2 * rs - mrs) * _tile(modc_ref[D + r0:D + r0 + OPR, :], OUW)
                          + _tile(modc_ref[MA + r0:MA + r0 + OPR, :], OUW))
                out_ref[r0:r0 + OPR, cols] = o.astype(BF16)
            return after_out_stores().astype(F32)

        r = _rb(r) + 0.0
        bits = pltpu.bitcast(r, jnp.int32)
        mono = bits ^ ((bits >> 31) & jnp.int32(0x7FFFFFFF))
        tok = (lax.broadcasted_iota(jnp.int32, (NSL, LANES), 0) * LANES
               + lax.broadcasted_iota(jnp.int32, (NSL, LANES), 1))
        keyi = (((mono >> 16) + 32768) * S + (S - 1 - tok)) + jnp.int32(1 << 29)
        key = pltpu.bitcast(keyi, F32)

        row16 = lax.broadcasted_iota(jnp.int32, (16, LANES), 0)
        rowc = lax.broadcasted_iota(jnp.int32, (16, 1), 0)
        sel_slab, sel_off = [], []
        tie, nunit = None, 0
        xsel = jnp.zeros((16, D), F32)
        mbsel = jnp.zeros((16, 1), F32)
        rssel = jnp.zeros((16, 1), F32)
        ksel = jnp.zeros((16, 1), F32)
        for t in range(TOPC):
            kmax = jnp.max(jnp.max(key, axis=0, keepdims=True), axis=1, keepdims=True)
            hit = key == kmax
            key = jnp.where(hit, 0.0, key)
            pick = lambda z: jnp.sum(jnp.sum(jnp.where(hit, z, 0.0), axis=0, keepdims=True),
                                     axis=1, keepdims=True)
            mbsel = jnp.where(rowc == t, pick(mb), mbsel)
            rssel = jnp.where(rowc == t, pick(rs), rssel)
            for _ in range(TK_TIES.count(t)):
                tie = out_unit(nunit)
                nunit += 1
                key = jnp.where(never, tie, key)
            ksel = jnp.where(rowc == t, kmax, ksel)
            ki = pltpu.bitcast(kmax, jnp.int32)[0, 0]
            idx = (S - 1) - (ki & (S - 1))
            slab = idx >> 7
            off = idx & (LANES - 1)
            onehot = jnp.where((row16 == t) & (lane16 == off), 1.0, 0.0).astype(BF16)
            dslab = xb_ref[:, pl.ds(pl.multiple_of(slab * LANES, LANES), LANES)]
            xsel = xsel + lax.dot_general(onehot, pltpu.bitcast(dslab, BF16), _NT,
                                          preferred_element_type=F32)
            sel_slab.append(slab)
            sel_off.append(off)
        nsel = _rb(_rb(xsel - mbsel) * rssel)
        hsel = _rb(_rb(nsel * mrow_ref[1, 0:1, :]) + mrow_ref[0, 0:1, :])
        hi = ((pltpu.bitcast(ksel, jnp.int32) - jnp.int32(1 << 29)) // S - 32768) << 16
        rbits = hi ^ ((hi >> 31) & jnp.int32(0x7FFF0000))
        gate = _rb(_sigmoid(jnp.where(rowc < TOPC, pltpu.bitcast(rbits, F32), 0.0)))

        def out_copy(sl, r0, nr):
            c0 = pl.multiple_of(sl * LANES, LANES)
            return cp(out_ref.at[r0:r0 + nr, pl.ds(c0, LANES)],
                      out_hbm.at[r0:r0 + nr, pl.ds(c0, LANES)], S_O)

        fresh = []
        seen = jnp.int32(0)
        for t in range(TOPC):
            fresh.append(((seen >> sel_slab[t]) & 1) == 0)
            seen = seen | (1 << sel_slab[t])
        plain = [((seen >> sl) & 1) == 0 for sl in range(NSL)]

        for n in range(nunit, NSL // OUW):
            tie = out_unit(n)
        for sl in range(NSL):
            pl.when(plain[sl])(lambda sl=sl: out_copy(sl, 0, D).start())

        h0 = jnp.where(never, tie, hsel[:, 0:LANES])
        hs = jnp.concatenate([h0, hsel[:, LANES:]], axis=1).astype(BF16)
        gpre = _rb(jnp.dot(hs, wg_ref[...], preferred_element_type=F32))
        u = _rb(jnp.dot(hs, wu_ref[...], preferred_element_type=F32))
        a = (_rb(gpre * _sigmoid(gpre)) * u).astype(BF16)

        pieces = PIECES

        gb = mrow_ref[2, 0:1, :]

        def down(r0, nr, tied):
            lhs = a
            if tied:
                a0 = jnp.where(never[0:8, :], pltpu.bitcast(after_out_stores(), U32),
                               pltpu.bitcast(a[:, TIEC:TIEC + LANES], U32))
                lhs = jnp.concatenate(([a[:, 0:TIEC]] if TIEC else []) + [pltpu.bitcast(a0, BF16)] + ([a[:, TIEC + LANES:]] if TIEC + LANES < FF else []), axis=1)
            y = jnp.dot(lhs, pltpu.bitcast(wd_ref[0:FF // 2, r0:r0 + nr], BF16),
                        preferred_element_type=F32)
            c = slice(r0, r0 + nr)
            return xsel[:, c] + gb[:, c] * (hsel[:, c] + y * gate)

        def patch(r0, nr, new):
            lane = lax.broadcasted_iota(jnp.int32, (nr // 2, LANES), 1)
            for t in range(TOPC):
                cols = pl.ds(pl.multiple_of(sel_slab[t] * LANES, LANES), LANES)
                old = pltpu.bitcast(out_ref[r0:r0 + nr, cols], U32)
                upd = pltpu.bitcast(_as_cols(new[t:t + 1, :]), U32)
                out_ref[r0:r0 + nr, cols] = pltpu.bitcast(jnp.where(lane == sel_off[t], upd, old), BF16)
            for t in range(TOPC):
                pl.when(fresh[t])(lambda t=t: out_copy(sel_slab[t], r0, nr).start())

        if DIST == 1:
            for n in range(len(pieces)):
                patch(*pieces[n], down(*pieces[n], n > 0))
        else:
            yts = [down(*pieces[0], False)]
            for n in range(len(pieces)):
                if n + 1 < len(pieces):
                    yts.append(down(*pieces[n + 1], n > 0))
                patch(*pieces[n], yts[n])

        cp(out_ref, out_hbm, S_O).wait()


@jax.jit
def pallas_adaLN_cond__gqa_block_cached__moe_arch_mod__prompt_kernel(
    A_x: jax.Array,
    A_k_cache: jax.Array,
    A_v_cache: jax.Array,
    A_wq: jax.Array,
    A_wo: jax.Array,
    B_x: jax.Array,
    B_w_r: jax.Array,
    B_w_gate: jax.Array,
    B_w_up: jax.Array,
    B_w_down: jax.Array,
    c: jax.Array,
    w_mod: jax.Array,
):
    del B_x
    B, S, D = A_x.shape
    assert B == 1
    NG, SK = A_k_cache.shape[1], A_k_cache.shape[2]
    REP = HQ // NG
    FF = B_w_gate.shape[1]
    GW = REP * DH

    xt = A_x.reshape(S, D).T
    wot = A_wo.T
    wdt = B_w_down.T
    k = A_k_cache.reshape(NG, SK, DH)
    v = A_v_cache.reshape(NG, SK, DH)

    hbm = pl.BlockSpec(memory_space=pl.ANY)
    out_t = pl.pallas_call(
        functools.partial(_kernel, S=S, SK=SK, D=D, FF=FF, NG=NG, REP=REP),
        grid=(NG,),
        in_specs=[hbm] * 11,
        out_specs=hbm,
        out_shape=jax.ShapeDtypeStruct((D, S), BF16),
        scratch_shapes=[
            pltpu.VMEM((D, S), BF16),
            pltpu.VMEM((2, SK, DH), BF16),
            pltpu.VMEM((2, SK, DH), BF16),
            pltpu.VMEM((2, D, GW), BF16),
            pltpu.VMEM((2, D, GW), BF16),
            pltpu.VMEM((D,), BF16),
            pltpu.VMEM((1, D), BF16),
            pltpu.VMEM((D, 6 * D), BF16),
            pltpu.VMEM((D, FF), BF16),
            pltpu.VMEM((D, FF), BF16),
            pltpu.VMEM((D, FF + WT_W), BF16),
            pltpu.VMEM(((FF + WT_W) // 2, D), U32),
            pltpu.VMEM((D, S), BF16),
            pltpu.VMEM((3 * D, LANES), F32),
            pltpu.VMEM((3, 8, D), F32),
            pltpu.VMEM((16, D), BF16),
            pltpu.VMEM((8, LANES), F32),
            pltpu.VMEM((S // 2, D), U32),
            pltpu.VMEM((D, S), F32),
            pltpu.VMEM((D // 2, S), U32),
            pltpu.VMEM((7, S // LANES, LANES), F32),
            pltpu.SemaphoreType.DMA((N_SEMS,)),
        ],
        compiler_params=pltpu.CompilerParams(
            dimension_semantics=("arbitrary",),
            vmem_limit_bytes=100 * 1024 * 1024,
            disable_bounds_checks=True,
        ),
    )(xt, k, v, A_wq, wot, B_w_r, c, w_mod, B_w_gate, B_w_up, wdt)
    return out_t.T.reshape(B, S, D)
```

```python
import functools
import math

import jax
import jax.numpy as jnp
from jax import lax
import jax.experimental.pallas as pl
import jax.experimental.pallas.tpu as pltpu

F32 = jnp.float32
BF16 = jnp.bfloat16
U32 = jnp.uint32

HQ = 32
DH = 128
TOPC = 8
LN_EPS = 1e-5
BQ = 256
LANES = 128
HEAD = [768, 512, 512, 1024, 768, 512, 512, 512, 768, 768, 512, 512, 512, 512, 512, 0]
MODE = [2, 1, 2, 2, 0, 0, 0, 0, 0, 1, 0, 0, 0, 2, 0, 1]
QP_POS = [-1, -1, -1, -1, -1, 3, -1, -1]
OP_POS = [11, 15, 21, 23, 30, 31, 31, 31]
XCH = 4
DIST = 2
TIEC = 2048
PIECES = [(0, 128), (128, 128), (256, 128), (384, 128), (512, 64)]
OUW = 2
TK_TIES = [0, 2, 3, 5, 6]
OPR = 16
MT_W = 384
MT_R = 8
WT_W = 384
WT_R = 256
WT_TIE = 0
MOD_STEP = 4

_NT = (((1,), (1,)), ((), ()))

S_C, S_WMA, S_WMB, S_WR, S_WG, S_WU, S_WD = range(7)
S_X = 7
S_G = S_X + XCH
S_O = S_G + 2
N_SEMS = S_O + 1


def _rb(x):
    return x.astype(BF16).astype(F32)


def _sigmoid(x):
    return 1.0 / (1.0 + jnp.exp(-x))


def _ln_rows(mean, var):
    eps = _rb(jnp.full((1, 1), LN_EPS, F32))
    return _rb(mean), _rb(jnp.sqrt(_rb(_rb(var) + eps)))


def _tile(col, n):
    return jnp.concatenate([col] * n, axis=1)


def _as_cols(row):
    return jnp.broadcast_to(row, (LANES, row.shape[1])).astype(BF16).T


def _kernel(xt_hbm, k_hbm, v_hbm, wq_hbm, wot_hbm, wr_hbm, c_hbm, wmod_hbm,
            wg_hbm, wu_hbm, wdt_hbm,
            out_hbm,
            xt_ref, k_buf, v_buf, wq_buf, wot_buf, wr_ref, c_ref, wmod_ref,
            wg_ref, wu_ref, wdt_ref, wd_ref, out_ref,
            modc_ref, mrow_ref, scc_ref, fold_ref, mb_ref, lhs_ref, rc_ref, h_ref, acc_ref, xb_ref, st_ref,
            sems,
            *, S, SK, D, FF, NG, REP):
    step = pl.program_id(0)
    qscale = (DH ** -0.5) * math.log2(math.e)
    NB = S // BQ
    GW = REP * DH
    TCH = S // XCH
    MA = 2 * D
    NSL = S // LANES

    def cp(src, dst, sem):
        return pltpu.make_async_copy(src, dst, sems.at[sem])

    def x_copy(i):
        cols = pl.ds(pl.multiple_of(i * TCH, TCH), TCH)
        return cp(xt_hbm.at[:, cols], xt_ref.at[:, cols], S_X + i)

    def group_copies(grp):
        slot = grp % 2
        cols = pl.ds(pl.multiple_of(grp * GW, GW), GW)
        return (cp(wq_hbm.at[:, cols], wq_buf.at[slot], S_G + slot),
                cp(k_hbm.at[grp], k_buf.at[slot], S_G + slot),
                cp(v_hbm.at[grp], v_buf.at[slot], S_G + slot),
                cp(wot_hbm.at[:, cols], wot_buf.at[slot], S_G + slot))

    c_cp = lambda: cp(c_hbm, c_ref, S_C)
    wma_cp = lambda: cp(wmod_hbm.at[:, 0:MA], wmod_ref.at[:, 0:MA], S_WMA)
    wmb_cp = lambda: cp(wmod_hbm.at[:, MA:6 * D], wmod_ref.at[:, MA:6 * D], S_WMB)
    wr_cp = lambda: cp(wr_hbm, wr_ref, S_WR)
    wg_cp = lambda: cp(wg_hbm, wg_ref, S_WG)
    wu_cp = lambda: cp(wu_hbm, wu_ref, S_WU)
    wd_cp = lambda: cp(wdt_hbm, wdt_ref.at[:, 0:FF], S_WD)

    def modcol(i):
        return modc_ref[i * D:(i + 1) * D, :]

    def finish_mod(mod, col0):
        mod = _rb(mod)
        lane = lax.broadcasted_iota(jnp.int32, mod.shape, 1) + col0
        is_scale = ((lane >= D) & (lane < 2 * D)) | ((lane >= 4 * D) & (lane < 5 * D))
        return jnp.where(is_scale, _rb(1.0 + mod), mod)

    @pl.when(step == 0)
    def _prologue():
        wma_cp().start()
        c_cp().start()
        for i in range(XCH):
            x_copy(i).start()
        for d in group_copies(0) + group_copies(1):
            d.start()
        wr_cp().start()
        acc_ref[...] = jnp.zeros((D, S), F32)
        wma_cp().wait()
        c_cp().wait()
        c = c_ref[...].astype(F32)
        sc = _rb(c * _sigmoid(c))
        mod = jnp.dot(jnp.broadcast_to(sc, (8, D)).astype(BF16), wmod_ref[:, 0:MA],
                      preferred_element_type=F32)
        modc_ref[0:MA, :] = _as_cols(finish_mod(mod, 0)[0:1, :]).astype(F32)

        def ln1(i, carry):
            x_copy(i).wait()
            x = xt_ref[:, pl.ds(pl.multiple_of(i * TCH, TCH), TCH)].astype(F32)
            piv = x[0:1, :]
            d = x - piv
            md = jnp.mean(d, axis=0, keepdims=True)
            var = jnp.maximum(jnp.mean(d * d, axis=0, keepdims=True) - md * md, 0.0)
            mb, sd = _ln_rows(piv + md, var)
            rs = 1.0 / sd
            n = TCH // LANES
            for u in range(n):
                st_ref[0, pl.ds(n * i + u, 1), :] = mb[:, u * LANES:(u + 1) * LANES]
            ht = (x * rs - mb * rs) * _tile(modcol(1), n) + _tile(modcol(0), n)
            h_ref[pl.ds(pl.multiple_of(i * (TCH // 2), TCH // 2), TCH // 2), :] = pltpu.bitcast(
                ht.astype(BF16).T, U32)
            return carry
        lax.fori_loop(0, XCH, ln1, 0)
        scc_ref[...] = _as_cols(sc).astype(F32)

    @pl.when(step == MOD_STEP)
    def _():
        wr_cp().wait()
        wmb_cp().wait()
        wg_cp().wait()
        wu_cp().wait()
        wd_cp().wait()

    @pl.when(step == NG - 1)
    def _fold_modulation():
        sb, cb, gb = (mrow_ref[0:1, i * D:(i + 1) * D] for i in (3, 4, 5))
        for i, z in enumerate((sb, cb, gb)):
            mb_ref[i] = jnp.broadcast_to(z, (8, D))
        fold_ref[0:D, :] = modcol(5) * modcol(4)
        fold_ref[D:MA, :] = modcol(5) * modcol(3)
        wr = wr_ref[...].astype(F32).reshape(1, D)
        wc = wr * cb
        whi = _rb(wc)
        wlo = _rb(wc - whi)
        row = lax.broadcasted_iota(jnp.int32, (16, D), 0)
        lhs_ref[...] = jnp.where(row == 0, 1.0, jnp.where(row == 1, whi, jnp.where(
            row == 2, wlo, 0.0))).astype(BF16)
        rc_ref[0:1, :] = jnp.broadcast_to(jnp.sum(whi + wlo, axis=1, keepdims=True), (1, LANES))
        rc_ref[1:2, :] = jnp.broadcast_to(jnp.sum(wr * sb, axis=1, keepdims=True), (1, LANES))

    for d in group_copies(step):
        d.wait()

    slot = step % 2
    k = k_buf[slot]
    v = v_buf[slot]
    wq = wq_buf[slot]
    wot = wot_buf[slot]

    def qproj(j):
        hb = pltpu.bitcast(h_ref[j * (BQ // 2):(j + 1) * (BQ // 2), :], BF16)
        q2 = jnp.dot(hb, wq, preferred_element_type=F32)
        return (q2 * qscale).astype(BF16)

    def qk(ci, lo, hi):
        return lax.dot_general(qs[ci], k[lo:hi], _NT, preferred_element_type=F32)

    def softmax_pv(s, mode):
        m = jnp.max(s, axis=1, keepdims=True)
        p = jnp.exp2(s - m)
        parts = [p[:, i * LANES:(i + 1) * LANES] for i in range(SK // LANES)]
        if mode == 2:
            lp = None
            for c in range(0, len(parts), 4):
                t = (parts[c] + parts[c + 1]) + (parts[c + 2] + parts[c + 3])
                lp = t if lp is None else lp + t
                parts[c + 3] = jnp.where(lp < 0.0, lp, parts[c + 3])
            p = jnp.concatenate(parts, axis=1)
        o = jnp.dot(p.astype(BF16), v, preferred_element_type=F32)
        if mode == 0:
            l = jnp.sum(p, axis=1, keepdims=True)
        elif mode == 1:
            lp = functools.reduce(lambda x, y: x + y, parts)
            l = jnp.sum(jnp.where(lp < 0.0, o, lp), axis=1, keepdims=True)
        else:
            l = jnp.sum(lp, axis=1, keepdims=True)
        rl = pl.reciprocal(l, approx=True)
        rl = rl * (2.0 - l * rl)
        return (o * rl).astype(BF16)

    def oproj(j):
        o2 = jnp.concatenate([outs[REP * j + r] for r in range(REP)], axis=1)
        acc_ref[:, j * BQ:(j + 1) * BQ] += lax.dot_general(wot, o2, _NT, preferred_element_type=F32)

    qs, outs = {}, []

    def fill(pos):
        for j in range(NB):
            if QP_POS[j] == pos:
                q2 = qproj(j)
                for r in range(REP):
                    qs[REP * j + r] = q2[:, r * DH:(r + 1) * DH]
        for j in range(NB):
            if OP_POS[j] == pos:
                oproj(j)

    NC = NB * REP
    assert (NG - MOD_STEP) * WT_W == FF
    wc0 = jnp.where(step >= MOD_STEP, (step - MOD_STEP) * WT_W, FF)
    never8 = lax.broadcasted_iota(jnp.int32, (8, LANES), 1) > step + LANES
    wtie = None
    for t0 in range(0, WT_W, LANES):
        for r0 in range(0, D, WT_R):
            r1 = min(r0 + WT_R, D)
            blk = pltpu.bitcast(wdt_ref[r0:r1, pl.ds(pl.multiple_of(wc0 + t0, LANES), LANES)], U32)
            if wtie is not None:
                blk = jnp.concatenate([jnp.where(never8, wtie, blk[0:8]), blk[8:]], axis=0)
            tb = pltpu.bitcast(pltpu.bitcast(blk, BF16).T, U32)
            wd_ref[pl.ds(pl.multiple_of((wc0 + t0) // 2, LANES // 2), LANES // 2), r0:r1] = tb
            wtie = wd_ref[pl.ds(pl.multiple_of(wc0 // 2, LANES // 2), 8), 0:LANES]
    nms = 4 * D // MT_W
    assert nms * MT_W == 4 * D and MOD_STEP + nms < NG
    in_win = (step >= MOD_STEP) & (step < MOD_STEP + nms)
    mc0 = pl.multiple_of(jnp.where(in_win, MA + (step - MOD_STEP) * MT_W, 0), LANES)
    gate8 = pltpu.bitcast(wtie, F32)
    for r0 in range(0, D, MT_R):
        sc8 = scc_ref[r0:r0 + MT_R, :]
        sc8 = jnp.concatenate([jnp.where(never8, gate8, sc8[0:8])] + ([sc8[8:]] if MT_R > 8 else []), axis=0)
        t = wmod_ref[r0:r0 + MT_R, pl.ds(mc0, MT_W)].astype(F32) * _tile(sc8, MT_W // LANES)
        macc = t if r0 == 0 else macc + t
        gate8 = macc[0:8, 0:LANES]
    mrow = finish_mod(jnp.sum(macc, axis=0, keepdims=True), mc0)
    mrow_ref[0:1, pl.ds(mc0, MT_W)] = mrow
    modc_ref[pl.ds(mc0, MT_W), :] = _as_cols(mrow).astype(F32)
    wtie = pltpu.bitcast(modc_ref[0:8, :], U32)
    fill(-1)
    qt = pltpu.bitcast(qs[WT_TIE], U32)
    qs[WT_TIE] = pltpu.bitcast(
        jnp.concatenate([jnp.where(never8, wtie, qt[0:8]), qt[8:]], axis=0), BF16)
    s_head = None
    for ci in range(NC):
        lo = HEAD[ci - 1] if ci else 0
        s = qk(ci, lo, SK)
        if lo:
            s = jnp.concatenate([s_head, s], axis=1)
        fill(2 * ci)
        if HEAD[ci]:
            s_head = qk(ci + 1, 0, HEAD[ci])
        outs.append(softmax_pv(s, MODE[ci]))
        fill(2 * ci + 1)

    @pl.when(step + 2 < NG)
    def _():
        for d in group_copies(step + 2):
            d.start()

    @pl.when(step == 0)
    def _():
        wmb_cp().start()
        wg_cp().start()

    @pl.when(step == 1)
    def _():
        wu_cp().start()

    @pl.when(step == 2)
    def _():
        wd_cp().start()

    @pl.when(step == NG - 1)
    def _epilogue():
        @pl.when(step > 0)
        def _ln2_sums():
            for sl in range(NSL):
                cols = slice(sl * LANES, (sl + 1) * LANES)
                piv = st_ref[0, sl:sl + 1, :]
                for r0 in range(0, D, LANES):
                    r1 = min(r0 + LANES, D)
                    x2 = xt_ref[r0:r1, cols].astype(F32) + modc_ref[MA + r0:MA + r1, :] * acc_ref[r0:r1, cols]
                    acc_ref[r0:r1, cols] = x2
                    xb = x2.astype(BF16)
                    xb_ref[r0 // 2:r1 // 2, cols] = pltpu.bitcast(xb, U32)
                    d = x2 - piv
                    lhs = lhs_ref[:, r0:r1]
                    t1 = jnp.dot(lhs, xb, preferred_element_type=F32)[0:8, :]
                    t2 = jnp.dot(lhs, (d * d).astype(BF16), preferred_element_type=F32)[0:8, :]
                    s1, s2 = (t1, t2) if r0 == 0 else (s1 + t1, s2 + t2)
                for n in range(3):
                    st_ref[1 + n, sl:sl + 1, :] = s1[n:n + 1, :]
                st_ref[4, sl:sl + 1, :] = s2[0:1, :]

        mean = st_ref[1] * (1.0 / D)
        md = mean - st_ref[0]
        mb, sd = _ln_rows(mean, jnp.maximum(st_ref[4] * (1.0 / D) - md * md, 0.0))
        rs = 1.0 / sd
        st_ref[5] = rs
        st_ref[6] = mb * rs
        r = (st_ref[2] + st_ref[3] - mb * rc_ref[0:1, :]) * rs + rc_ref[1:2, :]

        lane16 = lax.broadcasted_iota(jnp.int32, (16, LANES), 1)
        never = lane16 > step + LANES

        def after_out_stores():
            dyn0 = pl.multiple_of((step - (NG - 1)) * LANES, LANES)
            return out_ref[0:16, pl.ds(dyn0, LANES)]

        def out_unit(n):
            w = OUW * LANES
            cols = slice(n * w, (n + 1) * w)
            rs, mrs = (jnp.concatenate([st_ref[k, n * OUW + u:n * OUW + u + 1, :]
                                        for u in range(OUW)], axis=1) for k in (5, 6))
            for r0 in range(0, D, OPR):
                x2 = acc_ref[r0:r0 + OPR, cols]
                o = x2 + ((x2 * rs - mrs) * _tile(fold_ref[r0:r0 + OPR, :], OUW)
                          + _tile(fold_ref[D + r0:D + r0 + OPR, :], OUW))
                out_ref[r0:r0 + OPR, cols] = o.astype(BF16)
            return after_out_stores().astype(F32)

        r = _rb(r) + 0.0
        bits = pltpu.bitcast(r, jnp.int32)
        mono = bits ^ ((bits >> 31) & jnp.int32(0x7FFFFFFF))
        tok = (lax.broadcasted_iota(jnp.int32, (NSL, LANES), 0) * LANES
               + lax.broadcasted_iota(jnp.int32, (NSL, LANES), 1))
        keyi = (((mono >> 16) + 32768) * S + (S - 1 - tok)) + jnp.int32(1 << 29)
        key = pltpu.bitcast(keyi, F32)

        row16 = lax.broadcasted_iota(jnp.int32, (16, LANES), 0)
        rowc = lax.broadcasted_iota(jnp.int32, (16, 1), 0)
        sel_slab, sel_off = [], []
        tie, nunit = None, 0
        xsel = jnp.zeros((16, D), F32)
        mbsel = jnp.zeros((16, 1), F32)
        rssel = jnp.zeros((16, 1), F32)
        ksel = jnp.zeros((16, 1), F32)
        for t in range(TOPC):
            kmax = jnp.max(jnp.max(key, axis=0, keepdims=True), axis=1, keepdims=True)
            hit = key == kmax
            key = jnp.where(hit, 0.0, key)
            pick = lambda z: jnp.sum(jnp.sum(jnp.where(hit, z, 0.0), axis=0, keepdims=True),
                                     axis=1, keepdims=True)
            mbsel = jnp.where(rowc == t, pick(mb), mbsel)
            rssel = jnp.where(rowc == t, pick(rs), rssel)
            for _ in range(TK_TIES.count(t)):
                tie = out_unit(nunit)
                nunit += 1
                key = jnp.where(never, tie, key)
            ksel = jnp.where(rowc == t, kmax, ksel)
            ki = pltpu.bitcast(kmax, jnp.int32)[0, 0]
            idx = (S - 1) - (ki & (S - 1))
            slab = idx >> 7
            off = idx & (LANES - 1)
            onehot = jnp.where((row16 == t) & (lane16 == off), 1.0, 0.0).astype(BF16)
            dslab = xb_ref[:, pl.ds(pl.multiple_of(slab * LANES, LANES), LANES)]
            xsel = xsel + lax.dot_general(onehot, pltpu.bitcast(dslab, BF16), _NT,
                                          preferred_element_type=F32)
            sel_slab.append(slab)
            sel_off.append(off)
        nsel = _rb(_rb(xsel - mbsel) * rssel)
        hsel = _rb(_rb(nsel * mb_ref[1, 0:1, :]) + mb_ref[0, 0:1, :])
        hi = ((pltpu.bitcast(ksel, jnp.int32) - jnp.int32(1 << 29)) // S - 32768) << 16
        rbits = hi ^ ((hi >> 31) & jnp.int32(0x7FFF0000))
        gate = _rb(_sigmoid(jnp.where(rowc < TOPC, pltpu.bitcast(rbits, F32), 0.0)))

        def out_copy(sl, r0, nr):
            c0 = pl.multiple_of(sl * LANES, LANES)
            return cp(out_ref.at[r0:r0 + nr, pl.ds(c0, LANES)],
                      out_hbm.at[r0:r0 + nr, pl.ds(c0, LANES)], S_O)

        fresh = []
        seen = jnp.int32(0)
        for t in range(TOPC):
            fresh.append(((seen >> sel_slab[t]) & 1) == 0)
            seen = seen | (1 << sel_slab[t])
        plain = [((seen >> sl) & 1) == 0 for sl in range(NSL)]

        for n in range(nunit, NSL // OUW):
            tie = out_unit(n)
        for sl in range(NSL):
            pl.when(plain[sl])(lambda sl=sl: out_copy(sl, 0, D).start())

        h0 = jnp.where(never, tie, hsel[:, 0:LANES])
        hs = jnp.concatenate([h0, hsel[:, LANES:]], axis=1).astype(BF16)
        gpre = _rb(jnp.dot(hs, wg_ref[...], preferred_element_type=F32))
        u = _rb(jnp.dot(hs, wu_ref[...], preferred_element_type=F32))
        a = (_rb(gpre * _sigmoid(gpre)) * u).astype(BF16)

        pieces = PIECES

        gb = mb_ref[2, 0:1, :]

        def down(r0, nr, tied):
            lhs = a
            if tied:
                a0 = jnp.where(never[0:8, :], pltpu.bitcast(after_out_stores(), U32),
                               pltpu.bitcast(a[:, TIEC:TIEC + LANES], U32))
                lhs = jnp.concatenate(([a[:, 0:TIEC]] if TIEC else []) + [pltpu.bitcast(a0, BF16)] + ([a[:, TIEC + LANES:]] if TIEC + LANES < FF else []), axis=1)
            y = jnp.dot(lhs, pltpu.bitcast(wd_ref[0:FF // 2, r0:r0 + nr], BF16),
                        preferred_element_type=F32)
            c = slice(r0, r0 + nr)
            return xsel[:, c] + gb[:, c] * (hsel[:, c] + y * gate)

        def patch(r0, nr, new):
            lane = lax.broadcasted_iota(jnp.int32, (nr // 2, LANES), 1)
            for t in range(TOPC):
                cols = pl.ds(pl.multiple_of(sel_slab[t] * LANES, LANES), LANES)
                old = pltpu.bitcast(out_ref[r0:r0 + nr, cols], U32)
                upd = pltpu.bitcast(_as_cols(new[t:t + 1, :]), U32)
                out_ref[r0:r0 + nr, cols] = pltpu.bitcast(jnp.where(lane == sel_off[t], upd, old), BF16)
            for t in range(TOPC):
                pl.when(fresh[t])(lambda t=t: out_copy(sel_slab[t], r0, nr).start())

        if DIST == 1:
            for n in range(len(pieces)):
                patch(*pieces[n], down(*pieces[n], n > 0))
        else:
            yts = [down(*pieces[0], False)]
            for n in range(len(pieces)):
                if n + 1 < len(pieces):
                    yts.append(down(*pieces[n + 1], n > 0))
                patch(*pieces[n], yts[n])

        cp(out_ref, out_hbm, S_O).wait()


@jax.jit
def pallas_adaLN_cond__gqa_block_cached__moe_arch_mod__prompt_kernel(
    A_x: jax.Array,
    A_k_cache: jax.Array,
    A_v_cache: jax.Array,
    A_wq: jax.Array,
    A_wo: jax.Array,
    B_x: jax.Array,
    B_w_r: jax.Array,
    B_w_gate: jax.Array,
    B_w_up: jax.Array,
    B_w_down: jax.Array,
    c: jax.Array,
    w_mod: jax.Array,
):
    del B_x
    B, S, D = A_x.shape
    assert B == 1
    NG, SK = A_k_cache.shape[1], A_k_cache.shape[2]
    REP = HQ // NG
    FF = B_w_gate.shape[1]
    GW = REP * DH

    xt = A_x.reshape(S, D).T
    wot = A_wo.T
    wdt = B_w_down.T
    k = A_k_cache.reshape(NG, SK, DH)
    v = A_v_cache.reshape(NG, SK, DH)

    hbm = pl.BlockSpec(memory_space=pl.ANY)
    out_t = pl.pallas_call(
        functools.partial(_kernel, S=S, SK=SK, D=D, FF=FF, NG=NG, REP=REP),
        grid=(NG,),
        in_specs=[hbm] * 11,
        out_specs=hbm,
        out_shape=jax.ShapeDtypeStruct((D, S), BF16),
        scratch_shapes=[
            pltpu.VMEM((D, S), BF16),
            pltpu.VMEM((2, SK, DH), BF16),
            pltpu.VMEM((2, SK, DH), BF16),
            pltpu.VMEM((2, D, GW), BF16),
            pltpu.VMEM((2, D, GW), BF16),
            pltpu.VMEM((D,), BF16),
            pltpu.VMEM((1, D), BF16),
            pltpu.VMEM((D, 6 * D), BF16),
            pltpu.VMEM((D, FF), BF16),
            pltpu.VMEM((D, FF), BF16),
            pltpu.VMEM((D, FF + WT_W), BF16),
            pltpu.VMEM(((FF + WT_W) // 2, D), U32),
            pltpu.VMEM((D, S), BF16),
            pltpu.VMEM((6 * D, LANES), F32),
            pltpu.VMEM((8, 6 * D), F32),
            pltpu.VMEM((D, LANES), F32),
            pltpu.VMEM((2 * D, LANES), F32),
            pltpu.VMEM((3, 8, D), F32),
            pltpu.VMEM((16, D), BF16),
            pltpu.VMEM((8, LANES), F32),
            pltpu.VMEM((S // 2, D), U32),
            pltpu.VMEM((D, S), F32),
            pltpu.VMEM((D // 2, S), U32),
            pltpu.VMEM((7, S // LANES, LANES), F32),
            pltpu.SemaphoreType.DMA((N_SEMS,)),
        ],
        compiler_params=pltpu.CompilerParams(
            dimension_semantics=("arbitrary",),
            vmem_limit_bytes=100 * 1024 * 1024,
            disable_bounds_checks=True,
        ),
    )(xt, k, v, A_wq, wot, B_w_r, c, w_mod, B_w_gate, B_w_up, wdt)
    return out_t.T.reshape(B, S, D)
```

```python
import functools
import math

import jax
import jax.numpy as jnp
from jax import lax
import jax.experimental.pallas as pl
import jax.experimental.pallas.tpu as pltpu

F32 = jnp.float32
BF16 = jnp.bfloat16
U32 = jnp.uint32

HQ = 32
DH = 128
TOPC = 8
LN_EPS = 1e-5
BQ = 256
LANES = 128
HEAD = [768, 512, 512, 1024, 768, 512, 512, 512, 768, 768, 512, 512, 512, 512, 512, 0]
MODE = [2, 1, 2, 2, 0, 0, 0, 0, 0, 1, 0, 0, 0, 2, 0, 1]
QP_POS = [-1, -1, -1, -1, -1, 3, -1, -1]
OP_POS = [11, 15, 21, 23, 30, 31, 31, 31]
XCH = 4
DIST = 2
TIEC = 2048
PIECES = [(0, 128), (128, 128), (256, 128), (384, 128), (512, 64)]
OUW = 2
TK_TIES = [0, 2, 3, 5, 6]
OPR = 16
MT_W = 384
MT_R = 8
WT_W = 384
WT_R = 256
WT_TIE = 0
MOD_STEP = 4

_NT = (((1,), (1,)), ((), ()))

S_C = S_WMA = 0
S_WMB = S_WD = 1
S_WR = 2
S_WG = S_WU = 3
S_X = 4
S_G = S_X + XCH
S_O = S_G + 2
N_SEMS = S_O + 1


def _rb(x):
    return x.astype(BF16).astype(F32)


def _sigmoid(x):
    return 1.0 / (1.0 + jnp.exp(-x))


def _ln_rows(mean, var):
    eps = _rb(jnp.full((1, 1), LN_EPS, F32))
    return _rb(mean), _rb(jnp.sqrt(_rb(_rb(var) + eps)))


def _tile(col, n):
    return jnp.concatenate([col] * n, axis=1)


def _as_cols(row):
    return jnp.broadcast_to(row, (LANES, row.shape[1])).astype(BF16).T


def _kernel(xt_hbm, k_hbm, v_hbm, wq_hbm, wot_hbm, wr_hbm, c_hbm, wmod_hbm,
            wg_hbm, wu_hbm, wdt_hbm,
            out_hbm,
            xt_ref, k_buf, v_buf, wq_buf, wot_buf, wr_ref, c_ref, wmod_ref,
            wg_ref, wu_ref, wdt_ref, wd_ref, out_ref,
            modc_ref, mrow_ref, scc_ref, fold_ref, mb_ref, lhs_ref, rc_ref, h_ref, acc_ref, xb_ref, st_ref,
            sems,
            *, S, SK, D, FF, NG, REP):
    qscale = (DH ** -0.5) * math.log2(math.e)
    NB = S // BQ
    GW = REP * DH
    TCH = S // XCH
    MA = 2 * D
    NSL = S // LANES

    def cp(src, dst, sem):
        return pltpu.make_async_copy(src, dst, sems.at[sem])

    def x_copy(i):
        cols = pl.ds(pl.multiple_of(i * TCH, TCH), TCH)
        return cp(xt_hbm.at[:, cols], xt_ref.at[:, cols], S_X + i)

    def group_copies(grp):
        slot = grp % 2
        cols = pl.ds(pl.multiple_of(grp * GW, GW), GW)
        return (cp(wq_hbm.at[:, cols], wq_buf.at[slot], S_G + slot),
                cp(k_hbm.at[grp], k_buf.at[slot], S_G + slot),
                cp(v_hbm.at[grp], v_buf.at[slot], S_G + slot),
                cp(wot_hbm.at[:, cols], wot_buf.at[slot], S_G + slot))

    c_cp = lambda: cp(c_hbm, c_ref, S_C)
    wma_cp = lambda: cp(wmod_hbm.at[:, 0:MA], wmod_ref.at[:, 0:MA], S_WMA)
    wmb_cp = lambda: cp(wmod_hbm.at[:, MA:6 * D], wmod_ref.at[:, MA:6 * D], S_WMB)
    wr_cp = lambda: cp(wr_hbm, wr_ref, S_WR)
    wg_cp = lambda: cp(wg_hbm, wg_ref, S_WG)
    wu_cp = lambda: cp(wu_hbm, wu_ref, S_WU)
    wd_cp = lambda: cp(wdt_hbm, wdt_ref.at[:, 0:FF], S_WD)

    def modcol(i):
        return modc_ref[i * D:(i + 1) * D, :]

    def finish_mod(mod, col0):
        mod = _rb(mod)
        lane = lax.broadcasted_iota(jnp.int32, mod.shape, 1) + col0
        is_scale = ((lane >= D) & (lane < 2 * D)) | ((lane >= 4 * D) & (lane < 5 * D))
        return jnp.where(is_scale, _rb(1.0 + mod), mod)

    wma_cp().start()
    c_cp().start()
    for i in range(XCH):
        x_copy(i).start()
    for d in group_copies(0) + group_copies(1):
        d.start()
    wr_cp().start()
    acc_ref[...] = jnp.zeros((D, S), F32)
    wma_cp().wait()
    c_cp().wait()
    c = c_ref[...].astype(F32)
    sc = _rb(c * _sigmoid(c))
    mod = jnp.dot(jnp.broadcast_to(sc, (8, D)).astype(BF16), wmod_ref[:, 0:MA],
                  preferred_element_type=F32)
    modc_ref[0:MA, :] = _as_cols(finish_mod(mod, 0)[0:1, :]).astype(F32)

    def ln1(i, carry):
        x_copy(i).wait()
        x = xt_ref[:, pl.ds(pl.multiple_of(i * TCH, TCH), TCH)].astype(F32)
        piv = x[0:1, :]
        d = x - piv
        md = jnp.mean(d, axis=0, keepdims=True)
        var = jnp.maximum(jnp.mean(d * d, axis=0, keepdims=True) - md * md, 0.0)
        mb, sd = _ln_rows(piv + md, var)
        rs = 1.0 / sd
        n = TCH // LANES
        for u in range(n):
            st_ref[0, pl.ds(n * i + u, 1), :] = mb[:, u * LANES:(u + 1) * LANES]
        ht = (x * rs - mb * rs) * _tile(modcol(1), n) + _tile(modcol(0), n)
        h_ref[pl.ds(pl.multiple_of(i * (TCH // 2), TCH // 2), TCH // 2), :] = pltpu.bitcast(
            ht.astype(BF16).T, U32)
        return carry
    lax.fori_loop(0, XCH, ln1, 0)
    scc_ref[...] = _as_cols(sc).astype(F32)

    def fold_modulation():
        sb, cb, gb = (mrow_ref[0:1, i * D:(i + 1) * D] for i in (3, 4, 5))
        for i, z in enumerate((sb, cb, gb)):
            mb_ref[i] = jnp.broadcast_to(z, (8, D))
        fold_ref[0:D, :] = modcol(5) * modcol(4)
        fold_ref[D:MA, :] = modcol(5) * modcol(3)
        wr = wr_ref[...].astype(F32).reshape(1, D)
        wc = wr * cb
        whi = _rb(wc)
        wlo = _rb(wc - whi)
        row = lax.broadcasted_iota(jnp.int32, (16, D), 0)
        lhs_ref[...] = jnp.where(row == 0, 1.0, jnp.where(row == 1, whi, jnp.where(
            row == 2, wlo, 0.0))).astype(BF16)
        rc_ref[0:1, :] = jnp.broadcast_to(jnp.sum(whi + wlo, axis=1, keepdims=True), (1, LANES))
        rc_ref[1:2, :] = jnp.broadcast_to(jnp.sum(wr * sb, axis=1, keepdims=True), (1, LANES))

    def group_step(step, carry):
        @pl.when(step == MOD_STEP)
        def _():
            wmb_cp().wait()
            wd_cp().wait()

        for d in group_copies(step):
            d.wait()

        slot = step % 2
        k = k_buf[slot]
        v = v_buf[slot]
        wq = wq_buf[slot]
        wot = wot_buf[slot]

        def qproj(j):
            hb = pltpu.bitcast(h_ref[j * (BQ // 2):(j + 1) * (BQ // 2), :], BF16)
            q2 = jnp.dot(hb, wq, preferred_element_type=F32)
            return (q2 * qscale).astype(BF16)

        def qk(ci, lo, hi):
            return lax.dot_general(qs[ci], k[lo:hi], _NT, preferred_element_type=F32)

        def softmax_pv(s, mode):
            m = jnp.max(s, axis=1, keepdims=True)
            p = jnp.exp2(s - m)
            parts = [p[:, i * LANES:(i + 1) * LANES] for i in range(SK // LANES)]
            if mode == 2:
                lp = None
                for c in range(0, len(parts), 4):
                    t = (parts[c] + parts[c + 1]) + (parts[c + 2] + parts[c + 3])
                    lp = t if lp is None else lp + t
                    parts[c + 3] = jnp.where(lp < 0.0, lp, parts[c + 3])
                p = jnp.concatenate(parts, axis=1)
            o = jnp.dot(p.astype(BF16), v, preferred_element_type=F32)
            if mode == 0:
                l = jnp.sum(p, axis=1, keepdims=True)
            elif mode == 1:
                lp = functools.reduce(lambda x, y: x + y, parts)
                l = jnp.sum(jnp.where(lp < 0.0, o, lp), axis=1, keepdims=True)
            else:
                l = jnp.sum(lp, axis=1, keepdims=True)
            rl = pl.reciprocal(l, approx=True)
            rl = rl * (2.0 - l * rl)
            return (o * rl).astype(BF16)

        def oproj(j):
            o2 = jnp.concatenate([outs[REP * j + r] for r in range(REP)], axis=1)
            acc_ref[:, j * BQ:(j + 1) * BQ] += lax.dot_general(wot, o2, _NT, preferred_element_type=F32)

        qs, outs = {}, []

        def fill(pos):
            for j in range(NB):
                if QP_POS[j] == pos:
                    q2 = qproj(j)
                    for r in range(REP):
                        qs[REP * j + r] = q2[:, r * DH:(r + 1) * DH]
            for j in range(NB):
                if OP_POS[j] == pos:
                    oproj(j)

        NC = NB * REP
        assert (NG - MOD_STEP) * WT_W == FF
        wc0 = jnp.where(step >= MOD_STEP, (step - MOD_STEP) * WT_W, FF)
        never8 = lax.broadcasted_iota(jnp.int32, (8, LANES), 1) > step + LANES
        wtie = None
        for t0 in range(0, WT_W, LANES):
            for r0 in range(0, D, WT_R):
                r1 = min(r0 + WT_R, D)
                blk = pltpu.bitcast(wdt_ref[r0:r1, pl.ds(pl.multiple_of(wc0 + t0, LANES), LANES)], U32)
                if wtie is not None:
                    blk = jnp.concatenate([jnp.where(never8, wtie, blk[0:8]), blk[8:]], axis=0)
                tb = pltpu.bitcast(pltpu.bitcast(blk, BF16).T, U32)
                wd_ref[pl.ds(pl.multiple_of((wc0 + t0) // 2, LANES // 2), LANES // 2), r0:r1] = tb
                wtie = wd_ref[pl.ds(pl.multiple_of(wc0 // 2, LANES // 2), 8), 0:LANES]
        nms = 4 * D // MT_W
        assert nms * MT_W == 4 * D and MOD_STEP + nms < NG
        in_win = (step >= MOD_STEP) & (step < MOD_STEP + nms)
        mc0 = pl.multiple_of(jnp.where(in_win, MA + (step - MOD_STEP) * MT_W, 0), LANES)
        gate8 = pltpu.bitcast(wtie, F32)
        for r0 in range(0, D, MT_R):
            sc8 = scc_ref[r0:r0 + MT_R, :]
            sc8 = jnp.concatenate([jnp.where(never8, gate8, sc8[0:8])] + ([sc8[8:]] if MT_R > 8 else []), axis=0)
            t = wmod_ref[r0:r0 + MT_R, pl.ds(mc0, MT_W)].astype(F32) * _tile(sc8, MT_W // LANES)
            macc = t if r0 == 0 else macc + t
            gate8 = macc[0:8, 0:LANES]
        mrow = finish_mod(jnp.sum(macc, axis=0, keepdims=True), mc0)
        mrow_ref[0:1, pl.ds(mc0, MT_W)] = mrow
        modc_ref[pl.ds(mc0, MT_W), :] = _as_cols(mrow).astype(F32)
        wtie = pltpu.bitcast(modc_ref[0:8, :], U32)
        fill(-1)
        qt = pltpu.bitcast(qs[WT_TIE], U32)
        qs[WT_TIE] = pltpu.bitcast(
            jnp.concatenate([jnp.where(never8, wtie, qt[0:8]), qt[8:]], axis=0), BF16)
        s_head = None
        for ci in range(NC):
            lo = HEAD[ci - 1] if ci else 0
            s = qk(ci, lo, SK)
            if lo:
                s = jnp.concatenate([s_head, s], axis=1)
            fill(2 * ci)
            if HEAD[ci]:
                s_head = qk(ci + 1, 0, HEAD[ci])
            outs.append(softmax_pv(s, MODE[ci]))
            fill(2 * ci + 1)

        @pl.when(step + 2 < NG)
        def _():
            for d in group_copies(step + 2):
                d.start()

        @pl.when(step == 0)
        def _():
            wmb_cp().start()
            wg_cp().start()

        @pl.when(step == 1)
        def _():
            wu_cp().start()

        @pl.when(step == 2)
        def _():
            wd_cp().start()

        return step

    step = lax.fori_loop(0, NG, group_step, 0)

    wr_cp().wait()
    fold_modulation()
    for sl in range(NSL):
        cols = slice(sl * LANES, (sl + 1) * LANES)
        piv = st_ref[0, sl:sl + 1, :]
        for r0 in range(0, D, LANES):
            r1 = min(r0 + LANES, D)
            x2 = xt_ref[r0:r1, cols].astype(F32) + modc_ref[MA + r0:MA + r1, :] * acc_ref[r0:r1, cols]
            acc_ref[r0:r1, cols] = x2
            xb = x2.astype(BF16)
            xb_ref[r0 // 2:r1 // 2, cols] = pltpu.bitcast(xb, U32)
            d = x2 - piv
            lhs = lhs_ref[:, r0:r1]
            t1 = jnp.dot(lhs, xb, preferred_element_type=F32)[0:8, :]
            t2 = jnp.dot(lhs, (d * d).astype(BF16), preferred_element_type=F32)[0:8, :]
            s1, s2 = (t1, t2) if r0 == 0 else (s1 + t1, s2 + t2)
        for n in range(3):
            st_ref[1 + n, sl:sl + 1, :] = s1[n:n + 1, :]
        st_ref[4, sl:sl + 1, :] = s2[0:1, :]

    wg_cp().wait()
    wu_cp().wait()

    mean = st_ref[1] * (1.0 / D)
    md = mean - st_ref[0]
    mb, sd = _ln_rows(mean, jnp.maximum(st_ref[4] * (1.0 / D) - md * md, 0.0))
    rs = 1.0 / sd
    st_ref[5] = rs
    st_ref[6] = mb * rs
    r = (st_ref[2] + st_ref[3] - mb * rc_ref[0:1, :]) * rs + rc_ref[1:2, :]

    lane16 = lax.broadcasted_iota(jnp.int32, (16, LANES), 1)
    never = lane16 > step + LANES

    def after_out_stores():
        dyn0 = pl.multiple_of((step - (NG - 1)) * LANES, LANES)
        return out_ref[0:16, pl.ds(dyn0, LANES)]

    def out_unit(n):
        w = OUW * LANES
        cols = slice(n * w, (n + 1) * w)
        rs, mrs = (jnp.concatenate([st_ref[k, n * OUW + u:n * OUW + u + 1, :]
                                    for u in range(OUW)], axis=1) for k in (5, 6))
        for r0 in range(0, D, OPR):
            x2 = acc_ref[r0:r0 + OPR, cols]
            o = x2 + ((x2 * rs - mrs) * _tile(fold_ref[r0:r0 + OPR, :], OUW)
                      + _tile(fold_ref[D + r0:D + r0 + OPR, :], OUW))
            out_ref[r0:r0 + OPR, cols] = o.astype(BF16)
        return after_out_stores().astype(F32)

    r = _rb(r) + 0.0
    bits = pltpu.bitcast(r, jnp.int32)
    mono = bits ^ ((bits >> 31) & jnp.int32(0x7FFFFFFF))
    tok = (lax.broadcasted_iota(jnp.int32, (NSL, LANES), 0) * LANES
           + lax.broadcasted_iota(jnp.int32, (NSL, LANES), 1))
    keyi = (((mono >> 16) + 32768) * S + (S - 1 - tok)) + jnp.int32(1 << 29)
    key = pltpu.bitcast(keyi, F32)

    row16 = lax.broadcasted_iota(jnp.int32, (16, LANES), 0)
    rowc = lax.broadcasted_iota(jnp.int32, (16, 1), 0)
    sel_slab, sel_off = [], []
    tie, nunit = None, 0
    xsel = jnp.zeros((16, D), F32)
    mbsel = jnp.zeros((16, 1), F32)
    rssel = jnp.zeros((16, 1), F32)
    ksel = jnp.zeros((16, 1), F32)
    for t in range(TOPC):
        kmax = jnp.max(jnp.max(key, axis=0, keepdims=True), axis=1, keepdims=True)
        hit = key == kmax
        key = jnp.where(hit, 0.0, key)
        pick = lambda z: jnp.sum(jnp.sum(jnp.where(hit, z, 0.0), axis=0, keepdims=True),
                                 axis=1, keepdims=True)
        mbsel = jnp.where(rowc == t, pick(mb), mbsel)
        rssel = jnp.where(rowc == t, pick(rs), rssel)
        for _ in range(TK_TIES.count(t)):
            tie = out_unit(nunit)
            nunit += 1
            key = jnp.where(never, tie, key)
        ksel = jnp.where(rowc == t, kmax, ksel)
        ki = pltpu.bitcast(kmax, jnp.int32)[0, 0]
        idx = (S - 1) - (ki & (S - 1))
        slab = idx >> 7
        off = idx & (LANES - 1)
        onehot = jnp.where((row16 == t) & (lane16 == off), 1.0, 0.0).astype(BF16)
        dslab = xb_ref[:, pl.ds(pl.multiple_of(slab * LANES, LANES), LANES)]
        xsel = xsel + lax.dot_general(onehot, pltpu.bitcast(dslab, BF16), _NT,
                                      preferred_element_type=F32)
        sel_slab.append(slab)
        sel_off.append(off)
    nsel = _rb(_rb(xsel - mbsel) * rssel)
    hsel = _rb(_rb(nsel * mb_ref[1, 0:1, :]) + mb_ref[0, 0:1, :])
    hi = ((pltpu.bitcast(ksel, jnp.int32) - jnp.int32(1 << 29)) // S - 32768) << 16
    rbits = hi ^ ((hi >> 31) & jnp.int32(0x7FFF0000))
    gate = _rb(_sigmoid(jnp.where(rowc < TOPC, pltpu.bitcast(rbits, F32), 0.0)))

    def out_copy(sl, r0, nr):
        c0 = pl.multiple_of(sl * LANES, LANES)
        return cp(out_ref.at[r0:r0 + nr, pl.ds(c0, LANES)],
                  out_hbm.at[r0:r0 + nr, pl.ds(c0, LANES)], S_O)

    fresh = []
    seen = jnp.int32(0)
    for t in range(TOPC):
        fresh.append(((seen >> sel_slab[t]) & 1) == 0)
        seen = seen | (1 << sel_slab[t])
    plain = [((seen >> sl) & 1) == 0 for sl in range(NSL)]

    for n in range(nunit, NSL // OUW):
        tie = out_unit(n)
    for sl in range(NSL):
        pl.when(plain[sl])(lambda sl=sl: out_copy(sl, 0, D).start())

    h0 = jnp.where(never, tie, hsel[:, 0:LANES])
    hs = jnp.concatenate([h0, hsel[:, LANES:]], axis=1).astype(BF16)
    gpre = _rb(jnp.dot(hs, wg_ref[...], preferred_element_type=F32))
    u = _rb(jnp.dot(hs, wu_ref[...], preferred_element_type=F32))
    a = (_rb(gpre * _sigmoid(gpre)) * u).astype(BF16)

    pieces = PIECES

    gb = mb_ref[2, 0:1, :]

    def down(r0, nr, tied):
        lhs = a
        if tied:
            a0 = jnp.where(never[0:8, :], pltpu.bitcast(after_out_stores(), U32),
                           pltpu.bitcast(a[:, TIEC:TIEC + LANES], U32))
            lhs = jnp.concatenate(([a[:, 0:TIEC]] if TIEC else []) + [pltpu.bitcast(a0, BF16)] + ([a[:, TIEC + LANES:]] if TIEC + LANES < FF else []), axis=1)
        y = jnp.dot(lhs, pltpu.bitcast(wd_ref[0:FF // 2, r0:r0 + nr], BF16),
                    preferred_element_type=F32)
        c = slice(r0, r0 + nr)
        return xsel[:, c] + gb[:, c] * (hsel[:, c] + y * gate)

    def patch(r0, nr, new):
        lane = lax.broadcasted_iota(jnp.int32, (nr // 2, LANES), 1)
        for t in range(TOPC):
            cols = pl.ds(pl.multiple_of(sel_slab[t] * LANES, LANES), LANES)
            old = pltpu.bitcast(out_ref[r0:r0 + nr, cols], U32)
            upd = pltpu.bitcast(_as_cols(new[t:t + 1, :]), U32)
            out_ref[r0:r0 + nr, cols] = pltpu.bitcast(jnp.where(lane == sel_off[t], upd, old), BF16)
        for t in range(TOPC):
            pl.when(fresh[t])(lambda t=t: out_copy(sel_slab[t], r0, nr).start())

    if DIST == 1:
        for n in range(len(pieces)):
            patch(*pieces[n], down(*pieces[n], n > 0))
    else:
        yts = [down(*pieces[0], False)]
        for n in range(len(pieces)):
            if n + 1 < len(pieces):
                yts.append(down(*pieces[n + 1], n > 0))
            patch(*pieces[n], yts[n])

    cp(out_ref, out_hbm, S_O).wait()


@jax.jit
def pallas_adaLN_cond__gqa_block_cached__moe_arch_mod__prompt_kernel(
    A_x: jax.Array,
    A_k_cache: jax.Array,
    A_v_cache: jax.Array,
    A_wq: jax.Array,
    A_wo: jax.Array,
    B_x: jax.Array,
    B_w_r: jax.Array,
    B_w_gate: jax.Array,
    B_w_up: jax.Array,
    B_w_down: jax.Array,
    c: jax.Array,
    w_mod: jax.Array,
):
    del B_x
    B, S, D = A_x.shape
    assert B == 1
    NG, SK = A_k_cache.shape[1], A_k_cache.shape[2]
    REP = HQ // NG
    FF = B_w_gate.shape[1]
    GW = REP * DH

    xt = A_x.reshape(S, D).T
    wot = A_wo.T
    wdt = B_w_down.T
    k = A_k_cache.reshape(NG, SK, DH)
    v = A_v_cache.reshape(NG, SK, DH)

    hbm = pl.BlockSpec(memory_space=pl.ANY)
    out_t = pl.pallas_call(
        functools.partial(_kernel, S=S, SK=SK, D=D, FF=FF, NG=NG, REP=REP),
        in_specs=[hbm] * 11,
        out_specs=hbm,
        out_shape=jax.ShapeDtypeStruct((D, S), BF16),
        scratch_shapes=[
            pltpu.VMEM((D, S), BF16),
            pltpu.VMEM((2, SK, DH), BF16),
            pltpu.VMEM((2, SK, DH), BF16),
            pltpu.VMEM((2, D, GW), BF16),
            pltpu.VMEM((2, D, GW), BF16),
            pltpu.VMEM((D,), BF16),
            pltpu.VMEM((1, D), BF16),
            pltpu.VMEM((D, 6 * D), BF16),
            pltpu.VMEM((D, FF), BF16),
            pltpu.VMEM((D, FF), BF16),
            pltpu.VMEM((D, FF + WT_W), BF16),
            pltpu.VMEM(((FF + WT_W) // 2, D), U32),
            pltpu.VMEM((D, S), BF16),
            pltpu.VMEM((6 * D, LANES), F32),
            pltpu.VMEM((8, 6 * D), F32),
            pltpu.VMEM((D, LANES), F32),
            pltpu.VMEM((2 * D, LANES), F32),
            pltpu.VMEM((3, 8, D), F32),
            pltpu.VMEM((16, D), BF16),
            pltpu.VMEM((8, LANES), F32),
            pltpu.VMEM((S // 2, D), U32),
            pltpu.VMEM((D, S), F32),
            pltpu.VMEM((D // 2, S), U32),
            pltpu.VMEM((7, S // LANES, LANES), F32),
            pltpu.SemaphoreType.DMA((N_SEMS,)),
        ],
        compiler_params=pltpu.CompilerParams(
            vmem_limit_bytes=100 * 1024 * 1024,
            disable_bounds_checks=True,
        ),
    )(xt, k, v, A_wq, wot, B_w_r, c, w_mod, B_w_gate, B_w_up, wdt)
    return out_t.T.reshape(B, S, D)
```

```python
import functools
import math

import jax
import jax.numpy as jnp
from jax import lax
import jax.experimental.pallas as pl
import jax.experimental.pallas.tpu as pltpu

F32 = jnp.float32
BF16 = jnp.bfloat16
U32 = jnp.uint32

HQ = 32
DH = 128
TOPC = 8
LN_EPS = 1e-5
BQ = 256
LANES = 128
HEAD = [768, 512, 512, 1024, 768, 512, 512, 512, 768, 768, 512, 512, 512, 512, 512, 0]
MODE = [2, 1, 2, 2, 0, 0, 0, 0, 0, 1, 0, 0, 0, 2, 0, 1]
QP_POS = [-1, -1, -1, -1, -1, 3, -1, -1]
OP_POS = [11, 15, 21, 23, 30, 31, 31, 31]
XCH = 4
DIST = 2
TIEC = 2048
PIECES = [(0, 128), (128, 128), (256, 128), (384, 128), (512, 64)]
OUW = 2
TK_TIES = [0, 1, 2, 3, 4, 5, 6]
OPR = 16
PIV0 = 0
MT_W = 384
MT_R = 8
WT_W = 384
WT_R = 256
WT_TIE = 0
MOD_STEP = 4

_NT = (((1,), (1,)), ((), ()))

S_C = S_WMA = 0
S_WMB = S_WD = 1
S_WR = 2
S_WG = S_WU = 3
S_X = 4
S_G = S_X + XCH
S_O = S_G + 2
N_SEMS = S_O + 1


def _rb(x):
    return x.astype(BF16).astype(F32)


def _sigmoid(x):
    return 1.0 / (1.0 + jnp.exp(-x))


def _ln_rows(mean, var):
    eps = _rb(jnp.full((1, 1), LN_EPS, F32))
    return _rb(mean), _rb(jnp.sqrt(_rb(_rb(var) + eps)))


def _tile(col, n):
    return jnp.concatenate([col] * n, axis=1)


def _as_cols(row):
    return jnp.broadcast_to(row, (LANES, row.shape[1])).astype(BF16).T


def _kernel(xt_hbm, k_hbm, v_hbm, wq_hbm, wot_hbm, wr_hbm, c_hbm, wmod_hbm,
            wg_hbm, wu_hbm, wdt_hbm,
            out_hbm,
            xt_ref, k_buf, v_buf, wq_buf, wot_buf, wr_ref, c_ref, wmod_ref,
            wg_ref, wu_ref, wdt_ref, wd_ref, out_ref,
            modc_ref, mrow_ref, scc_ref, fold_ref, mb_ref, lhs_ref, rc_ref, h_ref, acc_ref, xb_ref, st_ref,
            sems,
            *, S, SK, D, FF, NG, REP):
    qscale = (DH ** -0.5) * math.log2(math.e)
    NB = S // BQ
    GW = REP * DH
    TCH = S // XCH
    MA = 2 * D
    NSL = S // LANES

    def cp(src, dst, sem):
        return pltpu.make_async_copy(src, dst, sems.at[sem])

    def x_copy(i):
        cols = pl.ds(pl.multiple_of(i * TCH, TCH), TCH)
        return cp(xt_hbm.at[:, cols], xt_ref.at[:, cols], S_X + i)

    def group_copies(grp):
        slot = grp % 2
        cols = pl.ds(pl.multiple_of(grp * GW, GW), GW)
        return (cp(wq_hbm.at[:, cols], wq_buf.at[slot], S_G + slot),
                cp(k_hbm.at[grp], k_buf.at[slot], S_G + slot),
                cp(v_hbm.at[grp], v_buf.at[slot], S_G + slot),
                cp(wot_hbm.at[:, cols], wot_buf.at[slot], S_G + slot))

    c_cp = lambda: cp(c_hbm, c_ref, S_C)
    wma_cp = lambda: cp(wmod_hbm.at[:, 0:MA], wmod_ref.at[:, 0:MA], S_WMA)
    wmb_cp = lambda: cp(wmod_hbm.at[:, MA:6 * D], wmod_ref.at[:, MA:6 * D], S_WMB)
    wr_cp = lambda: cp(wr_hbm, wr_ref, S_WR)
    wg_cp = lambda: cp(wg_hbm, wg_ref, S_WG)
    wu_cp = lambda: cp(wu_hbm, wu_ref, S_WU)
    wd_cp = lambda: cp(wdt_hbm, wdt_ref.at[:, 0:FF], S_WD)

    def modcol(i):
        return modc_ref[i * D:(i + 1) * D, :]

    def finish_mod(mod, col0):
        mod = _rb(mod)
        lane = lax.broadcasted_iota(jnp.int32, mod.shape, 1) + col0
        is_scale = ((lane >= D) & (lane < 2 * D)) | ((lane >= 4 * D) & (lane < 5 * D))
        return jnp.where(is_scale, _rb(1.0 + mod), mod)

    wma_cp().start()
    c_cp().start()
    for i in range(XCH):
        x_copy(i).start()
    for d in group_copies(0) + group_copies(1):
        d.start()
    wr_cp().start()
    acc_ref[...] = jnp.zeros((D, S), F32)
    wdt_ref[:, FF:FF + WT_W] = jnp.zeros((D, WT_W), BF16)
    wma_cp().wait()
    c_cp().wait()
    c = c_ref[...].astype(F32)
    sc = _rb(c * _sigmoid(c))
    mod = jnp.dot(jnp.broadcast_to(sc, (8, D)).astype(BF16), wmod_ref[:, 0:MA],
                  preferred_element_type=F32)
    modc_ref[0:MA, :] = _as_cols(finish_mod(mod, 0)[0:1, :]).astype(F32)

    def ln1(i, carry):
        x_copy(i).wait()
        x = xt_ref[:, pl.ds(pl.multiple_of(i * TCH, TCH), TCH)].astype(F32)
        piv = x[0:1, :]
        d = x - piv
        md = jnp.mean(d, axis=0, keepdims=True)
        var = jnp.maximum(jnp.mean(d * d, axis=0, keepdims=True) - md * md, 0.0)
        mb, sd = _ln_rows(piv + md, var)
        rs = 1.0 / sd
        n = TCH // LANES
        ht = (x * rs - mb * rs) * _tile(modcol(1), n) + _tile(modcol(0), n)
        h_ref[pl.ds(pl.multiple_of(i * (TCH // 2), TCH // 2), TCH // 2), :] = pltpu.bitcast(
            ht.astype(BF16).T, U32)
        return carry
    lax.fori_loop(0, XCH, ln1, 0)
    scc_ref[...] = _as_cols(sc).astype(F32)

    def fold_modulation():
        sb, cb, gb = (mrow_ref[0:1, i * D:(i + 1) * D] for i in (3, 4, 5))
        for i, z in enumerate((sb, cb, gb)):
            mb_ref[i] = jnp.broadcast_to(z, (8, D))
        fold_ref[0:D, :] = modcol(5) * modcol(4)
        fold_ref[D:MA, :] = modcol(5) * modcol(3)
        wr = wr_ref[...].astype(F32).reshape(1, D)
        wc = wr * cb
        whi = _rb(wc)
        wlo = _rb(wc - whi)
        row = lax.broadcasted_iota(jnp.int32, (16, D), 0)
        lhs_ref[...] = jnp.where(row == 0, 1.0, jnp.where(row == 1, whi, jnp.where(
            row == 2, wlo, 0.0))).astype(BF16)
        rc_ref[0:1, :] = jnp.broadcast_to(jnp.sum(whi + wlo, axis=1, keepdims=True), (1, LANES))
        rc_ref[1:2, :] = jnp.broadcast_to(jnp.sum(wr * sb, axis=1, keepdims=True), (1, LANES))

    def group_step(step, carry):
        @pl.when(step == MOD_STEP)
        def _():
            wmb_cp().wait()
            wd_cp().wait()

        for d in group_copies(step):
            d.wait()

        slot = step % 2
        k = k_buf[slot]
        v = v_buf[slot]
        wq = wq_buf[slot]
        wot = wot_buf[slot]

        def qproj(j):
            hb = pltpu.bitcast(h_ref[j * (BQ // 2):(j + 1) * (BQ // 2), :], BF16)
            q2 = jnp.dot(hb, wq, preferred_element_type=F32)
            return (q2 * qscale).astype(BF16)

        def qk(ci, lo, hi):
            return lax.dot_general(qs[ci], k[lo:hi], _NT, preferred_element_type=F32)

        def softmax_pv(s, mode):
            m = jnp.max(s, axis=1, keepdims=True)
            p = jnp.exp2(s - m)
            parts = [p[:, i * LANES:(i + 1) * LANES] for i in range(SK // LANES)]
            if mode == 2:
                lp = None
                for c in range(0, len(parts), 4):
                    t = (parts[c] + parts[c + 1]) + (parts[c + 2] + parts[c + 3])
                    lp = t if lp is None else lp + t
                    parts[c + 3] = jnp.where(lp < 0.0, lp, parts[c + 3])
                p = jnp.concatenate(parts, axis=1)
            o = jnp.dot(p.astype(BF16), v, preferred_element_type=F32)
            if mode == 0:
                l = jnp.sum(p, axis=1, keepdims=True)
            elif mode == 1:
                lp = functools.reduce(lambda x, y: x + y, parts)
                l = jnp.sum(jnp.where(lp < 0.0, o, lp), axis=1, keepdims=True)
            else:
                l = jnp.sum(lp, axis=1, keepdims=True)
            rl = pl.reciprocal(l, approx=True)
            rl = rl * (2.0 - l * rl)
            return (o * rl).astype(BF16)

        def oproj(j):
            o2 = jnp.concatenate([outs[REP * j + r] for r in range(REP)], axis=1)
            acc_ref[:, j * BQ:(j + 1) * BQ] += lax.dot_general(wot, o2, _NT, preferred_element_type=F32)

        qs, outs = {}, []

        def fill(pos):
            for j in range(NB):
                if QP_POS[j] == pos:
                    q2 = qproj(j)
                    for r in range(REP):
                        qs[REP * j + r] = q2[:, r * DH:(r + 1) * DH]
            for j in range(NB):
                if OP_POS[j] == pos:
                    oproj(j)

        NC = NB * REP
        assert (NG - MOD_STEP) * WT_W == FF
        wc0 = jnp.where(step >= MOD_STEP, (step - MOD_STEP) * WT_W, FF)
        never8 = lax.broadcasted_iota(jnp.int32, (8, LANES), 1) > step + LANES
        wtie = None
        for t0 in range(0, WT_W, LANES):
            for r0 in range(0, D, WT_R):
                r1 = min(r0 + WT_R, D)
                blk = pltpu.bitcast(wdt_ref[r0:r1, pl.ds(pl.multiple_of(wc0 + t0, LANES), LANES)], U32)
                if wtie is not None:
                    blk = jnp.concatenate([jnp.where(never8, wtie, blk[0:8]), blk[8:]], axis=0)
                tb = pltpu.bitcast(pltpu.bitcast(blk, BF16).T, U32)
                wd_ref[pl.ds(pl.multiple_of((wc0 + t0) // 2, LANES // 2), LANES // 2), r0:r1] = tb
                wtie = wd_ref[pl.ds(pl.multiple_of(wc0 // 2, LANES // 2), 8), 0:LANES]
        nms = 4 * D // MT_W
        assert nms * MT_W == 4 * D and MOD_STEP + nms < NG
        in_win = (step >= MOD_STEP) & (step < MOD_STEP + nms)
        mc0 = pl.multiple_of(jnp.where(in_win, MA + (step - MOD_STEP) * MT_W, 0), LANES)
        gate8 = pltpu.bitcast(wtie, F32)
        for r0 in range(0, D, MT_R):
            sc8 = scc_ref[r0:r0 + MT_R, :]
            sc8 = jnp.concatenate([jnp.where(never8, gate8, sc8[0:8])] + ([sc8[8:]] if MT_R > 8 else []), axis=0)
            t = wmod_ref[r0:r0 + MT_R, pl.ds(mc0, MT_W)].astype(F32) * _tile(sc8, MT_W // LANES)
            macc = t if r0 == 0 else macc + t
            gate8 = macc[0:8, 0:LANES]
        mrow = finish_mod(jnp.sum(macc, axis=0, keepdims=True), mc0)
        mrow_ref[0:1, pl.ds(mc0, MT_W)] = mrow
        modc_ref[pl.ds(mc0, MT_W), :] = _as_cols(mrow).astype(F32)
        wtie = pltpu.bitcast(modc_ref[0:8, :], U32)
        fill(-1)
        qt = pltpu.bitcast(qs[WT_TIE], U32)
        qs[WT_TIE] = pltpu.bitcast(
            jnp.concatenate([jnp.where(never8, wtie, qt[0:8]), qt[8:]], axis=0), BF16)
        s_head = None
        for ci in range(NC):
            lo = HEAD[ci - 1] if ci else 0
            s = qk(ci, lo, SK)
            if lo:
                s = jnp.concatenate([s_head, s], axis=1)
            fill(2 * ci)
            if HEAD[ci]:
                s_head = qk(ci + 1, 0, HEAD[ci])
            outs.append(softmax_pv(s, MODE[ci]))
            fill(2 * ci + 1)

        @pl.when(step + 2 < NG)
        def _():
            for d in group_copies(step + 2):
                d.start()

        @pl.when(step == 0)
        def _():
            wmb_cp().start()
            wg_cp().start()

        @pl.when(step == 1)
        def _():
            wu_cp().start()

        @pl.when(step == 2)
        def _():
            wd_cp().start()

        return step

    step = lax.fori_loop(0, NG, group_step, 0)

    wr_cp().wait()
    fold_modulation()
    for sl in range(NSL):
        cols = slice(sl * LANES, (sl + 1) * LANES)
        for r0 in range(0, D, LANES):
            r1 = min(r0 + LANES, D)
            x2 = xt_ref[r0:r1, cols].astype(F32) + modc_ref[MA + r0:MA + r1, :] * acc_ref[r0:r1, cols]
            acc_ref[r0:r1, cols] = x2
            xb = x2.astype(BF16)
            xb_ref[r0 // 2:r1 // 2, cols] = pltpu.bitcast(xb, U32)
            if r0 == 0:
                piv = jnp.mean(x2[PIV0:PIV0 + 8, :], axis=0, keepdims=True)
                st_ref[0, sl:sl + 1, :] = piv
            d = x2 - piv
            lhs = lhs_ref[:, r0:r1]
            t1 = jnp.dot(lhs, xb, preferred_element_type=F32)[0:8, :]
            t2 = jnp.dot(lhs, (d * d).astype(BF16), preferred_element_type=F32)[0:8, :]
            s1, s2 = (t1, t2) if r0 == 0 else (s1 + t1, s2 + t2)
        for n in range(3):
            st_ref[1 + n, sl:sl + 1, :] = s1[n:n + 1, :]
        st_ref[4, sl:sl + 1, :] = s2[0:1, :]

    wg_cp().wait()
    wu_cp().wait()

    mean = st_ref[1] * (1.0 / D)
    md = mean - st_ref[0]
    mb, sd = _ln_rows(mean, jnp.maximum(st_ref[4] * (1.0 / D) - md * md, 0.0))
    rs = 1.0 / sd
    st_ref[5] = rs
    st_ref[6] = mb * rs
    r = (st_ref[2] + st_ref[3] - mb * rc_ref[0:1, :]) * rs + rc_ref[1:2, :]

    lane16 = lax.broadcasted_iota(jnp.int32, (16, LANES), 1)
    never = lane16 > step + LANES

    def after_out_stores():
        dyn0 = pl.multiple_of((step - (NG - 1)) * LANES, LANES)
        return out_ref[0:16, pl.ds(dyn0, LANES)]

    def out_unit(n):
        w = OUW * LANES
        cols = slice(n * w, (n + 1) * w)
        rs, mrs = (jnp.concatenate([st_ref[k, n * OUW + u:n * OUW + u + 1, :]
                                    for u in range(OUW)], axis=1) for k in (5, 6))
        for r0 in range(0, D, OPR):
            x2 = acc_ref[r0:r0 + OPR, cols]
            o = x2 + ((x2 * rs - mrs) * _tile(fold_ref[r0:r0 + OPR, :], OUW)
                      + _tile(fold_ref[D + r0:D + r0 + OPR, :], OUW))
            out_ref[r0:r0 + OPR, cols] = o.astype(BF16)
        return after_out_stores().astype(F32)

    r = _rb(r) + 0.0
    bits = pltpu.bitcast(r, jnp.int32)
    mono = bits ^ ((bits >> 31) & jnp.int32(0x7FFFFFFF))
    tok = (lax.broadcasted_iota(jnp.int32, (NSL, LANES), 0) * LANES
           + lax.broadcasted_iota(jnp.int32, (NSL, LANES), 1))
    keyi = (((mono >> 16) + 32768) * S + (S - 1 - tok)) + jnp.int32(1 << 29)
    key = pltpu.bitcast(keyi, F32)

    row16 = lax.broadcasted_iota(jnp.int32, (16, LANES), 0)
    rowc = lax.broadcasted_iota(jnp.int32, (16, 1), 0)
    sel_slab, sel_off = [], []
    tie, nunit = None, 0
    xsel = jnp.zeros((16, D), F32)
    mbsel = jnp.zeros((16, 1), F32)
    rssel = jnp.zeros((16, 1), F32)
    ksel = jnp.zeros((16, 1), F32)
    for t in range(TOPC):
        kmax = jnp.max(jnp.max(key, axis=0, keepdims=True), axis=1, keepdims=True)
        hit = key == kmax
        key = jnp.where(hit, 0.0, key)
        pick = lambda z: jnp.sum(jnp.sum(jnp.where(hit, z, 0.0), axis=0, keepdims=True),
                                 axis=1, keepdims=True)
        mbsel = jnp.where(rowc == t, pick(mb), mbsel)
        rssel = jnp.where(rowc == t, pick(rs), rssel)
        for _ in range(TK_TIES.count(t)):
            tie = out_unit(nunit)
            nunit += 1
            key = jnp.where(never, tie, key)
        ksel = jnp.where(rowc == t, kmax, ksel)
        ki = pltpu.bitcast(kmax, jnp.int32)[0, 0]
        idx = (S - 1) - (ki & (S - 1))
        slab = idx >> 7
        off = idx & (LANES - 1)
        onehot = jnp.where((row16 == t) & (lane16 == off), 1.0, 0.0).astype(BF16)
        dslab = xb_ref[:, pl.ds(pl.multiple_of(slab * LANES, LANES), LANES)]
        xsel = xsel + lax.dot_general(onehot, pltpu.bitcast(dslab, BF16), _NT,
                                      preferred_element_type=F32)
        sel_slab.append(slab)
        sel_off.append(off)
    nsel = _rb(_rb(xsel - mbsel) * rssel)
    hsel = _rb(_rb(nsel * mb_ref[1, 0:1, :]) + mb_ref[0, 0:1, :])
    hi = ((pltpu.bitcast(ksel, jnp.int32) - jnp.int32(1 << 29)) // S - 32768) << 16
    rbits = hi ^ ((hi >> 31) & jnp.int32(0x7FFF0000))
    gate = _rb(_sigmoid(jnp.where(rowc < TOPC, pltpu.bitcast(rbits, F32), 0.0)))

    def out_copy(sl, r0, nr):
        c0 = pl.multiple_of(sl * LANES, LANES)
        return cp(out_ref.at[r0:r0 + nr, pl.ds(c0, LANES)],
                  out_hbm.at[r0:r0 + nr, pl.ds(c0, LANES)], S_O)

    fresh = []
    seen = jnp.int32(0)
    for t in range(TOPC):
        fresh.append(((seen >> sel_slab[t]) & 1) == 0)
        seen = seen | (1 << sel_slab[t])
    plain = [((seen >> sl) & 1) == 0 for sl in range(NSL)]

    for n in range(nunit, NSL // OUW):
        tie = out_unit(n)
    for sl in range(NSL):
        pl.when(plain[sl])(lambda sl=sl: out_copy(sl, 0, D).start())

    h0 = jnp.where(never, tie, hsel[:, 0:LANES])
    hs = jnp.concatenate([h0, hsel[:, LANES:]], axis=1).astype(BF16)
    gpre = _rb(jnp.dot(hs, wg_ref[...], preferred_element_type=F32))
    u = _rb(jnp.dot(hs, wu_ref[...], preferred_element_type=F32))
    a = (_rb(gpre * _sigmoid(gpre)) * u).astype(BF16)

    pieces = PIECES

    gb = mb_ref[2, 0:1, :]

    def down(r0, nr, tied):
        lhs = a
        if tied:
            a0 = jnp.where(never[0:8, :], pltpu.bitcast(after_out_stores(), U32),
                           pltpu.bitcast(a[:, TIEC:TIEC + LANES], U32))
            lhs = jnp.concatenate(([a[:, 0:TIEC]] if TIEC else []) + [pltpu.bitcast(a0, BF16)] + ([a[:, TIEC + LANES:]] if TIEC + LANES < FF else []), axis=1)
        y = jnp.dot(lhs, pltpu.bitcast(wd_ref[0:FF // 2, r0:r0 + nr], BF16),
                    preferred_element_type=F32)
        c = slice(r0, r0 + nr)
        return xsel[:, c] + gb[:, c] * (hsel[:, c] + y * gate)

    def patch(r0, nr, new):
        lane = lax.broadcasted_iota(jnp.int32, (nr // 2, LANES), 1)
        for t in range(TOPC):
            cols = pl.ds(pl.multiple_of(sel_slab[t] * LANES, LANES), LANES)
            old = pltpu.bitcast(out_ref[r0:r0 + nr, cols], U32)
            upd = pltpu.bitcast(_as_cols(new[t:t + 1, :]), U32)
            out_ref[r0:r0 + nr, cols] = pltpu.bitcast(jnp.where(lane == sel_off[t], upd, old), BF16)
        for t in range(TOPC):
            pl.when(fresh[t])(lambda t=t: out_copy(sel_slab[t], r0, nr).start())

    if DIST == 1:
        for n in range(len(pieces)):
            patch(*pieces[n], down(*pieces[n], n > 0))
    else:
        yts = [down(*pieces[0], False)]
        for n in range(len(pieces)):
            if n + 1 < len(pieces):
                yts.append(down(*pieces[n + 1], n > 0))
            patch(*pieces[n], yts[n])

    cp(out_ref, out_hbm, S_O).wait()


@jax.jit
def pallas_adaLN_cond__gqa_block_cached__moe_arch_mod__prompt_kernel(
    A_x: jax.Array,
    A_k_cache: jax.Array,
    A_v_cache: jax.Array,
    A_wq: jax.Array,
    A_wo: jax.Array,
    B_x: jax.Array,
    B_w_r: jax.Array,
    B_w_gate: jax.Array,
    B_w_up: jax.Array,
    B_w_down: jax.Array,
    c: jax.Array,
    w_mod: jax.Array,
):
    del B_x
    B, S, D = A_x.shape
    assert B == 1
    NG, SK = A_k_cache.shape[1], A_k_cache.shape[2]
    REP = HQ // NG
    FF = B_w_gate.shape[1]
    GW = REP * DH

    xt = A_x.reshape(S, D).T
    wot = A_wo.T
    wdt = B_w_down.T
    k = A_k_cache.reshape(NG, SK, DH)
    v = A_v_cache.reshape(NG, SK, DH)

    hbm = pl.BlockSpec(memory_space=pl.ANY)
    out_t = pl.pallas_call(
        functools.partial(_kernel, S=S, SK=SK, D=D, FF=FF, NG=NG, REP=REP),
        in_specs=[hbm] * 11,
        out_specs=hbm,
        out_shape=jax.ShapeDtypeStruct((D, S), BF16),
        scratch_shapes=[
            pltpu.VMEM((D, S), BF16),
            pltpu.VMEM((2, SK, DH), BF16),
            pltpu.VMEM((2, SK, DH), BF16),
            pltpu.VMEM((2, D, GW), BF16),
            pltpu.VMEM((2, D, GW), BF16),
            pltpu.VMEM((D,), BF16),
            pltpu.VMEM((1, D), BF16),
            pltpu.VMEM((D, 6 * D), BF16),
            pltpu.VMEM((D, FF), BF16),
            pltpu.VMEM((D, FF), BF16),
            pltpu.VMEM((D, FF + WT_W), BF16),
            pltpu.VMEM(((FF + WT_W) // 2, D), U32),
            pltpu.VMEM((D, S), BF16),
            pltpu.VMEM((6 * D, LANES), F32),
            pltpu.VMEM((8, 6 * D), F32),
            pltpu.VMEM((D, LANES), F32),
            pltpu.VMEM((2 * D, LANES), F32),
            pltpu.VMEM((3, 8, D), F32),
            pltpu.VMEM((16, D), BF16),
            pltpu.VMEM((8, LANES), F32),
            pltpu.VMEM((S // 2, D), U32),
            pltpu.VMEM((D, S), F32),
            pltpu.VMEM((D // 2, S), U32),
            pltpu.VMEM((7, S // LANES, LANES), F32),
            pltpu.SemaphoreType.DMA((N_SEMS,)),
        ],
        compiler_params=pltpu.CompilerParams(
            vmem_limit_bytes=100 * 1024 * 1024,
            disable_bounds_checks=True,
        ),
    )(xt, k, v, A_wq, wot, B_w_r, c, w_mod, B_w_gate, B_w_up, wdt)
    return out_t.T.reshape(B, S, D)
```

```python
import functools
import math

import jax
import jax.numpy as jnp
from jax import lax
import jax.experimental.pallas as pl
import jax.experimental.pallas.tpu as pltpu

F32 = jnp.float32
BF16 = jnp.bfloat16
U32 = jnp.uint32

HQ = 32
DH = 128
TOPC = 8
LN_EPS = 1e-5
BQ = 256
LANES = 128
HEAD = [0, 512, 768, 1024, 768, 512, 512, 768, 768, 640, 1280, 512, 640, 1280, 512, 0]
MODE = [2, 1, 2, 2, 0, 0, 0, 0, 0, 1, 2, 0, 0, 2, 1, 1]
QP_POS = [-1, -1, -1, -1, -1, 3, 18, -1]
OP_POS = [11, 15, 19, 24, 30, 31, 31, 31]
XCH = 4
DIST = 2
TIEC = 2048
PIECES = [(0, 128), (128, 128), (256, 128), (384, 128), (512, 64)]
OUW = 2
TK_TIES = [0, 1, 2, 3, 4, 5, 6]
OPR = 16
VB = [4, 5, 6, 7]
PK0 = 56
ZC = 1024
DBG_PREP = 1
PL = 4
PALL = 0
PT0 = 30000
PPER = 498
VA = 16
VG = 1
VPER = 450
VMARG = 300
PINPV = 0
PIV0 = 0
MT_W = 384
MT_R = 8
WT_W = 384
WT_R = 256
WT_TIE = 0
MOD_STEP = 4

_NT = (((1,), (1,)), ((), ()))

S_C = S_WMA = 0
S_WMB = S_WD = 1
S_WR = 2
S_WG = S_WU = 3
S_WQ0 = 4
S_X = 5
S_G = S_X + XCH
S_O = S_G + 2
N_SEMS = S_O + 1


def _rb(x):
    return x.astype(BF16).astype(F32)


def _sigmoid(x):
    return 1.0 / (1.0 + jnp.exp(-x))


def _ln_rows(mean, var):
    eps = _rb(jnp.full((1, 1), LN_EPS, F32))
    return _rb(mean), _rb(jnp.sqrt(_rb(_rb(var) + eps)))


def _tile(col, n):
    return jnp.concatenate([col] * n, axis=1)


def _as_cols(row):
    return jnp.broadcast_to(row, (LANES, row.shape[1])).astype(BF16).T


def _kernel(xt_hbm, k_hbm, v_hbm, wq_hbm, wot_hbm, wr_hbm, c_hbm, wmod_hbm,
            wg_hbm, wu_hbm, wdt_hbm,
            out_hbm,
            xt_ref, k_buf, v_buf, wq_buf, wot_buf, wqn_buf, wr_ref, c_ref, wmod_ref,
            wg_ref, wu_ref, wdt_ref, wd_ref, out_ref,
            modc_ref, mrow_ref, scc_ref, fold_ref, mb_ref, lhs_ref, rc_ref, h_ref, acc_ref, xb_ref, st_ref, hr_ref, ht_ref, bp_ref,
            sems,
            *, S, SK, D, FF, NG, REP):
    qscale = (DH ** -0.5) * math.log2(math.e)
    NB = S // BQ
    GW = REP * DH
    TCH = S // XCH
    MA = 2 * D
    NSL = S // LANES
    KM = D // LANES * LANES
    KR = D - KM

    def cp(src, dst, sem):
        return pltpu.make_async_copy(src, dst, sems.at[sem])

    def x_copy(i):
        cols = pl.ds(pl.multiple_of(i * TCH, TCH), TCH)
        return cp(xt_hbm.at[:, cols], xt_ref.at[:, cols], S_X + i)

    def group_copies(grp):
        slot = grp % 2
        nxt = jnp.minimum(grp + 1, NG - 1)
        cols = pl.ds(pl.multiple_of(grp * GW, GW), GW)
        return (cp(wq_hbm.at[:, cols], wq_buf.at[slot], S_G + slot),
                cp(k_hbm.at[grp], k_buf.at[slot], S_G + slot),
                cp(v_hbm.at[grp], v_buf.at[slot], S_G + slot),
                cp(wot_hbm.at[:, cols], wot_buf.at[slot], S_G + slot),
                cp(wq_hbm.at[KM:D, pl.ds(pl.multiple_of(nxt * GW, GW), GW)], wqn_buf.at[slot], S_G + slot))

    wq0_cp = lambda: cp(wq_hbm.at[KM:D, 0:GW], wqn_buf.at[2], S_WQ0)
    c_cp = lambda: cp(c_hbm, c_ref, S_C)
    wma_cp = lambda: cp(wmod_hbm.at[:, 0:MA], wmod_ref.at[:, 0:MA], S_WMA)
    wmb_cp = lambda: cp(wmod_hbm.at[:, MA:6 * D], wmod_ref.at[:, MA:6 * D], S_WMB)
    wr_cp = lambda: cp(wr_hbm, wr_ref, S_WR)
    wg_cp = lambda: cp(wg_hbm, wg_ref, S_WG)
    wu_cp = lambda: cp(wu_hbm, wu_ref, S_WU)
    wd_cp = lambda: cp(wdt_hbm, wdt_ref.at[:, 0:FF], S_WD)

    def modcol(i):
        return modc_ref[i * D:(i + 1) * D, :]

    def finish_mod(mod, col0):
        mod = _rb(mod)
        lane = lax.broadcasted_iota(jnp.int32, mod.shape, 1) + col0
        is_scale = ((lane >= D) & (lane < 2 * D)) | ((lane >= 4 * D) & (lane < 5 * D))
        return jnp.where(is_scale, _rb(1.0 + mod), mod)

    def prep_cols(w, k0, k1):
        for kk in range(k0, k1):
            bp_ref[kk * GW:(kk + 1) * GW, :] = _as_cols(w[kk:kk + 1, :]).astype(F32)

    wq0_cp().start()
    wma_cp().start()
    c_cp().start()
    for i in range(XCH):
        x_copy(i).start()
    for d in group_copies(0) + group_copies(1):
        d.start()
    wr_cp().start()
    acc_ref[:, 0:ZC] = jnp.zeros((D, ZC), F32)
    wq0_cp().wait()
    prep_cols(wqn_buf[2].astype(F32), 0, PK0)
    wma_cp().wait()
    c_cp().wait()
    c = c_ref[...].astype(F32)
    sc = _rb(c * _sigmoid(c))
    mod = jnp.dot(jnp.broadcast_to(sc, (8, D)).astype(BF16), wmod_ref[:, 0:MA],
                  preferred_element_type=F32)
    modc_ref[0:MA, :] = _as_cols(finish_mod(mod, 0)[0:1, :]).astype(F32)

    def ln1(i, carry):
        x_copy(i).wait()
        x = xt_ref[:, pl.ds(pl.multiple_of(i * TCH, TCH), TCH)].astype(F32)
        piv = x[0:1, :]
        d = x - piv
        md = jnp.mean(d, axis=0, keepdims=True)
        var = jnp.maximum(jnp.mean(d * d, axis=0, keepdims=True) - md * md, 0.0)
        mb, sd = _ln_rows(piv + md, var)
        rs = 1.0 / sd
        n = TCH // LANES
        ht = (x * rs - mb * rs) * _tile(modcol(1), n) + _tile(modcol(0), n)
        h_ref[pl.ds(pl.multiple_of(i * (TCH // 2), TCH // 2), TCH // 2), :] = pltpu.bitcast(
            ht.astype(BF16).T, U32)
        hr_ref[:, pl.ds(pl.multiple_of(i * TCH, TCH), TCH)] = _rb(ht[KM:D, :])
        return carry
    lax.fori_loop(0, XCH, ln1, 0)
    scc_ref[...] = _as_cols(sc).astype(F32)
    prep_cols(wqn_buf[2].astype(F32), PK0, KR)
    acc_ref[:, ZC:S] = jnp.zeros((D, S - ZC), F32)
    wdt_ref[:, FF:FF + WT_W] = jnp.zeros((D, WT_W), BF16)
    for n, j in enumerate(VB):
        for kk in range(KR):
            ht_ref[8 * kk:8 * kk + 8, n * BQ:(n + 1) * BQ] = jnp.broadcast_to(
                hr_ref[kk:kk + 1, j * BQ:(j + 1) * BQ], (8, BQ))

    def fold_modulation():
        sb, cb, gb = (mrow_ref[0:1, i * D:(i + 1) * D] for i in (3, 4, 5))
        for i, z in enumerate((sb, cb, gb)):
            mb_ref[i] = jnp.broadcast_to(z, (8, D))
        fold_ref[0:D, :] = modcol(5) * modcol(4)
        fold_ref[D:MA, :] = modcol(5) * modcol(3)
        wr = wr_ref[...].astype(F32).reshape(1, D)
        wc = wr * cb
        whi = _rb(wc)
        wlo = _rb(wc - whi)
        row = lax.broadcasted_iota(jnp.int32, (16, D), 0)
        lhs_ref[...] = jnp.where(row == 0, 1.0, jnp.where(row == 1, whi, jnp.where(
            row == 2, wlo, 0.0))).astype(BF16)
        rc_ref[0:1, :] = jnp.broadcast_to(jnp.sum(whi + wlo, axis=1, keepdims=True), (1, LANES))
        rc_ref[1:2, :] = jnp.broadcast_to(jnp.sum(wr * sb, axis=1, keepdims=True), (1, LANES))

    def group_step(step, carry):
        @pl.when(step == MOD_STEP)
        def _():
            wmb_cp().wait()
            wd_cp().wait()

        for d in group_copies(step):
            d.wait()

        slot = step % 2
        k = k_buf[slot]
        v = v_buf[slot]
        wq = wq_buf[slot]
        wot = wot_buf[slot]

        nev = lax.broadcasted_iota(jnp.int32, (8, BQ), 1) > step + BQ
        gates, qrem = [], {}
        gate = None
        for nb, j in enumerate(VB):
            res = []
            for n0 in range(0, GW, VA):
                acc = None
                for kk in range(KR):
                    a = ht_ref[8 * kk:8 * kk + 8, nb * BQ:(nb + 1) * BQ]
                    if gate is not None and kk % VG == 0:
                        a = jnp.where(nev, gate, a)
                    b = bp_ref[kk * GW + n0:kk * GW + n0 + VA, :]
                    t = _tile(b, BQ // LANES) * jnp.concatenate([a] * (VA // 8), axis=0)
                    acc = t if acc is None else acc + t
                    g0 = 8 * ((kk // VG) % (VA // 8))
                    g1 = 8 * ((kk // VG + 1) % (VA // 8))
                    gate = jnp.concatenate([acc[g0:g0 + 8, LANES:], acc[g1:g1 + 8, 0:LANES]], axis=1)
                res.append(acc)
                gates.append(gate)
            qrem[j] = jnp.concatenate(res, axis=0).T
        dues = [VMARG + (i + 1) * VPER for i in range(len(gates))]
        wn = wqn_buf[slot].astype(F32)
        for k0 in range(0, KR if DBG_PREP else 0, PL):
            r0 = k0 // 8 * 8
            blk = jnp.where(nev, gate, wn[r0:r0 + 8, :])
            gate = None
            for kk in range(k0, k0 + PL):
                last = _as_cols(blk[kk - r0:kk - r0 + 1, :]).astype(F32)
                bp_ref[kk * GW:(kk + 1) * GW, :] = last
                g = jnp.concatenate([last[GW - 8:GW], last[LANES - 8:LANES]], axis=1)
                gate = g if (gate is None or not PALL) else jnp.where(nev, gate, g)
            gates.append(gate)
            dues.append(PT0 + (k0 // PL + 1) * PPER)
        clock = [0]
        pinned = [0]

        def pin(x, final=False):
            due = len(gates) if final else sum(1 for t in dues if t <= clock[0])
            if due <= pinned[0]:
                return x
            pinned[0] = due
            g = pltpu.bitcast(gates[due - 1], U32)
            xu = pltpu.bitcast(x, U32)
            top = xu[0:8, 0:LANES]
            top = jnp.where(nev[:, 0:LANES], g[:, 0:LANES], jnp.where(nev[:, LANES:], g[:, LANES:], top))
            if xu.shape[1] > LANES:
                top = jnp.concatenate([top, xu[0:8, LANES:]], axis=1)
            return pltpu.bitcast(jnp.concatenate([top, xu[8:]], axis=0), BF16)

        def qproj(j):
            hb = pin(pltpu.bitcast(h_ref[j * (BQ // 2):(j + 1) * (BQ // 2), :], BF16))
            if j in VB:
                clock[0] += 512
                q2 = jnp.dot(hb[:, 0:KM], wq[0:KM], preferred_element_type=F32) + qrem[j]
            else:
                clock[0] += 640
                q2 = jnp.dot(hb, wq, preferred_element_type=F32)
            return (q2 * qscale).astype(BF16)

        def qk(ci, lo, hi):
            q = pin(qs[ci])
            clock[0] += (hi - lo) // 2
            return lax.dot_general(q, k[lo:hi], _NT, preferred_element_type=F32)

        def softmax_pv(s, mode):
            m = jnp.max(s, axis=1, keepdims=True)
            p = jnp.exp2(s - m)
            parts = [p[:, i * LANES:(i + 1) * LANES] for i in range(SK // LANES)]
            if mode == 2:
                lp = None
                for c in range(0, len(parts), 4):
                    t = (parts[c] + parts[c + 1]) + (parts[c + 2] + parts[c + 3])
                    lp = t if lp is None else lp + t
                    parts[c + 3] = jnp.where(lp < 0.0, lp, parts[c + 3])
                p = jnp.concatenate(parts, axis=1)
            pb = p.astype(BF16)
            if PINPV:
                pb = pin(pb)
            clock[0] += 1024
            o = jnp.dot(pb, v, preferred_element_type=F32)
            if mode == 0:
                l = jnp.sum(p, axis=1, keepdims=True)
            elif mode == 1:
                lp = functools.reduce(lambda x, y: x + y, parts)
                l = jnp.sum(jnp.where(lp < 0.0, o, lp), axis=1, keepdims=True)
            else:
                l = jnp.sum(lp, axis=1, keepdims=True)
            rl = pl.reciprocal(l, approx=True)
            rl = rl * (2.0 - l * rl)
            return (o * rl).astype(BF16)

        def oproj(j):
            o2 = jnp.concatenate([outs[REP * j + r] for r in range(REP)], axis=1)
            w = pin(wot, final=(j == NB - 1))
            clock[0] += 576
            acc_ref[:, j * BQ:(j + 1) * BQ] += lax.dot_general(w, o2, _NT, preferred_element_type=F32)

        qs, outs = {}, []

        def fill(pos):
            for j in range(NB):
                if QP_POS[j] == pos:
                    q2 = qproj(j)
                    for r in range(REP):
                        qs[REP * j + r] = q2[:, r * DH:(r + 1) * DH]
            for j in range(NB):
                if OP_POS[j] == pos:
                    oproj(j)

        NC = NB * REP
        assert (NG - MOD_STEP) * WT_W == FF
        wc0 = jnp.where(step >= MOD_STEP, (step - MOD_STEP) * WT_W, FF)
        never8 = lax.broadcasted_iota(jnp.int32, (8, LANES), 1) > step + LANES
        wtie = None
        for t0 in range(0, WT_W, LANES):
            for r0 in range(0, D, WT_R):
                r1 = min(r0 + WT_R, D)
                blk = pltpu.bitcast(wdt_ref[r0:r1, pl.ds(pl.multiple_of(wc0 + t0, LANES), LANES)], U32)
                if wtie is not None:
                    blk = jnp.concatenate([jnp.where(never8, wtie, blk[0:8]), blk[8:]], axis=0)
                tb = pltpu.bitcast(pltpu.bitcast(blk, BF16).T, U32)
                wd_ref[pl.ds(pl.multiple_of((wc0 + t0) // 2, LANES // 2), LANES // 2), r0:r1] = tb
                wtie = wd_ref[pl.ds(pl.multiple_of(wc0 // 2, LANES // 2), 8), 0:LANES]
        nms = 4 * D // MT_W
        assert nms * MT_W == 4 * D and MOD_STEP + nms < NG
        in_win = (step >= MOD_STEP) & (step < MOD_STEP + nms)
        mc0 = pl.multiple_of(jnp.where(in_win, MA + (step - MOD_STEP) * MT_W, 0), LANES)
        gate8 = pltpu.bitcast(wtie, F32)
        for r0 in range(0, D, MT_R):
            sc8 = scc_ref[r0:r0 + MT_R, :]
            sc8 = jnp.concatenate([jnp.where(never8, gate8, sc8[0:8])] + ([sc8[8:]] if MT_R > 8 else []), axis=0)
            t = wmod_ref[r0:r0 + MT_R, pl.ds(mc0, MT_W)].astype(F32) * _tile(sc8, MT_W // LANES)
            macc = t if r0 == 0 else macc + t
            gate8 = macc[0:8, 0:LANES]
        mrow = finish_mod(jnp.sum(macc, axis=0, keepdims=True), mc0)
        mrow_ref[0:1, pl.ds(mc0, MT_W)] = mrow
        modc_ref[pl.ds(mc0, MT_W), :] = _as_cols(mrow).astype(F32)
        wtie = pltpu.bitcast(modc_ref[0:8, :], U32)
        fill(-1)
        qt = pltpu.bitcast(qs[WT_TIE], U32)
        qs[WT_TIE] = pltpu.bitcast(
            jnp.concatenate([jnp.where(never8, wtie, qt[0:8]), qt[8:]], axis=0), BF16)
        s_head = None
        for ci in range(NC):
            lo = HEAD[ci - 1] if ci else 0
            s = qk(ci, lo, SK)
            if lo:
                s = jnp.concatenate([s_head, s], axis=1)
            fill(2 * ci)
            if HEAD[ci]:
                s_head = qk(ci + 1, 0, HEAD[ci])
            outs.append(softmax_pv(s, MODE[ci]))
            fill(2 * ci + 1)

        @pl.when(step + 2 < NG)
        def _():
            for d in group_copies(step + 2):
                d.start()

        @pl.when(step == 0)
        def _():
            wmb_cp().start()
            wg_cp().start()

        @pl.when(step == 1)
        def _():
            wu_cp().start()

        @pl.when(step == 2)
        def _():
            wd_cp().start()

        return step

    step = lax.fori_loop(0, NG, group_step, 0)

    wr_cp().wait()
    fold_modulation()
    for sl in range(NSL):
        cols = slice(sl * LANES, (sl + 1) * LANES)
        for r0 in range(0, D, LANES):
            r1 = min(r0 + LANES, D)
            x2 = xt_ref[r0:r1, cols].astype(F32) + modc_ref[MA + r0:MA + r1, :] * acc_ref[r0:r1, cols]
            acc_ref[r0:r1, cols] = x2
            xb = x2.astype(BF16)
            xb_ref[r0 // 2:r1 // 2, cols] = pltpu.bitcast(xb, U32)
            if r0 == 0:
                piv = jnp.mean(x2[PIV0:PIV0 + 8, :], axis=0, keepdims=True)
                st_ref[0, sl:sl + 1, :] = piv
            d = x2 - piv
            lhs = lhs_ref[:, r0:r1]
            t1 = jnp.dot(lhs, xb, preferred_element_type=F32)[0:8, :]
            t2 = jnp.dot(lhs, (d * d).astype(BF16), preferred_element_type=F32)[0:8, :]
            s1, s2 = (t1, t2) if r0 == 0 else (s1 + t1, s2 + t2)
        for n in range(3):
            st_ref[1 + n, sl:sl + 1, :] = s1[n:n + 1, :]
        st_ref[4, sl:sl + 1, :] = s2[0:1, :]

    wg_cp().wait()
    wu_cp().wait()

    mean = st_ref[1] * (1.0 / D)
    md = mean - st_ref[0]
    mb, sd = _ln_rows(mean, jnp.maximum(st_ref[4] * (1.0 / D) - md * md, 0.0))
    rs = 1.0 / sd
    st_ref[5] = rs
    st_ref[6] = mb * rs
    r = (st_ref[2] + st_ref[3] - mb * rc_ref[0:1, :]) * rs + rc_ref[1:2, :]

    lane16 = lax.broadcasted_iota(jnp.int32, (16, LANES), 1)
    never = lane16 > step + LANES

    def after_out_stores():
        dyn0 = pl.multiple_of((step - (NG - 1)) * LANES, LANES)
        return out_ref[0:16, pl.ds(dyn0, LANES)]

    def out_unit(n):
        w = OUW * LANES
        cols = slice(n * w, (n + 1) * w)
        rs, mrs = (jnp.concatenate([st_ref[k, n * OUW + u:n * OUW + u + 1, :]
                                    for u in range(OUW)], axis=1) for k in (5, 6))
        for r0 in range(0, D, OPR):
            x2 = acc_ref[r0:r0 + OPR, cols]
            o = x2 + ((x2 * rs - mrs) * _tile(fold_ref[r0:r0 + OPR, :], OUW)
                      + _tile(fold_ref[D + r0:D + r0 + OPR, :], OUW))
            out_ref[r0:r0 + OPR, cols] = o.astype(BF16)
        return after_out_stores().astype(F32)

    r = _rb(r) + 0.0
    bits = pltpu.bitcast(r, jnp.int32)
    mono = bits ^ ((bits >> 31) & jnp.int32(0x7FFFFFFF))
    tok = (lax.broadcasted_iota(jnp.int32, (NSL, LANES), 0) * LANES
           + lax.broadcasted_iota(jnp.int32, (NSL, LANES), 1))
    keyi = (((mono >> 16) + 32768) * S + (S - 1 - tok)) + jnp.int32(1 << 29)
    key = pltpu.bitcast(keyi, F32)

    row16 = lax.broadcasted_iota(jnp.int32, (16, LANES), 0)
    rowc = lax.broadcasted_iota(jnp.int32, (16, 1), 0)
    sel_slab, sel_off = [], []
    tie, nunit = None, 0
    xsel = jnp.zeros((16, D), F32)
    mbsel = jnp.zeros((16, 1), F32)
    rssel = jnp.zeros((16, 1), F32)
    ksel = jnp.zeros((16, 1), F32)
    for t in range(TOPC):
        kmax = jnp.max(jnp.max(key, axis=0, keepdims=True), axis=1, keepdims=True)
        hit = key == kmax
        key = jnp.where(hit, 0.0, key)
        pick = lambda z: jnp.sum(jnp.sum(jnp.where(hit, z, 0.0), axis=0, keepdims=True),
                                 axis=1, keepdims=True)
        mbsel = jnp.where(rowc == t, pick(mb), mbsel)
        rssel = jnp.where(rowc == t, pick(rs), rssel)
        for _ in range(TK_TIES.count(t)):
            tie = out_unit(nunit)
            nunit += 1
            key = jnp.where(never, tie, key)
        ksel = jnp.where(rowc == t, kmax, ksel)
        ki = pltpu.bitcast(kmax, jnp.int32)[0, 0]
        idx = (S - 1) - (ki & (S - 1))
        slab = idx >> 7
        off = idx & (LANES - 1)
        onehot = jnp.where((row16 == t) & (lane16 == off), 1.0, 0.0).astype(BF16)
        dslab = xb_ref[:, pl.ds(pl.multiple_of(slab * LANES, LANES), LANES)]
        xsel = xsel + lax.dot_general(onehot, pltpu.bitcast(dslab, BF16), _NT,
                                      preferred_element_type=F32)
        sel_slab.append(slab)
        sel_off.append(off)
    nsel = _rb(_rb(xsel - mbsel) * rssel)
    hsel = _rb(_rb(nsel * mb_ref[1, 0:1, :]) + mb_ref[0, 0:1, :])
    hi = ((pltpu.bitcast(ksel, jnp.int32) - jnp.int32(1 << 29)) // S - 32768) << 16
    rbits = hi ^ ((hi >> 31) & jnp.int32(0x7FFF0000))
    gate = _rb(_sigmoid(jnp.where(rowc < TOPC, pltpu.bitcast(rbits, F32), 0.0)))

    def out_copy(sl, r0, nr):
        c0 = pl.multiple_of(sl * LANES, LANES)
        return cp(out_ref.at[r0:r0 + nr, pl.ds(c0, LANES)],
                  out_hbm.at[r0:r0 + nr, pl.ds(c0, LANES)], S_O)

    fresh = []
    seen = jnp.int32(0)
    for t in range(TOPC):
        fresh.append(((seen >> sel_slab[t]) & 1) == 0)
        seen = seen | (1 << sel_slab[t])
    plain = [((seen >> sl) & 1) == 0 for sl in range(NSL)]

    for n in range(nunit, NSL // OUW):
        tie = out_unit(n)
    for sl in range(NSL):
        pl.when(plain[sl])(lambda sl=sl: out_copy(sl, 0, D).start())

    h0 = jnp.where(never, tie, hsel[:, 0:LANES])
    hs = jnp.concatenate([h0, hsel[:, LANES:]], axis=1).astype(BF16)
    gpre = _rb(jnp.dot(hs, wg_ref[...], preferred_element_type=F32))
    u = _rb(jnp.dot(hs, wu_ref[...], preferred_element_type=F32))
    a = (_rb(gpre * _sigmoid(gpre)) * u).astype(BF16)

    pieces = PIECES

    gb = mb_ref[2, 0:1, :]

    def down(r0, nr, tied):
        lhs = a
        if tied:
            a0 = jnp.where(never[0:8, :], pltpu.bitcast(after_out_stores(), U32),
                           pltpu.bitcast(a[:, TIEC:TIEC + LANES], U32))
            lhs = jnp.concatenate(([a[:, 0:TIEC]] if TIEC else []) + [pltpu.bitcast(a0, BF16)] + ([a[:, TIEC + LANES:]] if TIEC + LANES < FF else []), axis=1)
        y = jnp.dot(lhs, pltpu.bitcast(wd_ref[0:FF // 2, r0:r0 + nr], BF16),
                    preferred_element_type=F32)
        c = slice(r0, r0 + nr)
        return xsel[:, c] + gb[:, c] * (hsel[:, c] + y * gate)

    def patch(r0, nr, new):
        lane = lax.broadcasted_iota(jnp.int32, (nr // 2, LANES), 1)
        for t in range(TOPC):
            cols = pl.ds(pl.multiple_of(sel_slab[t] * LANES, LANES), LANES)
            old = pltpu.bitcast(out_ref[r0:r0 + nr, cols], U32)
            upd = pltpu.bitcast(_as_cols(new[t:t + 1, :]), U32)
            out_ref[r0:r0 + nr, cols] = pltpu.bitcast(jnp.where(lane == sel_off[t], upd, old), BF16)
        for t in range(TOPC):
            pl.when(fresh[t])(lambda t=t: out_copy(sel_slab[t], r0, nr).start())

    if DIST == 1:
        for n in range(len(pieces)):
            patch(*pieces[n], down(*pieces[n], n > 0))
    else:
        yts = [down(*pieces[0], False)]
        for n in range(len(pieces)):
            if n + 1 < len(pieces):
                yts.append(down(*pieces[n + 1], n > 0))
            patch(*pieces[n], yts[n])

    cp(out_ref, out_hbm, S_O).wait()


@jax.jit
def pallas_adaLN_cond__gqa_block_cached__moe_arch_mod__prompt_kernel(
    A_x: jax.Array,
    A_k_cache: jax.Array,
    A_v_cache: jax.Array,
    A_wq: jax.Array,
    A_wo: jax.Array,
    B_x: jax.Array,
    B_w_r: jax.Array,
    B_w_gate: jax.Array,
    B_w_up: jax.Array,
    B_w_down: jax.Array,
    c: jax.Array,
    w_mod: jax.Array,
):
    del B_x
    B, S, D = A_x.shape
    assert B == 1
    NG, SK = A_k_cache.shape[1], A_k_cache.shape[2]
    REP = HQ // NG
    FF = B_w_gate.shape[1]
    GW = REP * DH

    xt = A_x.reshape(S, D).T
    wot = A_wo.T
    wdt = B_w_down.T
    k = A_k_cache.reshape(NG, SK, DH)
    v = A_v_cache.reshape(NG, SK, DH)

    hbm = pl.BlockSpec(memory_space=pl.ANY)
    out_t = pl.pallas_call(
        functools.partial(_kernel, S=S, SK=SK, D=D, FF=FF, NG=NG, REP=REP),
        in_specs=[hbm] * 11,
        out_specs=hbm,
        out_shape=jax.ShapeDtypeStruct((D, S), BF16),
        scratch_shapes=[
            pltpu.VMEM((D, S), BF16),
            pltpu.VMEM((2, SK, DH), BF16),
            pltpu.VMEM((2, SK, DH), BF16),
            pltpu.VMEM((2, D, GW), BF16),
            pltpu.VMEM((2, D, GW), BF16),
            pltpu.VMEM((3, D % LANES, GW), BF16),
            pltpu.VMEM((D,), BF16),
            pltpu.VMEM((1, D), BF16),
            pltpu.VMEM((D, 6 * D), BF16),
            pltpu.VMEM((D, FF), BF16),
            pltpu.VMEM((D, FF), BF16),
            pltpu.VMEM((D, FF + WT_W), BF16),
            pltpu.VMEM(((FF + WT_W) // 2, D), U32),
            pltpu.VMEM((D, S), BF16),
            pltpu.VMEM((6 * D, LANES), F32),
            pltpu.VMEM((8, 6 * D), F32),
            pltpu.VMEM((D, LANES), F32),
            pltpu.VMEM((2 * D, LANES), F32),
            pltpu.VMEM((3, 8, D), F32),
            pltpu.VMEM((16, D), BF16),
            pltpu.VMEM((8, LANES), F32),
            pltpu.VMEM((S // 2, D), U32),
            pltpu.VMEM((D, S), F32),
            pltpu.VMEM((D // 2, S), U32),
            pltpu.VMEM((7, S // LANES, LANES), F32),
            pltpu.VMEM((D % LANES, S), F32),
            pltpu.VMEM((D % LANES * 8, len(VB) * BQ), F32),
            pltpu.VMEM((D % LANES * GW, LANES), F32),
            pltpu.SemaphoreType.DMA((N_SEMS,)),
        ],
        compiler_params=pltpu.CompilerParams(
            vmem_limit_bytes=100 * 1024 * 1024,
            disable_bounds_checks=True,
        ),
    )(xt, k, v, A_wq, wot, B_w_r, c, w_mod, B_w_gate, B_w_up, wdt)
    return out_t.T.reshape(B, S, D)
```

```python
import functools
import math

import jax
import jax.numpy as jnp
from jax import lax
import jax.experimental.pallas as pl
import jax.experimental.pallas.tpu as pltpu

F32 = jnp.float32
BF16 = jnp.bfloat16
U32 = jnp.uint32

HQ = 32
DH = 128
TOPC = 8
LN_EPS = 1e-5
BQ = 256
LANES = 128
HEAD = [0, 512, 768, 512, 768, 512, 512, 768, 1280, 768, 1536, 1024, 128, 1280, 512, 0]
MODE = [2, 1, 2, 1, 2, 0, 0, 0, 0, 1, 2, 0, 0, 0, 1, 1]
QP_POS = [-1, -1, -1, -1, -1, 3, 18, -1]
OP_POS = [12, 15, 19, 24, 30, 31, 31, 31]
XCH = 4
DIST = 2
TIEC = 2048
PIECES = [(0, 128), (128, 128), (256, 128), (384, 128), (512, 64)]
OUW = 2
TK_TIES = [0, 1, 2, 3, 4, 5, 6]
OPR = 16
VB = [4, 5, 6, 7]
PK0 = 56
ZC = 1024
DBG_PREP = 1
PL = 4
PALL = 0
PT0 = 30000
PPER = 498
VA = 16
VG = 1
ASSA = 1
BSSA = 0
VPER = 450
VMARG = 600
PINPV = 0
PIV0 = 0
MT_W = 384
MT_R = 8
WT_W = 384
WT_R = 256
WT_TIE = 0
MOD_STEP = 4

_NT = (((1,), (1,)), ((), ()))

S_C = S_WMA = 0
S_WMB = S_WD = 1
S_WR = 2
S_WG = S_WU = 3
S_WQ0 = 4
S_X = 5
S_G = S_X + XCH
S_O = S_G + 2
N_SEMS = S_O + 1


def _rb(x):
    return x.astype(BF16).astype(F32)


def _sigmoid(x):
    return 1.0 / (1.0 + jnp.exp(-x))


def _ln_rows(mean, var):
    eps = _rb(jnp.full((1, 1), LN_EPS, F32))
    return _rb(mean), _rb(jnp.sqrt(_rb(_rb(var) + eps)))


def _tile(col, n):
    return jnp.concatenate([col] * n, axis=1)


def _as_cols(row):
    return jnp.broadcast_to(row, (LANES, row.shape[1])).astype(BF16).T


def _kernel(xt_hbm, k_hbm, v_hbm, wq_hbm, wot_hbm, wr_hbm, c_hbm, wmod_hbm,
            wg_hbm, wu_hbm, wdt_hbm,
            out_hbm,
            xt_ref, k_buf, v_buf, wq_buf, wot_buf, wqn_buf, wr_ref, c_ref, wmod_ref,
            wg_ref, wu_ref, wdt_ref, wd_ref, out_ref,
            modc_ref, mrow_ref, scc_ref, fold_ref, mb_ref, lhs_ref, rc_ref, h_ref, acc_ref, xb_ref, st_ref, hr_ref, ht_ref, bp_ref,
            sems,
            *, S, SK, D, FF, NG, REP):
    qscale = (DH ** -0.5) * math.log2(math.e)
    NB = S // BQ
    GW = REP * DH
    TCH = S // XCH
    MA = 2 * D
    NSL = S // LANES
    KM = D // LANES * LANES
    KR = D - KM

    def cp(src, dst, sem):
        return pltpu.make_async_copy(src, dst, sems.at[sem])

    def x_copy(i):
        cols = pl.ds(pl.multiple_of(i * TCH, TCH), TCH)
        return cp(xt_hbm.at[:, cols], xt_ref.at[:, cols], S_X + i)

    def group_copies(grp):
        slot = grp % 2
        nxt = jnp.minimum(grp + 1, NG - 1)
        cols = pl.ds(pl.multiple_of(grp * GW, GW), GW)
        return (cp(wq_hbm.at[:, cols], wq_buf.at[slot], S_G + slot),
                cp(k_hbm.at[grp], k_buf.at[slot], S_G + slot),
                cp(v_hbm.at[grp], v_buf.at[slot], S_G + slot),
                cp(wot_hbm.at[:, cols], wot_buf.at[slot], S_G + slot),
                cp(wq_hbm.at[KM:D, pl.ds(pl.multiple_of(nxt * GW, GW), GW)], wqn_buf.at[slot], S_G + slot))

    wq0_cp = lambda: cp(wq_hbm.at[KM:D, 0:GW], wqn_buf.at[2], S_WQ0)
    c_cp = lambda: cp(c_hbm, c_ref, S_C)
    wma_cp = lambda: cp(wmod_hbm.at[:, 0:MA], wmod_ref.at[:, 0:MA], S_WMA)
    wmb_cp = lambda: cp(wmod_hbm.at[:, MA:6 * D], wmod_ref.at[:, MA:6 * D], S_WMB)
    wr_cp = lambda: cp(wr_hbm, wr_ref, S_WR)
    wg_cp = lambda: cp(wg_hbm, wg_ref, S_WG)
    wu_cp = lambda: cp(wu_hbm, wu_ref, S_WU)
    wd_cp = lambda: cp(wdt_hbm, wdt_ref.at[:, 0:FF], S_WD)

    def modcol(i):
        return modc_ref[i * D:(i + 1) * D, :]

    def finish_mod(mod, col0):
        mod = _rb(mod)
        lane = lax.broadcasted_iota(jnp.int32, mod.shape, 1) + col0
        is_scale = ((lane >= D) & (lane < 2 * D)) | ((lane >= 4 * D) & (lane < 5 * D))
        return jnp.where(is_scale, _rb(1.0 + mod), mod)

    def prep_cols(w, k0, k1):
        for kk in range(k0, k1):
            bp_ref[kk * GW:(kk + 1) * GW, :] = _as_cols(w[kk:kk + 1, :]).astype(F32)

    wq0_cp().start()
    wma_cp().start()
    c_cp().start()
    for i in range(XCH):
        x_copy(i).start()
    for d in group_copies(0) + group_copies(1):
        d.start()
    wr_cp().start()
    acc_ref[:, 0:ZC] = jnp.zeros((D, ZC), F32)
    wq0_cp().wait()
    prep_cols(wqn_buf[2].astype(F32), 0, PK0)
    wma_cp().wait()
    c_cp().wait()
    c = c_ref[...].astype(F32)
    sc = _rb(c * _sigmoid(c))
    mod = jnp.dot(jnp.broadcast_to(sc, (8, D)).astype(BF16), wmod_ref[:, 0:MA],
                  preferred_element_type=F32)
    modc_ref[0:MA, :] = _as_cols(finish_mod(mod, 0)[0:1, :]).astype(F32)

    def ln1(i, carry):
        x_copy(i).wait()
        x = xt_ref[:, pl.ds(pl.multiple_of(i * TCH, TCH), TCH)].astype(F32)
        piv = x[0:1, :]
        d = x - piv
        md = jnp.mean(d, axis=0, keepdims=True)
        var = jnp.maximum(jnp.mean(d * d, axis=0, keepdims=True) - md * md, 0.0)
        mb, sd = _ln_rows(piv + md, var)
        rs = 1.0 / sd
        n = TCH // LANES
        ht = (x * rs - mb * rs) * _tile(modcol(1), n) + _tile(modcol(0), n)
        h_ref[pl.ds(pl.multiple_of(i * (TCH // 2), TCH // 2), TCH // 2), :] = pltpu.bitcast(
            ht.astype(BF16).T, U32)
        hr_ref[:, pl.ds(pl.multiple_of(i * TCH, TCH), TCH)] = _rb(ht[KM:D, :])
        return carry
    lax.fori_loop(0, XCH, ln1, 0)
    scc_ref[...] = _as_cols(sc).astype(F32)
    prep_cols(wqn_buf[2].astype(F32), PK0, KR)
    acc_ref[:, ZC:S] = jnp.zeros((D, S - ZC), F32)
    wdt_ref[:, FF:FF + WT_W] = jnp.zeros((D, WT_W), BF16)
    for n, j in enumerate(VB):
        for kk in range(KR):
            ht_ref[8 * kk:8 * kk + 8, n * BQ:(n + 1) * BQ] = jnp.broadcast_to(
                hr_ref[kk:kk + 1, j * BQ:(j + 1) * BQ], (8, BQ))

    def fold_modulation():
        sb, cb, gb = (mrow_ref[0:1, i * D:(i + 1) * D] for i in (3, 4, 5))
        for i, z in enumerate((sb, cb, gb)):
            mb_ref[i] = jnp.broadcast_to(z, (8, D))
        fold_ref[0:D, :] = modcol(5) * modcol(4)
        fold_ref[D:MA, :] = modcol(5) * modcol(3)
        wr = wr_ref[...].astype(F32).reshape(1, D)
        wc = wr * cb
        whi = _rb(wc)
        wlo = _rb(wc - whi)
        row = lax.broadcasted_iota(jnp.int32, (16, D), 0)
        lhs_ref[...] = jnp.where(row == 0, 1.0, jnp.where(row == 1, whi, jnp.where(
            row == 2, wlo, 0.0))).astype(BF16)
        rc_ref[0:1, :] = jnp.broadcast_to(jnp.sum(whi + wlo, axis=1, keepdims=True), (1, LANES))
        rc_ref[1:2, :] = jnp.broadcast_to(jnp.sum(wr * sb, axis=1, keepdims=True), (1, LANES))

    def group_step(step, carry):
        @pl.when(step == MOD_STEP)
        def _():
            wmb_cp().wait()
            wd_cp().wait()

        for d in group_copies(step):
            d.wait()

        slot = step % 2
        k = k_buf[slot]
        v = v_buf[slot]
        wq = wq_buf[slot]
        wot = wot_buf[slot]

        nev = lax.broadcasted_iota(jnp.int32, (8, BQ), 1) > step + BQ
        gates, qrem, avals, bvals = [], {}, {}, {}
        nev2 = lax.broadcasted_iota(jnp.int32, (8, BQ), 1) > step + 2 * BQ
        nev3 = lax.broadcasted_iota(jnp.int32, (VA, LANES), 1) > step + 2 * BQ
        gate = None
        for nb, j in enumerate(VB):
            res = []
            for n0 in range(0, GW, VA):
                acc = None
                for kk in range(KR):
                    if n0 == 0 or not ASSA:
                        avals[kk] = ht_ref[8 * kk:8 * kk + 8, nb * BQ:(nb + 1) * BQ]
                        if ASSA:
                            avals[kk] = jnp.where(nev2, 0.0, avals[kk])
                    a = avals[kk]
                    if gate is not None and kk % VG == 0:
                        a = jnp.where(nev, gate, a)
                    if nb == 0 or not BSSA:
                        bvals[n0, kk] = bp_ref[kk * GW + n0:kk * GW + n0 + VA, :]
                        if BSSA:
                            bvals[n0, kk] = jnp.where(nev3, 0.0, bvals[n0, kk])
                    b = bvals[n0, kk]
                    t = _tile(b, BQ // LANES) * jnp.concatenate([a] * (VA // 8), axis=0)
                    acc = t if acc is None else acc + t
                    g0 = 8 * ((kk // VG) % (VA // 8))
                    g1 = 8 * ((kk // VG + 1) % (VA // 8))
                    gate = jnp.concatenate([acc[g0:g0 + 8, LANES:], acc[g1:g1 + 8, 0:LANES]], axis=1)
                res.append(acc)
                gates.append(gate)
            qrem[j] = jnp.concatenate(res, axis=0).T
        dues = [VMARG + (i + 1) * VPER for i in range(len(gates))]
        wn = wqn_buf[slot].astype(F32)
        for k0 in range(0, KR if DBG_PREP else 0, PL):
            r0 = k0 // 8 * 8
            blk = jnp.where(nev, gate, wn[r0:r0 + 8, :])
            gate = None
            for kk in range(k0, k0 + PL):
                last = _as_cols(blk[kk - r0:kk - r0 + 1, :]).astype(F32)
                bp_ref[kk * GW:(kk + 1) * GW, :] = last
                g = jnp.concatenate([last[GW - 8:GW], last[LANES - 8:LANES]], axis=1)
                gate = g if (gate is None or not PALL) else jnp.where(nev, gate, g)
            gates.append(gate)
            dues.append(PT0 + (k0 // PL + 1) * PPER)
        clock = [0]
        pinned = [0]

        def pin(x, final=False):
            due = len(gates) if final else sum(1 for t in dues if t <= clock[0])
            if due <= pinned[0]:
                return x
            pinned[0] = due
            g = pltpu.bitcast(gates[due - 1], U32)
            xu = pltpu.bitcast(x, U32)
            top = xu[0:8, 0:LANES]
            top = jnp.where(nev[:, 0:LANES], g[:, 0:LANES], jnp.where(nev[:, LANES:], g[:, LANES:], top))
            if xu.shape[1] > LANES:
                top = jnp.concatenate([top, xu[0:8, LANES:]], axis=1)
            return pltpu.bitcast(jnp.concatenate([top, xu[8:]], axis=0), BF16)

        def qproj(j):
            hb = pin(pltpu.bitcast(h_ref[j * (BQ // 2):(j + 1) * (BQ // 2), :], BF16))
            if j in VB:
                clock[0] += 512
                q2 = jnp.dot(hb[:, 0:KM], wq[0:KM], preferred_element_type=F32) + qrem[j]
            else:
                clock[0] += 640
                q2 = jnp.dot(hb, wq, preferred_element_type=F32)
            return (q2 * qscale).astype(BF16)

        def qk(ci, lo, hi):
            q = pin(qs[ci])
            clock[0] += (hi - lo) // 2
            return lax.dot_general(q, k[lo:hi], _NT, preferred_element_type=F32)

        def softmax_pv(s, mode):
            m = jnp.max(s, axis=1, keepdims=True)
            p = jnp.exp2(s - m)
            parts = [p[:, i * LANES:(i + 1) * LANES] for i in range(SK // LANES)]
            if mode == 2:
                lp = None
                for c in range(0, len(parts), 4):
                    t = (parts[c] + parts[c + 1]) + (parts[c + 2] + parts[c + 3])
                    lp = t if lp is None else lp + t
                    parts[c + 3] = jnp.where(lp < 0.0, lp, parts[c + 3])
                p = jnp.concatenate(parts, axis=1)
            pb = p.astype(BF16)
            if PINPV:
                pb = pin(pb)
            clock[0] += 1024
            o = jnp.dot(pb, v, preferred_element_type=F32)
            if mode == 0:
                l = jnp.sum(p, axis=1, keepdims=True)
            elif mode == 1:
                lp = functools.reduce(lambda x, y: x + y, parts)
                l = jnp.sum(jnp.where(lp < 0.0, o, lp), axis=1, keepdims=True)
            else:
                l = jnp.sum(lp, axis=1, keepdims=True)
            rl = pl.reciprocal(l, approx=True)
            rl = rl * (2.0 - l * rl)
            return (o * rl).astype(BF16)

        def oproj(j):
            o2 = jnp.concatenate([outs[REP * j + r] for r in range(REP)], axis=1)
            w = pin(wot, final=(j == NB - 1))
            clock[0] += 576
            acc_ref[:, j * BQ:(j + 1) * BQ] += lax.dot_general(w, o2, _NT, preferred_element_type=F32)

        qs, outs = {}, []

        def fill(pos):
            for j in range(NB):
                if QP_POS[j] == pos:
                    q2 = qproj(j)
                    for r in range(REP):
                        qs[REP * j + r] = q2[:, r * DH:(r + 1) * DH]
            for j in range(NB):
                if OP_POS[j] == pos:
                    oproj(j)

        NC = NB * REP
        assert (NG - MOD_STEP) * WT_W == FF
        wc0 = jnp.where(step >= MOD_STEP, (step - MOD_STEP) * WT_W, FF)
        never8 = lax.broadcasted_iota(jnp.int32, (8, LANES), 1) > step + LANES
        wtie = None
        for t0 in range(0, WT_W, LANES):
            for r0 in range(0, D, WT_R):
                r1 = min(r0 + WT_R, D)
                blk = pltpu.bitcast(wdt_ref[r0:r1, pl.ds(pl.multiple_of(wc0 + t0, LANES), LANES)], U32)
                if wtie is not None:
                    blk = jnp.concatenate([jnp.where(never8, wtie, blk[0:8]), blk[8:]], axis=0)
                tb = pltpu.bitcast(pltpu.bitcast(blk, BF16).T, U32)
                wd_ref[pl.ds(pl.multiple_of((wc0 + t0) // 2, LANES // 2), LANES // 2), r0:r1] = tb
                wtie = wd_ref[pl.ds(pl.multiple_of(wc0 // 2, LANES // 2), 8), 0:LANES]
        nms = 4 * D // MT_W
        assert nms * MT_W == 4 * D and MOD_STEP + nms < NG
        in_win = (step >= MOD_STEP) & (step < MOD_STEP + nms)
        mc0 = pl.multiple_of(jnp.where(in_win, MA + (step - MOD_STEP) * MT_W, 0), LANES)
        gate8 = pltpu.bitcast(wtie, F32)
        for r0 in range(0, D, MT_R):
            sc8 = scc_ref[r0:r0 + MT_R, :]
            sc8 = jnp.concatenate([jnp.where(never8, gate8, sc8[0:8])] + ([sc8[8:]] if MT_R > 8 else []), axis=0)
            t = wmod_ref[r0:r0 + MT_R, pl.ds(mc0, MT_W)].astype(F32) * _tile(sc8, MT_W // LANES)
            macc = t if r0 == 0 else macc + t
            gate8 = macc[0:8, 0:LANES]
        mrow = finish_mod(jnp.sum(macc, axis=0, keepdims=True), mc0)
        mrow_ref[0:1, pl.ds(mc0, MT_W)] = mrow
        modc_ref[pl.ds(mc0, MT_W), :] = _as_cols(mrow).astype(F32)
        wtie = pltpu.bitcast(modc_ref[0:8, :], U32)
        fill(-1)
        qt = pltpu.bitcast(qs[WT_TIE], U32)
        qs[WT_TIE] = pltpu.bitcast(
            jnp.concatenate([jnp.where(never8, wtie, qt[0:8]), qt[8:]], axis=0), BF16)
        s_head = None
        for ci in range(NC):
            lo = HEAD[ci - 1] if ci else 0
            s = qk(ci, lo, SK)
            if lo:
                s = jnp.concatenate([s_head, s], axis=1)
            fill(2 * ci)
            if HEAD[ci]:
                s_head = qk(ci + 1, 0, HEAD[ci])
            outs.append(softmax_pv(s, MODE[ci]))
            fill(2 * ci + 1)

        @pl.when(step + 2 < NG)
        def _():
            for d in group_copies(step + 2):
                d.start()

        @pl.when(step == 0)
        def _():
            wmb_cp().start()
            wg_cp().start()

        @pl.when(step == 1)
        def _():
            wu_cp().start()

        @pl.when(step == 2)
        def _():
            wd_cp().start()

        return step

    step = lax.fori_loop(0, NG, group_step, 0)

    wr_cp().wait()
    fold_modulation()
    for sl in range(NSL):
        cols = slice(sl * LANES, (sl + 1) * LANES)
        for r0 in range(0, D, LANES):
            r1 = min(r0 + LANES, D)
            x2 = xt_ref[r0:r1, cols].astype(F32) + modc_ref[MA + r0:MA + r1, :] * acc_ref[r0:r1, cols]
            acc_ref[r0:r1, cols] = x2
            xb = x2.astype(BF16)
            xb_ref[r0 // 2:r1 // 2, cols] = pltpu.bitcast(xb, U32)
            if r0 == 0:
                piv = jnp.mean(x2[PIV0:PIV0 + 8, :], axis=0, keepdims=True)
                st_ref[0, sl:sl + 1, :] = piv
            d = x2 - piv
            lhs = lhs_ref[:, r0:r1]
            t1 = jnp.dot(lhs, xb, preferred_element_type=F32)[0:8, :]
            t2 = jnp.dot(lhs, (d * d).astype(BF16), preferred_element_type=F32)[0:8, :]
            s1, s2 = (t1, t2) if r0 == 0 else (s1 + t1, s2 + t2)
        for n in range(3):
            st_ref[1 + n, sl:sl + 1, :] = s1[n:n + 1, :]
        st_ref[4, sl:sl + 1, :] = s2[0:1, :]

    wg_cp().wait()
    wu_cp().wait()

    mean = st_ref[1] * (1.0 / D)
    md = mean - st_ref[0]
    mb, sd = _ln_rows(mean, jnp.maximum(st_ref[4] * (1.0 / D) - md * md, 0.0))
    rs = 1.0 / sd
    st_ref[5] = rs
    st_ref[6] = mb * rs
    r = (st_ref[2] + st_ref[3] - mb * rc_ref[0:1, :]) * rs + rc_ref[1:2, :]

    lane16 = lax.broadcasted_iota(jnp.int32, (16, LANES), 1)
    never = lane16 > step + LANES

    def after_out_stores():
        dyn0 = pl.multiple_of((step - (NG - 1)) * LANES, LANES)
        return out_ref[0:16, pl.ds(dyn0, LANES)]

    def out_unit(n):
        w = OUW * LANES
        cols = slice(n * w, (n + 1) * w)
        rs, mrs = (jnp.concatenate([st_ref[k, n * OUW + u:n * OUW + u + 1, :]
                                    for u in range(OUW)], axis=1) for k in (5, 6))
        for r0 in range(0, D, OPR):
            x2 = acc_ref[r0:r0 + OPR, cols]
            o = x2 + ((x2 * rs - mrs) * _tile(fold_ref[r0:r0 + OPR, :], OUW)
                      + _tile(fold_ref[D + r0:D + r0 + OPR, :], OUW))
            out_ref[r0:r0 + OPR, cols] = o.astype(BF16)
        return after_out_stores().astype(F32)

    r = _rb(r) + 0.0
    bits = pltpu.bitcast(r, jnp.int32)
    mono = bits ^ ((bits >> 31) & jnp.int32(0x7FFFFFFF))
    tok = (lax.broadcasted_iota(jnp.int32, (NSL, LANES), 0) * LANES
           + lax.broadcasted_iota(jnp.int32, (NSL, LANES), 1))
    keyi = (((mono >> 16) + 32768) * S + (S - 1 - tok)) + jnp.int32(1 << 29)
    key = pltpu.bitcast(keyi, F32)

    row16 = lax.broadcasted_iota(jnp.int32, (16, LANES), 0)
    rowc = lax.broadcasted_iota(jnp.int32, (16, 1), 0)
    sel_slab, sel_off = [], []
    tie, nunit = None, 0
    xsel = jnp.zeros((16, D), F32)
    mbsel = jnp.zeros((16, 1), F32)
    rssel = jnp.zeros((16, 1), F32)
    ksel = jnp.zeros((16, 1), F32)
    for t in range(TOPC):
        kmax = jnp.max(jnp.max(key, axis=0, keepdims=True), axis=1, keepdims=True)
        hit = key == kmax
        key = jnp.where(hit, 0.0, key)
        pick = lambda z: jnp.sum(jnp.sum(jnp.where(hit, z, 0.0), axis=0, keepdims=True),
                                 axis=1, keepdims=True)
        mbsel = jnp.where(rowc == t, pick(mb), mbsel)
        rssel = jnp.where(rowc == t, pick(rs), rssel)
        for _ in range(TK_TIES.count(t)):
            tie = out_unit(nunit)
            nunit += 1
            key = jnp.where(never, tie, key)
        ksel = jnp.where(rowc == t, kmax, ksel)
        ki = pltpu.bitcast(kmax, jnp.int32)[0, 0]
        idx = (S - 1) - (ki & (S - 1))
        slab = idx >> 7
        off = idx & (LANES - 1)
        onehot = jnp.where((row16 == t) & (lane16 == off), 1.0, 0.0).astype(BF16)
        dslab = xb_ref[:, pl.ds(pl.multiple_of(slab * LANES, LANES), LANES)]
        xsel = xsel + lax.dot_general(onehot, pltpu.bitcast(dslab, BF16), _NT,
                                      preferred_element_type=F32)
        sel_slab.append(slab)
        sel_off.append(off)
    nsel = _rb(_rb(xsel - mbsel) * rssel)
    hsel = _rb(_rb(nsel * mb_ref[1, 0:1, :]) + mb_ref[0, 0:1, :])
    hi = ((pltpu.bitcast(ksel, jnp.int32) - jnp.int32(1 << 29)) // S - 32768) << 16
    rbits = hi ^ ((hi >> 31) & jnp.int32(0x7FFF0000))
    gate = _rb(_sigmoid(jnp.where(rowc < TOPC, pltpu.bitcast(rbits, F32), 0.0)))

    def out_copy(sl, r0, nr):
        c0 = pl.multiple_of(sl * LANES, LANES)
        return cp(out_ref.at[r0:r0 + nr, pl.ds(c0, LANES)],
                  out_hbm.at[r0:r0 + nr, pl.ds(c0, LANES)], S_O)

    fresh = []
    seen = jnp.int32(0)
    for t in range(TOPC):
        fresh.append(((seen >> sel_slab[t]) & 1) == 0)
        seen = seen | (1 << sel_slab[t])
    plain = [((seen >> sl) & 1) == 0 for sl in range(NSL)]

    for n in range(nunit, NSL // OUW):
        tie = out_unit(n)
    for sl in range(NSL):
        pl.when(plain[sl])(lambda sl=sl: out_copy(sl, 0, D).start())

    h0 = jnp.where(never, tie, hsel[:, 0:LANES])
    hs = jnp.concatenate([h0, hsel[:, LANES:]], axis=1).astype(BF16)
    gpre = _rb(jnp.dot(hs, wg_ref[...], preferred_element_type=F32))
    u = _rb(jnp.dot(hs, wu_ref[...], preferred_element_type=F32))
    a = (_rb(gpre * _sigmoid(gpre)) * u).astype(BF16)

    pieces = PIECES

    gb = mb_ref[2, 0:1, :]

    def down(r0, nr, tied):
        lhs = a
        if tied:
            a0 = jnp.where(never[0:8, :], pltpu.bitcast(after_out_stores(), U32),
                           pltpu.bitcast(a[:, TIEC:TIEC + LANES], U32))
            lhs = jnp.concatenate(([a[:, 0:TIEC]] if TIEC else []) + [pltpu.bitcast(a0, BF16)] + ([a[:, TIEC + LANES:]] if TIEC + LANES < FF else []), axis=1)
        y = jnp.dot(lhs, pltpu.bitcast(wd_ref[0:FF // 2, r0:r0 + nr], BF16),
                    preferred_element_type=F32)
        c = slice(r0, r0 + nr)
        return xsel[:, c] + gb[:, c] * (hsel[:, c] + y * gate)

    def patch(r0, nr, new):
        lane = lax.broadcasted_iota(jnp.int32, (nr // 2, LANES), 1)
        for t in range(TOPC):
            cols = pl.ds(pl.multiple_of(sel_slab[t] * LANES, LANES), LANES)
            old = pltpu.bitcast(out_ref[r0:r0 + nr, cols], U32)
            upd = pltpu.bitcast(_as_cols(new[t:t + 1, :]), U32)
            out_ref[r0:r0 + nr, cols] = pltpu.bitcast(jnp.where(lane == sel_off[t], upd, old), BF16)
        for t in range(TOPC):
            pl.when(fresh[t])(lambda t=t: out_copy(sel_slab[t], r0, nr).start())

    if DIST == 1:
        for n in range(len(pieces)):
            patch(*pieces[n], down(*pieces[n], n > 0))
    else:
        yts = [down(*pieces[0], False)]
        for n in range(len(pieces)):
            if n + 1 < len(pieces):
                yts.append(down(*pieces[n + 1], n > 0))
            patch(*pieces[n], yts[n])

    cp(out_ref, out_hbm, S_O).wait()


@jax.jit
def pallas_adaLN_cond__gqa_block_cached__moe_arch_mod__prompt_kernel(
    A_x: jax.Array,
    A_k_cache: jax.Array,
    A_v_cache: jax.Array,
    A_wq: jax.Array,
    A_wo: jax.Array,
    B_x: jax.Array,
    B_w_r: jax.Array,
    B_w_gate: jax.Array,
    B_w_up: jax.Array,
    B_w_down: jax.Array,
    c: jax.Array,
    w_mod: jax.Array,
):
    del B_x
    B, S, D = A_x.shape
    assert B == 1
    NG, SK = A_k_cache.shape[1], A_k_cache.shape[2]
    REP = HQ // NG
    FF = B_w_gate.shape[1]
    GW = REP * DH

    xt = A_x.reshape(S, D).T
    wot = A_wo.T
    wdt = B_w_down.T
    k = A_k_cache.reshape(NG, SK, DH)
    v = A_v_cache.reshape(NG, SK, DH)

    hbm = pl.BlockSpec(memory_space=pl.ANY)
    out_t = pl.pallas_call(
        functools.partial(_kernel, S=S, SK=SK, D=D, FF=FF, NG=NG, REP=REP),
        in_specs=[hbm] * 11,
        out_specs=hbm,
        out_shape=jax.ShapeDtypeStruct((D, S), BF16),
        scratch_shapes=[
            pltpu.VMEM((D, S), BF16),
            pltpu.VMEM((2, SK, DH), BF16),
            pltpu.VMEM((2, SK, DH), BF16),
            pltpu.VMEM((2, D, GW), BF16),
            pltpu.VMEM((2, D, GW), BF16),
            pltpu.VMEM((3, D % LANES, GW), BF16),
            pltpu.VMEM((D,), BF16),
            pltpu.VMEM((1, D), BF16),
            pltpu.VMEM((D, 6 * D), BF16),
            pltpu.VMEM((D, FF), BF16),
            pltpu.VMEM((D, FF), BF16),
            pltpu.VMEM((D, FF + WT_W), BF16),
            pltpu.VMEM(((FF + WT_W) // 2, D), U32),
            pltpu.VMEM((D, S), BF16),
            pltpu.VMEM((6 * D, LANES), F32),
            pltpu.VMEM((8, 6 * D), F32),
            pltpu.VMEM((D, LANES), F32),
            pltpu.VMEM((2 * D, LANES), F32),
            pltpu.VMEM((3, 8, D), F32),
            pltpu.VMEM((16, D), BF16),
            pltpu.VMEM((8, LANES), F32),
            pltpu.VMEM((S // 2, D), U32),
            pltpu.VMEM((D, S), F32),
            pltpu.VMEM((D // 2, S), U32),
            pltpu.VMEM((7, S // LANES, LANES), F32),
            pltpu.VMEM((D % LANES, S), F32),
            pltpu.VMEM((D % LANES * 8, len(VB) * BQ), F32),
            pltpu.VMEM((D % LANES * GW, LANES), F32),
            pltpu.SemaphoreType.DMA((N_SEMS,)),
        ],
        compiler_params=pltpu.CompilerParams(
            vmem_limit_bytes=100 * 1024 * 1024,
            disable_bounds_checks=True,
        ),
    )(xt, k, v, A_wq, wot, B_w_r, c, w_mod, B_w_gate, B_w_up, wdt)
    return out_t.T.reshape(B, S, D)
```

```python
import functools
import math

import jax
import jax.numpy as jnp
from jax import lax
import jax.experimental.pallas as pl
import jax.experimental.pallas.tpu as pltpu

F32 = jnp.float32
BF16 = jnp.bfloat16
U32 = jnp.uint32

HQ = 32
DH = 128
TOPC = 8
LN_EPS = 1e-5
BQ = 256
LANES = 128
XCH = 4
MOD_STEP = 4

HEAD = [0, 512, 512, 512, 768, 512, 512, 768, 1280, 768, 1536, 1024, 128, 1280, 512, 0]
MODE = [2, 1, 2, 1, 2, 0, 1, 2, 1, 1, 2, 0, 0, 0, 0, 1]
QP_POS = [-1, -1, -1, -1, -1, 3, -1, -1]
OP_POS = [12, 20, 19, 24, 30, 31, 31, 31]
VB = [4, 5, 6, 7]
VA = 16
VG = 1
VPER = 450
VMARG = 600
PL = 4
PT0 = 29959
PPER = 502
WT_W = 384
WT_R = 256
WT_TIE = 0
MT_W = 384
MT_R = 8
PK0 = 56
ZC = 1024
OUW = 2
OPR = 16
TK_TIES = [0, 1, 2, 3, 4, 5, 6]
PIECES = [(0, 128), (128, 128), (256, 128), (384, 128), (512, 64)]
TIEC = 2048

_NT = (((1,), (1,)), ((), ()))

S_C = S_WMA = 0
S_WMB = S_WD = 1
S_WR = 2
S_WG = S_WU = 3
S_WQ0 = 4
S_X = 5
S_G = S_X + XCH
S_O = S_G + 2
N_SEMS = S_O + 1


def _rb(x):
    return x.astype(BF16).astype(F32)


def _sigmoid(x):
    return 1.0 / (1.0 + jnp.exp(-x))


def _ln_rows(mean, var):
    eps = _rb(jnp.full((1, 1), LN_EPS, F32))
    return _rb(mean), _rb(jnp.sqrt(_rb(_rb(var) + eps)))


def _tile(col, n):
    return jnp.concatenate([col] * n, axis=1)


def _as_cols(row):
    return jnp.broadcast_to(row, (LANES, row.shape[1])).astype(BF16).T


def _kernel(xt_hbm, k_hbm, v_hbm, wq_hbm, wot_hbm, wr_hbm, c_hbm, wmod_hbm,
            wg_hbm, wu_hbm, wdt_hbm,
            out_hbm,
            xt_ref, k_buf, v_buf, wq_buf, wot_buf, wqn_buf, wr_ref, c_ref, wmod_ref,
            wg_ref, wu_ref, wdt_ref, wd_ref, out_ref,
            modc_ref, mrow_ref, scc_ref, fold_ref, mb_ref, lhs_ref, rc_ref, h_ref, acc_ref, xb_ref, st_ref, hr_ref, ht_ref, bp_ref, rem_ref, gate_ref,
            sems,
            *, S, SK, D, FF, NG, REP):
    qscale = (DH ** -0.5) * math.log2(math.e)
    NB = S // BQ
    GW = REP * DH
    TCH = S // XCH
    MA = 2 * D
    NSL = S // LANES
    KM = D // LANES * LANES
    KR = D - KM

    def cp(src, dst, sem):
        return pltpu.make_async_copy(src, dst, sems.at[sem])

    def x_copy(i):
        cols = pl.ds(pl.multiple_of(i * TCH, TCH), TCH)
        return cp(xt_hbm.at[:, cols], xt_ref.at[:, cols], S_X + i)

    def group_copies(grp):
        slot = grp % 2
        nxt = jnp.minimum(grp + 1, NG - 1)
        cols = pl.ds(pl.multiple_of(grp * GW, GW), GW)
        return (cp(wq_hbm.at[:, cols], wq_buf.at[slot], S_G + slot),
                cp(k_hbm.at[grp], k_buf.at[slot], S_G + slot),
                cp(v_hbm.at[grp], v_buf.at[slot], S_G + slot),
                cp(wot_hbm.at[:, cols], wot_buf.at[slot], S_G + slot),
                cp(wq_hbm.at[KM:D, pl.ds(pl.multiple_of(nxt * GW, GW), GW)], wqn_buf.at[slot], S_G + slot))

    wq0_cp = lambda: cp(wq_hbm.at[KM:D, 0:GW], wqn_buf.at[2], S_WQ0)
    c_cp = lambda: cp(c_hbm, c_ref, S_C)
    wma_cp = lambda: cp(wmod_hbm.at[:, 0:MA], wmod_ref.at[:, 0:MA], S_WMA)
    wmb_cp = lambda: cp(wmod_hbm.at[:, MA:6 * D], wmod_ref.at[:, MA:6 * D], S_WMB)
    wr_cp = lambda: cp(wr_hbm, wr_ref, S_WR)
    wg_cp = lambda: cp(wg_hbm, wg_ref, S_WG)
    wu_cp = lambda: cp(wu_hbm, wu_ref, S_WU)
    wd_cp = lambda: cp(wdt_hbm, wdt_ref.at[:, 0:FF], S_WD)

    def modcol(i):
        return modc_ref[i * D:(i + 1) * D, :]

    def finish_mod(mod, col0):
        mod = _rb(mod)
        lane = lax.broadcasted_iota(jnp.int32, mod.shape, 1) + col0
        is_scale = ((lane >= D) & (lane < 2 * D)) | ((lane >= 4 * D) & (lane < 5 * D))
        return jnp.where(is_scale, _rb(1.0 + mod), mod)

    def prep_cols(w, k0, k1):
        for kk in range(k0, k1):
            bp_ref[kk] = _as_cols(w[kk:kk + 1, :]).astype(F32)

    wq0_cp().start()
    wma_cp().start()
    c_cp().start()
    for i in range(XCH):
        x_copy(i).start()
    for d in group_copies(0) + group_copies(1):
        d.start()
    wr_cp().start()
    acc_ref[:, 0:ZC] = jnp.zeros((D, ZC), F32)
    wq0_cp().wait()
    prep_cols(wqn_buf[2].astype(F32), 0, PK0)
    wma_cp().wait()
    c_cp().wait()
    c = c_ref[...].astype(F32)
    sc = _rb(c * _sigmoid(c))
    mod = jnp.dot(jnp.broadcast_to(sc, (8, D)).astype(BF16), wmod_ref[:, 0:MA],
                  preferred_element_type=F32)
    modc_ref[0:MA, :] = _as_cols(finish_mod(mod, 0)[0:1, :]).astype(F32)

    def ln1(i, carry):
        x_copy(i).wait()
        x = xt_ref[:, pl.ds(pl.multiple_of(i * TCH, TCH), TCH)].astype(F32)
        piv = x[0:1, :]
        d = x - piv
        md = jnp.mean(d, axis=0, keepdims=True)
        var = jnp.maximum(jnp.mean(d * d, axis=0, keepdims=True) - md * md, 0.0)
        mb, sd = _ln_rows(piv + md, var)
        rs = 1.0 / sd
        n = TCH // LANES
        ht = (x * rs - mb * rs) * _tile(modcol(1), n) + _tile(modcol(0), n)
        h_ref[pl.ds(pl.multiple_of(i * (TCH // 2), TCH // 2), TCH // 2), :] = pltpu.bitcast(
            ht.astype(BF16).T, U32)
        hr_ref[:, pl.ds(pl.multiple_of(i * TCH, TCH), TCH)] = _rb(ht[KM:D, :])
        return carry
    lax.fori_loop(0, XCH, ln1, 0)
    scc_ref[...] = _as_cols(sc).astype(F32)
    prep_cols(wqn_buf[2].astype(F32), PK0, KR)
    acc_ref[:, ZC:S] = jnp.zeros((D, S - ZC), F32)
    wdt_ref[:, FF:FF + WT_W] = jnp.zeros((D, WT_W), BF16)
    for n, j in enumerate(VB):
        for kk in range(KR):
            ht_ref[n, 8 * kk:8 * kk + 8, :] = jnp.broadcast_to(
                hr_ref[kk:kk + 1, j * BQ:(j + 1) * BQ], (8, BQ))

    def fold_modulation():
        sb, cb, gb = (mrow_ref[0:1, i * D:(i + 1) * D] for i in (3, 4, 5))
        for i, z in enumerate((sb, cb, gb)):
            mb_ref[i] = jnp.broadcast_to(z, (8, D))
        fold_ref[0:D, :] = modcol(5) * modcol(4)
        fold_ref[D:MA, :] = modcol(5) * modcol(3)
        wr = wr_ref[...].astype(F32).reshape(1, D)
        wc = wr * cb
        whi = _rb(wc)
        wlo = _rb(wc - whi)
        row = lax.broadcasted_iota(jnp.int32, (16, D), 0)
        lhs_ref[...] = jnp.where(row == 0, 1.0, jnp.where(row == 1, whi, jnp.where(
            row == 2, wlo, 0.0))).astype(BF16)
        rc_ref[0:1, :] = jnp.broadcast_to(jnp.sum(whi + wlo, axis=1, keepdims=True), (1, LANES))
        rc_ref[1:2, :] = jnp.broadcast_to(jnp.sum(wr * sb, axis=1, keepdims=True), (1, LANES))

    def group_step(step, carry):
        @pl.when(step == MOD_STEP)
        def _():
            wmb_cp().wait()
            wd_cp().wait()

        for d in group_copies(step):
            d.wait()

        slot = step % 2
        k = k_buf[slot]
        v = v_buf[slot]
        wq = wq_buf[slot]
        wot = wot_buf[slot]

        nev = lax.broadcasted_iota(jnp.int32, (8, BQ), 1) > step + BQ
        assert VA == 16 and BQ == 2 * LANES
        npb = GW // VA

        def link(i, gate):
            av = ht_ref[i // npb]
            bv = bp_ref[:, pl.ds(pl.multiple_of((i % npb) * VA, VA), VA), :]
            bv = jnp.concatenate([bv, bv], axis=2)
            acc = None
            for kk in range(KR):
                a = av[8 * kk:8 * kk + 8]
                if kk % VG == 0:
                    a = jnp.where(nev, gate, a)
                t = bv[kk] * jnp.concatenate([a, a], axis=0)
                acc = t if acc is None else acc + t
                g0 = 8 * (kk // VG % 2)
                g1 = 8 - g0
                gate = jnp.concatenate([acc[g0:g0 + 8, LANES:], acc[g1:g1 + 8, 0:LANES]], axis=1)
            rem_ref[pl.ds(pl.multiple_of(i * VA, VA), VA), :] = acc
            gate_ref[i] = gate
            return gate

        gate = lax.fori_loop(0, len(VB) * npb, link, jnp.zeros((8, BQ), F32), unroll=True)
        gates = [functools.partial(lambda i: gate_ref[i], i) for i in range(len(VB) * npb)]
        qrem = {j: rem_ref[nb * GW:(nb + 1) * GW, :].T for nb, j in enumerate(VB)}
        dues = [VMARG + (i + 1) * VPER for i in range(len(gates))]
        wn = wqn_buf[slot].astype(F32)
        for k0 in range(0, KR, PL):
            r0 = k0 // 8 * 8
            blk = jnp.where(nev, gate, wn[r0:r0 + 8, :])
            for kk in range(k0, k0 + PL):
                last = _as_cols(blk[kk - r0:kk - r0 + 1, :]).astype(F32)
                bp_ref[kk] = last
            gate = jnp.concatenate([last[GW - 8:GW], last[LANES - 8:LANES]], axis=1)
            gates.append(functools.partial(lambda g: g, gate))
            dues.append(PT0 + (k0 // PL + 1) * PPER)
        clock = [0]
        pinned = [0]

        def pin(x, final=False):
            due = len(gates) if final else sum(1 for t in dues if t <= clock[0])
            if due <= pinned[0]:
                return x
            pinned[0] = due
            g = pltpu.bitcast(gates[due - 1](), U32)
            xu = pltpu.bitcast(x, U32)
            top = xu[0:8, 0:LANES]
            top = jnp.where(nev[:, 0:LANES], g[:, 0:LANES], jnp.where(nev[:, LANES:], g[:, LANES:], top))
            if xu.shape[1] > LANES:
                top = jnp.concatenate([top, xu[0:8, LANES:]], axis=1)
            return pltpu.bitcast(jnp.concatenate([top, xu[8:]], axis=0), BF16)

        def qproj(j):
            hb = pin(pltpu.bitcast(h_ref[j * (BQ // 2):(j + 1) * (BQ // 2), :], BF16))
            if j in VB:
                clock[0] += 512
                q2 = jnp.dot(hb[:, 0:KM], wq[0:KM], preferred_element_type=F32) + qrem[j]
            else:
                clock[0] += 640
                q2 = jnp.dot(hb, wq, preferred_element_type=F32)
            return (q2 * qscale).astype(BF16)

        def qk(ci, lo, hi):
            q = pin(qs[ci])
            clock[0] += (hi - lo) // 2
            return lax.dot_general(q, k[lo:hi], _NT, preferred_element_type=F32)

        def softmax_pv(s, mode):
            m = jnp.max(s, axis=1, keepdims=True)
            p = jnp.exp2(s - m)
            parts = [p[:, i * LANES:(i + 1) * LANES] for i in range(SK // LANES)]
            if mode == 2:
                lp = None
                for c in range(0, len(parts), 4):
                    t = (parts[c] + parts[c + 1]) + (parts[c + 2] + parts[c + 3])
                    lp = t if lp is None else lp + t
                    parts[c + 3] = jnp.where(lp < 0.0, lp, parts[c + 3])
                p = jnp.concatenate(parts, axis=1)
            clock[0] += SK // 2
            o = jnp.dot(p.astype(BF16), v, preferred_element_type=F32)
            if mode == 0:
                l = jnp.sum(p, axis=1, keepdims=True)
            elif mode == 1:
                lp = functools.reduce(lambda x, y: x + y, parts)
                l = jnp.sum(jnp.where(lp < 0.0, o, lp), axis=1, keepdims=True)
            else:
                l = jnp.sum(lp, axis=1, keepdims=True)
            rl = pl.reciprocal(l, approx=True)
            rl = rl * (2.0 - l * rl)
            return (o * rl).astype(BF16)

        def oproj(j):
            o2 = jnp.concatenate([outs[REP * j + r] for r in range(REP)], axis=1)
            w = pin(wot, final=(j == NB - 1))
            clock[0] += 576
            acc_ref[:, j * BQ:(j + 1) * BQ] += lax.dot_general(w, o2, _NT, preferred_element_type=F32)

        qs, outs = {}, []

        def fill(pos):
            for j in range(NB):
                if QP_POS[j] == pos:
                    q2 = qproj(j)
                    for r in range(REP):
                        qs[REP * j + r] = q2[:, r * DH:(r + 1) * DH]
            for j in range(NB):
                if OP_POS[j] == pos:
                    oproj(j)

        NC = NB * REP
        assert (NG - MOD_STEP) * WT_W == FF
        wc0 = jnp.where(step >= MOD_STEP, (step - MOD_STEP) * WT_W, FF)
        never8 = lax.broadcasted_iota(jnp.int32, (8, LANES), 1) > step + LANES
        wtie = None
        for t0 in range(0, WT_W, LANES):
            for r0 in range(0, D, WT_R):
                r1 = min(r0 + WT_R, D)
                blk = pltpu.bitcast(wdt_ref[r0:r1, pl.ds(pl.multiple_of(wc0 + t0, LANES), LANES)], U32)
                if wtie is not None:
                    blk = jnp.concatenate([jnp.where(never8, wtie, blk[0:8]), blk[8:]], axis=0)
                tb = pltpu.bitcast(pltpu.bitcast(blk, BF16).T, U32)
                wd_ref[pl.ds(pl.multiple_of((wc0 + t0) // 2, LANES // 2), LANES // 2), r0:r1] = tb
                wtie = wd_ref[pl.ds(pl.multiple_of(wc0 // 2, LANES // 2), 8), 0:LANES]
        nms = 4 * D // MT_W
        assert nms * MT_W == 4 * D and MOD_STEP + nms < NG
        in_win = (step >= MOD_STEP) & (step < MOD_STEP + nms)
        mc0 = pl.multiple_of(jnp.where(in_win, MA + (step - MOD_STEP) * MT_W, 0), LANES)
        gate8 = pltpu.bitcast(wtie, F32)
        for r0 in range(0, D, MT_R):
            sc8 = scc_ref[r0:r0 + MT_R, :]
            sc8 = jnp.concatenate([jnp.where(never8, gate8, sc8[0:8])] + ([sc8[8:]] if MT_R > 8 else []), axis=0)
            t = wmod_ref[r0:r0 + MT_R, pl.ds(mc0, MT_W)].astype(F32) * _tile(sc8, MT_W // LANES)
            macc = t if r0 == 0 else macc + t
            gate8 = macc[0:8, 0:LANES]
        mrow = finish_mod(jnp.sum(macc, axis=0, keepdims=True), mc0)
        mrow_ref[0:1, pl.ds(mc0, MT_W)] = mrow
        modc_ref[pl.ds(mc0, MT_W), :] = _as_cols(mrow).astype(F32)
        wtie = pltpu.bitcast(modc_ref[0:8, :], U32)
        fill(-1)
        qt = pltpu.bitcast(qs[WT_TIE], U32)
        qs[WT_TIE] = pltpu.bitcast(
            jnp.concatenate([jnp.where(never8, wtie, qt[0:8]), qt[8:]], axis=0), BF16)
        s_head = None
        for ci in range(NC):
            lo = HEAD[ci - 1] if ci else 0
            s = qk(ci, lo, SK)
            if lo:
                s = jnp.concatenate([s_head, s], axis=1)
            fill(2 * ci)
            if HEAD[ci]:
                s_head = qk(ci + 1, 0, HEAD[ci])
            outs.append(softmax_pv(s, MODE[ci]))
            fill(2 * ci + 1)

        @pl.when(step + 2 < NG)
        def _():
            for d in group_copies(step + 2):
                d.start()

        @pl.when(step == 0)
        def _():
            wmb_cp().start()
            wg_cp().start()

        @pl.when(step == 1)
        def _():
            wu_cp().start()

        @pl.when(step == 2)
        def _():
            wd_cp().start()

        return step

    step = lax.fori_loop(0, NG, group_step, 0)

    wr_cp().wait()
    fold_modulation()
    for sl in range(NSL):
        cols = slice(sl * LANES, (sl + 1) * LANES)
        for r0 in range(0, D, LANES):
            r1 = min(r0 + LANES, D)
            x2 = xt_ref[r0:r1, cols].astype(F32) + modc_ref[MA + r0:MA + r1, :] * acc_ref[r0:r1, cols]
            acc_ref[r0:r1, cols] = x2
            xb = x2.astype(BF16)
            xb_ref[r0 // 2:r1 // 2, cols] = pltpu.bitcast(xb, U32)
            if r0 == 0:
                piv = jnp.mean(x2[0:8, :], axis=0, keepdims=True)
                st_ref[0, sl:sl + 1, :] = piv
            d = x2 - piv
            lhs = lhs_ref[:, r0:r1]
            t1 = jnp.dot(lhs, xb, preferred_element_type=F32)[0:8, :]
            t2 = jnp.dot(lhs, (d * d).astype(BF16), preferred_element_type=F32)[0:8, :]
            s1, s2 = (t1, t2) if r0 == 0 else (s1 + t1, s2 + t2)
        for n in range(3):
            st_ref[1 + n, sl:sl + 1, :] = s1[n:n + 1, :]
        st_ref[4, sl:sl + 1, :] = s2[0:1, :]

    wg_cp().wait()
    wu_cp().wait()

    mean = st_ref[1] * (1.0 / D)
    md = mean - st_ref[0]
    mb, sd = _ln_rows(mean, jnp.maximum(st_ref[4] * (1.0 / D) - md * md, 0.0))
    rs = 1.0 / sd
    st_ref[5] = rs
    st_ref[6] = mb * rs
    r = (st_ref[2] + st_ref[3] - mb * rc_ref[0:1, :]) * rs + rc_ref[1:2, :]

    lane16 = lax.broadcasted_iota(jnp.int32, (16, LANES), 1)
    never = lane16 > step + LANES

    def after_out_stores():
        dyn0 = pl.multiple_of((step - (NG - 1)) * LANES, LANES)
        return out_ref[0:16, pl.ds(dyn0, LANES)]

    def out_unit(n):
        w = OUW * LANES
        cols = slice(n * w, (n + 1) * w)
        rs, mrs = (jnp.concatenate([st_ref[k, n * OUW + u:n * OUW + u + 1, :]
                                    for u in range(OUW)], axis=1) for k in (5, 6))
        for r0 in range(0, D, OPR):
            x2 = acc_ref[r0:r0 + OPR, cols]
            o = x2 + ((x2 * rs - mrs) * _tile(fold_ref[r0:r0 + OPR, :], OUW)
                      + _tile(fold_ref[D + r0:D + r0 + OPR, :], OUW))
            out_ref[r0:r0 + OPR, cols] = o.astype(BF16)
        return after_out_stores().astype(F32)

    r = _rb(r) + 0.0
    bits = pltpu.bitcast(r, jnp.int32)
    mono = bits ^ ((bits >> 31) & jnp.int32(0x7FFFFFFF))
    tok = (lax.broadcasted_iota(jnp.int32, (NSL, LANES), 0) * LANES
           + lax.broadcasted_iota(jnp.int32, (NSL, LANES), 1))
    keyi = (((mono >> 16) + 32768) * S + (S - 1 - tok)) + jnp.int32(1 << 29)
    key = pltpu.bitcast(keyi, F32)

    row16 = lax.broadcasted_iota(jnp.int32, (16, LANES), 0)
    rowc = lax.broadcasted_iota(jnp.int32, (16, 1), 0)
    sel_slab, sel_off = [], []
    tie, nunit = None, 0
    xsel = jnp.zeros((16, D), F32)
    mbsel = jnp.zeros((16, 1), F32)
    rssel = jnp.zeros((16, 1), F32)
    ksel = jnp.zeros((16, 1), F32)
    for t in range(TOPC):
        kmax = jnp.max(jnp.max(key, axis=0, keepdims=True), axis=1, keepdims=True)
        hit = key == kmax
        key = jnp.where(hit, 0.0, key)
        pick = lambda z: jnp.sum(jnp.sum(jnp.where(hit, z, 0.0), axis=0, keepdims=True),
                                 axis=1, keepdims=True)
        mbsel = jnp.where(rowc == t, pick(mb), mbsel)
        rssel = jnp.where(rowc == t, pick(rs), rssel)
        for _ in range(TK_TIES.count(t)):
            tie = out_unit(nunit)
            nunit += 1
            key = jnp.where(never, tie, key)
        ksel = jnp.where(rowc == t, kmax, ksel)
        ki = pltpu.bitcast(kmax, jnp.int32)[0, 0]
        idx = (S - 1) - (ki & (S - 1))
        slab = idx >> 7
        off = idx & (LANES - 1)
        onehot = jnp.where((row16 == t) & (lane16 == off), 1.0, 0.0).astype(BF16)
        dslab = xb_ref[:, pl.ds(pl.multiple_of(slab * LANES, LANES), LANES)]
        xsel = xsel + lax.dot_general(onehot, pltpu.bitcast(dslab, BF16), _NT,
                                      preferred_element_type=F32)
        sel_slab.append(slab)
        sel_off.append(off)
    nsel = _rb(_rb(xsel - mbsel) * rssel)
    hsel = _rb(_rb(nsel * mb_ref[1, 0:1, :]) + mb_ref[0, 0:1, :])
    hi = ((pltpu.bitcast(ksel, jnp.int32) - jnp.int32(1 << 29)) // S - 32768) << 16
    rbits = hi ^ ((hi >> 31) & jnp.int32(0x7FFF0000))
    gate = _rb(_sigmoid(jnp.where(rowc < TOPC, pltpu.bitcast(rbits, F32), 0.0)))

    def out_copy(sl, r0, nr):
        c0 = pl.multiple_of(sl * LANES, LANES)
        return cp(out_ref.at[r0:r0 + nr, pl.ds(c0, LANES)],
                  out_hbm.at[r0:r0 + nr, pl.ds(c0, LANES)], S_O)

    fresh = []
    seen = jnp.int32(0)
    for t in range(TOPC):
        fresh.append(((seen >> sel_slab[t]) & 1) == 0)
        seen = seen | (1 << sel_slab[t])
    plain = [((seen >> sl) & 1) == 0 for sl in range(NSL)]

    for n in range(nunit, NSL // OUW):
        tie = out_unit(n)
    for sl in range(NSL):
        pl.when(plain[sl])(lambda sl=sl: out_copy(sl, 0, D).start())

    h0 = jnp.where(never, tie, hsel[:, 0:LANES])
    hs = jnp.concatenate([h0, hsel[:, LANES:]], axis=1).astype(BF16)
    gpre = _rb(jnp.dot(hs, wg_ref[...], preferred_element_type=F32))
    u = _rb(jnp.dot(hs, wu_ref[...], preferred_element_type=F32))
    a = (_rb(gpre * _sigmoid(gpre)) * u).astype(BF16)

    gb = mb_ref[2, 0:1, :]

    def down(r0, nr, tied):
        lhs = a
        if tied:
            a0 = jnp.where(never[0:8, :], pltpu.bitcast(after_out_stores(), U32),
                           pltpu.bitcast(a[:, TIEC:TIEC + LANES], U32))
            lhs = jnp.concatenate([a[:, 0:TIEC], pltpu.bitcast(a0, BF16), a[:, TIEC + LANES:]], axis=1)
        y = jnp.dot(lhs, pltpu.bitcast(wd_ref[0:FF // 2, r0:r0 + nr], BF16),
                    preferred_element_type=F32)
        c = slice(r0, r0 + nr)
        return xsel[:, c] + gb[:, c] * (hsel[:, c] + y * gate)

    def patch(r0, nr, new):
        lane = lax.broadcasted_iota(jnp.int32, (nr // 2, LANES), 1)
        for t in range(TOPC):
            cols = pl.ds(pl.multiple_of(sel_slab[t] * LANES, LANES), LANES)
            old = pltpu.bitcast(out_ref[r0:r0 + nr, cols], U32)
            upd = pltpu.bitcast(_as_cols(new[t:t + 1, :]), U32)
            out_ref[r0:r0 + nr, cols] = pltpu.bitcast(jnp.where(lane == sel_off[t], upd, old), BF16)
        for t in range(TOPC):
            pl.when(fresh[t])(lambda t=t: out_copy(sel_slab[t], r0, nr).start())

    news = [down(*PIECES[0], False)]
    for n in range(len(PIECES)):
        if n + 1 < len(PIECES):
            news.append(down(*PIECES[n + 1], n > 0))
        patch(*PIECES[n], news[n])

    cp(out_ref, out_hbm, S_O).wait()


@jax.jit
def pallas_adaLN_cond__gqa_block_cached__moe_arch_mod__prompt_kernel(
    A_x: jax.Array,
    A_k_cache: jax.Array,
    A_v_cache: jax.Array,
    A_wq: jax.Array,
    A_wo: jax.Array,
    B_x: jax.Array,
    B_w_r: jax.Array,
    B_w_gate: jax.Array,
    B_w_up: jax.Array,
    B_w_down: jax.Array,
    c: jax.Array,
    w_mod: jax.Array,
):
    del B_x
    B, S, D = A_x.shape
    assert B == 1
    NG, SK = A_k_cache.shape[1], A_k_cache.shape[2]
    REP = HQ // NG
    FF = B_w_gate.shape[1]
    GW = REP * DH

    xt = A_x.reshape(S, D).T
    wot = A_wo.T
    wdt = B_w_down.T
    k = A_k_cache.reshape(NG, SK, DH)
    v = A_v_cache.reshape(NG, SK, DH)

    hbm = pl.BlockSpec(memory_space=pl.ANY)
    out_t = pl.pallas_call(
        functools.partial(_kernel, S=S, SK=SK, D=D, FF=FF, NG=NG, REP=REP),
        in_specs=[hbm] * 11,
        out_specs=hbm,
        out_shape=jax.ShapeDtypeStruct((D, S), BF16),
        scratch_shapes=[
            pltpu.VMEM((D, S), BF16),
            pltpu.VMEM((2, SK, DH), BF16),
            pltpu.VMEM((2, SK, DH), BF16),
            pltpu.VMEM((2, D, GW), BF16),
            pltpu.VMEM((2, D, GW), BF16),
            pltpu.VMEM((3, D % LANES, GW), BF16),
            pltpu.VMEM((D,), BF16),
            pltpu.VMEM((1, D), BF16),
            pltpu.VMEM((D, 6 * D), BF16),
            pltpu.VMEM((D, FF), BF16),
            pltpu.VMEM((D, FF), BF16),
            pltpu.VMEM((D, FF + WT_W), BF16),
            pltpu.VMEM(((FF + WT_W) // 2, D), U32),
            pltpu.VMEM((D, S), BF16),
            pltpu.VMEM((6 * D, LANES), F32),
            pltpu.VMEM((8, 6 * D), F32),
            pltpu.VMEM((D, LANES), F32),
            pltpu.VMEM((2 * D, LANES), F32),
            pltpu.VMEM((3, 8, D), F32),
            pltpu.VMEM((16, D), BF16),
            pltpu.VMEM((8, LANES), F32),
            pltpu.VMEM((S // 2, D), U32),
            pltpu.VMEM((D, S), F32),
            pltpu.VMEM((D // 2, S), U32),
            pltpu.VMEM((7, S // LANES, LANES), F32),
            pltpu.VMEM((D % LANES, S), F32),
            pltpu.VMEM((len(VB), D % LANES * 8, BQ), F32),
            pltpu.VMEM((D % LANES, GW, LANES), F32),
            pltpu.VMEM((len(VB) * GW, BQ), F32),
            pltpu.VMEM((len(VB) * GW // VA, 8, BQ), F32),
            pltpu.SemaphoreType.DMA((N_SEMS,)),
        ],
        compiler_params=pltpu.CompilerParams(
            vmem_limit_bytes=100 * 1024 * 1024,
            disable_bounds_checks=True,
        ),
    )(xt, k, v, A_wq, wot, B_w_r, c, w_mod, B_w_gate, B_w_up, wdt)
    return out_t.T.reshape(B, S, D)
```

```python
import functools
import math

import jax
import jax.numpy as jnp
from jax import lax
import jax.experimental.pallas as pl
import jax.experimental.pallas.tpu as pltpu

F32 = jnp.float32
BF16 = jnp.bfloat16
U32 = jnp.uint32

HQ = 32
DH = 128
TOPC = 8
LN_EPS = 1e-5
BQ = 256
LANES = 128
XCH = 4
MOD_STEP = 4

HEAD = [0, 1024, 512, 640, 1536, 512, 768, 512, 1024, 1280, 1280, 1536, 384, 512, 512, 0]
MODE = [2, 0, 2, 2, 2, 2, 0, 0, 0, 0, 2, 0, 0, 2, 2, 2]
QP_POS = [-1, -1, -1, -1, -1, 3, 18, -1]
OP_POS = [7, 12, 19, 24, 30, 31, 31, 31]
VB = [3, 4, 5, 6, 7]
VA = 16
VG = 2
VPER = 358
VMARG = 300
PL = 4
PT0 = 30000
PPER = 482
WT_W = 384
WT_R = 256
WT_TIE = 0
MT_W = 384
MT_R = 8
PK0 = 56
ZC = 1024
OUW = 2
OPR = 16
TK_TIES = [0, 1, 2, 3, 4, 5, 6]
PIECES = [(0, 128), (128, 128), (256, 128), (384, 128), (512, 64)]
TIEC = 2048

_NT = (((1,), (1,)), ((), ()))

S_C = S_WMA = 0
S_WMB = S_WD = 1
S_WR = 2
S_WG = S_WU = 3
S_WQ0 = 4
S_X = 5
S_G = S_X + XCH
S_O = S_G + 2
N_SEMS = S_O + 1


def _rb(x):
    return x.astype(BF16).astype(F32)


def _sigmoid(x):
    return 1.0 / (1.0 + jnp.exp(-x))


def _ln_rows(mean, var):
    eps = _rb(jnp.full((1, 1), LN_EPS, F32))
    return _rb(mean), _rb(jnp.sqrt(_rb(_rb(var) + eps)))


def _tile(col, n):
    return jnp.concatenate([col] * n, axis=1)


def _as_cols(row):
    return jnp.broadcast_to(row, (LANES, row.shape[1])).astype(BF16).T


def _kernel(xt_hbm, k_hbm, v_hbm, wq_hbm, wot_hbm, wr_hbm, c_hbm, wmod_hbm,
            wg_hbm, wu_hbm, wdt_hbm,
            out_hbm,
            xt_ref, k_buf, v_buf, wq_buf, wot_buf, wqn_buf, wr_ref, c_ref, wmod_ref,
            wg_ref, wu_ref, wdt_ref, wd_ref, out_ref,
            modc_ref, mrow_ref, scc_ref, fold_ref, mb_ref, lhs_ref, rc_ref, h_ref, acc_ref, xb_ref, st_ref, hr_ref, ht_ref, bp_ref, rem_ref, gate_ref,
            sems,
            *, S, SK, D, FF, NG, REP):
    qscale = (DH ** -0.5) * math.log2(math.e)
    NB = S // BQ
    GW = REP * DH
    TCH = S // XCH
    MA = 2 * D
    NSL = S // LANES
    KM = D // LANES * LANES
    KR = D - KM

    def cp(src, dst, sem):
        return pltpu.make_async_copy(src, dst, sems.at[sem])

    def x_copy(i):
        cols = pl.ds(pl.multiple_of(i * TCH, TCH), TCH)
        return cp(xt_hbm.at[:, cols], xt_ref.at[:, cols], S_X + i)

    def group_copies(grp):
        slot = grp % 2
        nxt = jnp.minimum(grp + 1, NG - 1)
        cols = pl.ds(pl.multiple_of(grp * GW, GW), GW)
        return (cp(wq_hbm.at[:, cols], wq_buf.at[slot], S_G + slot),
                cp(k_hbm.at[grp], k_buf.at[slot], S_G + slot),
                cp(v_hbm.at[grp], v_buf.at[slot], S_G + slot),
                cp(wot_hbm.at[:, cols], wot_buf.at[slot], S_G + slot),
                cp(wq_hbm.at[KM:D, pl.ds(pl.multiple_of(nxt * GW, GW), GW)], wqn_buf.at[slot], S_G + slot))

    wq0_cp = lambda: cp(wq_hbm.at[KM:D, 0:GW], wqn_buf.at[2], S_WQ0)
    c_cp = lambda: cp(c_hbm, c_ref, S_C)
    wma_cp = lambda: cp(wmod_hbm.at[:, 0:MA], wmod_ref.at[:, 0:MA], S_WMA)
    wmb_cp = lambda: cp(wmod_hbm.at[:, MA:6 * D], wmod_ref.at[:, MA:6 * D], S_WMB)
    wr_cp = lambda: cp(wr_hbm, wr_ref, S_WR)
    wg_cp = lambda: cp(wg_hbm, wg_ref, S_WG)
    wu_cp = lambda: cp(wu_hbm, wu_ref, S_WU)
    wd_cp = lambda: cp(wdt_hbm, wdt_ref.at[:, 0:FF], S_WD)

    def modcol(i):
        return modc_ref[i * D:(i + 1) * D, :]

    def finish_mod(mod, col0):
        mod = _rb(mod)
        lane = lax.broadcasted_iota(jnp.int32, mod.shape, 1) + col0
        is_scale = ((lane >= D) & (lane < 2 * D)) | ((lane >= 4 * D) & (lane < 5 * D))
        return jnp.where(is_scale, _rb(1.0 + mod), mod)

    def prep_cols(w, k0, k1):
        for kk in range(k0, k1):
            bp_ref[kk] = _as_cols(w[kk:kk + 1, :]).astype(F32)

    wq0_cp().start()
    wma_cp().start()
    c_cp().start()
    for i in range(XCH):
        x_copy(i).start()
    for d in group_copies(0) + group_copies(1):
        d.start()
    wr_cp().start()
    acc_ref[:, 0:ZC] = jnp.zeros((D, ZC), F32)
    wq0_cp().wait()
    prep_cols(wqn_buf[2].astype(F32), 0, PK0)
    wma_cp().wait()
    c_cp().wait()
    c = c_ref[...].astype(F32)
    sc = _rb(c * _sigmoid(c))
    mod = jnp.dot(jnp.broadcast_to(sc, (8, D)).astype(BF16), wmod_ref[:, 0:MA],
                  preferred_element_type=F32)
    modc_ref[0:MA, :] = _as_cols(finish_mod(mod, 0)[0:1, :]).astype(F32)

    def ln1(i, carry):
        x_copy(i).wait()
        x = xt_ref[:, pl.ds(pl.multiple_of(i * TCH, TCH), TCH)].astype(F32)
        piv = x[0:1, :]
        d = x - piv
        md = jnp.mean(d, axis=0, keepdims=True)
        var = jnp.maximum(jnp.mean(d * d, axis=0, keepdims=True) - md * md, 0.0)
        mb, sd = _ln_rows(piv + md, var)
        rs = 1.0 / sd
        n = TCH // LANES
        ht = (x * rs - mb * rs) * _tile(modcol(1), n) + _tile(modcol(0), n)
        h_ref[pl.ds(pl.multiple_of(i * (TCH // 2), TCH // 2), TCH // 2), :] = pltpu.bitcast(
            ht.astype(BF16).T, U32)
        hr_ref[:, pl.ds(pl.multiple_of(i * TCH, TCH), TCH)] = _rb(ht[KM:D, :])
        return carry
    lax.fori_loop(0, XCH, ln1, 0)
    scc_ref[...] = _as_cols(sc).astype(F32)
    prep_cols(wqn_buf[2].astype(F32), PK0, KR)
    acc_ref[:, ZC:S] = jnp.zeros((D, S - ZC), F32)
    wdt_ref[:, FF:FF + WT_W] = jnp.zeros((D, WT_W), BF16)
    for n, j in enumerate(VB):
        for kk in range(KR):
            ht_ref[n, 8 * kk:8 * kk + 8, :] = jnp.broadcast_to(
                hr_ref[kk:kk + 1, j * BQ:(j + 1) * BQ], (8, BQ))

    def fold_modulation():
        sb, cb, gb = (mrow_ref[0:1, i * D:(i + 1) * D] for i in (3, 4, 5))
        for i, z in enumerate((sb, cb, gb)):
            mb_ref[i] = jnp.broadcast_to(z, (8, D))
        fold_ref[0:D, :] = modcol(5) * modcol(4)
        fold_ref[D:MA, :] = modcol(5) * modcol(3)
        wr = wr_ref[...].astype(F32).reshape(1, D)
        wc = wr * cb
        whi = _rb(wc)
        wlo = _rb(wc - whi)
        row = lax.broadcasted_iota(jnp.int32, (16, D), 0)
        lhs_ref[...] = jnp.where(row == 0, 1.0, jnp.where(row == 1, whi, jnp.where(
            row == 2, wlo, 0.0))).astype(BF16)
        rc_ref[0:1, :] = jnp.broadcast_to(jnp.sum(whi + wlo, axis=1, keepdims=True), (1, LANES))
        rc_ref[1:2, :] = jnp.broadcast_to(jnp.sum(wr * sb, axis=1, keepdims=True), (1, LANES))

    def group_step(step, carry):
        @pl.when(step == MOD_STEP)
        def _():
            wmb_cp().wait()
            wd_cp().wait()

        for d in group_copies(step):
            d.wait()

        slot = step % 2
        k = k_buf[slot]
        v = v_buf[slot]
        wq = wq_buf[slot]
        wot = wot_buf[slot]

        nev = lax.broadcasted_iota(jnp.int32, (8, BQ), 1) > step + BQ
        assert VA == 16 and BQ == 2 * LANES
        npb = GW // VA

        def link(i, gate):
            av = ht_ref[i // npb]
            bv = bp_ref[:, pl.ds(pl.multiple_of((i % npb) * VA, VA), VA), :]
            bv = jnp.concatenate([bv, bv], axis=2)
            acc = None
            for kk in range(KR):
                a = av[8 * kk:8 * kk + 8]
                if kk % VG == 0:
                    a = jnp.where(nev, gate, a)
                t = bv[kk] * jnp.concatenate([a, a], axis=0)
                acc = t if acc is None else acc + t
                g0 = 8 * (kk // VG % 2)
                g1 = 8 - g0
                gate = jnp.concatenate([acc[g0:g0 + 8, LANES:], acc[g1:g1 + 8, 0:LANES]], axis=1)
            rem_ref[pl.ds(pl.multiple_of(i * VA, VA), VA), :] = acc
            gate_ref[i] = gate
            return gate

        gate = lax.fori_loop(0, len(VB) * npb, link, jnp.zeros((8, BQ), F32), unroll=True)
        gates = [functools.partial(lambda i: gate_ref[i], i) for i in range(len(VB) * npb)]
        qrem = {j: rem_ref[nb * GW:(nb + 1) * GW, :].T for nb, j in enumerate(VB)}
        dues = [VMARG + (i + 1) * VPER for i in range(len(gates))]
        wn = wqn_buf[slot].astype(F32)
        for k0 in range(0, KR, PL):
            r0 = k0 // 8 * 8
            blk = jnp.where(nev, gate, wn[r0:r0 + 8, :])
            for kk in range(k0, k0 + PL):
                last = _as_cols(blk[kk - r0:kk - r0 + 1, :]).astype(F32)
                bp_ref[kk] = last
            gate = jnp.concatenate([last[GW - 8:GW], last[LANES - 8:LANES]], axis=1)
            gates.append(functools.partial(lambda g: g, gate))
            dues.append(PT0 + (k0 // PL + 1) * PPER)
        clock = [0]
        pinned = [0]

        def pin(x, final=False):
            due = len(gates) if final else sum(1 for t in dues if t <= clock[0])
            if due <= pinned[0]:
                return x
            pinned[0] = due
            g = pltpu.bitcast(gates[due - 1](), U32)
            xu = pltpu.bitcast(x, U32)
            top = xu[0:8, 0:LANES]
            top = jnp.where(nev[:, 0:LANES], g[:, 0:LANES], jnp.where(nev[:, LANES:], g[:, LANES:], top))
            if xu.shape[1] > LANES:
                top = jnp.concatenate([top, xu[0:8, LANES:]], axis=1)
            return pltpu.bitcast(jnp.concatenate([top, xu[8:]], axis=0), BF16)

        def qproj(j):
            hb = pin(pltpu.bitcast(h_ref[j * (BQ // 2):(j + 1) * (BQ // 2), :], BF16))
            if j in VB:
                clock[0] += 512
                q2 = jnp.dot(hb[:, 0:KM], wq[0:KM], preferred_element_type=F32) + qrem[j]
            else:
                clock[0] += 640
                q2 = jnp.dot(hb, wq, preferred_element_type=F32)
            return (q2 * qscale).astype(BF16)

        def qk(ci, lo, hi):
            q = pin(qs[ci])
            clock[0] += (hi - lo) // 2
            return lax.dot_general(q, k[lo:hi], _NT, preferred_element_type=F32)

        def softmax_pv(s, mode):
            m = jnp.max(s, axis=1, keepdims=True)
            p = jnp.exp2(s - m)
            parts = [p[:, i * LANES:(i + 1) * LANES] for i in range(SK // LANES)]
            if mode == 2:
                lp = None
                for c in range(0, len(parts), 4):
                    t = (parts[c] + parts[c + 1]) + (parts[c + 2] + parts[c + 3])
                    lp = t if lp is None else lp + t
                    parts[c + 3] = jnp.where(lp < 0.0, lp, parts[c + 3])
                p = jnp.concatenate(parts, axis=1)
            clock[0] += SK // 2
            o = jnp.dot(p.astype(BF16), v, preferred_element_type=F32)
            if mode == 0:
                l = jnp.sum(p, axis=1, keepdims=True)
            elif mode == 1:
                lp = functools.reduce(lambda x, y: x + y, parts)
                l = jnp.sum(jnp.where(lp < 0.0, o, lp), axis=1, keepdims=True)
            else:
                l = jnp.sum(lp, axis=1, keepdims=True)
            rl = pl.reciprocal(l, approx=True)
            rl = rl * (2.0 - l * rl)
            return (o * rl).astype(BF16)

        def oproj(j):
            o2 = jnp.concatenate([outs[REP * j + r] for r in range(REP)], axis=1)
            w = pin(wot, final=(j == NB - 1))
            clock[0] += 576
            acc_ref[:, j * BQ:(j + 1) * BQ] += lax.dot_general(w, o2, _NT, preferred_element_type=F32)

        qs, outs = {}, []

        def fill(pos):
            for j in range(NB):
                if QP_POS[j] == pos:
                    q2 = qproj(j)
                    for r in range(REP):
                        qs[REP * j + r] = q2[:, r * DH:(r + 1) * DH]
            for j in range(NB):
                if OP_POS[j] == pos:
                    oproj(j)

        NC = NB * REP
        assert (NG - MOD_STEP) * WT_W == FF
        wc0 = jnp.where(step >= MOD_STEP, (step - MOD_STEP) * WT_W, FF)
        never8 = lax.broadcasted_iota(jnp.int32, (8, LANES), 1) > step + LANES
        wtie = None
        for t0 in range(0, WT_W, LANES):
            for r0 in range(0, D, WT_R):
                r1 = min(r0 + WT_R, D)
                blk = pltpu.bitcast(wdt_ref[r0:r1, pl.ds(pl.multiple_of(wc0 + t0, LANES), LANES)], U32)
                if wtie is not None:
                    blk = jnp.concatenate([jnp.where(never8, wtie, blk[0:8]), blk[8:]], axis=0)
                tb = pltpu.bitcast(pltpu.bitcast(blk, BF16).T, U32)
                wd_ref[pl.ds(pl.multiple_of((wc0 + t0) // 2, LANES // 2), LANES // 2), r0:r1] = tb
                wtie = wd_ref[pl.ds(pl.multiple_of(wc0 // 2, LANES // 2), 8), 0:LANES]
        nms = 4 * D // MT_W
        assert nms * MT_W == 4 * D and MOD_STEP + nms < NG
        in_win = (step >= MOD_STEP) & (step < MOD_STEP + nms)
        mc0 = pl.multiple_of(jnp.where(in_win, MA + (step - MOD_STEP) * MT_W, 0), LANES)
        gate8 = pltpu.bitcast(wtie, F32)
        for r0 in range(0, D, MT_R):
            sc8 = scc_ref[r0:r0 + MT_R, :]
            sc8 = jnp.concatenate([jnp.where(never8, gate8, sc8[0:8])] + ([sc8[8:]] if MT_R > 8 else []), axis=0)
            t = wmod_ref[r0:r0 + MT_R, pl.ds(mc0, MT_W)].astype(F32) * _tile(sc8, MT_W // LANES)
            macc = t if r0 == 0 else macc + t
            gate8 = macc[0:8, 0:LANES]
        mrow = finish_mod(jnp.sum(macc, axis=0, keepdims=True), mc0)
        mrow_ref[0:1, pl.ds(mc0, MT_W)] = mrow
        modc_ref[pl.ds(mc0, MT_W), :] = _as_cols(mrow).astype(F32)
        wtie = pltpu.bitcast(modc_ref[0:8, :], U32)
        fill(-1)
        qt = pltpu.bitcast(qs[WT_TIE], U32)
        qs[WT_TIE] = pltpu.bitcast(
            jnp.concatenate([jnp.where(never8, wtie, qt[0:8]), qt[8:]], axis=0), BF16)
        s_head = None
        for ci in range(NC):
            lo = HEAD[ci - 1] if ci else 0
            s = qk(ci, lo, SK)
            if lo:
                s = jnp.concatenate([s_head, s], axis=1)
            fill(2 * ci)
            if HEAD[ci]:
                s_head = qk(ci + 1, 0, HEAD[ci])
            outs.append(softmax_pv(s, MODE[ci]))
            fill(2 * ci + 1)

        @pl.when(step + 2 < NG)
        def _():
            for d in group_copies(step + 2):
                d.start()

        @pl.when(step == 0)
        def _():
            wmb_cp().start()
            wg_cp().start()

        @pl.when(step == 1)
        def _():
            wu_cp().start()

        @pl.when(step == 2)
        def _():
            wd_cp().start()

        return step

    step = lax.fori_loop(0, NG, group_step, 0)

    wr_cp().wait()
    fold_modulation()
    for sl in range(NSL):
        cols = slice(sl * LANES, (sl + 1) * LANES)
        for r0 in range(0, D, LANES):
            r1 = min(r0 + LANES, D)
            x2 = xt_ref[r0:r1, cols].astype(F32) + modc_ref[MA + r0:MA + r1, :] * acc_ref[r0:r1, cols]
            acc_ref[r0:r1, cols] = x2
            xb = x2.astype(BF16)
            xb_ref[r0 // 2:r1 // 2, cols] = pltpu.bitcast(xb, U32)
            if r0 == 0:
                piv = jnp.mean(x2[0:8, :], axis=0, keepdims=True)
                st_ref[0, sl:sl + 1, :] = piv
            d = x2 - piv
            lhs = lhs_ref[:, r0:r1]
            t1 = jnp.dot(lhs, xb, preferred_element_type=F32)[0:8, :]
            t2 = jnp.dot(lhs, (d * d).astype(BF16), preferred_element_type=F32)[0:8, :]
            s1, s2 = (t1, t2) if r0 == 0 else (s1 + t1, s2 + t2)
        for n in range(3):
            st_ref[1 + n, sl:sl + 1, :] = s1[n:n + 1, :]
        st_ref[4, sl:sl + 1, :] = s2[0:1, :]

    wg_cp().wait()
    wu_cp().wait()

    mean = st_ref[1] * (1.0 / D)
    md = mean - st_ref[0]
    mb, sd = _ln_rows(mean, jnp.maximum(st_ref[4] * (1.0 / D) - md * md, 0.0))
    rs = 1.0 / sd
    st_ref[5] = rs
    st_ref[6] = mb * rs
    r = (st_ref[2] + st_ref[3] - mb * rc_ref[0:1, :]) * rs + rc_ref[1:2, :]

    lane16 = lax.broadcasted_iota(jnp.int32, (16, LANES), 1)
    never = lane16 > step + LANES

    def after_out_stores():
        dyn0 = pl.multiple_of((step - (NG - 1)) * LANES, LANES)
        return out_ref[0:16, pl.ds(dyn0, LANES)]

    def out_unit(n):
        w = OUW * LANES
        cols = slice(n * w, (n + 1) * w)
        rs, mrs = (jnp.concatenate([st_ref[k, n * OUW + u:n * OUW + u + 1, :]
                                    for u in range(OUW)], axis=1) for k in (5, 6))
        for r0 in range(0, D, OPR):
            x2 = acc_ref[r0:r0 + OPR, cols]
            o = x2 + ((x2 * rs - mrs) * _tile(fold_ref[r0:r0 + OPR, :], OUW)
                      + _tile(fold_ref[D + r0:D + r0 + OPR, :], OUW))
            out_ref[r0:r0 + OPR, cols] = o.astype(BF16)
        return after_out_stores().astype(F32)

    r = _rb(r) + 0.0
    bits = pltpu.bitcast(r, jnp.int32)
    mono = bits ^ ((bits >> 31) & jnp.int32(0x7FFFFFFF))
    tok = (lax.broadcasted_iota(jnp.int32, (NSL, LANES), 0) * LANES
           + lax.broadcasted_iota(jnp.int32, (NSL, LANES), 1))
    keyi = (((mono >> 16) + 32768) * S + (S - 1 - tok)) + jnp.int32(1 << 29)
    key = pltpu.bitcast(keyi, F32)

    row16 = lax.broadcasted_iota(jnp.int32, (16, LANES), 0)
    rowc = lax.broadcasted_iota(jnp.int32, (16, 1), 0)
    sel_slab, sel_off = [], []
    tie, nunit = None, 0
    xsel = jnp.zeros((16, D), F32)
    mbsel = jnp.zeros((16, 1), F32)
    rssel = jnp.zeros((16, 1), F32)
    ksel = jnp.zeros((16, 1), F32)
    for t in range(TOPC):
        kmax = jnp.max(jnp.max(key, axis=0, keepdims=True), axis=1, keepdims=True)
        hit = key == kmax
        key = jnp.where(hit, 0.0, key)
        pick = lambda z: jnp.sum(jnp.sum(jnp.where(hit, z, 0.0), axis=0, keepdims=True),
                                 axis=1, keepdims=True)
        mbsel = jnp.where(rowc == t, pick(mb), mbsel)
        rssel = jnp.where(rowc == t, pick(rs), rssel)
        for _ in range(TK_TIES.count(t)):
            tie = out_unit(nunit)
            nunit += 1
            key = jnp.where(never, tie, key)
        ksel = jnp.where(rowc == t, kmax, ksel)
        ki = pltpu.bitcast(kmax, jnp.int32)[0, 0]
        idx = (S - 1) - (ki & (S - 1))
        slab = idx >> 7
        off = idx & (LANES - 1)
        onehot = jnp.where((row16 == t) & (lane16 == off), 1.0, 0.0).astype(BF16)
        dslab = xb_ref[:, pl.ds(pl.multiple_of(slab * LANES, LANES), LANES)]
        xsel = xsel + lax.dot_general(onehot, pltpu.bitcast(dslab, BF16), _NT,
                                      preferred_element_type=F32)
        sel_slab.append(slab)
        sel_off.append(off)
    nsel = _rb(_rb(xsel - mbsel) * rssel)
    hsel = _rb(_rb(nsel * mb_ref[1, 0:1, :]) + mb_ref[0, 0:1, :])
    hi = ((pltpu.bitcast(ksel, jnp.int32) - jnp.int32(1 << 29)) // S - 32768) << 16
    rbits = hi ^ ((hi >> 31) & jnp.int32(0x7FFF0000))
    gate = _rb(_sigmoid(jnp.where(rowc < TOPC, pltpu.bitcast(rbits, F32), 0.0)))

    def out_copy(sl, r0, nr):
        c0 = pl.multiple_of(sl * LANES, LANES)
        return cp(out_ref.at[r0:r0 + nr, pl.ds(c0, LANES)],
                  out_hbm.at[r0:r0 + nr, pl.ds(c0, LANES)], S_O)

    fresh = []
    seen = jnp.int32(0)
    for t in range(TOPC):
        fresh.append(((seen >> sel_slab[t]) & 1) == 0)
        seen = seen | (1 << sel_slab[t])
    plain = [((seen >> sl) & 1) == 0 for sl in range(NSL)]

    for n in range(nunit, NSL // OUW):
        tie = out_unit(n)
    for sl in range(NSL):
        pl.when(plain[sl])(lambda sl=sl: out_copy(sl, 0, D).start())

    h0 = jnp.where(never, tie, hsel[:, 0:LANES])
    hs = jnp.concatenate([h0, hsel[:, LANES:]], axis=1).astype(BF16)
    gpre = _rb(jnp.dot(hs, wg_ref[...], preferred_element_type=F32))
    u = _rb(jnp.dot(hs, wu_ref[...], preferred_element_type=F32))
    a = (_rb(gpre * _sigmoid(gpre)) * u).astype(BF16)

    gb = mb_ref[2, 0:1, :]

    def down(r0, nr, tied):
        lhs = a
        if tied:
            a0 = jnp.where(never[0:8, :], pltpu.bitcast(after_out_stores(), U32),
                           pltpu.bitcast(a[:, TIEC:TIEC + LANES], U32))
            lhs = jnp.concatenate([a[:, 0:TIEC], pltpu.bitcast(a0, BF16), a[:, TIEC + LANES:]], axis=1)
        y = jnp.dot(lhs, pltpu.bitcast(wd_ref[0:FF // 2, r0:r0 + nr], BF16),
                    preferred_element_type=F32)
        c = slice(r0, r0 + nr)
        return xsel[:, c] + gb[:, c] * (hsel[:, c] + y * gate)

    def patch(r0, nr, new):
        lane = lax.broadcasted_iota(jnp.int32, (nr // 2, LANES), 1)
        for t in range(TOPC):
            cols = pl.ds(pl.multiple_of(sel_slab[t] * LANES, LANES), LANES)
            old = pltpu.bitcast(out_ref[r0:r0 + nr, cols], U32)
            upd = pltpu.bitcast(_as_cols(new[t:t + 1, :]), U32)
            out_ref[r0:r0 + nr, cols] = pltpu.bitcast(jnp.where(lane == sel_off[t], upd, old), BF16)
        for t in range(TOPC):
            pl.when(fresh[t])(lambda t=t: out_copy(sel_slab[t], r0, nr).start())

    news = [down(*PIECES[0], False)]
    for n in range(len(PIECES)):
        if n + 1 < len(PIECES):
            news.append(down(*PIECES[n + 1], n > 0))
        patch(*PIECES[n], news[n])

    cp(out_ref, out_hbm, S_O).wait()


@jax.jit
def pallas_adaLN_cond__gqa_block_cached__moe_arch_mod__prompt_kernel(
    A_x: jax.Array,
    A_k_cache: jax.Array,
    A_v_cache: jax.Array,
    A_wq: jax.Array,
    A_wo: jax.Array,
    B_x: jax.Array,
    B_w_r: jax.Array,
    B_w_gate: jax.Array,
    B_w_up: jax.Array,
    B_w_down: jax.Array,
    c: jax.Array,
    w_mod: jax.Array,
):
    del B_x
    B, S, D = A_x.shape
    assert B == 1
    NG, SK = A_k_cache.shape[1], A_k_cache.shape[2]
    REP = HQ // NG
    FF = B_w_gate.shape[1]
    GW = REP * DH

    xt = A_x.reshape(S, D).T
    wot = A_wo.T
    wdt = B_w_down.T
    k = A_k_cache.reshape(NG, SK, DH)
    v = A_v_cache.reshape(NG, SK, DH)

    hbm = pl.BlockSpec(memory_space=pl.ANY)
    out_t = pl.pallas_call(
        functools.partial(_kernel, S=S, SK=SK, D=D, FF=FF, NG=NG, REP=REP),
        in_specs=[hbm] * 11,
        out_specs=hbm,
        out_shape=jax.ShapeDtypeStruct((D, S), BF16),
        scratch_shapes=[
            pltpu.VMEM((D, S), BF16),
            pltpu.VMEM((2, SK, DH), BF16),
            pltpu.VMEM((2, SK, DH), BF16),
            pltpu.VMEM((2, D, GW), BF16),
            pltpu.VMEM((2, D, GW), BF16),
            pltpu.VMEM((3, D % LANES, GW), BF16),
            pltpu.VMEM((D,), BF16),
            pltpu.VMEM((1, D), BF16),
            pltpu.VMEM((D, 6 * D), BF16),
            pltpu.VMEM((D, FF), BF16),
            pltpu.VMEM((D, FF), BF16),
            pltpu.VMEM((D, FF + WT_W), BF16),
            pltpu.VMEM(((FF + WT_W) // 2, D), U32),
            pltpu.VMEM((D, S), BF16),
            pltpu.VMEM((6 * D, LANES), F32),
            pltpu.VMEM((8, 6 * D), F32),
            pltpu.VMEM((D, LANES), F32),
            pltpu.VMEM((2 * D, LANES), F32),
            pltpu.VMEM((3, 8, D), F32),
            pltpu.VMEM((16, D), BF16),
            pltpu.VMEM((8, LANES), F32),
            pltpu.VMEM((S // 2, D), U32),
            pltpu.VMEM((D, S), F32),
            pltpu.VMEM((D // 2, S), U32),
            pltpu.VMEM((7, S // LANES, LANES), F32),
            pltpu.VMEM((D % LANES, S), F32),
            pltpu.VMEM((len(VB), D % LANES * 8, BQ), F32),
            pltpu.VMEM((D % LANES, GW, LANES), F32),
            pltpu.VMEM((len(VB) * GW, BQ), F32),
            pltpu.VMEM((len(VB) * GW // VA, 8, BQ), F32),
            pltpu.SemaphoreType.DMA((N_SEMS,)),
        ],
        compiler_params=pltpu.CompilerParams(
            vmem_limit_bytes=100 * 1024 * 1024,
            disable_bounds_checks=True,
        ),
    )(xt, k, v, A_wq, wot, B_w_r, c, w_mod, B_w_gate, B_w_up, wdt)
    return out_t.T.reshape(B, S, D)
```

```python
import functools
import math

import jax
import jax.numpy as jnp
from jax import lax
import jax.experimental.pallas as pl
import jax.experimental.pallas.tpu as pltpu

F32 = jnp.float32
BF16 = jnp.bfloat16
U32 = jnp.uint32

HQ = 32
DH = 128
TOPC = 8
LN_EPS = 1e-5
BQ = 256
LANES = 128
XCH = 4
MOD_STEP = 4

HEAD = [0, 1024, 1536, 1280, 1536, 640, 768, 1024, 1536, 1536, 1280, 1536, 384, 512, 512, 0]
MODE = [2, 2, 2, 2, 0, 2, 0, 0, 0, 1, 2, 2, 0, 2, 0, 2]
QP_POS = [-1, -1, -1, 5, -1, 3, 18, -1]
OP_POS = [7, 12, 17, 25, 30, 31, 31, 31]
VB = [2, 3, 4, 5, 6, 7]
VA = 16
VG = 4
VPER = 300
VMARG = 300
PL = 4
PT0 = 29864
PPER = 482
WT_W = 384
WT_R = 256
WT_TIE = 0
MT_W = 384
MT_R = 8
PK0 = 56
ZC = 1024
OUW = 2
OPR = 16
TK_TIES = [0, 1, 2, 3, 4, 5, 6]
PIECES = [(0, 128), (128, 128), (256, 128), (384, 128), (512, 64)]
TIEC = 2048

_NT = (((1,), (1,)), ((), ()))

S_C = S_WMA = 0
S_WMB = S_WD = 1
S_WR = 2
S_WG = S_WU = 3
S_WQ0 = 4
S_X = 5
S_G = S_X + XCH
S_O = S_G + 2
N_SEMS = S_O + 1


def _rb(x):
    return x.astype(BF16).astype(F32)


def _sigmoid(x):
    return 1.0 / (1.0 + jnp.exp(-x))


def _ln_rows(mean, var):
    eps = _rb(jnp.full((1, 1), LN_EPS, F32))
    return _rb(mean), _rb(jnp.sqrt(_rb(_rb(var) + eps)))


def _tile(col, n):
    return jnp.concatenate([col] * n, axis=1)


def _as_cols(row):
    return jnp.broadcast_to(row, (LANES, row.shape[1])).astype(BF16).T


def _kernel(xt_hbm, k_hbm, v_hbm, wq_hbm, wot_hbm, wr_hbm, c_hbm, wmod_hbm,
            wg_hbm, wu_hbm, wdt_hbm,
            out_hbm,
            xt_ref, k_buf, v_buf, wq_buf, wot_buf, wqn_buf, wr_ref, c_ref, wmod_ref,
            wg_ref, wu_ref, wdt_ref, wd_ref, out_ref,
            modc_ref, mrow_ref, scc_ref, fold_ref, mb_ref, lhs_ref, rc_ref, h_ref, acc_ref, xb_ref, st_ref, hr_ref, ht_ref, bp_ref, rem_ref, gate_ref,
            sems,
            *, S, SK, D, FF, NG, REP):
    qscale = (DH ** -0.5) * math.log2(math.e)
    NB = S // BQ
    GW = REP * DH
    TCH = S // XCH
    MA = 2 * D
    NSL = S // LANES
    KM = D // LANES * LANES
    KR = D - KM

    def cp(src, dst, sem):
        return pltpu.make_async_copy(src, dst, sems.at[sem])

    def x_copy(i):
        cols = pl.ds(pl.multiple_of(i * TCH, TCH), TCH)
        return cp(xt_hbm.at[:, cols], xt_ref.at[:, cols], S_X + i)

    def group_copies(grp):
        slot = grp % 2
        nxt = jnp.minimum(grp + 1, NG - 1)
        cols = pl.ds(pl.multiple_of(grp * GW, GW), GW)
        return (cp(wq_hbm.at[:, cols], wq_buf.at[slot], S_G + slot),
                cp(k_hbm.at[grp], k_buf.at[slot], S_G + slot),
                cp(v_hbm.at[grp], v_buf.at[slot], S_G + slot),
                cp(wot_hbm.at[:, cols], wot_buf.at[slot], S_G + slot),
                cp(wq_hbm.at[KM:D, pl.ds(pl.multiple_of(nxt * GW, GW), GW)], wqn_buf.at[slot], S_G + slot))

    wq0_cp = lambda: cp(wq_hbm.at[KM:D, 0:GW], wqn_buf.at[2], S_WQ0)
    c_cp = lambda: cp(c_hbm, c_ref, S_C)
    wma_cp = lambda: cp(wmod_hbm.at[:, 0:MA], wmod_ref.at[:, 0:MA], S_WMA)
    wmb_cp = lambda: cp(wmod_hbm.at[:, MA:6 * D], wmod_ref.at[:, MA:6 * D], S_WMB)
    wr_cp = lambda: cp(wr_hbm, wr_ref, S_WR)
    wg_cp = lambda: cp(wg_hbm, wg_ref, S_WG)
    wu_cp = lambda: cp(wu_hbm, wu_ref, S_WU)
    wd_cp = lambda: cp(wdt_hbm, wdt_ref.at[:, 0:FF], S_WD)

    def modcol(i):
        return modc_ref[i * D:(i + 1) * D, :]

    def finish_mod(mod, col0):
        mod = _rb(mod)
        lane = lax.broadcasted_iota(jnp.int32, mod.shape, 1) + col0
        is_scale = ((lane >= D) & (lane < 2 * D)) | ((lane >= 4 * D) & (lane < 5 * D))
        return jnp.where(is_scale, _rb(1.0 + mod), mod)

    def prep_cols(w, k0, k1):
        for kk in range(k0, k1):
            bp_ref[kk] = _as_cols(w[kk:kk + 1, :]).astype(F32)

    wq0_cp().start()
    wma_cp().start()
    c_cp().start()
    for i in range(XCH):
        x_copy(i).start()
    for d in group_copies(0) + group_copies(1):
        d.start()
    wr_cp().start()
    acc_ref[:, 0:ZC] = jnp.zeros((D, ZC), F32)
    wq0_cp().wait()
    prep_cols(wqn_buf[2].astype(F32), 0, PK0)
    wma_cp().wait()
    c_cp().wait()
    c = c_ref[...].astype(F32)
    sc = _rb(c * _sigmoid(c))
    mod = jnp.dot(jnp.broadcast_to(sc, (8, D)).astype(BF16), wmod_ref[:, 0:MA],
                  preferred_element_type=F32)
    modc_ref[0:MA, :] = _as_cols(finish_mod(mod, 0)[0:1, :]).astype(F32)

    def ln1(i, carry):
        x_copy(i).wait()
        x = xt_ref[:, pl.ds(pl.multiple_of(i * TCH, TCH), TCH)].astype(F32)
        piv = x[0:1, :]
        d = x - piv
        md = jnp.mean(d, axis=0, keepdims=True)
        var = jnp.maximum(jnp.mean(d * d, axis=0, keepdims=True) - md * md, 0.0)
        mb, sd = _ln_rows(piv + md, var)
        rs = 1.0 / sd
        n = TCH // LANES
        ht = (x * rs - mb * rs) * _tile(modcol(1), n) + _tile(modcol(0), n)
        h_ref[pl.ds(pl.multiple_of(i * (TCH // 2), TCH // 2), TCH // 2), :] = pltpu.bitcast(
            ht.astype(BF16).T, U32)
        hr_ref[:, pl.ds(pl.multiple_of(i * TCH, TCH), TCH)] = _rb(ht[KM:D, :])
        return carry
    lax.fori_loop(0, XCH, ln1, 0)
    scc_ref[...] = _as_cols(sc).astype(F32)
    prep_cols(wqn_buf[2].astype(F32), PK0, KR)
    acc_ref[:, ZC:S] = jnp.zeros((D, S - ZC), F32)
    wdt_ref[:, FF:FF + WT_W] = jnp.zeros((D, WT_W), BF16)
    for n, j in enumerate(VB):
        for kk in range(KR):
            ht_ref[n, 8 * kk:8 * kk + 8, :] = jnp.broadcast_to(
                hr_ref[kk:kk + 1, j * BQ:(j + 1) * BQ], (8, BQ))

    def fold_modulation():
        sb, cb, gb = (mrow_ref[0:1, i * D:(i + 1) * D] for i in (3, 4, 5))
        for i, z in enumerate((sb, cb, gb)):
            mb_ref[i] = jnp.broadcast_to(z, (8, D))
        fold_ref[0:D, :] = modcol(5) * modcol(4)
        fold_ref[D:MA, :] = modcol(5) * modcol(3)
        wr = wr_ref[...].astype(F32).reshape(1, D)
        wc = wr * cb
        whi = _rb(wc)
        wlo = _rb(wc - whi)
        row = lax.broadcasted_iota(jnp.int32, (16, D), 0)
        lhs_ref[...] = jnp.where(row == 0, 1.0, jnp.where(row == 1, whi, jnp.where(
            row == 2, wlo, 0.0))).astype(BF16)
        rc_ref[0:1, :] = jnp.broadcast_to(jnp.sum(whi + wlo, axis=1, keepdims=True), (1, LANES))
        rc_ref[1:2, :] = jnp.broadcast_to(jnp.sum(wr * sb, axis=1, keepdims=True), (1, LANES))

    def group_step(step, carry):
        @pl.when(step == MOD_STEP)
        def _():
            wmb_cp().wait()
            wd_cp().wait()

        for d in group_copies(step):
            d.wait()

        slot = step % 2
        k = k_buf[slot]
        v = v_buf[slot]
        wq = wq_buf[slot]
        wot = wot_buf[slot]

        nev = lax.broadcasted_iota(jnp.int32, (8, BQ), 1) > step + BQ
        assert VA == 16 and BQ == 2 * LANES
        npb = GW // VA

        def link(i, gate):
            av = ht_ref[i // npb]
            bv = bp_ref[:, pl.ds(pl.multiple_of((i % npb) * VA, VA), VA), :]
            bv = jnp.concatenate([bv, bv], axis=2)
            acc = None
            for kk in range(KR):
                a = av[8 * kk:8 * kk + 8]
                if kk % VG == 0:
                    a = jnp.where(nev, gate, a)
                t = bv[kk] * jnp.concatenate([a, a], axis=0)
                acc = t if acc is None else acc + t
                g0 = 8 * (kk // VG % 2)
                g1 = 8 - g0
                gate = jnp.concatenate([acc[g0:g0 + 8, LANES:], acc[g1:g1 + 8, 0:LANES]], axis=1)
            rem_ref[pl.ds(pl.multiple_of(i * VA, VA), VA), :] = acc
            gate_ref[i] = gate
            return gate

        gate = lax.fori_loop(0, len(VB) * npb, link, jnp.zeros((8, BQ), F32), unroll=True)
        gates = [functools.partial(lambda i: gate_ref[i], i) for i in range(len(VB) * npb)]
        qrem = {j: rem_ref[nb * GW:(nb + 1) * GW, :].T for nb, j in enumerate(VB)}
        dues = [VMARG + (i + 1) * VPER for i in range(len(gates))]
        wn = wqn_buf[slot].astype(F32)
        for k0 in range(0, KR, PL):
            r0 = k0 // 8 * 8
            blk = jnp.where(nev, gate, wn[r0:r0 + 8, :])
            for kk in range(k0, k0 + PL):
                last = _as_cols(blk[kk - r0:kk - r0 + 1, :]).astype(F32)
                bp_ref[kk] = last
            gate = jnp.concatenate([last[GW - 8:GW], last[LANES - 8:LANES]], axis=1)
            gates.append(functools.partial(lambda g: g, gate))
            dues.append(PT0 + (k0 // PL + 1) * PPER)
        clock = [0]
        pinned = [0]

        def pin(x, final=False):
            due = len(gates) if final else sum(1 for t in dues if t <= clock[0])
            if due <= pinned[0]:
                return x
            pinned[0] = due
            g = pltpu.bitcast(gates[due - 1](), U32)
            xu = pltpu.bitcast(x, U32)
            top = xu[0:8, 0:LANES]
            top = jnp.where(nev[:, 0:LANES], g[:, 0:LANES], jnp.where(nev[:, LANES:], g[:, LANES:], top))
            if xu.shape[1] > LANES:
                top = jnp.concatenate([top, xu[0:8, LANES:]], axis=1)
            return pltpu.bitcast(jnp.concatenate([top, xu[8:]], axis=0), BF16)

        def qproj(j):
            hb = pin(pltpu.bitcast(h_ref[j * (BQ // 2):(j + 1) * (BQ // 2), :], BF16))
            if j in VB:
                clock[0] += 512
                q2 = jnp.dot(hb[:, 0:KM], wq[0:KM], preferred_element_type=F32) + qrem[j]
            else:
                clock[0] += 640
                q2 = jnp.dot(hb, wq, preferred_element_type=F32)
            return (q2 * qscale).astype(BF16)

        def qk(ci, lo, hi):
            q = pin(qs[ci])
            clock[0] += (hi - lo) // 2
            return lax.dot_general(q, k[lo:hi], _NT, preferred_element_type=F32)

        def softmax_pv(s, mode):
            m = jnp.max(s, axis=1, keepdims=True)
            p = jnp.exp2(s - m)
            parts = [p[:, i * LANES:(i + 1) * LANES] for i in range(SK // LANES)]
            if mode == 2:
                lp = None
                for c in range(0, len(parts), 4):
                    t = (parts[c] + parts[c + 1]) + (parts[c + 2] + parts[c + 3])
                    lp = t if lp is None else lp + t
                    parts[c + 3] = jnp.where(lp < 0.0, lp, parts[c + 3])
                p = jnp.concatenate(parts, axis=1)
            clock[0] += SK // 2
            o = jnp.dot(p.astype(BF16), v, preferred_element_type=F32)
            if mode == 0:
                l = jnp.sum(p, axis=1, keepdims=True)
            elif mode == 1:
                lp = functools.reduce(lambda x, y: x + y, parts)
                l = jnp.sum(jnp.where(lp < 0.0, o, lp), axis=1, keepdims=True)
            else:
                l = jnp.sum(lp, axis=1, keepdims=True)
            rl = pl.reciprocal(l, approx=True)
            rl = rl * (2.0 - l * rl)
            return (o * rl).astype(BF16)

        def oproj(j):
            o2 = jnp.concatenate([outs[REP * j + r] for r in range(REP)], axis=1)
            w = pin(wot, final=(j == NB - 1))
            clock[0] += 576
            acc_ref[:, j * BQ:(j + 1) * BQ] += lax.dot_general(w, o2, _NT, preferred_element_type=F32)

        qs, outs = {}, []

        def fill(pos):
            for j in range(NB):
                if QP_POS[j] == pos:
                    q2 = qproj(j)
                    for r in range(REP):
                        qs[REP * j + r] = q2[:, r * DH:(r + 1) * DH]
            for j in range(NB):
                if OP_POS[j] == pos:
                    oproj(j)

        NC = NB * REP
        assert (NG - MOD_STEP) * WT_W == FF
        wc0 = jnp.where(step >= MOD_STEP, (step - MOD_STEP) * WT_W, FF)
        never8 = lax.broadcasted_iota(jnp.int32, (8, LANES), 1) > step + LANES
        wtie = None
        for t0 in range(0, WT_W, LANES):
            for r0 in range(0, D, WT_R):
                r1 = min(r0 + WT_R, D)
                blk = pltpu.bitcast(wdt_ref[r0:r1, pl.ds(pl.multiple_of(wc0 + t0, LANES), LANES)], U32)
                if wtie is not None:
                    blk = jnp.concatenate([jnp.where(never8, wtie, blk[0:8]), blk[8:]], axis=0)
                tb = pltpu.bitcast(pltpu.bitcast(blk, BF16).T, U32)
                wd_ref[pl.ds(pl.multiple_of((wc0 + t0) // 2, LANES // 2), LANES // 2), r0:r1] = tb
                wtie = wd_ref[pl.ds(pl.multiple_of(wc0 // 2, LANES // 2), 8), 0:LANES]
        nms = 4 * D // MT_W
        assert nms * MT_W == 4 * D and MOD_STEP + nms < NG
        in_win = (step >= MOD_STEP) & (step < MOD_STEP + nms)
        mc0 = pl.multiple_of(jnp.where(in_win, MA + (step - MOD_STEP) * MT_W, 0), LANES)
        gate8 = pltpu.bitcast(wtie, F32)
        for r0 in range(0, D, MT_R):
            sc8 = scc_ref[r0:r0 + MT_R, :]
            sc8 = jnp.concatenate([jnp.where(never8, gate8, sc8[0:8])] + ([sc8[8:]] if MT_R > 8 else []), axis=0)
            t = wmod_ref[r0:r0 + MT_R, pl.ds(mc0, MT_W)].astype(F32) * _tile(sc8, MT_W // LANES)
            macc = t if r0 == 0 else macc + t
            gate8 = macc[0:8, 0:LANES]
        mrow = finish_mod(jnp.sum(macc, axis=0, keepdims=True), mc0)
        mrow_ref[0:1, pl.ds(mc0, MT_W)] = mrow
        modc_ref[pl.ds(mc0, MT_W), :] = _as_cols(mrow).astype(F32)
        wtie = pltpu.bitcast(modc_ref[0:8, :], U32)
        fill(-1)
        qt = pltpu.bitcast(qs[WT_TIE], U32)
        qs[WT_TIE] = pltpu.bitcast(
            jnp.concatenate([jnp.where(never8, wtie, qt[0:8]), qt[8:]], axis=0), BF16)
        s_head = None
        for ci in range(NC):
            lo = HEAD[ci - 1] if ci else 0
            s = qk(ci, lo, SK)
            if lo:
                s = jnp.concatenate([s_head, s], axis=1)
            fill(2 * ci)
            if HEAD[ci]:
                s_head = qk(ci + 1, 0, HEAD[ci])
            outs.append(softmax_pv(s, MODE[ci]))
            fill(2 * ci + 1)

        @pl.when(step + 2 < NG)
        def _():
            for d in group_copies(step + 2):
                d.start()

        @pl.when(step == 0)
        def _():
            wmb_cp().start()
            wg_cp().start()

        @pl.when(step == 1)
        def _():
            wu_cp().start()

        @pl.when(step == 2)
        def _():
            wd_cp().start()

        return step

    step = lax.fori_loop(0, NG, group_step, 0)

    wr_cp().wait()
    fold_modulation()
    for sl in range(NSL):
        cols = slice(sl * LANES, (sl + 1) * LANES)
        for r0 in range(0, D, LANES):
            r1 = min(r0 + LANES, D)
            x2 = xt_ref[r0:r1, cols].astype(F32) + modc_ref[MA + r0:MA + r1, :] * acc_ref[r0:r1, cols]
            acc_ref[r0:r1, cols] = x2
            xb = x2.astype(BF16)
            xb_ref[r0 // 2:r1 // 2, cols] = pltpu.bitcast(xb, U32)
            if r0 == 0:
                piv = jnp.mean(x2[0:8, :], axis=0, keepdims=True)
                st_ref[0, sl:sl + 1, :] = piv
            d = x2 - piv
            lhs = lhs_ref[:, r0:r1]
            t1 = jnp.dot(lhs, xb, preferred_element_type=F32)[0:8, :]
            t2 = jnp.dot(lhs, (d * d).astype(BF16), preferred_element_type=F32)[0:8, :]
            s1, s2 = (t1, t2) if r0 == 0 else (s1 + t1, s2 + t2)
        for n in range(3):
            st_ref[1 + n, sl:sl + 1, :] = s1[n:n + 1, :]
        st_ref[4, sl:sl + 1, :] = s2[0:1, :]

    wg_cp().wait()
    wu_cp().wait()

    mean = st_ref[1] * (1.0 / D)
    md = mean - st_ref[0]
    mb, sd = _ln_rows(mean, jnp.maximum(st_ref[4] * (1.0 / D) - md * md, 0.0))
    rs = 1.0 / sd
    st_ref[5] = rs
    st_ref[6] = mb * rs
    r = (st_ref[2] + st_ref[3] - mb * rc_ref[0:1, :]) * rs + rc_ref[1:2, :]

    lane16 = lax.broadcasted_iota(jnp.int32, (16, LANES), 1)
    never = lane16 > step + LANES

    def after_out_stores():
        dyn0 = pl.multiple_of((step - (NG - 1)) * LANES, LANES)
        return out_ref[0:16, pl.ds(dyn0, LANES)]

    def out_unit(n):
        w = OUW * LANES
        cols = slice(n * w, (n + 1) * w)
        rs, mrs = (jnp.concatenate([st_ref[k, n * OUW + u:n * OUW + u + 1, :]
                                    for u in range(OUW)], axis=1) for k in (5, 6))
        for r0 in range(0, D, OPR):
            x2 = acc_ref[r0:r0 + OPR, cols]
            o = x2 + ((x2 * rs - mrs) * _tile(fold_ref[r0:r0 + OPR, :], OUW)
                      + _tile(fold_ref[D + r0:D + r0 + OPR, :], OUW))
            out_ref[r0:r0 + OPR, cols] = o.astype(BF16)
        return after_out_stores().astype(F32)

    r = _rb(r) + 0.0
    bits = pltpu.bitcast(r, jnp.int32)
    mono = bits ^ ((bits >> 31) & jnp.int32(0x7FFFFFFF))
    tok = (lax.broadcasted_iota(jnp.int32, (NSL, LANES), 0) * LANES
           + lax.broadcasted_iota(jnp.int32, (NSL, LANES), 1))
    keyi = (((mono >> 16) + 32768) * S + (S - 1 - tok)) + jnp.int32(1 << 29)
    key = pltpu.bitcast(keyi, F32)

    row16 = lax.broadcasted_iota(jnp.int32, (16, LANES), 0)
    rowc = lax.broadcasted_iota(jnp.int32, (16, 1), 0)
    sel_slab, sel_off = [], []
    tie, nunit = None, 0
    xsel = jnp.zeros((16, D), F32)
    mbsel = jnp.zeros((16, 1), F32)
    rssel = jnp.zeros((16, 1), F32)
    ksel = jnp.zeros((16, 1), F32)
    for t in range(TOPC):
        kmax = jnp.max(jnp.max(key, axis=0, keepdims=True), axis=1, keepdims=True)
        hit = key == kmax
        key = jnp.where(hit, 0.0, key)
        pick = lambda z: jnp.sum(jnp.sum(jnp.where(hit, z, 0.0), axis=0, keepdims=True),
                                 axis=1, keepdims=True)
        mbsel = jnp.where(rowc == t, pick(mb), mbsel)
        rssel = jnp.where(rowc == t, pick(rs), rssel)
        for _ in range(TK_TIES.count(t)):
            tie = out_unit(nunit)
            nunit += 1
            key = jnp.where(never, tie, key)
        ksel = jnp.where(rowc == t, kmax, ksel)
        ki = pltpu.bitcast(kmax, jnp.int32)[0, 0]
        idx = (S - 1) - (ki & (S - 1))
        slab = idx >> 7
        off = idx & (LANES - 1)
        onehot = jnp.where((row16 == t) & (lane16 == off), 1.0, 0.0).astype(BF16)
        dslab = xb_ref[:, pl.ds(pl.multiple_of(slab * LANES, LANES), LANES)]
        xsel = xsel + lax.dot_general(onehot, pltpu.bitcast(dslab, BF16), _NT,
                                      preferred_element_type=F32)
        sel_slab.append(slab)
        sel_off.append(off)
    nsel = _rb(_rb(xsel - mbsel) * rssel)
    hsel = _rb(_rb(nsel * mb_ref[1, 0:1, :]) + mb_ref[0, 0:1, :])
    hi = ((pltpu.bitcast(ksel, jnp.int32) - jnp.int32(1 << 29)) // S - 32768) << 16
    rbits = hi ^ ((hi >> 31) & jnp.int32(0x7FFF0000))
    gate = _rb(_sigmoid(jnp.where(rowc < TOPC, pltpu.bitcast(rbits, F32), 0.0)))

    def out_copy(sl, r0, nr):
        c0 = pl.multiple_of(sl * LANES, LANES)
        return cp(out_ref.at[r0:r0 + nr, pl.ds(c0, LANES)],
                  out_hbm.at[r0:r0 + nr, pl.ds(c0, LANES)], S_O)

    fresh = []
    seen = jnp.int32(0)
    for t in range(TOPC):
        fresh.append(((seen >> sel_slab[t]) & 1) == 0)
        seen = seen | (1 << sel_slab[t])
    plain = [((seen >> sl) & 1) == 0 for sl in range(NSL)]

    for n in range(nunit, NSL // OUW):
        tie = out_unit(n)
    for sl in range(NSL):
        pl.when(plain[sl])(lambda sl=sl: out_copy(sl, 0, D).start())

    h0 = jnp.where(never, tie, hsel[:, 0:LANES])
    hs = jnp.concatenate([h0, hsel[:, LANES:]], axis=1).astype(BF16)
    gpre = _rb(jnp.dot(hs, wg_ref[...], preferred_element_type=F32))
    u = _rb(jnp.dot(hs, wu_ref[...], preferred_element_type=F32))
    a = (_rb(gpre * _sigmoid(gpre)) * u).astype(BF16)

    gb = mb_ref[2, 0:1, :]

    def down(r0, nr, tied):
        lhs = a
        if tied:
            a0 = jnp.where(never[0:8, :], pltpu.bitcast(after_out_stores(), U32),
                           pltpu.bitcast(a[:, TIEC:TIEC + LANES], U32))
            lhs = jnp.concatenate([a[:, 0:TIEC], pltpu.bitcast(a0, BF16), a[:, TIEC + LANES:]], axis=1)
        y = jnp.dot(lhs, pltpu.bitcast(wd_ref[0:FF // 2, r0:r0 + nr], BF16),
                    preferred_element_type=F32)
        c = slice(r0, r0 + nr)
        return xsel[:, c] + gb[:, c] * (hsel[:, c] + y * gate)

    def patch(r0, nr, new):
        lane = lax.broadcasted_iota(jnp.int32, (nr // 2, LANES), 1)
        for t in range(TOPC):
            cols = pl.ds(pl.multiple_of(sel_slab[t] * LANES, LANES), LANES)
            old = pltpu.bitcast(out_ref[r0:r0 + nr, cols], U32)
            upd = pltpu.bitcast(_as_cols(new[t:t + 1, :]), U32)
            out_ref[r0:r0 + nr, cols] = pltpu.bitcast(jnp.where(lane == sel_off[t], upd, old), BF16)
        for t in range(TOPC):
            pl.when(fresh[t])(lambda t=t: out_copy(sel_slab[t], r0, nr).start())

    news = [down(*PIECES[0], False)]
    for n in range(len(PIECES)):
        if n + 1 < len(PIECES):
            news.append(down(*PIECES[n + 1], n > 0))
        patch(*PIECES[n], news[n])

    cp(out_ref, out_hbm, S_O).wait()


@jax.jit
def pallas_adaLN_cond__gqa_block_cached__moe_arch_mod__prompt_kernel(
    A_x: jax.Array,
    A_k_cache: jax.Array,
    A_v_cache: jax.Array,
    A_wq: jax.Array,
    A_wo: jax.Array,
    B_x: jax.Array,
    B_w_r: jax.Array,
    B_w_gate: jax.Array,
    B_w_up: jax.Array,
    B_w_down: jax.Array,
    c: jax.Array,
    w_mod: jax.Array,
):
    del B_x
    B, S, D = A_x.shape
    assert B == 1
    NG, SK = A_k_cache.shape[1], A_k_cache.shape[2]
    REP = HQ // NG
    FF = B_w_gate.shape[1]
    GW = REP * DH

    xt = A_x.reshape(S, D).T
    wot = A_wo.T
    wdt = B_w_down.T
    k = A_k_cache.reshape(NG, SK, DH)
    v = A_v_cache.reshape(NG, SK, DH)

    hbm = pl.BlockSpec(memory_space=pl.ANY)
    out_t = pl.pallas_call(
        functools.partial(_kernel, S=S, SK=SK, D=D, FF=FF, NG=NG, REP=REP),
        in_specs=[hbm] * 11,
        out_specs=hbm,
        out_shape=jax.ShapeDtypeStruct((D, S), BF16),
        scratch_shapes=[
            pltpu.VMEM((D, S), BF16),
            pltpu.VMEM((2, SK, DH), BF16),
            pltpu.VMEM((2, SK, DH), BF16),
            pltpu.VMEM((2, D, GW), BF16),
            pltpu.VMEM((2, D, GW), BF16),
            pltpu.VMEM((3, D % LANES, GW), BF16),
            pltpu.VMEM((D,), BF16),
            pltpu.VMEM((1, D), BF16),
            pltpu.VMEM((D, 6 * D), BF16),
            pltpu.VMEM((D, FF), BF16),
            pltpu.VMEM((D, FF), BF16),
            pltpu.VMEM((D, FF + WT_W), BF16),
            pltpu.VMEM(((FF + WT_W) // 2, D), U32),
            pltpu.VMEM((D, S), BF16),
            pltpu.VMEM((6 * D, LANES), F32),
            pltpu.VMEM((8, 6 * D), F32),
            pltpu.VMEM((D, LANES), F32),
            pltpu.VMEM((2 * D, LANES), F32),
            pltpu.VMEM((3, 8, D), F32),
            pltpu.VMEM((16, D), BF16),
            pltpu.VMEM((8, LANES), F32),
            pltpu.VMEM((S // 2, D), U32),
            pltpu.VMEM((D, S), F32),
            pltpu.VMEM((D // 2, S), U32),
            pltpu.VMEM((7, S // LANES, LANES), F32),
            pltpu.VMEM((D % LANES, S), F32),
            pltpu.VMEM((len(VB), D % LANES * 8, BQ), F32),
            pltpu.VMEM((D % LANES, GW, LANES), F32),
            pltpu.VMEM((len(VB) * GW, BQ), F32),
            pltpu.VMEM((len(VB) * GW // VA, 8, BQ), F32),
            pltpu.SemaphoreType.DMA((N_SEMS,)),
        ],
        compiler_params=pltpu.CompilerParams(
            vmem_limit_bytes=100 * 1024 * 1024,
            disable_bounds_checks=True,
        ),
    )(xt, k, v, A_wq, wot, B_w_r, c, w_mod, B_w_gate, B_w_up, wdt)
    return out_t.T.reshape(B, S, D)
```

```python
import functools
import math

import jax
import jax.numpy as jnp
from jax import lax
import jax.experimental.pallas as pl
import jax.experimental.pallas.tpu as pltpu

F32 = jnp.float32
BF16 = jnp.bfloat16
U32 = jnp.uint32

HQ = 32
DH = 128
TOPC = 8
LN_EPS = 1e-5
BQ = 256
LANES = 128
XCH = 4
MOD_STEP = 4

HEAD = [0, 1024, 1536, 1280, 1536, 640, 768, 1024, 1536, 1536, 1280, 1536, 384, 512, 512, 0]
MODE = [2, 2, 2, 2, 0, 2, 0, 0, 0, 1, 2, 2, 0, 2, 0, 2]
QP_POS = [-1, -1, -1, 5, -1, 3, 18, -1]
OP_POS = [7, 12, 17, 25, 30, 31, 31, 31]
V0 = 4
VA = 16
GF = 2
VPER = 300
VMARG = 300
PL = 4
PA = 1
PT0 = 29864
PPER = 482
WT_W = 384
WT_R = 256
WT_TIE = 0
MT_W = 384
MT_R = 8
PK0 = 56
ZC = 1024
OUW = 2
OPR = 16
TK_TIES = [0, 1, 2, 3, 4, 5, 6]
PIECES = [(0, 128), (128, 128), (256, 128), (384, 128), (512, 64)]
TIEC = 2048

_NT = (((1,), (1,)), ((), ()))

S_C = S_WMA = 0
S_WMB = S_WD = 1
S_WR = 2
S_WG = S_WU = 3
S_WQ0 = 4
S_X = 5
S_G = S_X + XCH
S_O = S_G + 2
N_SEMS = S_O + 1


def _rb(x):
    return x.astype(BF16).astype(F32)


def _sigmoid(x):
    return 1.0 / (1.0 + jnp.exp(-x))


def _ln_rows(mean, var):
    eps = _rb(jnp.full((1, 1), LN_EPS, F32))
    return _rb(mean), _rb(jnp.sqrt(_rb(_rb(var) + eps)))


def _tile(col, n):
    return jnp.concatenate([col] * n, axis=1)


def _as_cols(row):
    return jnp.broadcast_to(row, (LANES, row.shape[1])).astype(BF16).T


def _kernel(xt_hbm, k_hbm, v_hbm, wq_hbm, wot_hbm, wr_hbm, c_hbm, wmod_hbm,
            wg_hbm, wu_hbm, wdt_hbm,
            out_hbm,
            xt_ref, k_buf, v_buf, wq_buf, wot_buf, wqn_buf, wr_ref, c_ref, wmod_ref,
            wg_ref, wu_ref, wdt_ref, wd_ref, out_ref,
            modc_ref, mrow_ref, scc_ref, fold_ref, mb_ref, lhs_ref, rc_ref, h_ref, acc_ref, xb_ref, st_ref, hr_ref, ht_ref, bp_ref, rem_ref, gate_ref,
            sems,
            *, S, SK, D, FF, NG, REP):
    qscale = (DH ** -0.5) * math.log2(math.e)
    NB = S // BQ
    GW = REP * DH
    TCH = S // XCH
    MA = 2 * D
    NSL = S // LANES
    KM = D // LANES * LANES
    KR = D - KM

    def cp(src, dst, sem):
        return pltpu.make_async_copy(src, dst, sems.at[sem])

    def x_copy(i):
        cols = pl.ds(pl.multiple_of(i * TCH, TCH), TCH)
        return cp(xt_hbm.at[:, cols], xt_ref.at[:, cols], S_X + i)

    def group_copies(grp):
        slot = grp % 2
        nxt = jnp.minimum(grp + 1, NG - 1)
        cols = pl.ds(pl.multiple_of(grp * GW, GW), GW)
        return (cp(wq_hbm.at[:, cols], wq_buf.at[slot], S_G + slot),
                cp(k_hbm.at[grp], k_buf.at[slot], S_G + slot),
                cp(v_hbm.at[grp], v_buf.at[slot], S_G + slot),
                cp(wot_hbm.at[:, cols], wot_buf.at[slot], S_G + slot),
                cp(wq_hbm.at[KM:D, pl.ds(pl.multiple_of(nxt * GW, GW), GW)], wqn_buf.at[slot], S_G + slot))

    wq0_cp = lambda: cp(wq_hbm.at[KM:D, 0:GW], wqn_buf.at[2], S_WQ0)
    c_cp = lambda: cp(c_hbm, c_ref, S_C)
    wma_cp = lambda: cp(wmod_hbm.at[:, 0:MA], wmod_ref.at[:, 0:MA], S_WMA)
    wmb_cp = lambda: cp(wmod_hbm.at[:, MA:6 * D], wmod_ref.at[:, MA:6 * D], S_WMB)
    wr_cp = lambda: cp(wr_hbm, wr_ref, S_WR)
    wg_cp = lambda: cp(wg_hbm, wg_ref, S_WG)
    wu_cp = lambda: cp(wu_hbm, wu_ref, S_WU)
    wd_cp = lambda: cp(wdt_hbm, wdt_ref.at[:, 0:FF], S_WD)

    def modcol(i):
        return modc_ref[i * D:(i + 1) * D, :]

    def finish_mod(mod, col0):
        mod = _rb(mod)
        lane = lax.broadcasted_iota(jnp.int32, mod.shape, 1) + col0
        is_scale = ((lane >= D) & (lane < 2 * D)) | ((lane >= 4 * D) & (lane < 5 * D))
        return jnp.where(is_scale, _rb(1.0 + mod), mod)

    def prep_cols(w, k0, k1):
        for kk in range(k0, k1):
            bp_ref[kk] = _as_cols(w[kk:kk + 1, :]).astype(F32)

    wq0_cp().start()
    wma_cp().start()
    c_cp().start()
    for i in range(XCH):
        x_copy(i).start()
    for d in group_copies(0) + group_copies(1):
        d.start()
    wr_cp().start()
    acc_ref[:, 0:ZC] = jnp.zeros((D, ZC), F32)
    wq0_cp().wait()
    prep_cols(wqn_buf[2].astype(F32), 0, PK0)
    wma_cp().wait()
    c_cp().wait()
    c = c_ref[...].astype(F32)
    sc = _rb(c * _sigmoid(c))
    mod = jnp.dot(jnp.broadcast_to(sc, (8, D)).astype(BF16), wmod_ref[:, 0:MA],
                  preferred_element_type=F32)
    modc_ref[0:MA, :] = _as_cols(finish_mod(mod, 0)[0:1, :]).astype(F32)

    def ln1(i, carry):
        x_copy(i).wait()
        x = xt_ref[:, pl.ds(pl.multiple_of(i * TCH, TCH), TCH)].astype(F32)
        piv = x[0:1, :]
        d = x - piv
        md = jnp.mean(d, axis=0, keepdims=True)
        var = jnp.maximum(jnp.mean(d * d, axis=0, keepdims=True) - md * md, 0.0)
        mb, sd = _ln_rows(piv + md, var)
        rs = 1.0 / sd
        n = TCH // LANES
        ht = (x * rs - mb * rs) * _tile(modcol(1), n) + _tile(modcol(0), n)
        h_ref[pl.ds(pl.multiple_of(i * (TCH // 2), TCH // 2), TCH // 2), :] = pltpu.bitcast(
            ht.astype(BF16).T, U32)
        hr_ref[:, pl.ds(pl.multiple_of(i * TCH, TCH), TCH)] = _rb(ht[KM:D, :])
        return carry
    lax.fori_loop(0, XCH, ln1, 0)
    scc_ref[...] = _as_cols(sc).astype(F32)
    prep_cols(wqn_buf[2].astype(F32), PK0, KR)
    acc_ref[:, ZC:S] = jnp.zeros((D, S - ZC), F32)
    wdt_ref[:, FF:FF + WT_W] = jnp.zeros((D, WT_W), BF16)
    for n, j in enumerate(range(V0 // REP, NB)):
        for kk in range(KR):
            ht_ref[n, 8 * kk:8 * kk + 8, :] = jnp.broadcast_to(
                hr_ref[kk:kk + 1, j * BQ:(j + 1) * BQ], (8, BQ))

    def fold_modulation():
        sb, cb, gb = (mrow_ref[0:1, i * D:(i + 1) * D] for i in (3, 4, 5))
        for i, z in enumerate((sb, cb, gb)):
            mb_ref[i] = jnp.broadcast_to(z, (8, D))
        fold_ref[0:D, :] = modcol(5) * modcol(4)
        fold_ref[D:MA, :] = modcol(5) * modcol(3)
        wr = wr_ref[...].astype(F32).reshape(1, D)
        wc = wr * cb
        whi = _rb(wc)
        wlo = _rb(wc - whi)
        row = lax.broadcasted_iota(jnp.int32, (16, D), 0)
        lhs_ref[...] = jnp.where(row == 0, 1.0, jnp.where(row == 1, whi, jnp.where(
            row == 2, wlo, 0.0))).astype(BF16)
        rc_ref[0:1, :] = jnp.broadcast_to(jnp.sum(whi + wlo, axis=1, keepdims=True), (1, LANES))
        rc_ref[1:2, :] = jnp.broadcast_to(jnp.sum(wr * sb, axis=1, keepdims=True), (1, LANES))

    def group_step(step, carry):
        @pl.when(step == MOD_STEP)
        def _():
            wmb_cp().wait()
            wd_cp().wait()

        for d in group_copies(step):
            d.wait()

        slot = step % 2
        k = k_buf[slot]
        v = v_buf[slot]
        wq = wq_buf[slot]
        wot = wot_buf[slot]

        nev = lax.broadcasted_iota(jnp.int32, (8, BQ), 1) > step + BQ
        assert VA == 16 and BQ == 2 * LANES
        npb = GW // VA
        L0, L1, B0 = V0 * DH // VA, NB * npb, V0 // REP

        def link(i, gate):
            av = ht_ref[i // npb - B0]
            bv = bp_ref[:, pl.ds(pl.multiple_of((i % npb) * VA, VA), VA), :]
            bv = jnp.concatenate([bv, bv], axis=2)
            acc = None
            for kk in range(KR):
                a = av[8 * kk:8 * kk + 8]
                if (kk * GF) % 8 < GF:
                    a = jnp.where(nev, gate, a)
                t = bv[kk] * jnp.concatenate([a, a], axis=0)
                acc = t if acc is None else acc + t
                g0 = 8 * ((kk * GF) // 8 % 2)
                g1 = 8 - g0
                gate = jnp.concatenate([acc[g0:g0 + 8, LANES:], acc[g1:g1 + 8, 0:LANES]], axis=1)
            rem_ref[pl.ds(pl.multiple_of((i - L0) * VA, VA), VA), :] = acc
            gate_ref[i - L0] = gate
            return gate

        gate = lax.fori_loop(L0, L1, link, jnp.zeros((8, BQ), F32), unroll=True)
        gates = [functools.partial(lambda i: gate_ref[i], i) for i in range(L1 - L0)]
        dues = [VMARG + (i + 1) * VPER for i in range(len(gates))]
        wn = wqn_buf[slot].astype(F32)
        for k0 in range(0, KR, PL):
            r0 = k0 // 8 * 8
            blk = jnp.where(nev, gate, wn[r0:r0 + 8, :])
            for kk in range(k0, k0 + PL):
                last = _as_cols(blk[kk - r0:kk - r0 + 1, :]).astype(F32)
                bp_ref[kk] = last
                g = jnp.concatenate([last[GW - 8:GW], last[LANES - 8:LANES]], axis=1)
                gate = gate + g if k0 + PL - PA < kk else g
            gates.append(functools.partial(lambda g: g, gate))
            dues.append(PT0 + (k0 // PL + 1) * PPER)
        clock = [0]
        pinned = [0]

        def pin(x, final=False):
            due = len(gates) if final else sum(1 for t in dues if t <= clock[0])
            if due <= pinned[0]:
                return x
            pinned[0] = due
            g = pltpu.bitcast(gates[due - 1](), U32)
            xu = pltpu.bitcast(x, U32)
            top = xu[0:8, 0:LANES]
            top = jnp.where(nev[:, 0:LANES], g[:, 0:LANES], jnp.where(nev[:, LANES:], g[:, LANES:], top))
            if xu.shape[1] > LANES:
                top = jnp.concatenate([top, xu[0:8, LANES:]], axis=1)
            return pltpu.bitcast(jnp.concatenate([top, xu[8:]], axis=0), BF16)

        def qproj(j):
            hb = pin(pltpu.bitcast(h_ref[j * (BQ // 2):(j + 1) * (BQ // 2), :], BF16))
            nm = min(max(V0 - REP * j, 0), REP)
            clock[0] += 512 + 64 * nm
            if nm == REP:
                q2 = jnp.dot(hb, wq, preferred_element_type=F32)
            else:
                rem = rem_ref[(REP * j + nm - V0) * DH:(REP * j + REP - V0) * DH, :].T
                if nm:
                    rem = jnp.concatenate([jnp.dot(hb[:, KM:D], wq[KM:D, 0:nm * DH],
                                                   preferred_element_type=F32), rem], axis=1)
                q2 = jnp.dot(hb[:, 0:KM], wq[0:KM], preferred_element_type=F32) + rem
            return (q2 * qscale).astype(BF16)

        def qk(ci, lo, hi):
            q = pin(qs[ci])
            clock[0] += (hi - lo) // 2
            return lax.dot_general(q, k[lo:hi], _NT, preferred_element_type=F32)

        def softmax_pv(s, mode):
            m = jnp.max(s, axis=1, keepdims=True)
            p = jnp.exp2(s - m)
            parts = [p[:, i * LANES:(i + 1) * LANES] for i in range(SK // LANES)]
            if mode == 2:
                lp = None
                for c in range(0, len(parts), 4):
                    t = (parts[c] + parts[c + 1]) + (parts[c + 2] + parts[c + 3])
                    lp = t if lp is None else lp + t
                    parts[c + 3] = jnp.where(lp < 0.0, lp, parts[c + 3])
                p = jnp.concatenate(parts, axis=1)
            clock[0] += SK // 2
            o = jnp.dot(p.astype(BF16), v, preferred_element_type=F32)
            if mode == 0:
                l = jnp.sum(p, axis=1, keepdims=True)
            elif mode == 1:
                lp = functools.reduce(lambda x, y: x + y, parts)
                l = jnp.sum(jnp.where(lp < 0.0, o, lp), axis=1, keepdims=True)
            else:
                l = jnp.sum(lp, axis=1, keepdims=True)
            rl = pl.reciprocal(l, approx=True)
            rl = rl * (2.0 - l * rl)
            return (o * rl).astype(BF16)

        def oproj(j):
            o2 = jnp.concatenate([outs[REP * j + r] for r in range(REP)], axis=1)
            w = pin(wot, final=(j == NB - 1))
            clock[0] += 576
            acc_ref[:, j * BQ:(j + 1) * BQ] += lax.dot_general(w, o2, _NT, preferred_element_type=F32)

        qs, outs = {}, []

        def fill(pos):
            for j in range(NB):
                if QP_POS[j] == pos:
                    q2 = qproj(j)
                    for r in range(REP):
                        qs[REP * j + r] = q2[:, r * DH:(r + 1) * DH]
            for j in range(NB):
                if OP_POS[j] == pos:
                    oproj(j)

        NC = NB * REP
        assert (NG - MOD_STEP) * WT_W == FF
        wc0 = jnp.where(step >= MOD_STEP, (step - MOD_STEP) * WT_W, FF)
        never8 = lax.broadcasted_iota(jnp.int32, (8, LANES), 1) > step + LANES
        wtie = None
        for t0 in range(0, WT_W, LANES):
            for r0 in range(0, D, WT_R):
                r1 = min(r0 + WT_R, D)
                blk = pltpu.bitcast(wdt_ref[r0:r1, pl.ds(pl.multiple_of(wc0 + t0, LANES), LANES)], U32)
                if wtie is not None:
                    blk = jnp.concatenate([jnp.where(never8, wtie, blk[0:8]), blk[8:]], axis=0)
                tb = pltpu.bitcast(pltpu.bitcast(blk, BF16).T, U32)
                wd_ref[pl.ds(pl.multiple_of((wc0 + t0) // 2, LANES // 2), LANES // 2), r0:r1] = tb
                wtie = wd_ref[pl.ds(pl.multiple_of(wc0 // 2, LANES // 2), 8), 0:LANES]
        nms = 4 * D // MT_W
        assert nms * MT_W == 4 * D and MOD_STEP + nms < NG
        in_win = (step >= MOD_STEP) & (step < MOD_STEP + nms)
        mc0 = pl.multiple_of(jnp.where(in_win, MA + (step - MOD_STEP) * MT_W, 0), LANES)
        gate8 = pltpu.bitcast(wtie, F32)
        for r0 in range(0, D, MT_R):
            sc8 = scc_ref[r0:r0 + MT_R, :]
            sc8 = jnp.concatenate([jnp.where(never8, gate8, sc8[0:8])] + ([sc8[8:]] if MT_R > 8 else []), axis=0)
            t = wmod_ref[r0:r0 + MT_R, pl.ds(mc0, MT_W)].astype(F32) * _tile(sc8, MT_W // LANES)
            macc = t if r0 == 0 else macc + t
            gate8 = macc[0:8, 0:LANES]
        mrow = finish_mod(jnp.sum(macc, axis=0, keepdims=True), mc0)
        mrow_ref[0:1, pl.ds(mc0, MT_W)] = mrow
        modc_ref[pl.ds(mc0, MT_W), :] = _as_cols(mrow).astype(F32)
        wtie = pltpu.bitcast(modc_ref[0:8, :], U32)
        fill(-1)
        qt = pltpu.bitcast(qs[WT_TIE], U32)
        qs[WT_TIE] = pltpu.bitcast(
            jnp.concatenate([jnp.where(never8, wtie, qt[0:8]), qt[8:]], axis=0), BF16)
        s_head = None
        for ci in range(NC):
            lo = HEAD[ci - 1] if ci else 0
            s = qk(ci, lo, SK)
            if lo:
                s = jnp.concatenate([s_head, s], axis=1)
            fill(2 * ci)
            if HEAD[ci]:
                s_head = qk(ci + 1, 0, HEAD[ci])
            outs.append(softmax_pv(s, MODE[ci]))
            fill(2 * ci + 1)

        @pl.when(step + 2 < NG)
        def _():
            for d in group_copies(step + 2):
                d.start()

        @pl.when(step == 0)
        def _():
            wmb_cp().start()
            wg_cp().start()

        @pl.when(step == 1)
        def _():
            wu_cp().start()

        @pl.when(step == 2)
        def _():
            wd_cp().start()

        return step

    step = lax.fori_loop(0, NG, group_step, 0)

    wr_cp().wait()
    fold_modulation()
    for sl in range(NSL):
        cols = slice(sl * LANES, (sl + 1) * LANES)
        for r0 in range(0, D, LANES):
            r1 = min(r0 + LANES, D)
            x2 = xt_ref[r0:r1, cols].astype(F32) + modc_ref[MA + r0:MA + r1, :] * acc_ref[r0:r1, cols]
            acc_ref[r0:r1, cols] = x2
            xb = x2.astype(BF16)
            xb_ref[r0 // 2:r1 // 2, cols] = pltpu.bitcast(xb, U32)
            if r0 == 0:
                piv = jnp.mean(x2[0:8, :], axis=0, keepdims=True)
                st_ref[0, sl:sl + 1, :] = piv
            d = x2 - piv
            lhs = lhs_ref[:, r0:r1]
            t1 = jnp.dot(lhs, xb, preferred_element_type=F32)[0:8, :]
            t2 = jnp.dot(lhs, (d * d).astype(BF16), preferred_element_type=F32)[0:8, :]
            s1, s2 = (t1, t2) if r0 == 0 else (s1 + t1, s2 + t2)
        for n in range(3):
            st_ref[1 + n, sl:sl + 1, :] = s1[n:n + 1, :]
        st_ref[4, sl:sl + 1, :] = s2[0:1, :]

    wg_cp().wait()
    wu_cp().wait()

    mean = st_ref[1] * (1.0 / D)
    md = mean - st_ref[0]
    mb, sd = _ln_rows(mean, jnp.maximum(st_ref[4] * (1.0 / D) - md * md, 0.0))
    rs = 1.0 / sd
    st_ref[5] = rs
    st_ref[6] = mb * rs
    r = (st_ref[2] + st_ref[3] - mb * rc_ref[0:1, :]) * rs + rc_ref[1:2, :]

    lane16 = lax.broadcasted_iota(jnp.int32, (16, LANES), 1)
    never = lane16 > step + LANES

    def after_out_stores():
        dyn0 = pl.multiple_of((step - (NG - 1)) * LANES, LANES)
        return out_ref[0:16, pl.ds(dyn0, LANES)]

    def out_unit(n):
        w = OUW * LANES
        cols = slice(n * w, (n + 1) * w)
        rs, mrs = (jnp.concatenate([st_ref[k, n * OUW + u:n * OUW + u + 1, :]
                                    for u in range(OUW)], axis=1) for k in (5, 6))
        for r0 in range(0, D, OPR):
            x2 = acc_ref[r0:r0 + OPR, cols]
            o = x2 + ((x2 * rs - mrs) * _tile(fold_ref[r0:r0 + OPR, :], OUW)
                      + _tile(fold_ref[D + r0:D + r0 + OPR, :], OUW))
            out_ref[r0:r0 + OPR, cols] = o.astype(BF16)
        return after_out_stores().astype(F32)

    r = _rb(r) + 0.0
    bits = pltpu.bitcast(r, jnp.int32)
    mono = bits ^ ((bits >> 31) & jnp.int32(0x7FFFFFFF))
    tok = (lax.broadcasted_iota(jnp.int32, (NSL, LANES), 0) * LANES
           + lax.broadcasted_iota(jnp.int32, (NSL, LANES), 1))
    keyi = (((mono >> 16) + 32768) * S + (S - 1 - tok)) + jnp.int32(1 << 29)
    key = pltpu.bitcast(keyi, F32)

    row16 = lax.broadcasted_iota(jnp.int32, (16, LANES), 0)
    rowc = lax.broadcasted_iota(jnp.int32, (16, 1), 0)
    sel_slab, sel_off = [], []
    tie, nunit = None, 0
    xsel = jnp.zeros((16, D), F32)
    mbsel = jnp.zeros((16, 1), F32)
    rssel = jnp.zeros((16, 1), F32)
    ksel = jnp.zeros((16, 1), F32)
    for t in range(TOPC):
        kmax = jnp.max(jnp.max(key, axis=0, keepdims=True), axis=1, keepdims=True)
        hit = key == kmax
        key = jnp.where(hit, 0.0, key)
        pick = lambda z: jnp.sum(jnp.sum(jnp.where(hit, z, 0.0), axis=0, keepdims=True),
                                 axis=1, keepdims=True)
        mbsel = jnp.where(rowc == t, pick(mb), mbsel)
        rssel = jnp.where(rowc == t, pick(rs), rssel)
        for _ in range(TK_TIES.count(t)):
            tie = out_unit(nunit)
            nunit += 1
            key = jnp.where(never, tie, key)
        ksel = jnp.where(rowc == t, kmax, ksel)
        ki = pltpu.bitcast(kmax, jnp.int32)[0, 0]
        idx = (S - 1) - (ki & (S - 1))
        slab = idx >> 7
        off = idx & (LANES - 1)
        onehot = jnp.where((row16 == t) & (lane16 == off), 1.0, 0.0).astype(BF16)
        dslab = xb_ref[:, pl.ds(pl.multiple_of(slab * LANES, LANES), LANES)]
        xsel = xsel + lax.dot_general(onehot, pltpu.bitcast(dslab, BF16), _NT,
                                      preferred_element_type=F32)
        sel_slab.append(slab)
        sel_off.append(off)
    nsel = _rb(_rb(xsel - mbsel) * rssel)
    hsel = _rb(_rb(nsel * mb_ref[1, 0:1, :]) + mb_ref[0, 0:1, :])
    hi = ((pltpu.bitcast(ksel, jnp.int32) - jnp.int32(1 << 29)) // S - 32768) << 16
    rbits = hi ^ ((hi >> 31) & jnp.int32(0x7FFF0000))
    gate = _rb(_sigmoid(jnp.where(rowc < TOPC, pltpu.bitcast(rbits, F32), 0.0)))

    def out_copy(sl, r0, nr):
        c0 = pl.multiple_of(sl * LANES, LANES)
        return cp(out_ref.at[r0:r0 + nr, pl.ds(c0, LANES)],
                  out_hbm.at[r0:r0 + nr, pl.ds(c0, LANES)], S_O)

    fresh = []
    seen = jnp.int32(0)
    for t in range(TOPC):
        fresh.append(((seen >> sel_slab[t]) & 1) == 0)
        seen = seen | (1 << sel_slab[t])
    plain = [((seen >> sl) & 1) == 0 for sl in range(NSL)]

    for n in range(nunit, NSL // OUW):
        tie = out_unit(n)
    for sl in range(NSL):
        pl.when(plain[sl])(lambda sl=sl: out_copy(sl, 0, D).start())

    h0 = jnp.where(never, tie, hsel[:, 0:LANES])
    hs = jnp.concatenate([h0, hsel[:, LANES:]], axis=1).astype(BF16)
    gpre = _rb(jnp.dot(hs, wg_ref[...], preferred_element_type=F32))
    u = _rb(jnp.dot(hs, wu_ref[...], preferred_element_type=F32))
    a = (_rb(gpre * _sigmoid(gpre)) * u).astype(BF16)

    gb = mb_ref[2, 0:1, :]

    def down(r0, nr, tied):
        lhs = a
        if tied:
            a0 = jnp.where(never[0:8, :], pltpu.bitcast(after_out_stores(), U32),
                           pltpu.bitcast(a[:, TIEC:TIEC + LANES], U32))
            lhs = jnp.concatenate([a[:, 0:TIEC], pltpu.bitcast(a0, BF16), a[:, TIEC + LANES:]], axis=1)
        y = jnp.dot(lhs, pltpu.bitcast(wd_ref[0:FF // 2, r0:r0 + nr], BF16),
                    preferred_element_type=F32)
        c = slice(r0, r0 + nr)
        return xsel[:, c] + gb[:, c] * (hsel[:, c] + y * gate)

    def patch(r0, nr, new):
        lane = lax.broadcasted_iota(jnp.int32, (nr // 2, LANES), 1)
        for t in range(TOPC):
            cols = pl.ds(pl.multiple_of(sel_slab[t] * LANES, LANES), LANES)
            old = pltpu.bitcast(out_ref[r0:r0 + nr, cols], U32)
            upd = pltpu.bitcast(_as_cols(new[t:t + 1, :]), U32)
            out_ref[r0:r0 + nr, cols] = pltpu.bitcast(jnp.where(lane == sel_off[t], upd, old), BF16)
        for t in range(TOPC):
            pl.when(fresh[t])(lambda t=t: out_copy(sel_slab[t], r0, nr).start())

    news = [down(*PIECES[0], False)]
    for n in range(len(PIECES)):
        if n + 1 < len(PIECES):
            news.append(down(*PIECES[n + 1], n > 0))
        patch(*PIECES[n], news[n])

    cp(out_ref, out_hbm, S_O).wait()


@jax.jit
def pallas_adaLN_cond__gqa_block_cached__moe_arch_mod__prompt_kernel(
    A_x: jax.Array,
    A_k_cache: jax.Array,
    A_v_cache: jax.Array,
    A_wq: jax.Array,
    A_wo: jax.Array,
    B_x: jax.Array,
    B_w_r: jax.Array,
    B_w_gate: jax.Array,
    B_w_up: jax.Array,
    B_w_down: jax.Array,
    c: jax.Array,
    w_mod: jax.Array,
):
    del B_x
    B, S, D = A_x.shape
    assert B == 1
    NG, SK = A_k_cache.shape[1], A_k_cache.shape[2]
    REP = HQ // NG
    FF = B_w_gate.shape[1]
    GW = REP * DH

    xt = A_x.reshape(S, D).T
    wot = A_wo.T
    wdt = B_w_down.T
    k = A_k_cache.reshape(NG, SK, DH)
    v = A_v_cache.reshape(NG, SK, DH)

    hbm = pl.BlockSpec(memory_space=pl.ANY)
    out_t = pl.pallas_call(
        functools.partial(_kernel, S=S, SK=SK, D=D, FF=FF, NG=NG, REP=REP),
        in_specs=[hbm] * 11,
        out_specs=hbm,
        out_shape=jax.ShapeDtypeStruct((D, S), BF16),
        scratch_shapes=[
            pltpu.VMEM((D, S), BF16),
            pltpu.VMEM((2, SK, DH), BF16),
            pltpu.VMEM((2, SK, DH), BF16),
            pltpu.VMEM((2, D, GW), BF16),
            pltpu.VMEM((2, D, GW), BF16),
            pltpu.VMEM((3, D % LANES, GW), BF16),
            pltpu.VMEM((D,), BF16),
            pltpu.VMEM((1, D), BF16),
            pltpu.VMEM((D, 6 * D), BF16),
            pltpu.VMEM((D, FF), BF16),
            pltpu.VMEM((D, FF), BF16),
            pltpu.VMEM((D, FF + WT_W), BF16),
            pltpu.VMEM(((FF + WT_W) // 2, D), U32),
            pltpu.VMEM((D, S), BF16),
            pltpu.VMEM((6 * D, LANES), F32),
            pltpu.VMEM((8, 6 * D), F32),
            pltpu.VMEM((D, LANES), F32),
            pltpu.VMEM((2 * D, LANES), F32),
            pltpu.VMEM((3, 8, D), F32),
            pltpu.VMEM((16, D), BF16),
            pltpu.VMEM((8, LANES), F32),
            pltpu.VMEM((S // 2, D), U32),
            pltpu.VMEM((D, S), F32),
            pltpu.VMEM((D // 2, S), U32),
            pltpu.VMEM((7, S // LANES, LANES), F32),
            pltpu.VMEM((D % LANES, S), F32),
            pltpu.VMEM((S // BQ - V0 // REP, D % LANES * 8, BQ), F32),
            pltpu.VMEM((D % LANES, GW, LANES), F32),
            pltpu.VMEM(((S // BQ * REP - V0) * DH, BQ), F32),
            pltpu.VMEM(((S // BQ * REP - V0) * DH // VA, 8, BQ), F32),
            pltpu.SemaphoreType.DMA((N_SEMS,)),
        ],
        compiler_params=pltpu.CompilerParams(
            vmem_limit_bytes=100 * 1024 * 1024,
            disable_bounds_checks=True,
        ),
    )(xt, k, v, A_wq, wot, B_w_r, c, w_mod, B_w_gate, B_w_up, wdt)
    return out_t.T.reshape(B, S, D)
```

```python
import functools
import math

import jax
import jax.numpy as jnp
from jax import lax
import jax.experimental.pallas as pl
import jax.experimental.pallas.tpu as pltpu

F32 = jnp.float32
BF16 = jnp.bfloat16
U32 = jnp.uint32

HQ = 32
DH = 128
TOPC = 8
LN_EPS = 1e-5
BQ = 256
LANES = 128
XCH = 4
MOD_STEP = 4

HEAD = [0, 1024, 1536, 1280, 1536, 640, 768, 1024, 1536, 1536, 1280, 1536, 384, 512, 512, 0]
MODE = [2, 2, 2, 2, 0, 2, 0, 0, 0, 1, 2, 2, 0, 2, 0, 2]
QP_POS = [-1, -1, -1, 5, -1, 3, 18, -1]
OP_POS = [7, 12, 17, 25, 30, 31, 31, 31]
V0 = 4
VA = 16
GF = 2
VPER = 300
VMARG = 300
PL = 4
PA = 1
PT0 = 29864
PPER = 482
WT_W = 384
WT_R = 256
WT_TIE = 0
MT_W = 384
MT_R = 8
PK0 = 56
ZC = 1024
Z2 = 2048
OUW = 2
OPR = 16
TK_TIES = [0, 1, 2, 3, 4, 5, 6]
PIECES = [(0, 128), (128, 128), (256, 128), (384, 128), (512, 64)]
TIEC = 2048

_NT = (((1,), (1,)), ((), ()))

S_C = S_WMA = 0
S_WMB = S_WD = 1
S_WR = 2
S_WG = S_WU = 3
S_WQ0 = 4
S_X = 5
S_G = S_X + XCH
S_O = S_G + 2
N_SEMS = S_O + 1


def _rb(x):
    return x.astype(BF16).astype(F32)


def _sigmoid(x):
    return 1.0 / (1.0 + jnp.exp(-x))


def _ln_rows(mean, var):
    eps = _rb(jnp.full((1, 1), LN_EPS, F32))
    return _rb(mean), _rb(jnp.sqrt(_rb(_rb(var) + eps)))


def _tile(col, n):
    return jnp.concatenate([col] * n, axis=1)


def _as_cols(row):
    return jnp.broadcast_to(row, (LANES, row.shape[1])).astype(BF16).T


def _kernel(xt_hbm, k_hbm, v_hbm, wq_hbm, wot_hbm, wr_hbm, c_hbm, wmod_hbm,
            wg_hbm, wu_hbm, wdt_hbm,
            out_hbm,
            xt_ref, k_buf, v_buf, wq_buf, wot_buf, wqn_buf, wr_ref, c_ref, wmod_ref,
            wg_ref, wu_ref, wdt_ref, wd_ref, out_ref,
            modc_ref, mrow_ref, scc_ref, fold_ref, mb_ref, lhs_ref, rc_ref, h_ref, acc_ref, xb_ref, st_ref, hr_ref, ht_ref, bp_ref, rem_ref, gate_ref,
            sems,
            *, S, SK, D, FF, NG, REP):
    qscale = (DH ** -0.5) * math.log2(math.e)
    NB = S // BQ
    GW = REP * DH
    TCH = S // XCH
    MA = 2 * D
    NSL = S // LANES
    KM = D // LANES * LANES
    KR = D - KM

    def cp(src, dst, sem):
        return pltpu.make_async_copy(src, dst, sems.at[sem])

    def x_copy(i):
        cols = pl.ds(pl.multiple_of(i * TCH, TCH), TCH)
        return cp(xt_hbm.at[:, cols], xt_ref.at[:, cols], S_X + i)

    def group_copies(grp):
        slot = grp % 2
        nxt = jnp.minimum(grp + 1, NG - 1)
        cols = pl.ds(pl.multiple_of(grp * GW, GW), GW)
        return (cp(wq_hbm.at[:, cols], wq_buf.at[slot], S_G + slot),
                cp(k_hbm.at[grp], k_buf.at[slot], S_G + slot),
                cp(v_hbm.at[grp], v_buf.at[slot], S_G + slot),
                cp(wot_hbm.at[:, cols], wot_buf.at[slot], S_G + slot),
                cp(wq_hbm.at[KM:D, pl.ds(pl.multiple_of(nxt * GW, GW), GW)], wqn_buf.at[slot], S_G + slot))

    wq0_cp = lambda: cp(wq_hbm.at[KM:D, 0:GW], wqn_buf.at[2], S_WQ0)
    c_cp = lambda: cp(c_hbm, c_ref, S_C)
    wma_cp = lambda: cp(wmod_hbm.at[:, 0:MA], wmod_ref.at[:, 0:MA], S_WMA)
    wmb_cp = lambda: cp(wmod_hbm.at[:, MA:6 * D], wmod_ref.at[:, MA:6 * D], S_WMB)
    wr_cp = lambda: cp(wr_hbm, wr_ref, S_WR)
    wg_cp = lambda: cp(wg_hbm, wg_ref, S_WG)
    wu_cp = lambda: cp(wu_hbm, wu_ref, S_WU)
    wd_cp = lambda: cp(wdt_hbm, wdt_ref.at[:, 0:FF], S_WD)

    def modcol(i):
        return modc_ref[i * D:(i + 1) * D, :]

    def finish_mod(mod, col0):
        mod = _rb(mod)
        lane = lax.broadcasted_iota(jnp.int32, mod.shape, 1) + col0
        is_scale = ((lane >= D) & (lane < 2 * D)) | ((lane >= 4 * D) & (lane < 5 * D))
        return jnp.where(is_scale, _rb(1.0 + mod), mod)

    def prep_cols(w, k0, k1):
        for kk in range(k0, k1):
            bp_ref[kk] = _as_cols(w[kk:kk + 1, :]).astype(F32)

    wq0_cp().start()
    wma_cp().start()
    c_cp().start()
    for i in range(XCH):
        x_copy(i).start()
    for d in group_copies(0) + group_copies(1):
        d.start()
    wr_cp().start()
    acc_ref[:, 0:ZC] = jnp.zeros((D, ZC), F32)
    wq0_cp().wait()
    acc_ref[:, ZC:Z2] = jnp.zeros((D, Z2 - ZC), F32)
    prep_cols(wqn_buf[2].astype(F32), 0, PK0)
    wma_cp().wait()
    c_cp().wait()
    c = c_ref[...].astype(F32)
    sc = _rb(c * _sigmoid(c))
    mod = jnp.dot(jnp.broadcast_to(sc, (8, D)).astype(BF16), wmod_ref[:, 0:MA],
                  preferred_element_type=F32)
    modc_ref[0:MA, :] = _as_cols(finish_mod(mod, 0)[0:1, :]).astype(F32)

    def ln1(i, carry):
        x_copy(i).wait()
        x = xt_ref[:, pl.ds(pl.multiple_of(i * TCH, TCH), TCH)].astype(F32)
        piv = x[0:1, :]
        d = x - piv
        md = jnp.mean(d, axis=0, keepdims=True)
        var = jnp.maximum(jnp.mean(d * d, axis=0, keepdims=True) - md * md, 0.0)
        mb, sd = _ln_rows(piv + md, var)
        rs = 1.0 / sd
        n = TCH // LANES
        ht = (x * rs - mb * rs) * _tile(modcol(1), n) + _tile(modcol(0), n)
        h_ref[pl.ds(pl.multiple_of(i * (TCH // 2), TCH // 2), TCH // 2), :] = pltpu.bitcast(
            ht.astype(BF16).T, U32)
        hr_ref[:, pl.ds(pl.multiple_of(i * TCH, TCH), TCH)] = _rb(ht[KM:D, :])
        return carry
    lax.fori_loop(0, XCH, ln1, 0)
    scc_ref[...] = _as_cols(sc).astype(F32)
    prep_cols(wqn_buf[2].astype(F32), PK0, KR)
    if Z2 < S:
        acc_ref[:, Z2:S] = jnp.zeros((D, S - Z2), F32)
    wdt_ref[:, FF:FF + WT_W] = jnp.zeros((D, WT_W), BF16)
    for n, j in enumerate(range(V0 // REP, NB)):
        for kk in range(KR):
            ht_ref[n, 8 * kk:8 * kk + 8, :] = jnp.broadcast_to(
                hr_ref[kk:kk + 1, j * BQ:(j + 1) * BQ], (8, BQ))

    def fold_modulation():
        sb, cb, gb = (mrow_ref[0:1, i * D:(i + 1) * D] for i in (3, 4, 5))
        for i, z in enumerate((sb, cb, gb)):
            mb_ref[i] = jnp.broadcast_to(z, (8, D))
        fold_ref[0:D, :] = modcol(5) * modcol(4)
        fold_ref[D:MA, :] = modcol(5) * modcol(3)
        wr = wr_ref[...].astype(F32).reshape(1, D)
        wc = wr * cb
        whi = _rb(wc)
        wlo = _rb(wc - whi)
        row = lax.broadcasted_iota(jnp.int32, (16, D), 0)
        lhs_ref[...] = jnp.where(row == 0, 1.0, jnp.where(row == 1, whi, jnp.where(
            row == 2, wlo, 0.0))).astype(BF16)
        rc_ref[0:1, :] = jnp.broadcast_to(jnp.sum(whi + wlo, axis=1, keepdims=True), (1, LANES))
        rc_ref[1:2, :] = jnp.broadcast_to(jnp.sum(wr * sb, axis=1, keepdims=True), (1, LANES))

    def group_step(step, carry):
        @pl.when(step == MOD_STEP)
        def _():
            wmb_cp().wait()
            wd_cp().wait()

        for d in group_copies(step):
            d.wait()

        slot = step % 2
        k = k_buf[slot]
        v = v_buf[slot]
        wq = wq_buf[slot]
        wot = wot_buf[slot]

        nev = lax.broadcasted_iota(jnp.int32, (8, BQ), 1) > step + BQ
        assert VA == 16 and BQ == 2 * LANES
        npb = GW // VA
        L0, L1, B0 = V0 * DH // VA, NB * npb, V0 // REP

        def link(i, gate):
            av = ht_ref[i // npb - B0]
            bv = bp_ref[:, pl.ds(pl.multiple_of((i % npb) * VA, VA), VA), :]
            bv = jnp.concatenate([bv, bv], axis=2)
            acc = None
            for kk in range(KR):
                a = av[8 * kk:8 * kk + 8]
                if (kk * GF) % 8 < GF:
                    a = jnp.where(nev, gate, a)
                t = bv[kk] * jnp.concatenate([a, a], axis=0)
                acc = t if acc is None else acc + t
                g0 = 8 * ((kk * GF) // 8 % 2)
                g1 = 8 - g0
                gate = jnp.concatenate([acc[g0:g0 + 8, LANES:], acc[g1:g1 + 8, 0:LANES]], axis=1)
            rem_ref[pl.ds(pl.multiple_of((i - L0) * VA, VA), VA), :] = acc
            gate_ref[i - L0] = gate
            return gate

        gate = lax.fori_loop(L0, L1, link, jnp.zeros((8, BQ), F32), unroll=True)
        gates = [functools.partial(lambda i: gate_ref[i], i) for i in range(L1 - L0)]
        dues = [VMARG + (i + 1) * VPER for i in range(len(gates))]
        wn = wqn_buf[slot].astype(F32)
        for k0 in range(0, KR, PL):
            k1 = min(k0 + PL, KR)
            blks = {r0: jnp.where(nev, gate, wn[r0:r0 + 8, :]) for r0 in range(k0 // 8 * 8, k1, 8)}
            for kk in range(k0, k1):
                last = _as_cols(blks[kk // 8 * 8][kk % 8:kk % 8 + 1, :]).astype(F32)
                bp_ref[kk] = last
                g = jnp.concatenate([last[GW - 8:GW], last[LANES - 8:LANES]], axis=1)
                gate = gate + g if max(k0, k1 - PA) < kk else g
            gates.append(functools.partial(lambda g: g, gate))
            dues.append(PT0 + (k0 // PL + 1) * PPER)
        clock = [0]
        pinned = [0]

        def pin(x, final=False):
            due = len(gates) if final else sum(1 for t in dues if t <= clock[0])
            if due <= pinned[0]:
                return x
            pinned[0] = due
            g = pltpu.bitcast(gates[due - 1](), U32)
            xu = pltpu.bitcast(x, U32)
            top = xu[0:8, 0:LANES]
            top = jnp.where(nev[:, 0:LANES], g[:, 0:LANES], jnp.where(nev[:, LANES:], g[:, LANES:], top))
            if xu.shape[1] > LANES:
                top = jnp.concatenate([top, xu[0:8, LANES:]], axis=1)
            return pltpu.bitcast(jnp.concatenate([top, xu[8:]], axis=0), BF16)

        def qproj(j):
            hb = pin(pltpu.bitcast(h_ref[j * (BQ // 2):(j + 1) * (BQ // 2), :], BF16))
            nm = min(max(V0 - REP * j, 0), REP)
            clock[0] += 512 + 64 * nm
            if nm == REP:
                q2 = jnp.dot(hb, wq, preferred_element_type=F32)
            else:
                rem = rem_ref[(REP * j + nm - V0) * DH:(REP * j + REP - V0) * DH, :].T
                if nm:
                    rem = jnp.concatenate([jnp.dot(hb[:, KM:D], wq[KM:D, 0:nm * DH],
                                                   preferred_element_type=F32), rem], axis=1)
                q2 = jnp.dot(hb[:, 0:KM], wq[0:KM], preferred_element_type=F32) + rem
            return (q2 * qscale).astype(BF16)

        def qk(ci, lo, hi):
            q = pin(qs[ci])
            clock[0] += (hi - lo) // 2
            return lax.dot_general(q, k[lo:hi], _NT, preferred_element_type=F32)

        def softmax_pv(s, mode):
            m = jnp.max(s, axis=1, keepdims=True)
            p = jnp.exp2(s - m)
            parts = [p[:, i * LANES:(i + 1) * LANES] for i in range(SK // LANES)]
            if mode == 2:
                lp = None
                for c in range(0, len(parts), 4):
                    t = (parts[c] + parts[c + 1]) + (parts[c + 2] + parts[c + 3])
                    lp = t if lp is None else lp + t
                    parts[c + 3] = jnp.where(lp < 0.0, lp, parts[c + 3])
                p = jnp.concatenate(parts, axis=1)
            clock[0] += SK // 2
            o = jnp.dot(p.astype(BF16), v, preferred_element_type=F32)
            if mode == 0:
                l = jnp.sum(p, axis=1, keepdims=True)
            elif mode == 1:
                lp = functools.reduce(lambda x, y: x + y, parts)
                l = jnp.sum(jnp.where(lp < 0.0, o, lp), axis=1, keepdims=True)
            else:
                l = jnp.sum(lp, axis=1, keepdims=True)
            rl = pl.reciprocal(l, approx=True)
            rl = rl * (2.0 - l * rl)
            return (o * rl).astype(BF16)

        def oproj(j):
            o2 = jnp.concatenate([outs[REP * j + r] for r in range(REP)], axis=1)
            w = pin(wot, final=(j == NB - 1))
            clock[0] += 576
            acc_ref[:, j * BQ:(j + 1) * BQ] += lax.dot_general(w, o2, _NT, preferred_element_type=F32)

        qs, outs = {}, []

        def fill(pos):
            for j in range(NB):
                if QP_POS[j] == pos:
                    q2 = qproj(j)
                    for r in range(REP):
                        qs[REP * j + r] = q2[:, r * DH:(r + 1) * DH]
            for j in range(NB):
                if OP_POS[j] == pos:
                    oproj(j)

        NC = NB * REP
        assert (NG - MOD_STEP) * WT_W == FF
        wc0 = jnp.where(step >= MOD_STEP, (step - MOD_STEP) * WT_W, FF)
        never8 = lax.broadcasted_iota(jnp.int32, (8, LANES), 1) > step + LANES
        wtie = None
        for t0 in range(0, WT_W, LANES):
            for r0 in range(0, D, WT_R):
                r1 = min(r0 + WT_R, D)
                blk = pltpu.bitcast(wdt_ref[r0:r1, pl.ds(pl.multiple_of(wc0 + t0, LANES), LANES)], U32)
                if wtie is not None:
                    blk = jnp.concatenate([jnp.where(never8, wtie, blk[0:8]), blk[8:]], axis=0)
                tb = pltpu.bitcast(pltpu.bitcast(blk, BF16).T, U32)
                wd_ref[pl.ds(pl.multiple_of((wc0 + t0) // 2, LANES // 2), LANES // 2), r0:r1] = tb
                wtie = wd_ref[pl.ds(pl.multiple_of(wc0 // 2, LANES // 2), 8), 0:LANES]
        nms = 4 * D // MT_W
        assert nms * MT_W == 4 * D and MOD_STEP + nms < NG
        in_win = (step >= MOD_STEP) & (step < MOD_STEP + nms)
        mc0 = pl.multiple_of(jnp.where(in_win, MA + (step - MOD_STEP) * MT_W, 0), LANES)
        gate8 = pltpu.bitcast(wtie, F32)
        for r0 in range(0, D, MT_R):
            sc8 = scc_ref[r0:r0 + MT_R, :]
            sc8 = jnp.concatenate([jnp.where(never8, gate8, sc8[0:8])] + ([sc8[8:]] if MT_R > 8 else []), axis=0)
            t = wmod_ref[r0:r0 + MT_R, pl.ds(mc0, MT_W)].astype(F32) * _tile(sc8, MT_W // LANES)
            macc = t if r0 == 0 else macc + t
            gate8 = macc[0:8, 0:LANES]
        mrow = finish_mod(jnp.sum(macc, axis=0, keepdims=True), mc0)
        mrow_ref[0:1, pl.ds(mc0, MT_W)] = mrow
        modc_ref[pl.ds(mc0, MT_W), :] = _as_cols(mrow).astype(F32)
        wtie = pltpu.bitcast(modc_ref[0:8, :], U32)
        fill(-1)
        qt = pltpu.bitcast(qs[WT_TIE], U32)
        qs[WT_TIE] = pltpu.bitcast(
            jnp.concatenate([jnp.where(never8, wtie, qt[0:8]), qt[8:]], axis=0), BF16)
        s_head = None
        for ci in range(NC):
            lo = HEAD[ci - 1] if ci else 0
            s = qk(ci, lo, SK)
            if lo:
                s = jnp.concatenate([s_head, s], axis=1)
            fill(2 * ci)
            if HEAD[ci]:
                s_head = qk(ci + 1, 0, HEAD[ci])
            outs.append(softmax_pv(s, MODE[ci]))
            fill(2 * ci + 1)

        @pl.when(step + 2 < NG)
        def _():
            for d in group_copies(step + 2):
                d.start()

        @pl.when(step == 0)
        def _():
            wmb_cp().start()
            wg_cp().start()

        @pl.when(step == 1)
        def _():
            wu_cp().start()

        @pl.when(step == 2)
        def _():
            wd_cp().start()

        return step

    step = lax.fori_loop(0, NG, group_step, 0)

    wr_cp().wait()
    fold_modulation()
    for sl in range(NSL):
        cols = slice(sl * LANES, (sl + 1) * LANES)
        for r0 in range(0, D, LANES):
            r1 = min(r0 + LANES, D)
            x2 = xt_ref[r0:r1, cols].astype(F32) + modc_ref[MA + r0:MA + r1, :] * acc_ref[r0:r1, cols]
            acc_ref[r0:r1, cols] = x2
            xb = x2.astype(BF16)
            xb_ref[r0 // 2:r1 // 2, cols] = pltpu.bitcast(xb, U32)
            if r0 == 0:
                piv = jnp.mean(x2[0:8, :], axis=0, keepdims=True)
                st_ref[0, sl:sl + 1, :] = piv
            d = x2 - piv
            lhs = lhs_ref[:, r0:r1]
            t1 = jnp.dot(lhs, xb, preferred_element_type=F32)[0:8, :]
            t2 = jnp.dot(lhs, (d * d).astype(BF16), preferred_element_type=F32)[0:8, :]
            s1, s2 = (t1, t2) if r0 == 0 else (s1 + t1, s2 + t2)
        for n in range(3):
            st_ref[1 + n, sl:sl + 1, :] = s1[n:n + 1, :]
        st_ref[4, sl:sl + 1, :] = s2[0:1, :]

    wg_cp().wait()
    wu_cp().wait()

    mean = st_ref[1] * (1.0 / D)
    md = mean - st_ref[0]
    mb, sd = _ln_rows(mean, jnp.maximum(st_ref[4] * (1.0 / D) - md * md, 0.0))
    rs = 1.0 / sd
    st_ref[5] = rs
    st_ref[6] = mb * rs
    r = (st_ref[2] + st_ref[3] - mb * rc_ref[0:1, :]) * rs + rc_ref[1:2, :]

    lane16 = lax.broadcasted_iota(jnp.int32, (16, LANES), 1)
    never = lane16 > step + LANES

    def after_out_stores():
        dyn0 = pl.multiple_of((step - (NG - 1)) * LANES, LANES)
        return out_ref[0:16, pl.ds(dyn0, LANES)]

    def out_unit(n):
        w = OUW * LANES
        cols = slice(n * w, (n + 1) * w)
        rs, mrs = (jnp.concatenate([st_ref[k, n * OUW + u:n * OUW + u + 1, :]
                                    for u in range(OUW)], axis=1) for k in (5, 6))
        for r0 in range(0, D, OPR):
            x2 = acc_ref[r0:r0 + OPR, cols]
            o = x2 + ((x2 * rs - mrs) * _tile(fold_ref[r0:r0 + OPR, :], OUW)
                      + _tile(fold_ref[D + r0:D + r0 + OPR, :], OUW))
            out_ref[r0:r0 + OPR, cols] = o.astype(BF16)
        return after_out_stores().astype(F32)

    r = _rb(r) + 0.0
    bits = pltpu.bitcast(r, jnp.int32)
    mono = bits ^ ((bits >> 31) & jnp.int32(0x7FFFFFFF))
    tok = (lax.broadcasted_iota(jnp.int32, (NSL, LANES), 0) * LANES
           + lax.broadcasted_iota(jnp.int32, (NSL, LANES), 1))
    keyi = (((mono >> 16) + 32768) * S + (S - 1 - tok)) + jnp.int32(1 << 29)
    key = pltpu.bitcast(keyi, F32)

    row16 = lax.broadcasted_iota(jnp.int32, (16, LANES), 0)
    rowc = lax.broadcasted_iota(jnp.int32, (16, 1), 0)
    sel_slab, sel_off = [], []
    tie, nunit = None, 0
    xsel = jnp.zeros((16, D), F32)
    mbsel = jnp.zeros((16, 1), F32)
    rssel = jnp.zeros((16, 1), F32)
    ksel = jnp.zeros((16, 1), F32)
    for t in range(TOPC):
        kmax = jnp.max(jnp.max(key, axis=0, keepdims=True), axis=1, keepdims=True)
        hit = key == kmax
        key = jnp.where(hit, 0.0, key)
        pick = lambda z: jnp.sum(jnp.sum(jnp.where(hit, z, 0.0), axis=0, keepdims=True),
                                 axis=1, keepdims=True)
        mbsel = jnp.where(rowc == t, pick(mb), mbsel)
        rssel = jnp.where(rowc == t, pick(rs), rssel)
        for _ in range(TK_TIES.count(t)):
            tie = out_unit(nunit)
            nunit += 1
            key = jnp.where(never, tie, key)
        ksel = jnp.where(rowc == t, kmax, ksel)
        ki = pltpu.bitcast(kmax, jnp.int32)[0, 0]
        idx = (S - 1) - (ki & (S - 1))
        slab = idx >> 7
        off = idx & (LANES - 1)
        onehot = jnp.where((row16 == t) & (lane16 == off), 1.0, 0.0).astype(BF16)
        dslab = xb_ref[:, pl.ds(pl.multiple_of(slab * LANES, LANES), LANES)]
        xsel = xsel + lax.dot_general(onehot, pltpu.bitcast(dslab, BF16), _NT,
                                      preferred_element_type=F32)
        sel_slab.append(slab)
        sel_off.append(off)
    nsel = _rb(_rb(xsel - mbsel) * rssel)
    hsel = _rb(_rb(nsel * mb_ref[1, 0:1, :]) + mb_ref[0, 0:1, :])
    hi = ((pltpu.bitcast(ksel, jnp.int32) - jnp.int32(1 << 29)) // S - 32768) << 16
    rbits = hi ^ ((hi >> 31) & jnp.int32(0x7FFF0000))
    gate = _rb(_sigmoid(jnp.where(rowc < TOPC, pltpu.bitcast(rbits, F32), 0.0)))

    def out_copy(sl, r0, nr):
        c0 = pl.multiple_of(sl * LANES, LANES)
        return cp(out_ref.at[r0:r0 + nr, pl.ds(c0, LANES)],
                  out_hbm.at[r0:r0 + nr, pl.ds(c0, LANES)], S_O)

    fresh = []
    seen = jnp.int32(0)
    for t in range(TOPC):
        fresh.append(((seen >> sel_slab[t]) & 1) == 0)
        seen = seen | (1 << sel_slab[t])
    plain = [((seen >> sl) & 1) == 0 for sl in range(NSL)]

    for n in range(nunit, NSL // OUW):
        tie = out_unit(n)
    for sl in range(NSL):
        pl.when(plain[sl])(lambda sl=sl: out_copy(sl, 0, D).start())

    h0 = jnp.where(never, tie, hsel[:, 0:LANES])
    hs = jnp.concatenate([h0, hsel[:, LANES:]], axis=1).astype(BF16)
    gpre = _rb(jnp.dot(hs, wg_ref[...], preferred_element_type=F32))
    u = _rb(jnp.dot(hs, wu_ref[...], preferred_element_type=F32))
    a = (_rb(gpre * _sigmoid(gpre)) * u).astype(BF16)

    gb = mb_ref[2, 0:1, :]

    def down(r0, nr, tied):
        lhs = a
        if tied:
            a0 = jnp.where(never[0:8, :], pltpu.bitcast(after_out_stores(), U32),
                           pltpu.bitcast(a[:, TIEC:TIEC + LANES], U32))
            lhs = jnp.concatenate([a[:, 0:TIEC], pltpu.bitcast(a0, BF16), a[:, TIEC + LANES:]], axis=1)
        y = jnp.dot(lhs, pltpu.bitcast(wd_ref[0:FF // 2, r0:r0 + nr], BF16),
                    preferred_element_type=F32)
        c = slice(r0, r0 + nr)
        return xsel[:, c] + gb[:, c] * (hsel[:, c] + y * gate)

    def patch(r0, nr, new):
        lane = lax.broadcasted_iota(jnp.int32, (nr // 2, LANES), 1)
        for t in range(TOPC):
            cols = pl.ds(pl.multiple_of(sel_slab[t] * LANES, LANES), LANES)
            old = pltpu.bitcast(out_ref[r0:r0 + nr, cols], U32)
            upd = pltpu.bitcast(_as_cols(new[t:t + 1, :]), U32)
            out_ref[r0:r0 + nr, cols] = pltpu.bitcast(jnp.where(lane == sel_off[t], upd, old), BF16)
        for t in range(TOPC):
            pl.when(fresh[t])(lambda t=t: out_copy(sel_slab[t], r0, nr).start())

    news = [down(*PIECES[0], False)]
    for n in range(len(PIECES)):
        if n + 1 < len(PIECES):
            news.append(down(*PIECES[n + 1], n > 0))
        patch(*PIECES[n], news[n])

    cp(out_ref, out_hbm, S_O).wait()


@jax.jit
def pallas_adaLN_cond__gqa_block_cached__moe_arch_mod__prompt_kernel(
    A_x: jax.Array,
    A_k_cache: jax.Array,
    A_v_cache: jax.Array,
    A_wq: jax.Array,
    A_wo: jax.Array,
    B_x: jax.Array,
    B_w_r: jax.Array,
    B_w_gate: jax.Array,
    B_w_up: jax.Array,
    B_w_down: jax.Array,
    c: jax.Array,
    w_mod: jax.Array,
):
    del B_x
    B, S, D = A_x.shape
    assert B == 1
    NG, SK = A_k_cache.shape[1], A_k_cache.shape[2]
    REP = HQ // NG
    FF = B_w_gate.shape[1]
    GW = REP * DH

    xt = A_x.reshape(S, D).T
    wot = A_wo.T
    wdt = B_w_down.T
    k = A_k_cache.reshape(NG, SK, DH)
    v = A_v_cache.reshape(NG, SK, DH)

    hbm = pl.BlockSpec(memory_space=pl.ANY)
    out_t = pl.pallas_call(
        functools.partial(_kernel, S=S, SK=SK, D=D, FF=FF, NG=NG, REP=REP),
        in_specs=[hbm] * 11,
        out_specs=hbm,
        out_shape=jax.ShapeDtypeStruct((D, S), BF16),
        scratch_shapes=[
            pltpu.VMEM((D, S), BF16),
            pltpu.VMEM((2, SK, DH), BF16),
            pltpu.VMEM((2, SK, DH), BF16),
            pltpu.VMEM((2, D, GW), BF16),
            pltpu.VMEM((2, D, GW), BF16),
            pltpu.VMEM((3, D % LANES, GW), BF16),
            pltpu.VMEM((D,), BF16),
            pltpu.VMEM((1, D), BF16),
            pltpu.VMEM((D, 6 * D), BF16),
            pltpu.VMEM((D, FF), BF16),
            pltpu.VMEM((D, FF), BF16),
            pltpu.VMEM((D, FF + WT_W), BF16),
            pltpu.VMEM(((FF + WT_W) // 2, D), U32),
            pltpu.VMEM((D, S), BF16),
            pltpu.VMEM((6 * D, LANES), F32),
            pltpu.VMEM((8, 6 * D), F32),
            pltpu.VMEM((D, LANES), F32),
            pltpu.VMEM((2 * D, LANES), F32),
            pltpu.VMEM((3, 8, D), F32),
            pltpu.VMEM((16, D), BF16),
            pltpu.VMEM((8, LANES), F32),
            pltpu.VMEM((S // 2, D), U32),
            pltpu.VMEM((D, S), F32),
            pltpu.VMEM((D // 2, S), U32),
            pltpu.VMEM((7, S // LANES, LANES), F32),
            pltpu.VMEM((D % LANES, S), F32),
            pltpu.VMEM((S // BQ - V0 // REP, D % LANES * 8, BQ), F32),
            pltpu.VMEM((D % LANES, GW, LANES), F32),
            pltpu.VMEM(((S // BQ * REP - V0) * DH, BQ), F32),
            pltpu.VMEM(((S // BQ * REP - V0) * DH // VA, 8, BQ), F32),
            pltpu.SemaphoreType.DMA((N_SEMS,)),
        ],
        compiler_params=pltpu.CompilerParams(
            vmem_limit_bytes=100 * 1024 * 1024,
            disable_bounds_checks=True,
        ),
    )(xt, k, v, A_wq, wot, B_w_r, c, w_mod, B_w_gate, B_w_up, wdt)
    return out_t.T.reshape(B, S, D)
```

```python
import functools
import math

import jax
import jax.numpy as jnp
from jax import lax
import jax.experimental.pallas as pl
import jax.experimental.pallas.tpu as pltpu

F32 = jnp.float32
BF16 = jnp.bfloat16
U32 = jnp.uint32

HQ = 32
DH = 128
TOPC = 8
LN_EPS = 1e-5
BQ = 256
LANES = 128
XCH = 4
MOD_STEP = 4

HEAD = [0, 1280, 1536, 1280, 1536, 1024, 768, 1024, 1536, 1280, 1536, 1536, 640, 1536, 512, 0]
MODE = [2, 2, 2, 2, 0, 2, 0, 0, 1, 1, 2, 0, 0, 2, 1, 2]
QP_POS = [-1, -1, -1, -1, -1, 3, 18, -1]
OP_POS = [7, 12, 17, 25, 30, 31, 31, 31]
V0 = 4
VA = 16
GF = 2
VPER = 300
VMARG = 300
PL = 4
PA = 1
PT0 = 29864
PPER = 515
WT_W = 384
WT_R = 256
WT_TIE = 0
MT_W = 384
MT_R = 8
PK0 = 56
ZC = 1024
DMA_AT = 14
PG0 = 5
PGI = 3
OUW = 2
OPR = 16
TK_TIES = [0, 1, 2, 3, 4, 5, 6]
PIECES = [(0, 128), (128, 128), (256, 128), (384, 128), (512, 64)]
TIEC = 2048

_NT = (((1,), (1,)), ((), ()))

S_C = S_WMA = 0
S_WMB = S_WD = 1
S_WR = 2
S_WG = S_WU = 3
S_WQ0 = 4
S_WQR = 5
S_X = 6
S_G = S_X + XCH
S_O = S_G + 2
N_SEMS = S_O + 1


def _rb(x):
    return x.astype(BF16).astype(F32)


def _sigmoid(x):
    return 1.0 / (1.0 + jnp.exp(-x))


def _ln_rows(mean, var):
    eps = _rb(jnp.full((1, 1), LN_EPS, F32))
    return _rb(mean), _rb(jnp.sqrt(_rb(_rb(var) + eps)))


def _tile(col, n):
    return jnp.concatenate([col] * n, axis=1)


def _as_cols(row):
    return jnp.broadcast_to(row, (LANES, row.shape[1])).astype(BF16).T


def _kernel(xt_hbm, k_hbm, v_hbm, wq_hbm, wot_hbm, wr_hbm, c_hbm, wmod_hbm,
            wg_hbm, wu_hbm, wdt_hbm,
            out_hbm,
            xt_ref, k_buf, v_buf, wq_buf, wot_buf, wqr_ref, wr_ref, c_ref, wmod_ref,
            wg_ref, wu_ref, wdt_ref, wd_ref, out_ref,
            modc_ref, mrow_ref, scc_ref, fold_ref, mb_ref, lhs_ref, rc_ref, h_ref, acc_ref, xb_ref, st_ref, hr_ref, ht_ref, bp_ref, rem_ref, gate_ref, pre_ref,
            sems,
            *, S, SK, D, FF, NG, REP):
    qscale = (DH ** -0.5) * math.log2(math.e)
    NB = S // BQ
    GW = REP * DH
    TCH = S // XCH
    MA = 2 * D
    NSL = S // LANES
    KM = D // LANES * LANES
    KR = D - KM

    def cp(src, dst, sem):
        return pltpu.make_async_copy(src, dst, sems.at[sem])

    def x_copy(i):
        cols = pl.ds(pl.multiple_of(i * TCH, TCH), TCH)
        return cp(xt_hbm.at[:, cols], xt_ref.at[:, cols], S_X + i)

    def group_copies(grp):
        slot = grp % 2
        cols = pl.ds(pl.multiple_of(grp * GW, GW), GW)
        return (cp(wq_hbm.at[0:KM, cols], wq_buf.at[slot, 0:KM], S_G + slot),
                cp(k_hbm.at[grp], k_buf.at[slot], S_G + slot),
                cp(v_hbm.at[grp], v_buf.at[slot], S_G + slot),
                cp(wot_hbm.at[:, cols], wot_buf.at[slot], S_G + slot))

    wq0_cp = lambda: cp(wq_hbm.at[KM:D, 0:GW], wqr_ref.at[:, 0:GW], S_WQ0)
    wqr_cp = lambda: cp(wq_hbm.at[KM:D, GW:NG * GW], wqr_ref.at[:, GW:NG * GW], S_WQR)
    c_cp = lambda: cp(c_hbm, c_ref, S_C)
    wma_cp = lambda: cp(wmod_hbm.at[:, 0:MA], wmod_ref.at[:, 0:MA], S_WMA)
    wmb_cp = lambda: cp(wmod_hbm.at[:, MA:6 * D], wmod_ref.at[:, MA:6 * D], S_WMB)
    wr_cp = lambda: cp(wr_hbm, wr_ref, S_WR)
    wg_cp = lambda: cp(wg_hbm, wg_ref, S_WG)
    wu_cp = lambda: cp(wu_hbm, wu_ref, S_WU)
    wd_cp = lambda: cp(wdt_hbm, wdt_ref.at[:, 0:FF], S_WD)

    def modcol(i):
        return modc_ref[i * D:(i + 1) * D, :]

    def finish_mod(mod, col0):
        mod = _rb(mod)
        lane = lax.broadcasted_iota(jnp.int32, mod.shape, 1) + col0
        is_scale = ((lane >= D) & (lane < 2 * D)) | ((lane >= 4 * D) & (lane < 5 * D))
        return jnp.where(is_scale, _rb(1.0 + mod), mod)

    def prep_cols(w, k0, k1):
        for kk in range(k0, k1):
            bp_ref[kk] = _as_cols(w[kk:kk + 1, :]).astype(F32)

    wq0_cp().start()
    wma_cp().start()
    c_cp().start()
    for i in range(XCH):
        x_copy(i).start()
        if i == 0:
            wqr_cp().start()
    for d in group_copies(0) + group_copies(1):
        d.start()
    wr_cp().start()
    acc_ref[:, 0:ZC] = jnp.zeros((D, ZC), F32)
    wq0_cp().wait()
    acc_ref[:, ZC:S] = jnp.zeros((D, S - ZC), F32)
    prep_cols(wqr_ref[:, 0:GW].astype(F32), 0, PK0)
    wma_cp().wait()
    c_cp().wait()
    c = c_ref[...].astype(F32)
    sc = _rb(c * _sigmoid(c))
    mod = jnp.dot(jnp.broadcast_to(sc, (8, D)).astype(BF16), wmod_ref[:, 0:MA],
                  preferred_element_type=F32)
    modc_ref[0:MA, :] = _as_cols(finish_mod(mod, 0)[0:1, :]).astype(F32)

    def pre(t0, t1, g0, ng):
        hb = pltpu.bitcast(h_ref[t0 // 2:t1 // 2, :], BF16)[:, KM:D]
        for u in range(ng):
            cols = pl.ds(pl.multiple_of((g0 + u) * GW, GW), GW)
            pre_ref[g0 + u, t0:t1, :] = jnp.dot(hb, wqr_ref[:, cols], preferred_element_type=F32)

    def ln1(i, carry):
        x_copy(i).wait()
        if not isinstance(i, int):
            pre(0, TCH, PG0 + (i - 1) * PGI, PGI)
        x = xt_ref[:, pl.ds(pl.multiple_of(i * TCH, TCH), TCH)].astype(F32)
        piv = x[0:1, :]
        d = x - piv
        md = jnp.mean(d, axis=0, keepdims=True)
        var = jnp.maximum(jnp.mean(d * d, axis=0, keepdims=True) - md * md, 0.0)
        mb, sd = _ln_rows(piv + md, var)
        rs = 1.0 / sd
        n = TCH // LANES
        ht = (x * rs - mb * rs) * _tile(modcol(1), n) + _tile(modcol(0), n)
        h_ref[pl.ds(pl.multiple_of(i * (TCH // 2), TCH // 2), TCH // 2), :] = pltpu.bitcast(
            ht.astype(BF16).T, U32)
        hr_ref[:, pl.ds(pl.multiple_of(i * TCH, TCH), TCH)] = _rb(ht[KM:D, :])
        return carry
    assert V0 % REP == 0 and V0 // REP * BQ >= TCH
    ln1(0, 0)
    wqr_cp().wait()
    pre(0, TCH, 0, PG0)
    scc_ref[...] = _as_cols(sc).astype(F32)
    prep_cols(wqr_ref[:, 0:GW].astype(F32), PK0, KR)
    wdt_ref[:, FF:FF + WT_W] = jnp.zeros((D, WT_W), BF16)
    wq_buf[:, KM:KM + 16, :] = jnp.zeros((2, 16, GW), BF16)
    lax.fori_loop(1, XCH, ln1, 0)
    gdone = PG0 + (XCH - 1) * PGI
    pre(0, TCH, gdone, NG - gdone)
    if V0 // REP * BQ > TCH:
        pre(TCH, V0 // REP * BQ, 0, NG)
    for n, j in enumerate(range(V0 // REP, NB)):
        for kk in range(KR):
            ht_ref[n, 8 * kk:8 * kk + 8, :] = jnp.broadcast_to(
                hr_ref[kk:kk + 1, j * BQ:(j + 1) * BQ], (8, BQ))

    def fold_modulation():
        sb, cb, gb = (mrow_ref[0:1, i * D:(i + 1) * D] for i in (3, 4, 5))
        for i, z in enumerate((sb, cb, gb)):
            mb_ref[i] = jnp.broadcast_to(z, (8, D))
        fold_ref[0:D, :] = modcol(5) * modcol(4)
        fold_ref[D:MA, :] = modcol(5) * modcol(3)
        wr = wr_ref[...].astype(F32).reshape(1, D)
        wc = wr * cb
        whi = _rb(wc)
        wlo = _rb(wc - whi)
        row = lax.broadcasted_iota(jnp.int32, (16, D), 0)
        lhs_ref[...] = jnp.where(row == 0, 1.0, jnp.where(row == 1, whi, jnp.where(
            row == 2, wlo, 0.0))).astype(BF16)
        rc_ref[0:1, :] = jnp.broadcast_to(jnp.sum(whi + wlo, axis=1, keepdims=True), (1, LANES))
        rc_ref[1:2, :] = jnp.broadcast_to(jnp.sum(wr * sb, axis=1, keepdims=True), (1, LANES))

    def group_step(step, carry):
        @pl.when(step == MOD_STEP)
        def _():
            wmb_cp().wait()
            wd_cp().wait()

        for d in group_copies(step):
            d.wait()

        slot = step % 2
        k = k_buf[slot]
        v = v_buf[slot]
        wq = wq_buf[slot, 0:KM]
        wot = wot_buf[slot]

        nev = lax.broadcasted_iota(jnp.int32, (8, BQ), 1) > step + BQ
        assert VA == 16 and BQ == 2 * LANES
        npb = GW // VA
        L0, L1, B0 = V0 * DH // VA, NB * npb, V0 // REP

        def link(i, gate):
            av = ht_ref[i // npb - B0]
            bv = bp_ref[:, pl.ds(pl.multiple_of((i % npb) * VA, VA), VA), :]
            bv = jnp.concatenate([bv, bv], axis=2)
            acc = None
            for kk in range(KR):
                a = av[8 * kk:8 * kk + 8]
                if (kk * GF) % 8 < GF:
                    a = jnp.where(nev, gate, a)
                t = bv[kk] * jnp.concatenate([a, a], axis=0)
                acc = t if acc is None else acc + t
                g0 = 8 * ((kk * GF) // 8 % 2)
                g1 = 8 - g0
                gate = jnp.concatenate([acc[g0:g0 + 8, LANES:], acc[g1:g1 + 8, 0:LANES]], axis=1)
            rem_ref[pl.ds(pl.multiple_of((i - L0) * VA, VA), VA), :] = acc
            gate_ref[i - L0] = gate
            return gate

        gate = lax.fori_loop(L0, L1, link, jnp.zeros((8, BQ), F32), unroll=True)
        gates = [functools.partial(lambda i: gate_ref[i], i) for i in range(L1 - L0)]
        dues = [VMARG + (i + 1) * VPER for i in range(len(gates))]
        wn = wqr_ref[:, pl.ds(pl.multiple_of(jnp.minimum(step + 1, NG - 1) * GW, GW), GW)].astype(F32)
        for k0 in range(0, KR, PL):
            k1 = min(k0 + PL, KR)
            blks = {r0: jnp.where(nev, gate, wn[r0:r0 + 8, :]) for r0 in range(k0 // 8 * 8, k1, 8)}
            for kk in range(k0, k1):
                last = _as_cols(blks[kk // 8 * 8][kk % 8:kk % 8 + 1, :]).astype(F32)
                bp_ref[kk] = last
                g = jnp.concatenate([last[GW - 8:GW], last[LANES - 8:LANES]], axis=1)
                gate = gate + g if max(k0, k1 - PA) < kk else g
            gates.append(functools.partial(lambda g: g, gate))
            dues.append(PT0 + (k0 // PL + 1) * PPER)
        clock = [0]
        pinned = [0]

        def pin(x, final=False):
            due = len(gates) if final else sum(1 for t in dues if t <= clock[0])
            if due <= pinned[0]:
                return x
            pinned[0] = due
            g = pltpu.bitcast(gates[due - 1](), U32)
            xu = pltpu.bitcast(x, U32)
            top = xu[0:8, 0:LANES]
            top = jnp.where(nev[:, 0:LANES], g[:, 0:LANES], jnp.where(nev[:, LANES:], g[:, LANES:], top))
            if xu.shape[1] > LANES:
                top = jnp.concatenate([top, xu[0:8, LANES:]], axis=1)
            return pltpu.bitcast(jnp.concatenate([top, xu[8:]], axis=0), BF16)

        def qproj(j):
            hb = pin(pltpu.bitcast(h_ref[j * (BQ // 2):(j + 1) * (BQ // 2), :], BF16))
            clock[0] += 512
            if REP * j < V0:
                rem = pre_ref[step, j * BQ:(j + 1) * BQ, :]
            else:
                rem = rem_ref[(REP * j - V0) * DH:(REP * j + REP - V0) * DH, :].T
            q2 = jnp.dot(hb[:, 0:KM], wq, preferred_element_type=F32) + rem
            return (q2 * qscale).astype(BF16)

        def qk(ci, lo, hi):
            q = pin(qs[ci])
            clock[0] += (hi - lo) // 2
            return lax.dot_general(q, k[lo:hi], _NT, preferred_element_type=F32)

        def softmax_pv(s, mode):
            m = jnp.max(s, axis=1, keepdims=True)
            p = jnp.exp2(s - m)
            parts = [p[:, i * LANES:(i + 1) * LANES] for i in range(SK // LANES)]
            if mode == 2:
                lp = None
                for c in range(0, len(parts), 4):
                    t = (parts[c] + parts[c + 1]) + (parts[c + 2] + parts[c + 3])
                    lp = t if lp is None else lp + t
                    parts[c + 3] = jnp.where(lp < 0.0, lp, parts[c + 3])
                p = jnp.concatenate(parts, axis=1)
            clock[0] += SK // 2
            o = jnp.dot(p.astype(BF16), v, preferred_element_type=F32)
            if mode == 0:
                l = jnp.sum(p, axis=1, keepdims=True)
            elif mode == 1:
                lp = functools.reduce(lambda x, y: x + y, parts)
                l = jnp.sum(jnp.where(lp < 0.0, o, lp), axis=1, keepdims=True)
            else:
                l = jnp.sum(lp, axis=1, keepdims=True)
            rl = pl.reciprocal(l, approx=True)
            rl = rl * (2.0 - l * rl)
            return (o * rl).astype(BF16)

        def oproj(j):
            o2 = jnp.concatenate([outs[REP * j + r] for r in range(REP)], axis=1)
            w = pin(wot, final=(j == NB - 1))
            clock[0] += 576
            acc_ref[:, j * BQ:(j + 1) * BQ] += lax.dot_general(w, o2, _NT, preferred_element_type=F32)

        qs, outs = {}, []

        def fill(pos):
            for j in range(NB):
                if QP_POS[j] == pos:
                    q2 = qproj(j)
                    for r in range(REP):
                        qs[REP * j + r] = q2[:, r * DH:(r + 1) * DH]
            for j in range(NB):
                if OP_POS[j] == pos:
                    oproj(j)

        NC = NB * REP
        assert (NG - MOD_STEP) * WT_W == FF
        wc0 = jnp.where(step >= MOD_STEP, (step - MOD_STEP) * WT_W, FF)
        never8 = lax.broadcasted_iota(jnp.int32, (8, LANES), 1) > step + LANES
        wtie = None
        for t0 in range(0, WT_W, LANES):
            for r0 in range(0, D, WT_R):
                r1 = min(r0 + WT_R, D)
                blk = pltpu.bitcast(wdt_ref[r0:r1, pl.ds(pl.multiple_of(wc0 + t0, LANES), LANES)], U32)
                if wtie is not None:
                    blk = jnp.concatenate([jnp.where(never8, wtie, blk[0:8]), blk[8:]], axis=0)
                tb = pltpu.bitcast(pltpu.bitcast(blk, BF16).T, U32)
                wd_ref[pl.ds(pl.multiple_of((wc0 + t0) // 2, LANES // 2), LANES // 2), r0:r1] = tb
                wtie = wd_ref[pl.ds(pl.multiple_of(wc0 // 2, LANES // 2), 8), 0:LANES]
        nms = 4 * D // MT_W
        assert nms * MT_W == 4 * D and MOD_STEP + nms < NG
        in_win = (step >= MOD_STEP) & (step < MOD_STEP + nms)
        mc0 = pl.multiple_of(jnp.where(in_win, MA + (step - MOD_STEP) * MT_W, 0), LANES)
        gate8 = pltpu.bitcast(wtie, F32)
        for r0 in range(0, D, MT_R):
            sc8 = scc_ref[r0:r0 + MT_R, :]
            sc8 = jnp.concatenate([jnp.where(never8, gate8, sc8[0:8])] + ([sc8[8:]] if MT_R > 8 else []), axis=0)
            t = wmod_ref[r0:r0 + MT_R, pl.ds(mc0, MT_W)].astype(F32) * _tile(sc8, MT_W // LANES)
            macc = t if r0 == 0 else macc + t
            gate8 = macc[0:8, 0:LANES]
        mrow = finish_mod(jnp.sum(macc, axis=0, keepdims=True), mc0)
        mrow_ref[0:1, pl.ds(mc0, MT_W)] = mrow
        modc_ref[pl.ds(mc0, MT_W), :] = _as_cols(mrow).astype(F32)
        wtie = pltpu.bitcast(modc_ref[0:8, :], U32)
        fill(-1)
        qt = pltpu.bitcast(qs[WT_TIE], U32)
        qs[WT_TIE] = pltpu.bitcast(
            jnp.concatenate([jnp.where(never8, wtie, qt[0:8]), qt[8:]], axis=0), BF16)
        s_head = None
        for ci in range(NC):
            lo = HEAD[ci - 1] if ci else 0
            if ci == DMA_AT:
                qt = pltpu.bitcast(qs[ci], U32)
                tok = pltpu.bitcast(wq_buf[slot, KM:KM + 16, 0:LANES], U32)
                qs[ci] = pltpu.bitcast(
                    jnp.concatenate([jnp.where(never8, tok, qt[0:8]), qt[8:]], axis=0), BF16)
            s = qk(ci, lo, SK)
            if lo:
                s = jnp.concatenate([s_head, s], axis=1)
            fill(2 * ci)
            if HEAD[ci]:
                s_head = qk(ci + 1, 0, HEAD[ci])
            outs.append(softmax_pv(s, MODE[ci]))
            fill(2 * ci + 1)

        @pl.when(step + 2 < NG)
        def _():
            for d in group_copies(step + 2):
                d.start()

        @pl.when(step == 0)
        def _():
            wmb_cp().start()
            wg_cp().start()

        @pl.when(step == 1)
        def _():
            wu_cp().start()

        @pl.when(step == 2)
        def _():
            wd_cp().start()

        return step

    step = lax.fori_loop(0, NG, group_step, 0)

    wr_cp().wait()
    fold_modulation()
    for sl in range(NSL):
        cols = slice(sl * LANES, (sl + 1) * LANES)
        for r0 in range(0, D, LANES):
            r1 = min(r0 + LANES, D)
            x2 = xt_ref[r0:r1, cols].astype(F32) + modc_ref[MA + r0:MA + r1, :] * acc_ref[r0:r1, cols]
            acc_ref[r0:r1, cols] = x2
            xb = x2.astype(BF16)
            xb_ref[r0 // 2:r1 // 2, cols] = pltpu.bitcast(xb, U32)
            if r0 == 0:
                piv = jnp.mean(x2[0:8, :], axis=0, keepdims=True)
                st_ref[0, sl:sl + 1, :] = piv
            d = x2 - piv
            lhs = lhs_ref[:, r0:r1]
            t1 = jnp.dot(lhs, xb, preferred_element_type=F32)[0:8, :]
            t2 = jnp.dot(lhs, (d * d).astype(BF16), preferred_element_type=F32)[0:8, :]
            s1, s2 = (t1, t2) if r0 == 0 else (s1 + t1, s2 + t2)
        for n in range(3):
            st_ref[1 + n, sl:sl + 1, :] = s1[n:n + 1, :]
        st_ref[4, sl:sl + 1, :] = s2[0:1, :]

    wg_cp().wait()
    wu_cp().wait()

    mean = st_ref[1] * (1.0 / D)
    md = mean - st_ref[0]
    mb, sd = _ln_rows(mean, jnp.maximum(st_ref[4] * (1.0 / D) - md * md, 0.0))
    rs = 1.0 / sd
    st_ref[5] = rs
    st_ref[6] = mb * rs
    r = (st_ref[2] + st_ref[3] - mb * rc_ref[0:1, :]) * rs + rc_ref[1:2, :]

    lane16 = lax.broadcasted_iota(jnp.int32, (16, LANES), 1)
    never = lane16 > step + LANES

    def after_out_stores():
        dyn0 = pl.multiple_of((step - (NG - 1)) * LANES, LANES)
        return out_ref[0:16, pl.ds(dyn0, LANES)]

    def out_unit(n):
        w = OUW * LANES
        cols = slice(n * w, (n + 1) * w)
        rs, mrs = (jnp.concatenate([st_ref[k, n * OUW + u:n * OUW + u + 1, :]
                                    for u in range(OUW)], axis=1) for k in (5, 6))
        for r0 in range(0, D, OPR):
            x2 = acc_ref[r0:r0 + OPR, cols]
            o = x2 + ((x2 * rs - mrs) * _tile(fold_ref[r0:r0 + OPR, :], OUW)
                      + _tile(fold_ref[D + r0:D + r0 + OPR, :], OUW))
            out_ref[r0:r0 + OPR, cols] = o.astype(BF16)
        return after_out_stores().astype(F32)

    r = _rb(r) + 0.0
    bits = pltpu.bitcast(r, jnp.int32)
    mono = bits ^ ((bits >> 31) & jnp.int32(0x7FFFFFFF))
    tok = (lax.broadcasted_iota(jnp.int32, (NSL, LANES), 0) * LANES
           + lax.broadcasted_iota(jnp.int32, (NSL, LANES), 1))
    keyi = (((mono >> 16) + 32768) * S + (S - 1 - tok)) + jnp.int32(1 << 29)
    key = pltpu.bitcast(keyi, F32)

    row16 = lax.broadcasted_iota(jnp.int32, (16, LANES), 0)
    rowc = lax.broadcasted_iota(jnp.int32, (16, 1), 0)
    sel_slab, sel_off = [], []
    tie, nunit = None, 0
    xsel = jnp.zeros((16, D), F32)
    mbsel = jnp.zeros((16, 1), F32)
    rssel = jnp.zeros((16, 1), F32)
    ksel = jnp.zeros((16, 1), F32)
    for t in range(TOPC):
        kmax = jnp.max(jnp.max(key, axis=0, keepdims=True), axis=1, keepdims=True)
        hit = key == kmax
        key = jnp.where(hit, 0.0, key)
        pick = lambda z: jnp.sum(jnp.sum(jnp.where(hit, z, 0.0), axis=0, keepdims=True),
                                 axis=1, keepdims=True)
        mbsel = jnp.where(rowc == t, pick(mb), mbsel)
        rssel = jnp.where(rowc == t, pick(rs), rssel)
        for _ in range(TK_TIES.count(t)):
            tie = out_unit(nunit)
            nunit += 1
            key = jnp.where(never, tie, key)
        ksel = jnp.where(rowc == t, kmax, ksel)
        ki = pltpu.bitcast(kmax, jnp.int32)[0, 0]
        idx = (S - 1) - (ki & (S - 1))
        slab = idx >> 7
        off = idx & (LANES - 1)
        onehot = jnp.where((row16 == t) & (lane16 == off), 1.0, 0.0).astype(BF16)
        dslab = xb_ref[:, pl.ds(pl.multiple_of(slab * LANES, LANES), LANES)]
        xsel = xsel + lax.dot_general(onehot, pltpu.bitcast(dslab, BF16), _NT,
                                      preferred_element_type=F32)
        sel_slab.append(slab)
        sel_off.append(off)
    nsel = _rb(_rb(xsel - mbsel) * rssel)
    hsel = _rb(_rb(nsel * mb_ref[1, 0:1, :]) + mb_ref[0, 0:1, :])
    hi = ((pltpu.bitcast(ksel, jnp.int32) - jnp.int32(1 << 29)) // S - 32768) << 16
    rbits = hi ^ ((hi >> 31) & jnp.int32(0x7FFF0000))
    gate = _rb(_sigmoid(jnp.where(rowc < TOPC, pltpu.bitcast(rbits, F32), 0.0)))

    def out_copy(sl, r0, nr):
        c0 = pl.multiple_of(sl * LANES, LANES)
        return cp(out_ref.at[r0:r0 + nr, pl.ds(c0, LANES)],
                  out_hbm.at[r0:r0 + nr, pl.ds(c0, LANES)], S_O)

    fresh = []
    seen = jnp.int32(0)
    for t in range(TOPC):
        fresh.append(((seen >> sel_slab[t]) & 1) == 0)
        seen = seen | (1 << sel_slab[t])
    plain = [((seen >> sl) & 1) == 0 for sl in range(NSL)]

    for n in range(nunit, NSL // OUW):
        tie = out_unit(n)
    for sl in range(NSL):
        pl.when(plain[sl])(lambda sl=sl: out_copy(sl, 0, D).start())

    h0 = jnp.where(never, tie, hsel[:, 0:LANES])
    hs = jnp.concatenate([h0, hsel[:, LANES:]], axis=1).astype(BF16)
    gpre = _rb(jnp.dot(hs, wg_ref[...], preferred_element_type=F32))
    u = _rb(jnp.dot(hs, wu_ref[...], preferred_element_type=F32))
    a = (_rb(gpre * _sigmoid(gpre)) * u).astype(BF16)

    gb = mb_ref[2, 0:1, :]

    def down(r0, nr, tied):
        lhs = a
        if tied:
            a0 = jnp.where(never[0:8, :], pltpu.bitcast(after_out_stores(), U32),
                           pltpu.bitcast(a[:, TIEC:TIEC + LANES], U32))
            lhs = jnp.concatenate([a[:, 0:TIEC], pltpu.bitcast(a0, BF16), a[:, TIEC + LANES:]], axis=1)
        y = jnp.dot(lhs, pltpu.bitcast(wd_ref[0:FF // 2, r0:r0 + nr], BF16),
                    preferred_element_type=F32)
        c = slice(r0, r0 + nr)
        return xsel[:, c] + gb[:, c] * (hsel[:, c] + y * gate)

    def patch(r0, nr, new):
        lane = lax.broadcasted_iota(jnp.int32, (nr // 2, LANES), 1)
        for t in range(TOPC):
            cols = pl.ds(pl.multiple_of(sel_slab[t] * LANES, LANES), LANES)
            old = pltpu.bitcast(out_ref[r0:r0 + nr, cols], U32)
            upd = pltpu.bitcast(_as_cols(new[t:t + 1, :]), U32)
            out_ref[r0:r0 + nr, cols] = pltpu.bitcast(jnp.where(lane == sel_off[t], upd, old), BF16)
        for t in range(TOPC):
            pl.when(fresh[t])(lambda t=t: out_copy(sel_slab[t], r0, nr).start())

    news = [down(*PIECES[0], False)]
    for n in range(len(PIECES)):
        if n + 1 < len(PIECES):
            news.append(down(*PIECES[n + 1], n > 0))
        patch(*PIECES[n], news[n])

    cp(out_ref, out_hbm, S_O).wait()


@jax.jit
def pallas_adaLN_cond__gqa_block_cached__moe_arch_mod__prompt_kernel(
    A_x: jax.Array,
    A_k_cache: jax.Array,
    A_v_cache: jax.Array,
    A_wq: jax.Array,
    A_wo: jax.Array,
    B_x: jax.Array,
    B_w_r: jax.Array,
    B_w_gate: jax.Array,
    B_w_up: jax.Array,
    B_w_down: jax.Array,
    c: jax.Array,
    w_mod: jax.Array,
):
    del B_x
    B, S, D = A_x.shape
    assert B == 1
    NG, SK = A_k_cache.shape[1], A_k_cache.shape[2]
    REP = HQ // NG
    FF = B_w_gate.shape[1]
    GW = REP * DH

    xt = A_x.reshape(S, D).T
    wot = A_wo.T
    wdt = B_w_down.T
    k = A_k_cache.reshape(NG, SK, DH)
    v = A_v_cache.reshape(NG, SK, DH)

    hbm = pl.BlockSpec(memory_space=pl.ANY)
    out_t = pl.pallas_call(
        functools.partial(_kernel, S=S, SK=SK, D=D, FF=FF, NG=NG, REP=REP),
        in_specs=[hbm] * 11,
        out_specs=hbm,
        out_shape=jax.ShapeDtypeStruct((D, S), BF16),
        scratch_shapes=[
            pltpu.VMEM((D, S), BF16),
            pltpu.VMEM((2, SK, DH), BF16),
            pltpu.VMEM((2, SK, DH), BF16),
            pltpu.VMEM((2, D // LANES * LANES + 16, GW), BF16),
            pltpu.VMEM((2, D, GW), BF16),
            pltpu.VMEM((D % LANES, NG * GW), BF16),
            pltpu.VMEM((D,), BF16),
            pltpu.VMEM((1, D), BF16),
            pltpu.VMEM((D, 6 * D), BF16),
            pltpu.VMEM((D, FF), BF16),
            pltpu.VMEM((D, FF), BF16),
            pltpu.VMEM((D, FF + WT_W), BF16),
            pltpu.VMEM(((FF + WT_W) // 2, D), U32),
            pltpu.VMEM((D, S), BF16),
            pltpu.VMEM((6 * D, LANES), F32),
            pltpu.VMEM((8, 6 * D), F32),
            pltpu.VMEM((D, LANES), F32),
            pltpu.VMEM((2 * D, LANES), F32),
            pltpu.VMEM((3, 8, D), F32),
            pltpu.VMEM((16, D), BF16),
            pltpu.VMEM((8, LANES), F32),
            pltpu.VMEM((S // 2, D), U32),
            pltpu.VMEM((D, S), F32),
            pltpu.VMEM((D // 2, S), U32),
            pltpu.VMEM((7, S // LANES, LANES), F32),
            pltpu.VMEM((D % LANES, S), F32),
            pltpu.VMEM((S // BQ - V0 // REP, D % LANES * 8, BQ), F32),
            pltpu.VMEM((D % LANES, GW, LANES), F32),
            pltpu.VMEM(((S // BQ * REP - V0) * DH, BQ), F32),
            pltpu.VMEM(((S // BQ * REP - V0) * DH // VA, 8, BQ), F32),
            pltpu.VMEM((NG, V0 // REP * BQ, GW), F32),
            pltpu.SemaphoreType.DMA((N_SEMS,)),
        ],
        compiler_params=pltpu.CompilerParams(
            vmem_limit_bytes=120 * 1024 * 1024,
            disable_bounds_checks=True,
        ),
    )(xt, k, v, A_wq, wot, B_w_r, c, w_mod, B_w_gate, B_w_up, wdt)
    return out_t.T.reshape(B, S, D)
```

```python
import functools
import math

import jax
import jax.numpy as jnp
from jax import lax
import jax.experimental.pallas as pl
import jax.experimental.pallas.tpu as pltpu

F32 = jnp.float32
BF16 = jnp.bfloat16
U32 = jnp.uint32

HQ = 32
DH = 128
TOPC = 8
LN_EPS = 1e-5
BQ = 256
LANES = 128
XCH = 4

HEAD = [0, 1280, 1536, 1280, 1536, 1024, 768, 1024, 1536, 1280, 1536, 1536, 640, 1536, 512, 0]
MODE = [2, 2, 2, 2, 0, 2, 0, 0, 1, 1, 2, 0, 0, 2, 1, 2]
QP_POS = [-1, -1, -1, -1, -1, 3, 18, -1]
OP_POS = [7, 12, 17, 25, 30, 31, 31, 31]
V0 = 4
VA = 16
GF = 2
VPER = 300
VMARG = 300
PL = 4
PA = 1
PT0 = 29864
PPER = 515
WT_W = 384
WT_R = 256
WT_TIE = 0
MT_W = 256
MT_R = 8
PK0 = 56
ZC = 1024
DMA_AT = 14
PG0 = 5
PGI = 3
OUW = 2
OPR = 16
TK_TIES = [0, 1, 2, 3, 4, 5, 6]
PIECES = [(0, 128), (128, 128), (256, 128), (384, 128), (512, 64)]
TIEC = 2048

_NT = (((1,), (1,)), ((), ()))

S_C = S_WMA = 0
S_ST = 1
S_WR = 2
S_WG = S_WU = 3
S_WQ0 = 4
S_WQR = 5
S_X = 6
S_G = S_X + XCH
S_O = S_G + 2
N_SEMS = S_O + 1


def _rb(x):
    return x.astype(BF16).astype(F32)


def _sigmoid(x):
    return 1.0 / (1.0 + jnp.exp(-x))


def _ln_rows(mean, var):
    eps = _rb(jnp.full((1, 1), LN_EPS, F32))
    return _rb(mean), _rb(jnp.sqrt(_rb(_rb(var) + eps)))


def _tile(col, n):
    return jnp.concatenate([col] * n, axis=1)


def _as_cols(row):
    return jnp.broadcast_to(row, (LANES, row.shape[1])).astype(BF16).T


def _kernel(xt_hbm, k_hbm, v_hbm, wq_hbm, wot_hbm, wr_hbm, c_hbm, wmod_hbm,
            wg_hbm, wu_hbm, wdt_hbm,
            out_hbm,
            xt_ref, k_buf, v_buf, wq_buf, wot_buf, wqr_ref, wr_ref, c_ref, wmod_ref, wms_ref,
            wg_ref, wu_ref, wdt_ref, wd_ref, out_ref,
            modc_ref, mrow_ref, scc_ref, fold_ref, mb_ref, lhs_ref, rc_ref, h_ref, acc_ref, xb_ref, st_ref, hr_ref, ht_ref, bp_ref, rem_ref, gate_ref, pre_ref,
            sems,
            *, S, SK, D, FF, NG, REP):
    qscale = (DH ** -0.5) * math.log2(math.e)
    NB = S // BQ
    GW = REP * DH
    TCH = S // XCH
    MA = 2 * D
    NSL = S // LANES
    KM = D // LANES * LANES
    KR = D - KM

    def cp(src, dst, sem):
        return pltpu.make_async_copy(src, dst, sems.at[sem])

    def x_copy(i):
        cols = pl.ds(pl.multiple_of(i * TCH, TCH), TCH)
        return cp(xt_hbm.at[:, cols], xt_ref.at[:, cols], S_X + i)

    def group_copies(grp, which=(0, 1, 2, 3)):
        slot = grp % 2
        cols = pl.ds(pl.multiple_of(grp * GW, GW), GW)
        ends = ((lambda: (wq_hbm.at[0:KM, cols], wq_buf.at[slot, 0:KM])),
                (lambda: (k_hbm.at[grp], k_buf.at[slot])),
                (lambda: (v_hbm.at[grp], v_buf.at[slot])),
                (lambda: (wot_hbm.at[:, cols], wot_buf.at[slot])))
        return [cp(*ends[i](), S_G + slot) for i in which]

    wq0_cp = lambda: cp(wq_hbm.at[KM:D, 0:GW], wqr_ref.at[:, 0:GW], S_WQ0)
    wqr_cp = lambda: cp(wq_hbm.at[KM:D, GW:NG * GW], wqr_ref.at[:, GW:NG * GW], S_WQR)
    c_cp = lambda: cp(c_hbm, c_ref, S_C)
    wma_cp = lambda: cp(wmod_hbm.at[:, 0:MA], wmod_ref, S_WMA)
    wr_cp = lambda: cp(wr_hbm, wr_ref, S_WR)
    wg_cp = lambda: cp(wg_hbm, wg_ref, S_WG)
    wu_cp = lambda: cp(wu_hbm, wu_ref, S_WU)

    def side_cols(step):
        return (pl.multiple_of(jnp.clip(step - 1, 0, FF // WT_W - 1) * WT_W, LANES),
                pl.multiple_of(MA + jnp.clip(step - 1, 0, 4 * D // MT_W - 1) * MT_W, LANES))

    def side_copies(step):
        wc, mc = side_cols(step)
        return (cp(wdt_hbm.at[:, pl.ds(wc, WT_W)], wdt_ref, S_ST),
                cp(wmod_hbm.at[:, pl.ds(mc, MT_W)], wms_ref, S_ST))

    def modcol(i):
        return modc_ref[i * D:(i + 1) * D, :]

    def finish_mod(mod, col0):
        mod = _rb(mod)
        lane = lax.broadcasted_iota(jnp.int32, mod.shape, 1) + col0
        is_scale = ((lane >= D) & (lane < 2 * D)) | ((lane >= 4 * D) & (lane < 5 * D))
        return jnp.where(is_scale, _rb(1.0 + mod), mod)

    def prep_cols(w, k0, k1):
        for kk in range(k0, k1):
            bp_ref[kk] = _as_cols(w[kk:kk + 1, :]).astype(F32)

    wq0_cp().start()
    wma_cp().start()
    c_cp().start()
    for i in range(XCH):
        x_copy(i).start()
        if i == 0:
            wqr_cp().start()
    for d in group_copies(0) + group_copies(1):
        d.start()
    wr_cp().start()
    acc_ref[:, 0:ZC] = jnp.zeros((D, ZC), F32)
    wq0_cp().wait()
    acc_ref[:, ZC:S] = jnp.zeros((D, S - ZC), F32)
    prep_cols(wqr_ref[:, 0:GW].astype(F32), 0, PK0)
    wma_cp().wait()
    c_cp().wait()
    c = c_ref[...].astype(F32)
    sc = _rb(c * _sigmoid(c))
    mod = jnp.dot(jnp.broadcast_to(sc, (8, D)).astype(BF16), wmod_ref[...],
                  preferred_element_type=F32)
    modc_ref[0:MA, :] = _as_cols(finish_mod(mod, 0)[0:1, :]).astype(F32)

    def pre(t0, t1, g0, ng):
        hb = pltpu.bitcast(h_ref[t0 // 2:t1 // 2, :], BF16)[:, KM:D]
        for u in range(ng):
            cols = pl.ds(pl.multiple_of((g0 + u) * GW, GW), GW)
            pre_ref[g0 + u, t0:t1, :] = jnp.dot(hb, wqr_ref[:, cols], preferred_element_type=F32)

    def ln1(i, carry):
        x_copy(i).wait()
        if not isinstance(i, int):
            pre(0, TCH, PG0 + (i - 1) * PGI, PGI)
        x = xt_ref[:, pl.ds(pl.multiple_of(i * TCH, TCH), TCH)].astype(F32)
        piv = x[0:1, :]
        d = x - piv
        md = jnp.mean(d, axis=0, keepdims=True)
        var = jnp.maximum(jnp.mean(d * d, axis=0, keepdims=True) - md * md, 0.0)
        mb, sd = _ln_rows(piv + md, var)
        rs = 1.0 / sd
        n = TCH // LANES
        ht = (x * rs - mb * rs) * _tile(modcol(1), n) + _tile(modcol(0), n)
        h_ref[pl.ds(pl.multiple_of(i * (TCH // 2), TCH // 2), TCH // 2), :] = pltpu.bitcast(
            ht.astype(BF16).T, U32)
        hr_ref[:, pl.ds(pl.multiple_of(i * TCH, TCH), TCH)] = _rb(ht[KM:D, :])
        return carry
    assert V0 % REP == 0 and V0 // REP * BQ >= TCH
    ln1(0, 0)
    wqr_cp().wait()
    pre(0, TCH, 0, PG0)
    scc_ref[...] = _as_cols(sc).astype(F32)
    prep_cols(wqr_ref[:, 0:GW].astype(F32), PK0, KR)
    wdt_ref[...] = jnp.zeros((D, WT_W), BF16)
    wms_ref[...] = jnp.zeros((D, MT_W), BF16)
    wq_buf[:, KM:KM + 16, :] = jnp.zeros((2, 16, GW), BF16)
    lax.fori_loop(1, XCH, ln1, 0)
    gdone = PG0 + (XCH - 1) * PGI
    pre(0, TCH, gdone, NG - gdone)
    if V0 // REP * BQ > TCH:
        pre(TCH, V0 // REP * BQ, 0, NG)
    for n, j in enumerate(range(V0 // REP, NB)):
        for kk in range(KR):
            ht_ref[n, 8 * kk:8 * kk + 8, :] = jnp.broadcast_to(
                hr_ref[kk:kk + 1, j * BQ:(j + 1) * BQ], (8, BQ))

    def fold_modulation():
        sb, cb, gb = (mrow_ref[0:1, i * D:(i + 1) * D] for i in (3, 4, 5))
        for i, z in enumerate((sb, cb, gb)):
            mb_ref[i] = jnp.broadcast_to(z, (8, D))
        fold_ref[0:D, :] = modcol(5) * modcol(4)
        fold_ref[D:MA, :] = modcol(5) * modcol(3)
        wr = wr_ref[...].astype(F32).reshape(1, D)
        wc = wr * cb
        whi = _rb(wc)
        wlo = _rb(wc - whi)
        row = lax.broadcasted_iota(jnp.int32, (16, D), 0)
        lhs_ref[...] = jnp.where(row == 0, 1.0, jnp.where(row == 1, whi, jnp.where(
            row == 2, wlo, 0.0))).astype(BF16)
        rc_ref[0:1, :] = jnp.broadcast_to(jnp.sum(whi + wlo, axis=1, keepdims=True), (1, LANES))
        rc_ref[1:2, :] = jnp.broadcast_to(jnp.sum(wr * sb, axis=1, keepdims=True), (1, LANES))

    def group_step(step, carry):
        @pl.when(step > 0)
        def _():
            for d in side_copies(step):
                d.wait()

        for d in group_copies(step):
            d.wait()

        slot = step % 2
        k = k_buf[slot]
        v = v_buf[slot]
        wq = wq_buf[slot, 0:KM]
        wot = wot_buf[slot]

        nev = lax.broadcasted_iota(jnp.int32, (8, BQ), 1) > step + BQ
        assert VA == 16 and BQ == 2 * LANES
        npb = GW // VA
        L0, L1, B0 = V0 * DH // VA, NB * npb, V0 // REP

        def link(i, gate):
            av = ht_ref[i // npb - B0]
            bv = bp_ref[:, pl.ds(pl.multiple_of((i % npb) * VA, VA), VA), :]
            bv = jnp.concatenate([bv, bv], axis=2)
            acc = None
            for kk in range(KR):
                a = av[8 * kk:8 * kk + 8]
                if (kk * GF) % 8 < GF:
                    a = jnp.where(nev, gate, a)
                t = bv[kk] * jnp.concatenate([a, a], axis=0)
                acc = t if acc is None else acc + t
                g0 = 8 * ((kk * GF) // 8 % 2)
                g1 = 8 - g0
                gate = jnp.concatenate([acc[g0:g0 + 8, LANES:], acc[g1:g1 + 8, 0:LANES]], axis=1)
            rem_ref[pl.ds(pl.multiple_of((i - L0) * VA, VA), VA), :] = acc
            gate_ref[i - L0] = gate
            return gate

        gate = lax.fori_loop(L0, L1, link, jnp.zeros((8, BQ), F32), unroll=True)
        gates = [functools.partial(lambda i: gate_ref[i], i) for i in range(L1 - L0)]
        dues = [VMARG + (i + 1) * VPER for i in range(len(gates))]
        wn = wqr_ref[:, pl.ds(pl.multiple_of(jnp.minimum(step + 1, NG - 1) * GW, GW), GW)].astype(F32)
        for k0 in range(0, KR, PL):
            k1 = min(k0 + PL, KR)
            blks = {r0: jnp.where(nev, gate, wn[r0:r0 + 8, :]) for r0 in range(k0 // 8 * 8, k1, 8)}
            for kk in range(k0, k1):
                last = _as_cols(blks[kk // 8 * 8][kk % 8:kk % 8 + 1, :]).astype(F32)
                bp_ref[kk] = last
                g = jnp.concatenate([last[GW - 8:GW], last[LANES - 8:LANES]], axis=1)
                gate = gate + g if max(k0, k1 - PA) < kk else g
            gates.append(functools.partial(lambda g: g, gate))
            dues.append(PT0 + (k0 // PL + 1) * PPER)
        clock = [0]
        pinned = [0]

        def pin(x, final=False):
            due = len(gates) if final else sum(1 for t in dues if t <= clock[0])
            if due <= pinned[0]:
                return x
            pinned[0] = due
            g = pltpu.bitcast(gates[due - 1](), U32)
            xu = pltpu.bitcast(x, U32)
            top = xu[0:8, 0:LANES]
            top = jnp.where(nev[:, 0:LANES], g[:, 0:LANES], jnp.where(nev[:, LANES:], g[:, LANES:], top))
            if xu.shape[1] > LANES:
                top = jnp.concatenate([top, xu[0:8, LANES:]], axis=1)
            return pltpu.bitcast(jnp.concatenate([top, xu[8:]], axis=0), BF16)

        def qproj(j):
            hb = pin(pltpu.bitcast(h_ref[j * (BQ // 2):(j + 1) * (BQ // 2), :], BF16))
            clock[0] += 512
            if REP * j < V0:
                rem = pre_ref[step, j * BQ:(j + 1) * BQ, :]
            else:
                rem = rem_ref[(REP * j - V0) * DH:(REP * j + REP - V0) * DH, :].T
            q2 = jnp.dot(hb[:, 0:KM], wq, preferred_element_type=F32) + rem
            return (q2 * qscale).astype(BF16)

        def qk(ci, lo, hi):
            q = pin(qs[ci])
            clock[0] += (hi - lo) // 2
            return lax.dot_general(q, k[lo:hi], _NT, preferred_element_type=F32)

        def softmax_pv(s, mode):
            m = jnp.max(s, axis=1, keepdims=True)
            p = jnp.exp2(s - m)
            parts = [p[:, i * LANES:(i + 1) * LANES] for i in range(SK // LANES)]
            if mode == 2:
                lp = None
                for c in range(0, len(parts), 4):
                    t = (parts[c] + parts[c + 1]) + (parts[c + 2] + parts[c + 3])
                    lp = t if lp is None else lp + t
                    parts[c + 3] = jnp.where(lp < 0.0, lp, parts[c + 3])
                p = jnp.concatenate(parts, axis=1)
            clock[0] += SK // 2
            o = jnp.dot(p.astype(BF16), v, preferred_element_type=F32)
            if mode == 0:
                l = jnp.sum(p, axis=1, keepdims=True)
            elif mode == 1:
                lp = functools.reduce(lambda x, y: x + y, parts)
                l = jnp.sum(jnp.where(lp < 0.0, o, lp), axis=1, keepdims=True)
            else:
                l = jnp.sum(lp, axis=1, keepdims=True)
            rl = pl.reciprocal(l, approx=True)
            rl = rl * (2.0 - l * rl)
            return (o * rl).astype(BF16)

        def oproj(j):
            o2 = jnp.concatenate([outs[REP * j + r] for r in range(REP)], axis=1)
            w = pin(wot, final=(j == NB - 1))
            clock[0] += 576
            acc_ref[:, j * BQ:(j + 1) * BQ] += lax.dot_general(w, o2, _NT, preferred_element_type=F32)

        qs, outs = {}, []

        def fill(pos):
            for j in range(NB):
                if QP_POS[j] == pos:
                    q2 = qproj(j)
                    for r in range(REP):
                        qs[REP * j + r] = q2[:, r * DH:(r + 1) * DH]
            for j in range(NB):
                if OP_POS[j] == pos:
                    oproj(j)

        NC = NB * REP
        assert FF % WT_W == 0 and FF // WT_W < NG and (4 * D) % MT_W == 0 and 4 * D // MT_W < NG
        wc0, mc0 = side_cols(step)
        never8 = lax.broadcasted_iota(jnp.int32, (8, LANES), 1) > step + LANES
        wtie = None
        for t0 in range(0, WT_W, LANES):
            for r0 in range(0, D, WT_R):
                r1 = min(r0 + WT_R, D)
                blk = pltpu.bitcast(wdt_ref[r0:r1, t0:t0 + LANES], U32)
                if wtie is not None:
                    blk = jnp.concatenate([jnp.where(never8, wtie, blk[0:8]), blk[8:]], axis=0)
                tb = pltpu.bitcast(pltpu.bitcast(blk, BF16).T, U32)
                wd_ref[pl.ds(pl.multiple_of((wc0 + t0) // 2, LANES // 2), LANES // 2), r0:r1] = tb
                wtie = wd_ref[pl.ds(pl.multiple_of(wc0 // 2, LANES // 2), 8), 0:LANES]
        gate8 = pltpu.bitcast(wtie, F32)
        for r0 in range(0, D, MT_R):
            sc8 = scc_ref[r0:r0 + MT_R, :]
            sc8 = jnp.concatenate([jnp.where(never8, gate8, sc8[0:8])] + ([sc8[8:]] if MT_R > 8 else []), axis=0)
            t = wms_ref[r0:r0 + MT_R, :].astype(F32) * _tile(sc8, MT_W // LANES)
            macc = t if r0 == 0 else macc + t
            gate8 = macc[0:8, 0:LANES]
        mrow = finish_mod(jnp.sum(macc, axis=0, keepdims=True), mc0)
        mrow_ref[0:1, pl.ds(mc0, MT_W)] = mrow
        modc_ref[pl.ds(mc0, MT_W), :] = _as_cols(mrow).astype(F32)
        wtie = pltpu.bitcast(modc_ref[0:8, :], U32)
        fill(-1)
        qt = pltpu.bitcast(qs[WT_TIE], U32)
        qs[WT_TIE] = pltpu.bitcast(
            jnp.concatenate([jnp.where(never8, wtie, qt[0:8]), qt[8:]], axis=0), BF16)
        s_head = None
        for ci in range(NC):
            lo = HEAD[ci - 1] if ci else 0
            if ci == DMA_AT:
                qt = pltpu.bitcast(qs[ci], U32)
                tok = pltpu.bitcast(wq_buf[slot, KM:KM + 16, 0:LANES], U32)
                qs[ci] = pltpu.bitcast(
                    jnp.concatenate([jnp.where(never8, tok, qt[0:8]), qt[8:]], axis=0), BF16)
            s = qk(ci, lo, SK)
            if lo:
                s = jnp.concatenate([s_head, s], axis=1)
            fill(2 * ci)
            if HEAD[ci]:
                s_head = qk(ci + 1, 0, HEAD[ci])
            outs.append(softmax_pv(s, MODE[ci]))
            fill(2 * ci + 1)

        pl.when(step + 2 < NG)(lambda: group_copies(step + 2, (0,))[0].start())

        @pl.when(step + 1 < NG)
        def _():
            for d in side_copies(step + 1):
                d.start()

        @pl.when(step + 2 < NG)
        def _():
            for d in group_copies(step + 2, (1, 2, 3)):
                d.start()

        @pl.when(step == 0)
        def _():
            wg_cp().start()

        @pl.when(step == 1)
        def _():
            wu_cp().start()

        return step

    step = lax.fori_loop(0, NG, group_step, 0)

    wr_cp().wait()
    fold_modulation()
    for sl in range(NSL):
        cols = slice(sl * LANES, (sl + 1) * LANES)
        for r0 in range(0, D, LANES):
            r1 = min(r0 + LANES, D)
            x2 = xt_ref[r0:r1, cols].astype(F32) + modc_ref[MA + r0:MA + r1, :] * acc_ref[r0:r1, cols]
            acc_ref[r0:r1, cols] = x2
            xb = x2.astype(BF16)
            xb_ref[r0 // 2:r1 // 2, cols] = pltpu.bitcast(xb, U32)
            if r0 == 0:
                piv = jnp.mean(x2[0:8, :], axis=0, keepdims=True)
                st_ref[0, sl:sl + 1, :] = piv
            d = x2 - piv
            lhs = lhs_ref[:, r0:r1]
            t1 = jnp.dot(lhs, xb, preferred_element_type=F32)[0:8, :]
            t2 = jnp.dot(lhs, (d * d).astype(BF16), preferred_element_type=F32)[0:8, :]
            s1, s2 = (t1, t2) if r0 == 0 else (s1 + t1, s2 + t2)
        for n in range(3):
            st_ref[1 + n, sl:sl + 1, :] = s1[n:n + 1, :]
        st_ref[4, sl:sl + 1, :] = s2[0:1, :]

    wg_cp().wait()
    wu_cp().wait()

    mean = st_ref[1] * (1.0 / D)
    md = mean - st_ref[0]
    mb, sd = _ln_rows(mean, jnp.maximum(st_ref[4] * (1.0 / D) - md * md, 0.0))
    rs = 1.0 / sd
    st_ref[5] = rs
    st_ref[6] = mb * rs
    r = (st_ref[2] + st_ref[3] - mb * rc_ref[0:1, :]) * rs + rc_ref[1:2, :]

    lane16 = lax.broadcasted_iota(jnp.int32, (16, LANES), 1)
    never = lane16 > step + LANES

    def after_out_stores():
        dyn0 = pl.multiple_of((step - (NG - 1)) * LANES, LANES)
        return out_ref[0:16, pl.ds(dyn0, LANES)]

    def out_unit(n):
        w = OUW * LANES
        cols = slice(n * w, (n + 1) * w)
        rs, mrs = (jnp.concatenate([st_ref[k, n * OUW + u:n * OUW + u + 1, :]
                                    for u in range(OUW)], axis=1) for k in (5, 6))
        for r0 in range(0, D, OPR):
            x2 = acc_ref[r0:r0 + OPR, cols]
            o = x2 + ((x2 * rs - mrs) * _tile(fold_ref[r0:r0 + OPR, :], OUW)
                      + _tile(fold_ref[D + r0:D + r0 + OPR, :], OUW))
            out_ref[r0:r0 + OPR, cols] = o.astype(BF16)
        return after_out_stores().astype(F32)

    r = _rb(r) + 0.0
    bits = pltpu.bitcast(r, jnp.int32)
    mono = bits ^ ((bits >> 31) & jnp.int32(0x7FFFFFFF))
    tok = (lax.broadcasted_iota(jnp.int32, (NSL, LANES), 0) * LANES
           + lax.broadcasted_iota(jnp.int32, (NSL, LANES), 1))
    keyi = (((mono >> 16) + 32768) * S + (S - 1 - tok)) + jnp.int32(1 << 29)
    key = pltpu.bitcast(keyi, F32)

    row16 = lax.broadcasted_iota(jnp.int32, (16, LANES), 0)
    rowc = lax.broadcasted_iota(jnp.int32, (16, 1), 0)
    sel_slab, sel_off = [], []
    tie, nunit = None, 0
    xsel = jnp.zeros((16, D), F32)
    mbsel = jnp.zeros((16, 1), F32)
    rssel = jnp.zeros((16, 1), F32)
    ksel = jnp.zeros((16, 1), F32)
    for t in range(TOPC):
        kmax = jnp.max(jnp.max(key, axis=0, keepdims=True), axis=1, keepdims=True)
        hit = key == kmax
        key = jnp.where(hit, 0.0, key)
        pick = lambda z: jnp.sum(jnp.sum(jnp.where(hit, z, 0.0), axis=0, keepdims=True),
                                 axis=1, keepdims=True)
        mbsel = jnp.where(rowc == t, pick(mb), mbsel)
        rssel = jnp.where(rowc == t, pick(rs), rssel)
        for _ in range(TK_TIES.count(t)):
            tie = out_unit(nunit)
            nunit += 1
            key = jnp.where(never, tie, key)
        ksel = jnp.where(rowc == t, kmax, ksel)
        ki = pltpu.bitcast(kmax, jnp.int32)[0, 0]
        idx = (S - 1) - (ki & (S - 1))
        slab = idx >> 7
        off = idx & (LANES - 1)
        onehot = jnp.where((row16 == t) & (lane16 == off), 1.0, 0.0).astype(BF16)
        dslab = xb_ref[:, pl.ds(pl.multiple_of(slab * LANES, LANES), LANES)]
        xsel = xsel + lax.dot_general(onehot, pltpu.bitcast(dslab, BF16), _NT,
                                      preferred_element_type=F32)
        sel_slab.append(slab)
        sel_off.append(off)
    nsel = _rb(_rb(xsel - mbsel) * rssel)
    hsel = _rb(_rb(nsel * mb_ref[1, 0:1, :]) + mb_ref[0, 0:1, :])
    hi = ((pltpu.bitcast(ksel, jnp.int32) - jnp.int32(1 << 29)) // S - 32768) << 16
    rbits = hi ^ ((hi >> 31) & jnp.int32(0x7FFF0000))
    gate = _rb(_sigmoid(jnp.where(rowc < TOPC, pltpu.bitcast(rbits, F32), 0.0)))

    def out_copy(sl, r0, nr):
        c0 = pl.multiple_of(sl * LANES, LANES)
        return cp(out_ref.at[r0:r0 + nr, pl.ds(c0, LANES)],
                  out_hbm.at[r0:r0 + nr, pl.ds(c0, LANES)], S_O)

    fresh = []
    seen = jnp.int32(0)
    for t in range(TOPC):
        fresh.append(((seen >> sel_slab[t]) & 1) == 0)
        seen = seen | (1 << sel_slab[t])
    plain = [((seen >> sl) & 1) == 0 for sl in range(NSL)]

    for n in range(nunit, NSL // OUW):
        tie = out_unit(n)
    for sl in range(NSL):
        pl.when(plain[sl])(lambda sl=sl: out_copy(sl, 0, D).start())

    h0 = jnp.where(never, tie, hsel[:, 0:LANES])
    hs = jnp.concatenate([h0, hsel[:, LANES:]], axis=1).astype(BF16)
    gpre = _rb(jnp.dot(hs, wg_ref[...], preferred_element_type=F32))
    u = _rb(jnp.dot(hs, wu_ref[...], preferred_element_type=F32))
    a = (_rb(gpre * _sigmoid(gpre)) * u).astype(BF16)

    gb = mb_ref[2, 0:1, :]

    def down(r0, nr, tied):
        lhs = a
        if tied:
            a0 = jnp.where(never[0:8, :], pltpu.bitcast(after_out_stores(), U32),
                           pltpu.bitcast(a[:, TIEC:TIEC + LANES], U32))
            lhs = jnp.concatenate([a[:, 0:TIEC], pltpu.bitcast(a0, BF16), a[:, TIEC + LANES:]], axis=1)
        y = jnp.dot(lhs, pltpu.bitcast(wd_ref[0:FF // 2, r0:r0 + nr], BF16),
                    preferred_element_type=F32)
        c = slice(r0, r0 + nr)
        return xsel[:, c] + gb[:, c] * (hsel[:, c] + y * gate)

    def patch(r0, nr, new):
        lane = lax.broadcasted_iota(jnp.int32, (nr // 2, LANES), 1)
        for t in range(TOPC):
            cols = pl.ds(pl.multiple_of(sel_slab[t] * LANES, LANES), LANES)
            old = pltpu.bitcast(out_ref[r0:r0 + nr, cols], U32)
            upd = pltpu.bitcast(_as_cols(new[t:t + 1, :]), U32)
            out_ref[r0:r0 + nr, cols] = pltpu.bitcast(jnp.where(lane == sel_off[t], upd, old), BF16)
        for t in range(TOPC):
            pl.when(fresh[t])(lambda t=t: out_copy(sel_slab[t], r0, nr).start())

    news = [down(*PIECES[0], False)]
    for n in range(len(PIECES)):
        if n + 1 < len(PIECES):
            news.append(down(*PIECES[n + 1], n > 0))
        patch(*PIECES[n], news[n])

    cp(out_ref, out_hbm, S_O).wait()


@jax.jit
def pallas_adaLN_cond__gqa_block_cached__moe_arch_mod__prompt_kernel(
    A_x: jax.Array,
    A_k_cache: jax.Array,
    A_v_cache: jax.Array,
    A_wq: jax.Array,
    A_wo: jax.Array,
    B_x: jax.Array,
    B_w_r: jax.Array,
    B_w_gate: jax.Array,
    B_w_up: jax.Array,
    B_w_down: jax.Array,
    c: jax.Array,
    w_mod: jax.Array,
):
    del B_x
    B, S, D = A_x.shape
    assert B == 1
    NG, SK = A_k_cache.shape[1], A_k_cache.shape[2]
    REP = HQ // NG
    FF = B_w_gate.shape[1]
    GW = REP * DH

    xt = A_x.reshape(S, D).T
    wot = A_wo.T
    wdt = B_w_down.T
    k = A_k_cache.reshape(NG, SK, DH)
    v = A_v_cache.reshape(NG, SK, DH)

    hbm = pl.BlockSpec(memory_space=pl.ANY)
    out_t = pl.pallas_call(
        functools.partial(_kernel, S=S, SK=SK, D=D, FF=FF, NG=NG, REP=REP),
        in_specs=[hbm] * 11,
        out_specs=hbm,
        out_shape=jax.ShapeDtypeStruct((D, S), BF16),
        scratch_shapes=[
            pltpu.VMEM((D, S), BF16),
            pltpu.VMEM((2, SK, DH), BF16),
            pltpu.VMEM((2, SK, DH), BF16),
            pltpu.VMEM((2, D // LANES * LANES + 16, GW), BF16),
            pltpu.VMEM((2, D, GW), BF16),
            pltpu.VMEM((D % LANES, NG * GW), BF16),
            pltpu.VMEM((D,), BF16),
            pltpu.VMEM((1, D), BF16),
            pltpu.VMEM((D, 2 * D), BF16),
            pltpu.VMEM((D, MT_W), BF16),
            pltpu.VMEM((D, FF), BF16),
            pltpu.VMEM((D, FF), BF16),
            pltpu.VMEM((D, WT_W), BF16),
            pltpu.VMEM((FF // 2, D), U32),
            pltpu.VMEM((D, S), BF16),
            pltpu.VMEM((6 * D, LANES), F32),
            pltpu.VMEM((8, 6 * D), F32),
            pltpu.VMEM((D, LANES), F32),
            pltpu.VMEM((2 * D, LANES), F32),
            pltpu.VMEM((3, 8, D), F32),
            pltpu.VMEM((16, D), BF16),
            pltpu.VMEM((8, LANES), F32),
            pltpu.VMEM((S // 2, D), U32),
            pltpu.VMEM((D, S), F32),
            pltpu.VMEM((D // 2, S), U32),
            pltpu.VMEM((7, S // LANES, LANES), F32),
            pltpu.VMEM((D % LANES, S), F32),
            pltpu.VMEM((S // BQ - V0 // REP, D % LANES * 8, BQ), F32),
            pltpu.VMEM((D % LANES, GW, LANES), F32),
            pltpu.VMEM(((S // BQ * REP - V0) * DH, BQ), F32),
            pltpu.VMEM(((S // BQ * REP - V0) * DH // VA, 8, BQ), F32),
            pltpu.VMEM((NG, V0 // REP * BQ, GW), F32),
            pltpu.SemaphoreType.DMA((N_SEMS,)),
        ],
        compiler_params=pltpu.CompilerParams(
            vmem_limit_bytes=120 * 1024 * 1024,
            disable_bounds_checks=True,
        ),
    )(xt, k, v, A_wq, wot, B_w_r, c, w_mod, B_w_gate, B_w_up, wdt)
    return out_t.T.reshape(B, S, D)
```

```python
import functools
import math

import jax
import jax.numpy as jnp
from jax import lax
import jax.experimental.pallas as pl
import jax.experimental.pallas.tpu as pltpu

F32 = jnp.float32
BF16 = jnp.bfloat16
U32 = jnp.uint32

HQ = 32
DH = 128
TOPC = 8
LN_EPS = 1e-5
BQ = 256
LANES = 128
XCH = 4

HEAD = [0, 1280, 1536, 1280, 1536, 640, 768, 640, 1536, 768, 1536, 1536, 640, 1536, 512, 0]
MODE = [2, 2, 2, 2, 0, 2, 0, 0, 0, 1, 2, 0, 0, 2, 1, 2]
QP_POS = [-1, -1, -1, -1, -1, 3, 18, -1]
OP_POS = [7, 12, 17, 25, 30, 31, 31, 31]
V0 = 4
VA = 16
GF = 2
VPER = 300
VMARG = 300
PL = 4
PA = 1
PT0 = 29864
PPER = 506
WT_W = 384
WT_R = 256
WT_TIE = 0
MT_W = 256
MT_R = 8
PK0 = 56
ZC = 1024
DMA_AT = 14
PG0 = 5
PGI = 3
OUW = 2
OPR = 16
TK_TIES = [0, 1, 2, 3, 4, 5, 6]
PIECES = [(0, 128), (128, 128), (256, 128), (384, 128), (512, 64)]
TIEC = 2048

_NT = (((1,), (1,)), ((), ()))

S_C = S_WMA = 0
S_ST = 1
S_WR = 2
S_WG = S_WU = 3
S_WQ0 = 4
S_WQR = 5
S_X = 6
S_G = S_X + XCH
S_O = S_G + 2
N_SEMS = S_O + 1


def _rb(x):
    return x.astype(BF16).astype(F32)


def _sigmoid(x):
    return 1.0 / (1.0 + jnp.exp(-x))


def _ln_rows(mean, var):
    eps = _rb(jnp.full((1, 1), LN_EPS, F32))
    return _rb(mean), _rb(jnp.sqrt(_rb(_rb(var) + eps)))


def _tile(col, n):
    return jnp.concatenate([col] * n, axis=1)


def _as_cols(row):
    return jnp.broadcast_to(row, (LANES, row.shape[1])).astype(BF16).T


def _kernel(xt_hbm, k_hbm, v_hbm, wq_hbm, wot_hbm, wr_hbm, c_hbm, wmod_hbm,
            wg_hbm, wu_hbm, wdt_hbm,
            out_hbm,
            xt_ref, k_buf, v_buf, wq_buf, wot_buf, wqr_ref, wr_ref, c_ref, wmod_ref, wms_ref,
            wg_ref, wu_ref, wdt_ref, wd_ref, out_ref,
            modc_ref, mrow_ref, scc_ref, fold_ref, mb_ref, lhs_ref, rc_ref, h_ref, acc_ref, xb_ref, st_ref, ht_ref, bp_ref, rem_ref, gate_ref, pre_ref,
            sems,
            *, S, SK, D, FF, NG, REP):
    qscale = (DH ** -0.5) * math.log2(math.e)
    NB = S // BQ
    GW = REP * DH
    TCH = S // XCH
    MA = 2 * D
    NSL = S // LANES
    KM = D // LANES * LANES
    KR = D - KM

    def cp(src, dst, sem):
        return pltpu.make_async_copy(src, dst, sems.at[sem])

    def x_copy(i):
        cols = pl.ds(pl.multiple_of(i * TCH, TCH), TCH)
        return cp(xt_hbm.at[:, cols], xt_ref.at[:, cols], S_X + i)

    def group_copies(grp, which=(0, 1, 2, 3)):
        slot = grp % 2
        cols = pl.ds(pl.multiple_of(grp * GW, GW), GW)
        ends = ((lambda: (wq_hbm.at[0:KM, cols], wq_buf.at[slot, 0:KM])),
                (lambda: (k_hbm.at[grp], k_buf.at[slot])),
                (lambda: (v_hbm.at[grp], v_buf.at[slot])),
                (lambda: (wot_hbm.at[:, cols], wot_buf.at[slot])))
        return [cp(*ends[i](), S_G + slot) for i in which]

    wq0_cp = lambda: cp(wq_hbm.at[KM:D, 0:GW], wqr_ref.at[:, 0:GW], S_WQ0)
    wqr_cp = lambda: cp(wq_hbm.at[KM:D, GW:NG * GW], wqr_ref.at[:, GW:NG * GW], S_WQR)
    c_cp = lambda: cp(c_hbm, c_ref, S_C)
    wma_cp = lambda: cp(wmod_hbm.at[:, 0:MA], wmod_ref, S_WMA)
    wr_cp = lambda: cp(wr_hbm, wr_ref, S_WR)
    wg_cp = lambda: cp(wg_hbm, wg_ref, S_WG)
    wu_cp = lambda: cp(wu_hbm, wu_ref, S_WU)

    def side_cols(step):
        return (pl.multiple_of(jnp.clip(step - 1, 0, FF // WT_W - 1) * WT_W, LANES),
                pl.multiple_of(MA + jnp.clip(step - 1, 0, 4 * D // MT_W - 1) * MT_W, LANES))

    def side_copies(step):
        wc, mc = side_cols(step)
        return (cp(wdt_hbm.at[:, pl.ds(wc, WT_W)], wdt_ref, S_ST),
                cp(wmod_hbm.at[:, pl.ds(mc, MT_W)], wms_ref, S_ST))

    def modcol(i):
        return modc_ref[i * D:(i + 1) * D, :]

    def finish_mod(mod, col0):
        mod = _rb(mod)
        lane = lax.broadcasted_iota(jnp.int32, mod.shape, 1) + col0
        is_scale = ((lane >= D) & (lane < 2 * D)) | ((lane >= 4 * D) & (lane < 5 * D))
        return jnp.where(is_scale, _rb(1.0 + mod), mod)

    def prep_cols(w, k0, k1):
        for kk in range(k0, k1):
            bp_ref[kk] = _as_cols(w[kk:kk + 1, :]).astype(F32)

    wq0_cp().start()
    wma_cp().start()
    c_cp().start()
    for i in range(XCH):
        x_copy(i).start()
        if i == 0:
            wqr_cp().start()
    for d in group_copies(0) + group_copies(1):
        d.start()
    wr_cp().start()
    acc_ref[:, 0:ZC] = jnp.zeros((D, ZC), F32)
    wq0_cp().wait()
    acc_ref[:, ZC:S] = jnp.zeros((D, S - ZC), F32)
    prep_cols(wqr_ref[:, 0:GW].astype(F32), 0, PK0)
    wma_cp().wait()
    c_cp().wait()
    c = c_ref[...].astype(F32)
    sc = _rb(c * _sigmoid(c))
    mod = jnp.dot(jnp.broadcast_to(sc, (8, D)).astype(BF16), wmod_ref[...],
                  preferred_element_type=F32)
    modc_ref[0:MA, :] = _as_cols(finish_mod(mod, 0)[0:1, :]).astype(F32)

    def pre(t0, t1, g0, ng):
        hb = pltpu.bitcast(h_ref[t0 // 2:t1 // 2, :], BF16)[:, KM:D]
        for u in range(ng):
            cols = pl.ds(pl.multiple_of((g0 + u) * GW, GW), GW)
            pre_ref[g0 + u, t0:t1, :] = jnp.dot(hb, wqr_ref[:, cols], preferred_element_type=F32)

    def ln1(i, carry):
        x_copy(i).wait()
        if not isinstance(i, int):
            pre(0, TCH, PG0 + (i - 1) * PGI, PGI)
        x = xt_ref[:, pl.ds(pl.multiple_of(i * TCH, TCH), TCH)].astype(F32)
        piv = x[0:1, :]
        d = x - piv
        md = jnp.mean(d, axis=0, keepdims=True)
        var = jnp.maximum(jnp.mean(d * d, axis=0, keepdims=True) - md * md, 0.0)
        mb, sd = _ln_rows(piv + md, var)
        rs = 1.0 / sd
        n = TCH // LANES
        ht = (x * rs - mb * rs) * _tile(modcol(1), n) + _tile(modcol(0), n)
        h_ref[pl.ds(pl.multiple_of(i * (TCH // 2), TCH // 2), TCH // 2), :] = pltpu.bitcast(
            ht.astype(BF16).T, U32)
        if not isinstance(i, int):
            hr = _rb(ht[KM:D, :])
            rep = jnp.concatenate([jnp.broadcast_to(hr[kk:kk + 1, :], (8, TCH)) for kk in range(KR)], axis=0)
            for u in range(TCH // BQ):
                ht_ref[(i - 1) * (TCH // BQ) + u] = rep[:, u * BQ:(u + 1) * BQ]
        return carry
    assert V0 * BQ == REP * TCH
    ln1(0, 0)
    wqr_cp().wait()
    pre(0, TCH, 0, PG0)
    scc_ref[...] = _as_cols(sc).astype(F32)
    prep_cols(wqr_ref[:, 0:GW].astype(F32), PK0, KR)
    wdt_ref[...] = jnp.zeros((D, WT_W), BF16)
    wms_ref[...] = jnp.zeros((D, MT_W), BF16)
    wq_buf[:, KM:KM + 16, :] = jnp.zeros((2, 16, GW), BF16)
    lax.fori_loop(1, XCH, ln1, 0)
    gdone = PG0 + (XCH - 1) * PGI
    if gdone < NG:
        pre(0, TCH, gdone, NG - gdone)

    def fold_modulation():
        sb, cb, gb = (mrow_ref[0:1, i * D:(i + 1) * D] for i in (3, 4, 5))
        for i, z in enumerate((sb, cb, gb)):
            mb_ref[i] = jnp.broadcast_to(z, (8, D))
        fold_ref[0:D, :] = modcol(5) * modcol(4)
        fold_ref[D:MA, :] = modcol(5) * modcol(3)
        wr = wr_ref[...].astype(F32).reshape(1, D)
        wc = wr * cb
        whi = _rb(wc)
        wlo = _rb(wc - whi)
        row = lax.broadcasted_iota(jnp.int32, (16, D), 0)
        lhs_ref[...] = jnp.where(row == 0, 1.0, jnp.where(row == 1, whi, jnp.where(
            row == 2, wlo, 0.0))).astype(BF16)
        rc_ref[0:1, :] = jnp.broadcast_to(jnp.sum(whi + wlo, axis=1, keepdims=True), (1, LANES))
        rc_ref[1:2, :] = jnp.broadcast_to(jnp.sum(wr * sb, axis=1, keepdims=True), (1, LANES))

    def group_step(step, carry):
        @pl.when(step > 0)
        def _():
            for d in side_copies(step):
                d.wait()

        for d in group_copies(step):
            d.wait()

        slot = step % 2
        k = k_buf[slot]
        v = v_buf[slot]
        wq = wq_buf[slot, 0:KM]
        wot = wot_buf[slot]

        nev = lax.broadcasted_iota(jnp.int32, (8, BQ), 1) > step + BQ
        assert VA == 16 and BQ == 2 * LANES
        npb = GW // VA
        L0, L1, B0 = V0 * DH // VA, NB * npb, V0 // REP

        def link(i, gate):
            av = ht_ref[i // npb - B0]
            bv = bp_ref[:, pl.ds(pl.multiple_of((i % npb) * VA, VA), VA), :]
            bv = jnp.concatenate([bv, bv], axis=2)
            acc = None
            for kk in range(KR):
                a = av[8 * kk:8 * kk + 8]
                if (kk * GF) % 8 < GF:
                    a = jnp.where(nev, gate, a)
                t = bv[kk] * jnp.concatenate([a, a], axis=0)
                acc = t if acc is None else acc + t
                g0 = 8 * ((kk * GF) // 8 % 2)
                g1 = 8 - g0
                gate = jnp.concatenate([acc[g0:g0 + 8, LANES:], acc[g1:g1 + 8, 0:LANES]], axis=1)
            rem_ref[pl.ds(pl.multiple_of((i - L0) * VA, VA), VA), :] = acc
            gate_ref[i - L0] = gate
            return gate

        gate = lax.fori_loop(L0, L1, link, jnp.zeros((8, BQ), F32), unroll=True)
        gates = [functools.partial(lambda i: gate_ref[i], i) for i in range(L1 - L0)]
        dues = [VMARG + (i + 1) * VPER for i in range(len(gates))]
        wn = wqr_ref[:, pl.ds(pl.multiple_of(jnp.minimum(step + 1, NG - 1) * GW, GW), GW)].astype(F32)
        for k0 in range(0, KR, PL):
            k1 = min(k0 + PL, KR)
            blks = {r0: jnp.where(nev, gate, wn[r0:r0 + 8, :]) for r0 in range(k0 // 8 * 8, k1, 8)}
            for kk in range(k0, k1):
                last = _as_cols(blks[kk // 8 * 8][kk % 8:kk % 8 + 1, :]).astype(F32)
                bp_ref[kk] = last
                g = jnp.concatenate([last[GW - 8:GW], last[LANES - 8:LANES]], axis=1)
                gate = gate + g if max(k0, k1 - PA) < kk else g
            gates.append(functools.partial(lambda g: g, gate))
            dues.append(PT0 + (k0 // PL + 1) * PPER)
        clock = [0]
        pinned = [0]

        def pin(x, final=False):
            due = len(gates) if final else sum(1 for t in dues if t <= clock[0])
            if due <= pinned[0]:
                return x
            pinned[0] = due
            g = pltpu.bitcast(gates[due - 1](), U32)
            xu = pltpu.bitcast(x, U32)
            top = xu[0:8, 0:LANES]
            top = jnp.where(nev[:, 0:LANES], g[:, 0:LANES], jnp.where(nev[:, LANES:], g[:, LANES:], top))
            if xu.shape[1] > LANES:
                top = jnp.concatenate([top, xu[0:8, LANES:]], axis=1)
            return pltpu.bitcast(jnp.concatenate([top, xu[8:]], axis=0), BF16)

        def qproj(j):
            hb = pin(pltpu.bitcast(h_ref[j * (BQ // 2):(j + 1) * (BQ // 2), :], BF16))
            clock[0] += 512
            if REP * j < V0:
                rem = pre_ref[step, j * BQ:(j + 1) * BQ, :]
            else:
                rem = rem_ref[(REP * j - V0) * DH:(REP * j + REP - V0) * DH, :].T
            q2 = jnp.dot(hb[:, 0:KM], wq, preferred_element_type=F32) + rem
            return (q2 * qscale).astype(BF16)

        def qk(ci, lo, hi):
            q = pin(qs[ci])
            clock[0] += (hi - lo) // 2
            return lax.dot_general(q, k[lo:hi], _NT, preferred_element_type=F32)

        def softmax_pv(s, mode):
            m = jnp.max(s, axis=1, keepdims=True)
            p = jnp.exp2(s - m)
            parts = [p[:, i * LANES:(i + 1) * LANES] for i in range(SK // LANES)]
            if mode == 2:
                lp = None
                for c in range(0, len(parts), 4):
                    t = (parts[c] + parts[c + 1]) + (parts[c + 2] + parts[c + 3])
                    lp = t if lp is None else lp + t
                    parts[c + 3] = jnp.where(lp < 0.0, lp, parts[c + 3])
                p = jnp.concatenate(parts, axis=1)
            clock[0] += SK // 2
            o = jnp.dot(p.astype(BF16), v, preferred_element_type=F32)
            if mode == 0:
                l = jnp.sum(p, axis=1, keepdims=True)
            elif mode == 1:
                lp = functools.reduce(lambda x, y: x + y, parts)
                l = jnp.sum(jnp.where(lp < 0.0, o, lp), axis=1, keepdims=True)
            else:
                l = jnp.sum(lp, axis=1, keepdims=True)
            rl = pl.reciprocal(l, approx=True)
            rl = rl * (2.0 - l * rl)
            return (o * rl).astype(BF16)

        def oproj(j):
            o2 = jnp.concatenate([outs[REP * j + r] for r in range(REP)], axis=1)
            w = pin(wot, final=(j == NB - 1))
            clock[0] += 576
            acc_ref[:, j * BQ:(j + 1) * BQ] += lax.dot_general(w, o2, _NT, preferred_element_type=F32)

        qs, outs = {}, []

        def fill(pos):
            for j in range(NB):
                if QP_POS[j] == pos:
                    q2 = qproj(j)
                    for r in range(REP):
                        qs[REP * j + r] = q2[:, r * DH:(r + 1) * DH]
            for j in range(NB):
                if OP_POS[j] == pos:
                    oproj(j)

        NC = NB * REP
        assert FF % WT_W == 0 and FF // WT_W < NG and (4 * D) % MT_W == 0 and 4 * D // MT_W < NG
        wc0, mc0 = side_cols(step)
        never8 = lax.broadcasted_iota(jnp.int32, (8, LANES), 1) > step + LANES
        wtie = None
        for t0 in range(0, WT_W, LANES):
            for r0 in range(0, D, WT_R):
                r1 = min(r0 + WT_R, D)
                blk = pltpu.bitcast(wdt_ref[r0:r1, t0:t0 + LANES], U32)
                if wtie is not None:
                    blk = jnp.concatenate([jnp.where(never8, wtie, blk[0:8]), blk[8:]], axis=0)
                tb = pltpu.bitcast(pltpu.bitcast(blk, BF16).T, U32)
                wd_ref[pl.ds(pl.multiple_of((wc0 + t0) // 2, LANES // 2), LANES // 2), r0:r1] = tb
                wtie = wd_ref[pl.ds(pl.multiple_of(wc0 // 2, LANES // 2), 8), 0:LANES]
        gate8 = pltpu.bitcast(wtie, F32)
        for r0 in range(0, D, MT_R):
            sc8 = scc_ref[r0:r0 + MT_R, :]
            sc8 = jnp.concatenate([jnp.where(never8, gate8, sc8[0:8])] + ([sc8[8:]] if MT_R > 8 else []), axis=0)
            t = wms_ref[r0:r0 + MT_R, :].astype(F32) * _tile(sc8, MT_W // LANES)
            macc = t if r0 == 0 else macc + t
            gate8 = macc[0:8, 0:LANES]
        mrow = finish_mod(jnp.sum(macc, axis=0, keepdims=True), mc0)
        mrow_ref[0:1, pl.ds(mc0, MT_W)] = mrow
        modc_ref[pl.ds(mc0, MT_W), :] = _as_cols(mrow).astype(F32)
        wtie = pltpu.bitcast(modc_ref[0:8, :], U32)
        fill(-1)
        qt = pltpu.bitcast(qs[WT_TIE], U32)
        qs[WT_TIE] = pltpu.bitcast(
            jnp.concatenate([jnp.where(never8, wtie, qt[0:8]), qt[8:]], axis=0), BF16)
        s_head = None
        for ci in range(NC):
            lo = HEAD[ci - 1] if ci else 0
            if ci == DMA_AT:
                qt = pltpu.bitcast(qs[ci], U32)
                tok = pltpu.bitcast(wq_buf[slot, KM:KM + 16, 0:LANES], U32)
                qs[ci] = pltpu.bitcast(
                    jnp.concatenate([jnp.where(never8, tok, qt[0:8]), qt[8:]], axis=0), BF16)
            s = qk(ci, lo, SK)
            if lo:
                s = jnp.concatenate([s_head, s], axis=1)
            fill(2 * ci)
            if HEAD[ci]:
                s_head = qk(ci + 1, 0, HEAD[ci])
            outs.append(softmax_pv(s, MODE[ci]))
            fill(2 * ci + 1)

        pl.when(step + 2 < NG)(lambda: group_copies(step + 2, (0,))[0].start())

        @pl.when(step + 1 < NG)
        def _():
            for d in side_copies(step + 1):
                d.start()

        @pl.when(step + 2 < NG)
        def _():
            for d in group_copies(step + 2, (1, 2, 3)):
                d.start()

        @pl.when(step == 0)
        def _():
            wg_cp().start()

        @pl.when(step == 1)
        def _():
            wu_cp().start()

        return step

    step = lax.fori_loop(0, NG, group_step, 0)

    wr_cp().wait()
    fold_modulation()
    for sl in range(NSL):
        cols = slice(sl * LANES, (sl + 1) * LANES)
        for r0 in range(0, D, LANES):
            r1 = min(r0 + LANES, D)
            x2 = xt_ref[r0:r1, cols].astype(F32) + modc_ref[MA + r0:MA + r1, :] * acc_ref[r0:r1, cols]
            acc_ref[r0:r1, cols] = x2
            xb = x2.astype(BF16)
            xb_ref[r0 // 2:r1 // 2, cols] = pltpu.bitcast(xb, U32)
            if r0 == 0:
                piv = jnp.mean(x2[0:8, :], axis=0, keepdims=True)
                st_ref[0, sl:sl + 1, :] = piv
            d = x2 - piv
            lhs = lhs_ref[:, r0:r1]
            t1 = jnp.dot(lhs, xb, preferred_element_type=F32)[0:8, :]
            t2 = jnp.dot(lhs, (d * d).astype(BF16), preferred_element_type=F32)[0:8, :]
            s1, s2 = (t1, t2) if r0 == 0 else (s1 + t1, s2 + t2)
        for n in range(3):
            st_ref[1 + n, sl:sl + 1, :] = s1[n:n + 1, :]
        st_ref[4, sl:sl + 1, :] = s2[0:1, :]

    wg_cp().wait()
    wu_cp().wait()

    mean = st_ref[1] * (1.0 / D)
    md = mean - st_ref[0]
    mb, sd = _ln_rows(mean, jnp.maximum(st_ref[4] * (1.0 / D) - md * md, 0.0))
    rs = 1.0 / sd
    st_ref[5] = rs
    st_ref[6] = mb * rs
    r = (st_ref[2] + st_ref[3] - mb * rc_ref[0:1, :]) * rs + rc_ref[1:2, :]

    lane16 = lax.broadcasted_iota(jnp.int32, (16, LANES), 1)
    never = lane16 > step + LANES

    def after_out_stores():
        dyn0 = pl.multiple_of((step - (NG - 1)) * LANES, LANES)
        return out_ref[0:16, pl.ds(dyn0, LANES)]

    def out_unit(n):
        w = OUW * LANES
        cols = slice(n * w, (n + 1) * w)
        rs, mrs = (jnp.concatenate([st_ref[k, n * OUW + u:n * OUW + u + 1, :]
                                    for u in range(OUW)], axis=1) for k in (5, 6))
        for r0 in range(0, D, OPR):
            x2 = acc_ref[r0:r0 + OPR, cols]
            o = x2 + ((x2 * rs - mrs) * _tile(fold_ref[r0:r0 + OPR, :], OUW)
                      + _tile(fold_ref[D + r0:D + r0 + OPR, :], OUW))
            out_ref[r0:r0 + OPR, cols] = o.astype(BF16)
        return after_out_stores().astype(F32)

    r = _rb(r) + 0.0
    bits = pltpu.bitcast(r, jnp.int32)
    mono = bits ^ ((bits >> 31) & jnp.int32(0x7FFFFFFF))
    tok = (lax.broadcasted_iota(jnp.int32, (NSL, LANES), 0) * LANES
           + lax.broadcasted_iota(jnp.int32, (NSL, LANES), 1))
    keyi = (((mono >> 16) + 32768) * S + (S - 1 - tok)) + jnp.int32(1 << 29)
    key = pltpu.bitcast(keyi, F32)

    row16 = lax.broadcasted_iota(jnp.int32, (16, LANES), 0)
    rowc = lax.broadcasted_iota(jnp.int32, (16, 1), 0)
    sel_slab, sel_off = [], []
    tie, nunit = None, 0
    xsel = jnp.zeros((16, D), F32)
    mbsel = jnp.zeros((16, 1), F32)
    rssel = jnp.zeros((16, 1), F32)
    ksel = jnp.zeros((16, 1), F32)
    for t in range(TOPC):
        kmax = jnp.max(jnp.max(key, axis=0, keepdims=True), axis=1, keepdims=True)
        hit = key == kmax
        key = jnp.where(hit, 0.0, key)
        pick = lambda z: jnp.sum(jnp.sum(jnp.where(hit, z, 0.0), axis=0, keepdims=True),
                                 axis=1, keepdims=True)
        mbsel = jnp.where(rowc == t, pick(mb), mbsel)
        rssel = jnp.where(rowc == t, pick(rs), rssel)
        for _ in range(TK_TIES.count(t)):
            tie = out_unit(nunit)
            nunit += 1
            key = jnp.where(never, tie, key)
        ksel = jnp.where(rowc == t, kmax, ksel)
        ki = pltpu.bitcast(kmax, jnp.int32)[0, 0]
        idx = (S - 1) - (ki & (S - 1))
        slab = idx >> 7
        off = idx & (LANES - 1)
        onehot = jnp.where((row16 == t) & (lane16 == off), 1.0, 0.0).astype(BF16)
        dslab = xb_ref[:, pl.ds(pl.multiple_of(slab * LANES, LANES), LANES)]
        xsel = xsel + lax.dot_general(onehot, pltpu.bitcast(dslab, BF16), _NT,
                                      preferred_element_type=F32)
        sel_slab.append(slab)
        sel_off.append(off)
    nsel = _rb(_rb(xsel - mbsel) * rssel)
    hsel = _rb(_rb(nsel * mb_ref[1, 0:1, :]) + mb_ref[0, 0:1, :])
    hi = ((pltpu.bitcast(ksel, jnp.int32) - jnp.int32(1 << 29)) // S - 32768) << 16
    rbits = hi ^ ((hi >> 31) & jnp.int32(0x7FFF0000))
    gate = _rb(_sigmoid(jnp.where(rowc < TOPC, pltpu.bitcast(rbits, F32), 0.0)))

    def out_copy(sl, r0, nr):
        c0 = pl.multiple_of(sl * LANES, LANES)
        return cp(out_ref.at[r0:r0 + nr, pl.ds(c0, LANES)],
                  out_hbm.at[r0:r0 + nr, pl.ds(c0, LANES)], S_O)

    fresh = []
    seen = jnp.int32(0)
    for t in range(TOPC):
        fresh.append(((seen >> sel_slab[t]) & 1) == 0)
        seen = seen | (1 << sel_slab[t])
    plain = [((seen >> sl) & 1) == 0 for sl in range(NSL)]

    for n in range(nunit, NSL // OUW):
        tie = out_unit(n)
    for sl in range(NSL):
        pl.when(plain[sl])(lambda sl=sl: out_copy(sl, 0, D).start())

    h0 = jnp.where(never, tie, hsel[:, 0:LANES])
    hs = jnp.concatenate([h0, hsel[:, LANES:]], axis=1).astype(BF16)
    gpre = _rb(jnp.dot(hs, wg_ref[...], preferred_element_type=F32))
    u = _rb(jnp.dot(hs, wu_ref[...], preferred_element_type=F32))
    a = (_rb(gpre * _sigmoid(gpre)) * u).astype(BF16)

    gb = mb_ref[2, 0:1, :]

    def down(r0, nr, tied):
        lhs = a
        if tied:
            a0 = jnp.where(never[0:8, :], pltpu.bitcast(after_out_stores(), U32),
                           pltpu.bitcast(a[:, TIEC:TIEC + LANES], U32))
            lhs = jnp.concatenate([a[:, 0:TIEC], pltpu.bitcast(a0, BF16), a[:, TIEC + LANES:]], axis=1)
        y = jnp.dot(lhs, pltpu.bitcast(wd_ref[0:FF // 2, r0:r0 + nr], BF16),
                    preferred_element_type=F32)
        c = slice(r0, r0 + nr)
        return xsel[:, c] + gb[:, c] * (hsel[:, c] + y * gate)

    def patch(r0, nr, new):
        lane = lax.broadcasted_iota(jnp.int32, (nr // 2, LANES), 1)
        for t in range(TOPC):
            cols = pl.ds(pl.multiple_of(sel_slab[t] * LANES, LANES), LANES)
            old = pltpu.bitcast(out_ref[r0:r0 + nr, cols], U32)
            upd = pltpu.bitcast(_as_cols(new[t:t + 1, :]), U32)
            out_ref[r0:r0 + nr, cols] = pltpu.bitcast(jnp.where(lane == sel_off[t], upd, old), BF16)
        for t in range(TOPC):
            pl.when(fresh[t])(lambda t=t: out_copy(sel_slab[t], r0, nr).start())

    news = [down(*PIECES[0], False)]
    for n in range(len(PIECES)):
        if n + 1 < len(PIECES):
            news.append(down(*PIECES[n + 1], n > 0))
        patch(*PIECES[n], news[n])

    cp(out_ref, out_hbm, S_O).wait()


@jax.jit
def pallas_adaLN_cond__gqa_block_cached__moe_arch_mod__prompt_kernel(
    A_x: jax.Array,
    A_k_cache: jax.Array,
    A_v_cache: jax.Array,
    A_wq: jax.Array,
    A_wo: jax.Array,
    B_x: jax.Array,
    B_w_r: jax.Array,
    B_w_gate: jax.Array,
    B_w_up: jax.Array,
    B_w_down: jax.Array,
    c: jax.Array,
    w_mod: jax.Array,
):
    del B_x
    B, S, D = A_x.shape
    assert B == 1
    NG, SK = A_k_cache.shape[1], A_k_cache.shape[2]
    REP = HQ // NG
    FF = B_w_gate.shape[1]
    GW = REP * DH

    xt = A_x.reshape(S, D).T
    wot = A_wo.T
    wdt = B_w_down.T
    k = A_k_cache.reshape(NG, SK, DH)
    v = A_v_cache.reshape(NG, SK, DH)

    hbm = pl.BlockSpec(memory_space=pl.ANY)
    out_t = pl.pallas_call(
        functools.partial(_kernel, S=S, SK=SK, D=D, FF=FF, NG=NG, REP=REP),
        in_specs=[hbm] * 11,
        out_specs=hbm,
        out_shape=jax.ShapeDtypeStruct((D, S), BF16),
        scratch_shapes=[
            pltpu.VMEM((D, S), BF16),
            pltpu.VMEM((2, SK, DH), BF16),
            pltpu.VMEM((2, SK, DH), BF16),
            pltpu.VMEM((2, D // LANES * LANES + 16, GW), BF16),
            pltpu.VMEM((2, D, GW), BF16),
            pltpu.VMEM((D % LANES, NG * GW), BF16),
            pltpu.VMEM((D,), BF16),
            pltpu.VMEM((1, D), BF16),
            pltpu.VMEM((D, 2 * D), BF16),
            pltpu.VMEM((D, MT_W), BF16),
            pltpu.VMEM((D, FF), BF16),
            pltpu.VMEM((D, FF), BF16),
            pltpu.VMEM((D, WT_W), BF16),
            pltpu.VMEM((FF // 2, D), U32),
            pltpu.VMEM((D, S), BF16),
            pltpu.VMEM((6 * D, LANES), F32),
            pltpu.VMEM((8, 6 * D), F32),
            pltpu.VMEM((D, LANES), F32),
            pltpu.VMEM((2 * D, LANES), F32),
            pltpu.VMEM((3, 8, D), F32),
            pltpu.VMEM((16, D), BF16),
            pltpu.VMEM((8, LANES), F32),
            pltpu.VMEM((S // 2, D), U32),
            pltpu.VMEM((D, S), F32),
            pltpu.VMEM((D // 2, S), U32),
            pltpu.VMEM((7, S // LANES, LANES), F32),
            pltpu.VMEM((S // BQ - V0 // REP, D % LANES * 8, BQ), F32),
            pltpu.VMEM((D % LANES, GW, LANES), F32),
            pltpu.VMEM(((S // BQ * REP - V0) * DH, BQ), F32),
            pltpu.VMEM(((S // BQ * REP - V0) * DH // VA, 8, BQ), F32),
            pltpu.VMEM((NG, V0 // REP * BQ, GW), F32),
            pltpu.SemaphoreType.DMA((N_SEMS,)),
        ],
        compiler_params=pltpu.CompilerParams(
            vmem_limit_bytes=120 * 1024 * 1024,
            disable_bounds_checks=True,
        ),
    )(xt, k, v, A_wq, wot, B_w_r, c, w_mod, B_w_gate, B_w_up, wdt)
    return out_t.T.reshape(B, S, D)
```

```python
import functools
import math

import jax
import jax.numpy as jnp
from jax import lax
import jax.experimental.pallas as pl
import jax.experimental.pallas.tpu as pltpu

F32 = jnp.float32
BF16 = jnp.bfloat16
U32 = jnp.uint32

HQ = 32
DH = 128
TOPC = 8
LN_EPS = 1e-5
BQ = 256
LANES = 128
XCH = 4

HEAD = [0, 1280, 1536, 1280, 1536, 640, 768, 640, 1536, 768, 1536, 1536, 640, 1536, 512, 0]
MODE = [2, 2, 2, 2, 0, 2, 0, 0, 0, 1, 2, 0, 0, 2, 1, 2]
QP_POS = [-1, -1, -1, -1, -1, 3, 18, -1]
OP_POS = [7, 12, 17, 25, 30, 31, 31, 31]
V0 = 4
VA = 16
GF = 2
VPER = 300
VMARG = 300
PL = 4
PA = 1
PT0 = 29864
PPER = 506
WT_W = 384
WT_R = 256
WT_TIE = 0
MT_W = 256
MT_R = 8
PK0 = 56
ZC = 1024
DMA_AT = 14
PG0 = 5
PGI = 3
OUW = 2
OPR = 16
TK_TIES = [0, 1, 2, 3, 4, 5, 6]
PIECES = [(0, 128), (128, 128), (256, 128), (384, 128), (512, 64)]
TIEC = 2048

_NT = (((1,), (1,)), ((), ()))

S_C = S_WMA = 0
S_ST = 1
S_WR = 2
S_WG = S_WU = 3
S_WQ0 = 4
S_WQR = 5
S_X = 6
S_G = S_X + XCH
S_O = S_G + 2
N_SEMS = S_O + 1


def _rb(x):
    return x.astype(BF16).astype(F32)


def _sigmoid(x):
    return 1.0 / (1.0 + jnp.exp(-x))


def _ln_rows(mean, var):
    eps = _rb(jnp.full((1, 1), LN_EPS, F32))
    return _rb(mean), _rb(jnp.sqrt(_rb(_rb(var) + eps)))


def _tile(col, n):
    return jnp.concatenate([col] * n, axis=1)


def _as_cols(row):
    return jnp.broadcast_to(row, (LANES, row.shape[1])).astype(BF16).T


def _kernel(xt_hbm, k_hbm, v_hbm, wq_hbm, wot_hbm, wr_hbm, c_hbm, wmod_hbm,
            wg_hbm, wu_hbm, wdt_hbm,
            out_hbm,
            xt_ref, k_buf, v_buf, wq_buf, wot_buf, wqr_ref, wr_ref, c_ref, wmod_ref, wms_ref,
            wg_ref, wu_ref, wdt_ref, wd_ref, out_ref,
            modc_ref, mrow_ref, scc_ref, fold_ref, mb_ref, lhs_ref, rc_ref, h_ref, acc_ref,
            xb_ref, st_ref, ht_ref, bp_ref, rem_ref, gate_ref, pre_ref,
            sems,
            *, S, SK, D, FF, NG, REP):
    qscale = (DH ** -0.5) * math.log2(math.e)
    NB = S // BQ
    GW = REP * DH
    TCH = S // XCH
    MA = 2 * D
    NSL = S // LANES
    KM = D // LANES * LANES
    KR = D - KM

    def cp(src, dst, sem):
        return pltpu.make_async_copy(src, dst, sems.at[sem])

    def x_copy(i):
        cols = pl.ds(pl.multiple_of(i * TCH, TCH), TCH)
        return cp(xt_hbm.at[:, cols], xt_ref.at[:, cols], S_X + i)

    def group_copies(grp, which=(0, 1, 2, 3)):
        slot = grp % 2
        cols = pl.ds(pl.multiple_of(grp * GW, GW), GW)
        ends = ((lambda: (wq_hbm.at[0:KM, cols], wq_buf.at[slot, 0:KM])),
                (lambda: (k_hbm.at[grp], k_buf.at[slot])),
                (lambda: (v_hbm.at[grp], v_buf.at[slot])),
                (lambda: (wot_hbm.at[:, cols], wot_buf.at[slot])))
        return [cp(*ends[i](), S_G + slot) for i in which]

    wq0_cp = lambda: cp(wq_hbm.at[KM:D, 0:GW], wqr_ref.at[:, 0:GW], S_WQ0)
    wqr_cp = lambda: cp(wq_hbm.at[KM:D, GW:NG * GW], wqr_ref.at[:, GW:NG * GW], S_WQR)
    c_cp = lambda: cp(c_hbm, c_ref, S_C)
    wma_cp = lambda: cp(wmod_hbm.at[:, 0:MA], wmod_ref, S_WMA)
    wr_cp = lambda: cp(wr_hbm, wr_ref, S_WR)
    wg_cp = lambda: cp(wg_hbm, wg_ref, S_WG)
    wu_cp = lambda: cp(wu_hbm, wu_ref, S_WU)

    def side_cols(step):
        return (pl.multiple_of(jnp.clip(step - 1, 0, FF // WT_W - 1) * WT_W, LANES),
                pl.multiple_of(MA + jnp.clip(step - 1, 0, 4 * D // MT_W - 1) * MT_W, LANES))

    def side_copies(step):
        wc, mc = side_cols(step)
        return (cp(wdt_hbm.at[:, pl.ds(wc, WT_W)], wdt_ref, S_ST),
                cp(wmod_hbm.at[:, pl.ds(mc, MT_W)], wms_ref, S_ST))

    def modcol(i):
        return modc_ref[i * D:(i + 1) * D, :]

    def finish_mod(mod, col0):
        mod = _rb(mod)
        lane = lax.broadcasted_iota(jnp.int32, mod.shape, 1) + col0
        is_scale = ((lane >= D) & (lane < 2 * D)) | ((lane >= 4 * D) & (lane < 5 * D))
        return jnp.where(is_scale, _rb(1.0 + mod), mod)

    def prep_cols(w, k0, k1):
        for kk in range(k0, k1):
            bp_ref[kk] = _as_cols(w[kk:kk + 1, :]).astype(F32)

    wq0_cp().start()
    wma_cp().start()
    c_cp().start()
    for i in range(XCH):
        x_copy(i).start()
        if i == 0:
            wqr_cp().start()
    for d in group_copies(0) + group_copies(1):
        d.start()
    wr_cp().start()
    acc_ref[:, 0:ZC] = jnp.zeros((D, ZC), F32)
    wq0_cp().wait()
    acc_ref[:, ZC:S] = jnp.zeros((D, S - ZC), F32)
    prep_cols(wqr_ref[:, 0:GW].astype(F32), 0, PK0)
    wma_cp().wait()
    c_cp().wait()
    c = c_ref[...].astype(F32)
    sc = _rb(c * _sigmoid(c))
    mod = jnp.dot(jnp.broadcast_to(sc, (8, D)).astype(BF16), wmod_ref[...],
                  preferred_element_type=F32)
    modc_ref[0:MA, :] = _as_cols(finish_mod(mod, 0)[0:1, :]).astype(F32)

    def pre(t0, t1, g0, ng):
        hb = pltpu.bitcast(h_ref[t0 // 2:t1 // 2, :], BF16)[:, KM:D]
        for u in range(ng):
            cols = pl.ds(pl.multiple_of((g0 + u) * GW, GW), GW)
            pre_ref[g0 + u, t0:t1, :] = jnp.dot(hb, wqr_ref[:, cols], preferred_element_type=F32)

    def ln1(i, carry):
        x_copy(i).wait()
        if not isinstance(i, int):
            pre(0, TCH, PG0 + (i - 1) * PGI, PGI)
        x = xt_ref[:, pl.ds(pl.multiple_of(i * TCH, TCH), TCH)].astype(F32)
        piv = x[0:1, :]
        d = x - piv
        md = jnp.mean(d, axis=0, keepdims=True)
        var = jnp.maximum(jnp.mean(d * d, axis=0, keepdims=True) - md * md, 0.0)
        mb, sd = _ln_rows(piv + md, var)
        rs = 1.0 / sd
        n = TCH // LANES
        ht = (x * rs - mb * rs) * _tile(modcol(1), n) + _tile(modcol(0), n)
        kt = D if isinstance(i, int) else KM
        h_ref[pl.ds(pl.multiple_of(i * (TCH // 2), TCH // 2), TCH // 2), 0:kt] = pltpu.bitcast(
            ht[0:kt].astype(BF16).T, U32)
        if not isinstance(i, int):
            hr = _rb(ht[KM:D, :])
            rep = jnp.concatenate([jnp.broadcast_to(hr[kk:kk + 1, :], (8, TCH)) for kk in range(KR)], axis=0)
            for u in range(TCH // BQ):
                ht_ref[(i - 1) * (TCH // BQ) + u] = rep[:, u * BQ:(u + 1) * BQ]
        return carry
    assert V0 * BQ == REP * TCH
    ln1(0, 0)
    wqr_cp().wait()
    pre(0, TCH, 0, PG0)
    scc_ref[...] = _as_cols(sc).astype(F32)
    prep_cols(wqr_ref[:, 0:GW].astype(F32), PK0, KR)
    wdt_ref[...] = jnp.zeros((D, WT_W), BF16)
    wms_ref[...] = jnp.zeros((D, MT_W), BF16)
    wq_buf[:, KM:KM + 16, :] = jnp.zeros((2, 16, GW), BF16)
    lax.fori_loop(1, XCH, ln1, 0)
    gdone = PG0 + (XCH - 1) * PGI
    if gdone < NG:
        pre(0, TCH, gdone, NG - gdone)

    def fold_modulation():
        sb, cb, gb = (mrow_ref[0:1, i * D:(i + 1) * D] for i in (3, 4, 5))
        for i, z in enumerate((sb, cb, gb)):
            mb_ref[i] = jnp.broadcast_to(z, (8, D))
        fold_ref[0:D, :] = modcol(5) * modcol(4)
        fold_ref[D:MA, :] = modcol(5) * modcol(3)
        wr = wr_ref[...].astype(F32).reshape(1, D)
        wc = wr * cb
        whi = _rb(wc)
        wlo = _rb(wc - whi)
        row = lax.broadcasted_iota(jnp.int32, (16, D), 0)
        lhs_ref[...] = jnp.where(row == 0, 1.0, jnp.where(row == 1, whi, jnp.where(
            row == 2, wlo, 0.0))).astype(BF16)
        rc_ref[0:1, :] = jnp.broadcast_to(jnp.sum(whi + wlo, axis=1, keepdims=True), (1, LANES))
        rc_ref[1:2, :] = jnp.broadcast_to(jnp.sum(wr * sb, axis=1, keepdims=True), (1, LANES))

    def group_step(step, carry):
        @pl.when(step > 0)
        def _():
            for d in side_copies(step):
                d.wait()

        for d in group_copies(step):
            d.wait()

        slot = step % 2
        k = k_buf[slot]
        v = v_buf[slot]
        wq = wq_buf[slot, 0:KM]
        wot = wot_buf[slot]

        nev = lax.broadcasted_iota(jnp.int32, (8, BQ), 1) > step + BQ
        assert VA == 16 and BQ == 2 * LANES
        npb = GW // VA
        L0, L1, B0 = V0 * DH // VA, NB * npb, V0 // REP

        def link(i, gate):
            av = ht_ref[i // npb - B0]
            bv = bp_ref[:, pl.ds(pl.multiple_of((i % npb) * VA, VA), VA), :]
            bv = jnp.concatenate([bv, bv], axis=2)
            acc = None
            for kk in range(KR):
                a = av[8 * kk:8 * kk + 8]
                if (kk * GF) % 8 < GF:
                    a = jnp.where(nev, gate, a)
                t = bv[kk] * jnp.concatenate([a, a], axis=0)
                acc = t if acc is None else acc + t
                g0 = 8 * ((kk * GF) // 8 % 2)
                g1 = 8 - g0
                gate = jnp.concatenate([acc[g0:g0 + 8, LANES:], acc[g1:g1 + 8, 0:LANES]], axis=1)
            rem_ref[pl.ds(pl.multiple_of((i - L0) * VA, VA), VA), :] = acc
            gate_ref[i - L0] = gate
            return gate

        gate = lax.fori_loop(L0, L1, link, jnp.zeros((8, BQ), F32), unroll=True)
        gates = [functools.partial(lambda i: gate_ref[i], i) for i in range(L1 - L0)]
        dues = [VMARG + (i + 1) * VPER for i in range(len(gates))]
        wn = wqr_ref[:, pl.ds(pl.multiple_of(jnp.minimum(step + 1, NG - 1) * GW, GW), GW)].astype(F32)
        for k0 in range(0, KR, PL):
            k1 = min(k0 + PL, KR)
            blks = {r0: jnp.where(nev, gate, wn[r0:r0 + 8, :]) for r0 in range(k0 // 8 * 8, k1, 8)}
            for kk in range(k0, k1):
                last = _as_cols(blks[kk // 8 * 8][kk % 8:kk % 8 + 1, :]).astype(F32)
                bp_ref[kk] = last
                g = jnp.concatenate([last[GW - 8:GW], last[LANES - 8:LANES]], axis=1)
                gate = gate + g if max(k0, k1 - PA) < kk else g
            gates.append(functools.partial(lambda g: g, gate))
            dues.append(PT0 + (k0 // PL + 1) * PPER)
        clock = [0]
        pinned = [0]

        def pin(x, final=False):
            due = len(gates) if final else sum(1 for t in dues if t <= clock[0])
            if due <= pinned[0]:
                return x
            pinned[0] = due
            g = pltpu.bitcast(gates[due - 1](), U32)
            xu = pltpu.bitcast(x, U32)
            top = xu[0:8, 0:LANES]
            top = jnp.where(nev[:, 0:LANES], g[:, 0:LANES], jnp.where(nev[:, LANES:], g[:, LANES:], top))
            if xu.shape[1] > LANES:
                top = jnp.concatenate([top, xu[0:8, LANES:]], axis=1)
            return pltpu.bitcast(jnp.concatenate([top, xu[8:]], axis=0), BF16)

        def qproj(j):
            hb = pin(pltpu.bitcast(h_ref[j * (BQ // 2):(j + 1) * (BQ // 2), 0:KM], BF16))
            clock[0] += 512
            if REP * j < V0:
                rem = pre_ref[step, j * BQ:(j + 1) * BQ, :]
            else:
                rem = rem_ref[(REP * j - V0) * DH:(REP * j + REP - V0) * DH, :].T
            q2 = jnp.dot(hb, wq, preferred_element_type=F32) + rem
            return (q2 * qscale).astype(BF16)

        def qk(ci, lo, hi):
            q = pin(qs[ci])
            clock[0] += (hi - lo) // 2
            return lax.dot_general(q, k[lo:hi], _NT, preferred_element_type=F32)

        def softmax_pv(s, mode):
            m = jnp.max(s, axis=1, keepdims=True)
            p = jnp.exp2(s - m)
            parts = [p[:, i * LANES:(i + 1) * LANES] for i in range(SK // LANES)]
            if mode == 2:
                lp = None
                for c in range(0, len(parts), 4):
                    t = (parts[c] + parts[c + 1]) + (parts[c + 2] + parts[c + 3])
                    lp = t if lp is None else lp + t
                    parts[c + 3] = jnp.where(lp < 0.0, lp, parts[c + 3])
                p = jnp.concatenate(parts, axis=1)
            clock[0] += SK // 2
            o = jnp.dot(p.astype(BF16), v, preferred_element_type=F32)
            if mode == 0:
                l = jnp.sum(p, axis=1, keepdims=True)
            elif mode == 1:
                lp = functools.reduce(lambda x, y: x + y, parts)
                l = jnp.sum(jnp.where(lp < 0.0, o, lp), axis=1, keepdims=True)
            else:
                l = jnp.sum(lp, axis=1, keepdims=True)
            rl = pl.reciprocal(l, approx=True)
            rl = rl * (2.0 - l * rl)
            return (o * rl).astype(BF16)

        def oproj(j):
            o2 = jnp.concatenate([outs[REP * j + r] for r in range(REP)], axis=1)
            w = pin(wot, final=(j == NB - 1))
            clock[0] += 576
            acc_ref[:, j * BQ:(j + 1) * BQ] += lax.dot_general(w, o2, _NT, preferred_element_type=F32)

        qs, outs = {}, []

        def fill(pos):
            for j in range(NB):
                if QP_POS[j] == pos:
                    q2 = qproj(j)
                    for r in range(REP):
                        qs[REP * j + r] = q2[:, r * DH:(r + 1) * DH]
            for j in range(NB):
                if OP_POS[j] == pos:
                    oproj(j)

        NC = NB * REP
        assert FF % WT_W == 0 and FF // WT_W < NG and (4 * D) % MT_W == 0 and 4 * D // MT_W < NG
        wc0, mc0 = side_cols(step)
        never8 = lax.broadcasted_iota(jnp.int32, (8, LANES), 1) > step + LANES
        wtie = None
        for t0 in range(0, WT_W, LANES):
            for r0 in range(0, D, WT_R):
                r1 = min(r0 + WT_R, D)
                blk = pltpu.bitcast(wdt_ref[r0:r1, t0:t0 + LANES], U32)
                if wtie is not None:
                    blk = jnp.concatenate([jnp.where(never8, wtie, blk[0:8]), blk[8:]], axis=0)
                tb = pltpu.bitcast(pltpu.bitcast(blk, BF16).T, U32)
                wd_ref[pl.ds(pl.multiple_of((wc0 + t0) // 2, LANES // 2), LANES // 2), r0:r1] = tb
                wtie = wd_ref[pl.ds(pl.multiple_of(wc0 // 2, LANES // 2), 8), 0:LANES]
        gate8 = pltpu.bitcast(wtie, F32)
        for r0 in range(0, D, MT_R):
            sc8 = scc_ref[r0:r0 + MT_R, :]
            sc8 = jnp.concatenate([jnp.where(never8, gate8, sc8[0:8])] + ([sc8[8:]] if MT_R > 8 else []), axis=0)
            t = wms_ref[r0:r0 + MT_R, :].astype(F32) * _tile(sc8, MT_W // LANES)
            macc = t if r0 == 0 else macc + t
            gate8 = macc[0:8, 0:LANES]
        mrow = finish_mod(jnp.sum(macc, axis=0, keepdims=True), mc0)
        mrow_ref[0:1, pl.ds(mc0, MT_W)] = mrow
        modc_ref[pl.ds(mc0, MT_W), :] = _as_cols(mrow).astype(F32)
        wtie = pltpu.bitcast(modc_ref[0:8, :], U32)
        fill(-1)
        qt = pltpu.bitcast(qs[WT_TIE], U32)
        qs[WT_TIE] = pltpu.bitcast(
            jnp.concatenate([jnp.where(never8, wtie, qt[0:8]), qt[8:]], axis=0), BF16)
        s_head = None
        for ci in range(NC):
            lo = HEAD[ci - 1] if ci else 0
            if ci == DMA_AT:
                qt = pltpu.bitcast(qs[ci], U32)
                tok = pltpu.bitcast(wq_buf[slot, KM:KM + 16, 0:LANES], U32)
                qs[ci] = pltpu.bitcast(
                    jnp.concatenate([jnp.where(never8, tok, qt[0:8]), qt[8:]], axis=0), BF16)
            s = qk(ci, lo, SK)
            if lo:
                s = jnp.concatenate([s_head, s], axis=1)
            fill(2 * ci)
            if HEAD[ci]:
                s_head = qk(ci + 1, 0, HEAD[ci])
            outs.append(softmax_pv(s, MODE[ci]))
            fill(2 * ci + 1)

        pl.when(step + 2 < NG)(lambda: group_copies(step + 2, (0,))[0].start())

        @pl.when(step + 1 < NG)
        def _():
            for d in side_copies(step + 1):
                d.start()

        @pl.when(step + 2 < NG)
        def _():
            for d in group_copies(step + 2, (1, 2, 3)):
                d.start()

        @pl.when(step == 0)
        def _():
            wg_cp().start()

        @pl.when(step == 1)
        def _():
            wu_cp().start()

        return step

    step = lax.fori_loop(0, NG, group_step, 0)

    wr_cp().wait()
    fold_modulation()
    for sl in range(NSL):
        cols = slice(sl * LANES, (sl + 1) * LANES)
        for r0 in range(0, D, LANES):
            r1 = min(r0 + LANES, D)
            x2 = xt_ref[r0:r1, cols].astype(F32) + modc_ref[MA + r0:MA + r1, :] * acc_ref[r0:r1, cols]
            acc_ref[r0:r1, cols] = x2
            xb = x2.astype(BF16)
            xb_ref[r0 // 2:r1 // 2, cols] = pltpu.bitcast(xb, U32)
            if r0 == 0:
                piv = jnp.mean(x2[0:8, :], axis=0, keepdims=True)
                st_ref[0, sl:sl + 1, :] = piv
            d = x2 - piv
            lhs = lhs_ref[:, r0:r1]
            t1 = jnp.dot(lhs, xb, preferred_element_type=F32)[0:8, :]
            t2 = jnp.dot(lhs, (d * d).astype(BF16), preferred_element_type=F32)[0:8, :]
            s1, s2 = (t1, t2) if r0 == 0 else (s1 + t1, s2 + t2)
        for n in range(3):
            st_ref[1 + n, sl:sl + 1, :] = s1[n:n + 1, :]
        st_ref[4, sl:sl + 1, :] = s2[0:1, :]

    wg_cp().wait()
    wu_cp().wait()

    mean = st_ref[1] * (1.0 / D)
    md = mean - st_ref[0]
    mb, sd = _ln_rows(mean, jnp.maximum(st_ref[4] * (1.0 / D) - md * md, 0.0))
    rs = 1.0 / sd
    st_ref[5] = rs
    st_ref[6] = mb * rs
    r = (st_ref[2] + st_ref[3] - mb * rc_ref[0:1, :]) * rs + rc_ref[1:2, :]

    lane16 = lax.broadcasted_iota(jnp.int32, (16, LANES), 1)
    never = lane16 > step + LANES

    def after_out_stores():
        dyn0 = pl.multiple_of((step - (NG - 1)) * LANES, LANES)
        return out_ref[0:16, pl.ds(dyn0, LANES)]

    def out_unit(n):
        w = OUW * LANES
        cols = slice(n * w, (n + 1) * w)
        rs, mrs = (jnp.concatenate([st_ref[k, n * OUW + u:n * OUW + u + 1, :]
                                    for u in range(OUW)], axis=1) for k in (5, 6))
        for r0 in range(0, D, OPR):
            x2 = acc_ref[r0:r0 + OPR, cols]
            o = x2 + ((x2 * rs - mrs) * _tile(fold_ref[r0:r0 + OPR, :], OUW)
                      + _tile(fold_ref[D + r0:D + r0 + OPR, :], OUW))
            out_ref[r0:r0 + OPR, cols] = o.astype(BF16)
        return after_out_stores().astype(F32)

    r = _rb(r) + 0.0
    bits = pltpu.bitcast(r, jnp.int32)
    mono = bits ^ ((bits >> 31) & jnp.int32(0x7FFFFFFF))
    tok = (lax.broadcasted_iota(jnp.int32, (NSL, LANES), 0) * LANES
           + lax.broadcasted_iota(jnp.int32, (NSL, LANES), 1))
    keyi = (((mono >> 16) + 32768) * S + (S - 1 - tok)) + jnp.int32(1 << 29)
    key = pltpu.bitcast(keyi, F32)

    row16 = lax.broadcasted_iota(jnp.int32, (16, LANES), 0)
    rowc = lax.broadcasted_iota(jnp.int32, (16, 1), 0)
    sel_slab, sel_off = [], []
    tie, nunit = None, 0
    xsel = jnp.zeros((16, D), F32)
    mbsel = jnp.zeros((16, 1), F32)
    rssel = jnp.zeros((16, 1), F32)
    ksel = jnp.zeros((16, 1), F32)
    for t in range(TOPC):
        kmax = jnp.max(jnp.max(key, axis=0, keepdims=True), axis=1, keepdims=True)
        hit = key == kmax
        key = jnp.where(hit, 0.0, key)
        pick = lambda z: jnp.sum(jnp.sum(jnp.where(hit, z, 0.0), axis=0, keepdims=True),
                                 axis=1, keepdims=True)
        mbsel = jnp.where(rowc == t, pick(mb), mbsel)
        rssel = jnp.where(rowc == t, pick(rs), rssel)
        for _ in range(TK_TIES.count(t)):
            tie = out_unit(nunit)
            nunit += 1
            key = jnp.where(never, tie, key)
        ksel = jnp.where(rowc == t, kmax, ksel)
        ki = pltpu.bitcast(kmax, jnp.int32)[0, 0]
        idx = (S - 1) - (ki & (S - 1))
        slab = idx >> 7
        off = idx & (LANES - 1)
        onehot = jnp.where((row16 == t) & (lane16 == off), 1.0, 0.0).astype(BF16)
        dslab = xb_ref[:, pl.ds(pl.multiple_of(slab * LANES, LANES), LANES)]
        xsel = xsel + lax.dot_general(onehot, pltpu.bitcast(dslab, BF16), _NT,
                                      preferred_element_type=F32)
        sel_slab.append(slab)
        sel_off.append(off)
    nsel = _rb(_rb(xsel - mbsel) * rssel)
    hsel = _rb(_rb(nsel * mb_ref[1, 0:1, :]) + mb_ref[0, 0:1, :])
    hi = ((pltpu.bitcast(ksel, jnp.int32) - jnp.int32(1 << 29)) // S - 32768) << 16
    rbits = hi ^ ((hi >> 31) & jnp.int32(0x7FFF0000))
    gate = _rb(_sigmoid(jnp.where(rowc < TOPC, pltpu.bitcast(rbits, F32), 0.0)))

    def out_copy(sl, r0, nr):
        c0 = pl.multiple_of(sl * LANES, LANES)
        return cp(out_ref.at[r0:r0 + nr, pl.ds(c0, LANES)],
                  out_hbm.at[r0:r0 + nr, pl.ds(c0, LANES)], S_O)

    fresh = []
    seen = jnp.int32(0)
    for t in range(TOPC):
        fresh.append(((seen >> sel_slab[t]) & 1) == 0)
        seen = seen | (1 << sel_slab[t])
    plain = [((seen >> sl) & 1) == 0 for sl in range(NSL)]

    for n in range(nunit, NSL // OUW):
        tie = out_unit(n)
    for sl in range(NSL):
        pl.when(plain[sl])(lambda sl=sl: out_copy(sl, 0, D).start())

    h0 = jnp.where(never, tie, hsel[:, 0:LANES])
    hs = jnp.concatenate([h0, hsel[:, LANES:]], axis=1).astype(BF16)
    gpre = _rb(jnp.dot(hs, wg_ref[...], preferred_element_type=F32))
    u = _rb(jnp.dot(hs, wu_ref[...], preferred_element_type=F32))
    a = (_rb(gpre * _sigmoid(gpre)) * u).astype(BF16)

    gb = mb_ref[2, 0:1, :]

    def down(r0, nr, tied):
        lhs = a
        if tied:
            a0 = jnp.where(never[0:8, :], pltpu.bitcast(after_out_stores(), U32),
                           pltpu.bitcast(a[:, TIEC:TIEC + LANES], U32))
            lhs = jnp.concatenate([a[:, 0:TIEC], pltpu.bitcast(a0, BF16), a[:, TIEC + LANES:]], axis=1)
        y = jnp.dot(lhs, pltpu.bitcast(wd_ref[0:FF // 2, r0:r0 + nr], BF16),
                    preferred_element_type=F32)
        c = slice(r0, r0 + nr)
        return xsel[:, c] + gb[:, c] * (hsel[:, c] + y * gate)

    def patch(r0, nr, new):
        lane = lax.broadcasted_iota(jnp.int32, (nr // 2, LANES), 1)
        for t in range(TOPC):
            cols = pl.ds(pl.multiple_of(sel_slab[t] * LANES, LANES), LANES)
            old = pltpu.bitcast(out_ref[r0:r0 + nr, cols], U32)
            upd = pltpu.bitcast(_as_cols(new[t:t + 1, :]), U32)
            out_ref[r0:r0 + nr, cols] = pltpu.bitcast(jnp.where(lane == sel_off[t], upd, old), BF16)
        for t in range(TOPC):
            pl.when(fresh[t])(lambda t=t: out_copy(sel_slab[t], r0, nr).start())

    news = [down(*PIECES[0], False)]
    for n in range(len(PIECES)):
        if n + 1 < len(PIECES):
            news.append(down(*PIECES[n + 1], n > 0))
        patch(*PIECES[n], news[n])

    cp(out_ref, out_hbm, S_O).wait()


@jax.jit
def pallas_adaLN_cond__gqa_block_cached__moe_arch_mod__prompt_kernel(
    A_x: jax.Array,
    A_k_cache: jax.Array,
    A_v_cache: jax.Array,
    A_wq: jax.Array,
    A_wo: jax.Array,
    B_x: jax.Array,
    B_w_r: jax.Array,
    B_w_gate: jax.Array,
    B_w_up: jax.Array,
    B_w_down: jax.Array,
    c: jax.Array,
    w_mod: jax.Array,
):
    del B_x
    B, S, D = A_x.shape
    assert B == 1
    NG, SK = A_k_cache.shape[1], A_k_cache.shape[2]
    REP = HQ // NG
    FF = B_w_gate.shape[1]
    GW = REP * DH

    xt = A_x.reshape(S, D).T
    wot = A_wo.T
    wdt = B_w_down.T
    k = A_k_cache.reshape(NG, SK, DH)
    v = A_v_cache.reshape(NG, SK, DH)

    hbm = pl.BlockSpec(memory_space=pl.ANY)
    out_t = pl.pallas_call(
        functools.partial(_kernel, S=S, SK=SK, D=D, FF=FF, NG=NG, REP=REP),
        in_specs=[hbm] * 11,
        out_specs=hbm,
        out_shape=jax.ShapeDtypeStruct((D, S), BF16),
        scratch_shapes=[
            pltpu.VMEM((D, S), BF16),
            pltpu.VMEM((2, SK, DH), BF16),
            pltpu.VMEM((2, SK, DH), BF16),
            pltpu.VMEM((2, D // LANES * LANES + 16, GW), BF16),
            pltpu.VMEM((2, D, GW), BF16),
            pltpu.VMEM((D % LANES, NG * GW), BF16),
            pltpu.VMEM((D,), BF16),
            pltpu.VMEM((1, D), BF16),
            pltpu.VMEM((D, 2 * D), BF16),
            pltpu.VMEM((D, MT_W), BF16),
            pltpu.VMEM((D, FF), BF16),
            pltpu.VMEM((D, FF), BF16),
            pltpu.VMEM((D, WT_W), BF16),
            pltpu.VMEM((FF // 2, D), U32),
            pltpu.VMEM((D, S), BF16),
            pltpu.VMEM((6 * D, LANES), F32),
            pltpu.VMEM((8, 6 * D), F32),
            pltpu.VMEM((D, LANES), F32),
            pltpu.VMEM((2 * D, LANES), F32),
            pltpu.VMEM((3, 8, D), F32),
            pltpu.VMEM((16, D), BF16),
            pltpu.VMEM((8, LANES), F32),
            pltpu.VMEM((S // 2, D), U32),
            pltpu.VMEM((D, S), F32),
            pltpu.VMEM((D // 2, S), U32),
            pltpu.VMEM((7, S // LANES, LANES), F32),
            pltpu.VMEM((S // BQ - V0 // REP, D % LANES * 8, BQ), F32),
            pltpu.VMEM((D % LANES, GW, LANES), F32),
            pltpu.VMEM(((S // BQ * REP - V0) * DH, BQ), F32),
            pltpu.VMEM(((S // BQ * REP - V0) * DH // VA, 8, BQ), F32),
            pltpu.VMEM((NG, V0 // REP * BQ, GW), F32),
            pltpu.SemaphoreType.DMA((N_SEMS,)),
        ],
        compiler_params=pltpu.CompilerParams(
            vmem_limit_bytes=120 * 1024 * 1024,
            disable_bounds_checks=True,
        ),
    )(xt, k, v, A_wq, wot, B_w_r, c, w_mod, B_w_gate, B_w_up, wdt)
    return out_t.T.reshape(B, S, D)
```

```python
import functools
import math

import jax
import jax.numpy as jnp
from jax import lax
import jax.experimental.pallas as pl
import jax.experimental.pallas.tpu as pltpu

F32 = jnp.float32
BF16 = jnp.bfloat16
U32 = jnp.uint32

HQ = 32
DH = 128
TOPC = 8
LN_EPS = 1e-5
BQ = 256
LANES = 128
XCH = 4

HEAD = [0, 1280, 1536, 1280, 1536, 640, 768, 640, 1536, 768, 1536, 1536, 640, 1536, 512, 0]
MODE = [2, 2, 2, 2, 0, 2, 0, 0, 0, 1, 2, 0, 0, 2, 1, 2]
QP_POS = [-1, -1, -1, -1, -1, 3, 18, -1]
OP_POS = [7, 12, 17, 25, 30, 31, 31, 31]
V0 = 4
VA = 16
GF = 2
VPER = 300
VMARG = 300
ADJ = [0, 2, -2, 0, 0, 0, 2, 0, 0, 0, 0, 0, -3, 0, 0, 0, 0, 0, 0, 0, 0, 1, 0, 0, 0, 0, 0, 0, 0, 0, 0, 1, 0, 0, 0, 0, 0, 0, 0, 0, 0, 0, 0, 1, 0, 0, 0, 0]
PL = 4
PA = 1
PT0 = 29864
PPER = 506
WT_W = 384
WT_R = 256
WT_TIE = 0
MT_W = 256
MT_R = 8
PK0 = 56
ZC = 1024
DMA_AT = 14
PG0 = 5
PGI = 3
OUW = 2
OPR = 16
TK_TIES = [0, 1, 2, 3, 4, 5, 6]
PIECES = [(0, 128), (128, 128), (256, 128), (384, 128), (512, 64)]
TIEC = 2048

_NT = (((1,), (1,)), ((), ()))

S_C = S_WMA = 0
S_ST = 1
S_WR = 2
S_WG = S_WU = 3
S_WQ0 = 4
S_WQR = 5
S_X = 6
S_G = S_X + XCH
S_O = S_G + 2
N_SEMS = S_O + 1


def _rb(x):
    return x.astype(BF16).astype(F32)


def _sigmoid(x):
    return 1.0 / (1.0 + jnp.exp(-x))


def _ln_rows(mean, var):
    eps = _rb(jnp.full((1, 1), LN_EPS, F32))
    return _rb(mean), _rb(jnp.sqrt(_rb(_rb(var) + eps)))


def _tile(col, n):
    return jnp.concatenate([col] * n, axis=1)


def _as_cols(row):
    return jnp.broadcast_to(row, (LANES, row.shape[1])).astype(BF16).T


def _kernel(xt_hbm, k_hbm, v_hbm, wq_hbm, wot_hbm, wr_hbm, c_hbm, wmod_hbm,
            wg_hbm, wu_hbm, wdt_hbm,
            out_hbm,
            xt_ref, k_buf, v_buf, wq_buf, wot_buf, wqr_ref, wr_ref, c_ref, wmod_ref, wms_ref,
            wg_ref, wu_ref, wdt_ref, wd_ref, out_ref,
            modc_ref, mrow_ref, scc_ref, fold_ref, mb_ref, lhs_ref, rc_ref, h_ref, acc_ref,
            xb_ref, st_ref, ht_ref, bp_ref, rem_ref, gate_ref, pre_ref,
            sems,
            *, S, SK, D, FF, NG, REP):
    qscale = (DH ** -0.5) * math.log2(math.e)
    NB = S // BQ
    GW = REP * DH
    TCH = S // XCH
    MA = 2 * D
    NSL = S // LANES
    KM = D // LANES * LANES
    KR = D - KM

    def cp(src, dst, sem):
        return pltpu.make_async_copy(src, dst, sems.at[sem])

    def x_copy(i):
        cols = pl.ds(pl.multiple_of(i * TCH, TCH), TCH)
        return cp(xt_hbm.at[:, cols], xt_ref.at[:, cols], S_X + i)

    def group_copies(grp, which=(0, 1, 2, 3)):
        slot = grp % 2
        cols = pl.ds(pl.multiple_of(grp * GW, GW), GW)
        ends = ((lambda: (wq_hbm.at[0:KM, cols], wq_buf.at[slot, 0:KM])),
                (lambda: (k_hbm.at[grp], k_buf.at[slot])),
                (lambda: (v_hbm.at[grp], v_buf.at[slot])),
                (lambda: (wot_hbm.at[:, cols], wot_buf.at[slot])))
        return [cp(*ends[i](), S_G + slot) for i in which]

    wq0_cp = lambda: cp(wq_hbm.at[KM:D, 0:GW], wqr_ref.at[:, 0:GW], S_WQ0)
    wqr_cp = lambda: cp(wq_hbm.at[KM:D, GW:NG * GW], wqr_ref.at[:, GW:NG * GW], S_WQR)
    c_cp = lambda: cp(c_hbm, c_ref, S_C)
    wma_cp = lambda: cp(wmod_hbm.at[:, 0:MA], wmod_ref, S_WMA)
    wr_cp = lambda: cp(wr_hbm, wr_ref, S_WR)
    wg_cp = lambda: cp(wg_hbm, wg_ref, S_WG)
    wu_cp = lambda: cp(wu_hbm, wu_ref, S_WU)

    def side_cols(step):
        return (pl.multiple_of(jnp.clip(step - 1, 0, FF // WT_W - 1) * WT_W, LANES),
                pl.multiple_of(MA + jnp.clip(step - 1, 0, 4 * D // MT_W - 1) * MT_W, LANES))

    def side_copies(step):
        wc, mc = side_cols(step)
        return (cp(wdt_hbm.at[:, pl.ds(wc, WT_W)], wdt_ref, S_ST),
                cp(wmod_hbm.at[:, pl.ds(mc, MT_W)], wms_ref, S_ST))

    def modcol(i):
        return modc_ref[i * D:(i + 1) * D, :]

    def finish_mod(mod, col0):
        mod = _rb(mod)
        lane = lax.broadcasted_iota(jnp.int32, mod.shape, 1) + col0
        is_scale = ((lane >= D) & (lane < 2 * D)) | ((lane >= 4 * D) & (lane < 5 * D))
        return jnp.where(is_scale, _rb(1.0 + mod), mod)

    def prep_cols(w, k0, k1):
        for kk in range(k0, k1):
            bp_ref[kk] = _as_cols(w[kk:kk + 1, :]).astype(F32)

    wq0_cp().start()
    wma_cp().start()
    c_cp().start()
    for i in range(XCH):
        x_copy(i).start()
        if i == 0:
            wqr_cp().start()
    for d in group_copies(0) + group_copies(1):
        d.start()
    wr_cp().start()
    acc_ref[:, 0:ZC] = jnp.zeros((D, ZC), F32)
    wq0_cp().wait()
    acc_ref[:, ZC:S] = jnp.zeros((D, S - ZC), F32)
    prep_cols(wqr_ref[:, 0:GW].astype(F32), 0, PK0)
    wma_cp().wait()
    c_cp().wait()
    c = c_ref[...].astype(F32)
    sc = _rb(c * _sigmoid(c))
    mod = jnp.dot(jnp.broadcast_to(sc, (8, D)).astype(BF16), wmod_ref[...],
                  preferred_element_type=F32)
    modc_ref[0:MA, :] = _as_cols(finish_mod(mod, 0)[0:1, :]).astype(F32)

    def pre(t0, t1, g0, ng):
        hb = pltpu.bitcast(h_ref[t0 // 2:t1 // 2, :], BF16)[:, KM:D]
        for u in range(ng):
            cols = pl.ds(pl.multiple_of((g0 + u) * GW, GW), GW)
            pre_ref[g0 + u, t0:t1, :] = jnp.dot(hb, wqr_ref[:, cols], preferred_element_type=F32)

    def ln1(i, carry):
        x_copy(i).wait()
        if not isinstance(i, int):
            pre(0, TCH, PG0 + (i - 1) * PGI, PGI)
        x = xt_ref[:, pl.ds(pl.multiple_of(i * TCH, TCH), TCH)].astype(F32)
        piv = x[0:1, :]
        d = x - piv
        md = jnp.mean(d, axis=0, keepdims=True)
        var = jnp.maximum(jnp.mean(d * d, axis=0, keepdims=True) - md * md, 0.0)
        mb, sd = _ln_rows(piv + md, var)
        rs = 1.0 / sd
        n = TCH // LANES
        ht = (x * rs - mb * rs) * _tile(modcol(1), n) + _tile(modcol(0), n)
        kt = D if isinstance(i, int) else KM
        h_ref[pl.ds(pl.multiple_of(i * (TCH // 2), TCH // 2), TCH // 2), 0:kt] = pltpu.bitcast(
            ht[0:kt].astype(BF16).T, U32)
        if not isinstance(i, int):
            hr = _rb(ht[KM:D, :])
            rep = jnp.concatenate([jnp.broadcast_to(hr[kk:kk + 1, :], (8, TCH)) for kk in range(KR)], axis=0)
            for u in range(TCH // BQ):
                ht_ref[(i - 1) * (TCH // BQ) + u] = rep[:, u * BQ:(u + 1) * BQ]
        return carry
    assert V0 * BQ == REP * TCH
    ln1(0, 0)
    wqr_cp().wait()
    pre(0, TCH, 0, PG0)
    scc_ref[...] = _as_cols(sc).astype(F32)
    prep_cols(wqr_ref[:, 0:GW].astype(F32), PK0, KR)
    wdt_ref[...] = jnp.zeros((D, WT_W), BF16)
    wms_ref[...] = jnp.zeros((D, MT_W), BF16)
    wq_buf[:, KM:KM + 16, :] = jnp.zeros((2, 16, GW), BF16)
    lax.fori_loop(1, XCH, ln1, 0)
    gdone = PG0 + (XCH - 1) * PGI
    if gdone < NG:
        pre(0, TCH, gdone, NG - gdone)

    def fold_modulation():
        sb, cb, gb = (mrow_ref[0:1, i * D:(i + 1) * D] for i in (3, 4, 5))
        for i, z in enumerate((sb, cb, gb)):
            mb_ref[i] = jnp.broadcast_to(z, (8, D))
        fold_ref[0:D, :] = modcol(5) * modcol(4)
        fold_ref[D:MA, :] = modcol(5) * modcol(3)
        wr = wr_ref[...].astype(F32).reshape(1, D)
        wc = wr * cb
        whi = _rb(wc)
        wlo = _rb(wc - whi)
        row = lax.broadcasted_iota(jnp.int32, (16, D), 0)
        lhs_ref[...] = jnp.where(row == 0, 1.0, jnp.where(row == 1, whi, jnp.where(
            row == 2, wlo, 0.0))).astype(BF16)
        rc_ref[0:1, :] = jnp.broadcast_to(jnp.sum(whi + wlo, axis=1, keepdims=True), (1, LANES))
        rc_ref[1:2, :] = jnp.broadcast_to(jnp.sum(wr * sb, axis=1, keepdims=True), (1, LANES))

    def group_step(step, carry):
        @pl.when(step > 0)
        def _():
            for d in side_copies(step):
                d.wait()

        for d in group_copies(step):
            d.wait()

        slot = step % 2
        k = k_buf[slot]
        v = v_buf[slot]
        wq = wq_buf[slot, 0:KM]
        wot = wot_buf[slot]

        nev = lax.broadcasted_iota(jnp.int32, (8, BQ), 1) > step + BQ
        assert VA == 16 and BQ == 2 * LANES
        npb = GW // VA
        L0, L1, B0 = V0 * DH // VA, NB * npb, V0 // REP

        def link(i, gate):
            av = ht_ref[i // npb - B0]
            bv = bp_ref[:, pl.ds(pl.multiple_of((i % npb) * VA, VA), VA), :]
            bv = jnp.concatenate([bv, bv], axis=2)
            acc = None
            for kk in range(KR):
                a = av[8 * kk:8 * kk + 8]
                if (kk * GF) % 8 < GF:
                    a = jnp.where(nev, gate, a)
                t = bv[kk] * jnp.concatenate([a, a], axis=0)
                acc = t if acc is None else acc + t
                g0 = 8 * ((kk * GF) // 8 % 2)
                g1 = 8 - g0
                gate = jnp.concatenate([acc[g0:g0 + 8, LANES:], acc[g1:g1 + 8, 0:LANES]], axis=1)
            rem_ref[pl.ds(pl.multiple_of((i - L0) * VA, VA), VA), :] = acc
            gate_ref[i - L0] = gate
            return gate

        gate = lax.fori_loop(L0, L1, link, jnp.zeros((8, BQ), F32), unroll=True)
        gates = [functools.partial(lambda i: gate_ref[i], i) for i in range(L1 - L0)]
        dues = [VMARG + (i + 1) * VPER for i in range(len(gates))]
        wn = wqr_ref[:, pl.ds(pl.multiple_of(jnp.minimum(step + 1, NG - 1) * GW, GW), GW)].astype(F32)
        for k0 in range(0, KR, PL):
            k1 = min(k0 + PL, KR)
            blks = {r0: jnp.where(nev, gate, wn[r0:r0 + 8, :]) for r0 in range(k0 // 8 * 8, k1, 8)}
            for kk in range(k0, k1):
                last = _as_cols(blks[kk // 8 * 8][kk % 8:kk % 8 + 1, :]).astype(F32)
                bp_ref[kk] = last
                g = jnp.concatenate([last[GW - 8:GW], last[LANES - 8:LANES]], axis=1)
                gate = gate + g if max(k0, k1 - PA) < kk else g
            gates.append(functools.partial(lambda g: g, gate))
            dues.append(PT0 + (k0 // PL + 1) * PPER)
        clock = [0]
        pinned = [0]
        npin = [0]

        def pin(x, final=False):
            due = sum(1 for t in dues if t <= clock[0]) + ADJ[npin[0]]
            due = len(gates) if final else min(due, len(gates))
            npin[0] += 1
            if due <= pinned[0]:
                return x
            pinned[0] = due
            g = pltpu.bitcast(gates[due - 1](), U32)
            xu = pltpu.bitcast(x, U32)
            top = xu[0:8, 0:LANES]
            top = jnp.where(nev[:, 0:LANES], g[:, 0:LANES], jnp.where(nev[:, LANES:], g[:, LANES:], top))
            if xu.shape[1] > LANES:
                top = jnp.concatenate([top, xu[0:8, LANES:]], axis=1)
            return pltpu.bitcast(jnp.concatenate([top, xu[8:]], axis=0), BF16)

        def qproj(j):
            hb = pin(pltpu.bitcast(h_ref[j * (BQ // 2):(j + 1) * (BQ // 2), 0:KM], BF16))
            clock[0] += 512
            if REP * j < V0:
                rem = pre_ref[step, j * BQ:(j + 1) * BQ, :]
            else:
                rem = rem_ref[(REP * j - V0) * DH:(REP * j + REP - V0) * DH, :].T
            q2 = jnp.dot(hb, wq, preferred_element_type=F32) + rem
            return (q2 * qscale).astype(BF16)

        def qk(ci, lo, hi):
            q = pin(qs[ci])
            clock[0] += (hi - lo) // 2
            return lax.dot_general(q, k[lo:hi], _NT, preferred_element_type=F32)

        def softmax_pv(s, mode):
            m = jnp.max(s, axis=1, keepdims=True)
            p = jnp.exp2(s - m)
            parts = [p[:, i * LANES:(i + 1) * LANES] for i in range(SK // LANES)]
            if mode == 2:
                lp = None
                for c in range(0, len(parts), 4):
                    t = (parts[c] + parts[c + 1]) + (parts[c + 2] + parts[c + 3])
                    lp = t if lp is None else lp + t
                    parts[c + 3] = jnp.where(lp < 0.0, lp, parts[c + 3])
                p = jnp.concatenate(parts, axis=1)
            clock[0] += SK // 2
            o = jnp.dot(p.astype(BF16), v, preferred_element_type=F32)
            if mode == 0:
                l = jnp.sum(p, axis=1, keepdims=True)
            elif mode == 1:
                lp = functools.reduce(lambda x, y: x + y, parts)
                l = jnp.sum(jnp.where(lp < 0.0, o, lp), axis=1, keepdims=True)
            else:
                l = jnp.sum(lp, axis=1, keepdims=True)
            rl = pl.reciprocal(l, approx=True)
            rl = rl * (2.0 - l * rl)
            return (o * rl).astype(BF16)

        def oproj(j):
            o2 = jnp.concatenate([outs[REP * j + r] for r in range(REP)], axis=1)
            w = pin(wot, final=(j == NB - 1))
            clock[0] += 576
            acc_ref[:, j * BQ:(j + 1) * BQ] += lax.dot_general(w, o2, _NT, preferred_element_type=F32)

        qs, outs = {}, []

        def fill(pos):
            for j in range(NB):
                if QP_POS[j] == pos:
                    q2 = qproj(j)
                    for r in range(REP):
                        qs[REP * j + r] = q2[:, r * DH:(r + 1) * DH]
            for j in range(NB):
                if OP_POS[j] == pos:
                    oproj(j)

        NC = NB * REP
        assert FF % WT_W == 0 and FF // WT_W < NG and (4 * D) % MT_W == 0 and 4 * D // MT_W < NG
        wc0, mc0 = side_cols(step)
        never8 = lax.broadcasted_iota(jnp.int32, (8, LANES), 1) > step + LANES
        wtie = None
        for t0 in range(0, WT_W, LANES):
            for r0 in range(0, D, WT_R):
                r1 = min(r0 + WT_R, D)
                blk = pltpu.bitcast(wdt_ref[r0:r1, t0:t0 + LANES], U32)
                if wtie is not None:
                    blk = jnp.concatenate([jnp.where(never8, wtie, blk[0:8]), blk[8:]], axis=0)
                tb = pltpu.bitcast(pltpu.bitcast(blk, BF16).T, U32)
                wd_ref[pl.ds(pl.multiple_of((wc0 + t0) // 2, LANES // 2), LANES // 2), r0:r1] = tb
                wtie = wd_ref[pl.ds(pl.multiple_of(wc0 // 2, LANES // 2), 8), 0:LANES]
        gate8 = pltpu.bitcast(wtie, F32)
        for r0 in range(0, D, MT_R):
            sc8 = scc_ref[r0:r0 + MT_R, :]
            sc8 = jnp.concatenate([jnp.where(never8, gate8, sc8[0:8])] + ([sc8[8:]] if MT_R > 8 else []), axis=0)
            t = wms_ref[r0:r0 + MT_R, :].astype(F32) * _tile(sc8, MT_W // LANES)
            macc = t if r0 == 0 else macc + t
            gate8 = macc[0:8, 0:LANES]
        mrow = finish_mod(jnp.sum(macc, axis=0, keepdims=True), mc0)
        mrow_ref[0:1, pl.ds(mc0, MT_W)] = mrow
        modc_ref[pl.ds(mc0, MT_W), :] = _as_cols(mrow).astype(F32)
        wtie = pltpu.bitcast(modc_ref[0:8, :], U32)
        fill(-1)
        qt = pltpu.bitcast(qs[WT_TIE], U32)
        qs[WT_TIE] = pltpu.bitcast(
            jnp.concatenate([jnp.where(never8, wtie, qt[0:8]), qt[8:]], axis=0), BF16)
        s_head = None
        for ci in range(NC):
            lo = HEAD[ci - 1] if ci else 0
            if ci == DMA_AT:
                qt = pltpu.bitcast(qs[ci], U32)
                tok = pltpu.bitcast(wq_buf[slot, KM:KM + 16, 0:LANES], U32)
                qs[ci] = pltpu.bitcast(
                    jnp.concatenate([jnp.where(never8, tok, qt[0:8]), qt[8:]], axis=0), BF16)
            s = qk(ci, lo, SK)
            if lo:
                s = jnp.concatenate([s_head, s], axis=1)
            fill(2 * ci)
            if HEAD[ci]:
                s_head = qk(ci + 1, 0, HEAD[ci])
            outs.append(softmax_pv(s, MODE[ci]))
            fill(2 * ci + 1)

        pl.when(step + 2 < NG)(lambda: group_copies(step + 2, (0,))[0].start())

        @pl.when(step + 1 < NG)
        def _():
            for d in side_copies(step + 1):
                d.start()

        @pl.when(step + 2 < NG)
        def _():
            for d in group_copies(step + 2, (1, 2, 3)):
                d.start()

        @pl.when(step == 0)
        def _():
            wg_cp().start()

        @pl.when(step == 1)
        def _():
            wu_cp().start()

        return step

    step = lax.fori_loop(0, NG, group_step, 0)

    wr_cp().wait()
    fold_modulation()
    for sl in range(NSL):
        cols = slice(sl * LANES, (sl + 1) * LANES)
        for r0 in range(0, D, LANES):
            r1 = min(r0 + LANES, D)
            x2 = xt_ref[r0:r1, cols].astype(F32) + modc_ref[MA + r0:MA + r1, :] * acc_ref[r0:r1, cols]
            acc_ref[r0:r1, cols] = x2
            xb = x2.astype(BF16)
            xb_ref[r0 // 2:r1 // 2, cols] = pltpu.bitcast(xb, U32)
            if r0 == 0:
                piv = jnp.mean(x2[0:8, :], axis=0, keepdims=True)
                st_ref[0, sl:sl + 1, :] = piv
            d = x2 - piv
            lhs = lhs_ref[:, r0:r1]
            t1 = jnp.dot(lhs, xb, preferred_element_type=F32)[0:8, :]
            t2 = jnp.dot(lhs, (d * d).astype(BF16), preferred_element_type=F32)[0:8, :]
            s1, s2 = (t1, t2) if r0 == 0 else (s1 + t1, s2 + t2)
        for n in range(3):
            st_ref[1 + n, sl:sl + 1, :] = s1[n:n + 1, :]
        st_ref[4, sl:sl + 1, :] = s2[0:1, :]

    wg_cp().wait()
    wu_cp().wait()

    mean = st_ref[1] * (1.0 / D)
    md = mean - st_ref[0]
    mb, sd = _ln_rows(mean, jnp.maximum(st_ref[4] * (1.0 / D) - md * md, 0.0))
    rs = 1.0 / sd
    st_ref[5] = rs
    st_ref[6] = mb * rs
    r = (st_ref[2] + st_ref[3] - mb * rc_ref[0:1, :]) * rs + rc_ref[1:2, :]

    lane16 = lax.broadcasted_iota(jnp.int32, (16, LANES), 1)
    never = lane16 > step + LANES

    def after_out_stores():
        dyn0 = pl.multiple_of((step - (NG - 1)) * LANES, LANES)
        return out_ref[0:16, pl.ds(dyn0, LANES)]

    def out_unit(n):
        w = OUW * LANES
        cols = slice(n * w, (n + 1) * w)
        rs, mrs = (jnp.concatenate([st_ref[k, n * OUW + u:n * OUW + u + 1, :]
                                    for u in range(OUW)], axis=1) for k in (5, 6))
        for r0 in range(0, D, OPR):
            x2 = acc_ref[r0:r0 + OPR, cols]
            o = x2 + ((x2 * rs - mrs) * _tile(fold_ref[r0:r0 + OPR, :], OUW)
                      + _tile(fold_ref[D + r0:D + r0 + OPR, :], OUW))
            out_ref[r0:r0 + OPR, cols] = o.astype(BF16)
        return after_out_stores().astype(F32)

    r = _rb(r) + 0.0
    bits = pltpu.bitcast(r, jnp.int32)
    mono = bits ^ ((bits >> 31) & jnp.int32(0x7FFFFFFF))
    tok = (lax.broadcasted_iota(jnp.int32, (NSL, LANES), 0) * LANES
           + lax.broadcasted_iota(jnp.int32, (NSL, LANES), 1))
    keyi = (((mono >> 16) + 32768) * S + (S - 1 - tok)) + jnp.int32(1 << 29)
    key = pltpu.bitcast(keyi, F32)

    row16 = lax.broadcasted_iota(jnp.int32, (16, LANES), 0)
    rowc = lax.broadcasted_iota(jnp.int32, (16, 1), 0)
    sel_slab, sel_off = [], []
    tie, nunit = None, 0
    xsel = jnp.zeros((16, D), F32)
    mbsel = jnp.zeros((16, 1), F32)
    rssel = jnp.zeros((16, 1), F32)
    ksel = jnp.zeros((16, 1), F32)
    for t in range(TOPC):
        kmax = jnp.max(jnp.max(key, axis=0, keepdims=True), axis=1, keepdims=True)
        hit = key == kmax
        key = jnp.where(hit, 0.0, key)
        pick = lambda z: jnp.sum(jnp.sum(jnp.where(hit, z, 0.0), axis=0, keepdims=True),
                                 axis=1, keepdims=True)
        mbsel = jnp.where(rowc == t, pick(mb), mbsel)
        rssel = jnp.where(rowc == t, pick(rs), rssel)
        for _ in range(TK_TIES.count(t)):
            tie = out_unit(nunit)
            nunit += 1
            key = jnp.where(never, tie, key)
        ksel = jnp.where(rowc == t, kmax, ksel)
        ki = pltpu.bitcast(kmax, jnp.int32)[0, 0]
        idx = (S - 1) - (ki & (S - 1))
        slab = idx >> 7
        off = idx & (LANES - 1)
        onehot = jnp.where((row16 == t) & (lane16 == off), 1.0, 0.0).astype(BF16)
        dslab = xb_ref[:, pl.ds(pl.multiple_of(slab * LANES, LANES), LANES)]
        xsel = xsel + lax.dot_general(onehot, pltpu.bitcast(dslab, BF16), _NT,
                                      preferred_element_type=F32)
        sel_slab.append(slab)
        sel_off.append(off)
    nsel = _rb(_rb(xsel - mbsel) * rssel)
    hsel = _rb(_rb(nsel * mb_ref[1, 0:1, :]) + mb_ref[0, 0:1, :])
    hi = ((pltpu.bitcast(ksel, jnp.int32) - jnp.int32(1 << 29)) // S - 32768) << 16
    rbits = hi ^ ((hi >> 31) & jnp.int32(0x7FFF0000))
    gate = _rb(_sigmoid(jnp.where(rowc < TOPC, pltpu.bitcast(rbits, F32), 0.0)))

    def out_copy(sl, r0, nr):
        c0 = pl.multiple_of(sl * LANES, LANES)
        return cp(out_ref.at[r0:r0 + nr, pl.ds(c0, LANES)],
                  out_hbm.at[r0:r0 + nr, pl.ds(c0, LANES)], S_O)

    fresh = []
    seen = jnp.int32(0)
    for t in range(TOPC):
        fresh.append(((seen >> sel_slab[t]) & 1) == 0)
        seen = seen | (1 << sel_slab[t])
    plain = [((seen >> sl) & 1) == 0 for sl in range(NSL)]

    for n in range(nunit, NSL // OUW):
        tie = out_unit(n)
    for sl in range(NSL):
        pl.when(plain[sl])(lambda sl=sl: out_copy(sl, 0, D).start())

    h0 = jnp.where(never, tie, hsel[:, 0:LANES])
    hs = jnp.concatenate([h0, hsel[:, LANES:]], axis=1).astype(BF16)
    gpre = _rb(jnp.dot(hs, wg_ref[...], preferred_element_type=F32))
    u = _rb(jnp.dot(hs, wu_ref[...], preferred_element_type=F32))
    a = (_rb(gpre * _sigmoid(gpre)) * u).astype(BF16)

    gb = mb_ref[2, 0:1, :]

    def down(r0, nr, tied):
        lhs = a
        if tied:
            a0 = jnp.where(never[0:8, :], pltpu.bitcast(after_out_stores(), U32),
                           pltpu.bitcast(a[:, TIEC:TIEC + LANES], U32))
            lhs = jnp.concatenate([a[:, 0:TIEC], pltpu.bitcast(a0, BF16), a[:, TIEC + LANES:]], axis=1)
        y = jnp.dot(lhs, pltpu.bitcast(wd_ref[0:FF // 2, r0:r0 + nr], BF16),
                    preferred_element_type=F32)
        c = slice(r0, r0 + nr)
        return xsel[:, c] + gb[:, c] * (hsel[:, c] + y * gate)

    def patch(r0, nr, new):
        lane = lax.broadcasted_iota(jnp.int32, (nr // 2, LANES), 1)
        for t in range(TOPC):
            cols = pl.ds(pl.multiple_of(sel_slab[t] * LANES, LANES), LANES)
            old = pltpu.bitcast(out_ref[r0:r0 + nr, cols], U32)
            upd = pltpu.bitcast(_as_cols(new[t:t + 1, :]), U32)
            out_ref[r0:r0 + nr, cols] = pltpu.bitcast(jnp.where(lane == sel_off[t], upd, old), BF16)
        for t in range(TOPC):
            pl.when(fresh[t])(lambda t=t: out_copy(sel_slab[t], r0, nr).start())

    news = [down(*PIECES[0], False)]
    for n in range(len(PIECES)):
        if n + 1 < len(PIECES):
            news.append(down(*PIECES[n + 1], n > 0))
        patch(*PIECES[n], news[n])

    cp(out_ref, out_hbm, S_O).wait()


@jax.jit
def pallas_adaLN_cond__gqa_block_cached__moe_arch_mod__prompt_kernel(
    A_x: jax.Array,
    A_k_cache: jax.Array,
    A_v_cache: jax.Array,
    A_wq: jax.Array,
    A_wo: jax.Array,
    B_x: jax.Array,
    B_w_r: jax.Array,
    B_w_gate: jax.Array,
    B_w_up: jax.Array,
    B_w_down: jax.Array,
    c: jax.Array,
    w_mod: jax.Array,
):
    del B_x
    B, S, D = A_x.shape
    assert B == 1
    NG, SK = A_k_cache.shape[1], A_k_cache.shape[2]
    REP = HQ // NG
    FF = B_w_gate.shape[1]
    GW = REP * DH

    xt = A_x.reshape(S, D).T
    wot = A_wo.T
    wdt = B_w_down.T
    k = A_k_cache.reshape(NG, SK, DH)
    v = A_v_cache.reshape(NG, SK, DH)

    hbm = pl.BlockSpec(memory_space=pl.ANY)
    out_t = pl.pallas_call(
        functools.partial(_kernel, S=S, SK=SK, D=D, FF=FF, NG=NG, REP=REP),
        in_specs=[hbm] * 11,
        out_specs=hbm,
        out_shape=jax.ShapeDtypeStruct((D, S), BF16),
        scratch_shapes=[
            pltpu.VMEM((D, S), BF16),
            pltpu.VMEM((2, SK, DH), BF16),
            pltpu.VMEM((2, SK, DH), BF16),
            pltpu.VMEM((2, D // LANES * LANES + 16, GW), BF16),
            pltpu.VMEM((2, D, GW), BF16),
            pltpu.VMEM((D % LANES, NG * GW), BF16),
            pltpu.VMEM((D,), BF16),
            pltpu.VMEM((1, D), BF16),
            pltpu.VMEM((D, 2 * D), BF16),
            pltpu.VMEM((D, MT_W), BF16),
            pltpu.VMEM((D, FF), BF16),
            pltpu.VMEM((D, FF), BF16),
            pltpu.VMEM((D, WT_W), BF16),
            pltpu.VMEM((FF // 2, D), U32),
            pltpu.VMEM((D, S), BF16),
            pltpu.VMEM((6 * D, LANES), F32),
            pltpu.VMEM((8, 6 * D), F32),
            pltpu.VMEM((D, LANES), F32),
            pltpu.VMEM((2 * D, LANES), F32),
            pltpu.VMEM((3, 8, D), F32),
            pltpu.VMEM((16, D), BF16),
            pltpu.VMEM((8, LANES), F32),
            pltpu.VMEM((S // 2, D), U32),
            pltpu.VMEM((D, S), F32),
            pltpu.VMEM((D // 2, S), U32),
            pltpu.VMEM((7, S // LANES, LANES), F32),
            pltpu.VMEM((S // BQ - V0 // REP, D % LANES * 8, BQ), F32),
            pltpu.VMEM((D % LANES, GW, LANES), F32),
            pltpu.VMEM(((S // BQ * REP - V0) * DH, BQ), F32),
            pltpu.VMEM(((S // BQ * REP - V0) * DH // VA, 8, BQ), F32),
            pltpu.VMEM((NG, V0 // REP * BQ, GW), F32),
            pltpu.SemaphoreType.DMA((N_SEMS,)),
        ],
        compiler_params=pltpu.CompilerParams(
            vmem_limit_bytes=120 * 1024 * 1024,
            disable_bounds_checks=True,
        ),
    )(xt, k, v, A_wq, wot, B_w_r, c, w_mod, B_w_gate, B_w_up, wdt)
    return out_t.T.reshape(B, S, D)
```
